```python
import jax
import jax.numpy as jnp

def _softmax(x, axis=-1):
    return jax.nn.softmax(x, axis=axis)
def _gelu(x):
    return jax.nn.gelu(x, approximate=True)
def _silu(x):
    return jax.nn.silu(x)
def _sigmoid(x):
    return jax.nn.sigmoid(x)
def _layernorm(x, axis=-1, eps=1e-5):
    m = jnp.mean(x, axis=axis, keepdims=True)
    v = jnp.var(x, axis=axis, keepdims=True)
    return (x - m) / jnp.sqrt(v + eps)
def _scatter_add(tgt, idx, src, axis=0):
    return tgt.at[idx].add(src)
def _segment_sum(src, seg, n):
    return jax.ops.segment_sum(src, seg, n)
class _Rng:
    def __init__(self, key):
        self._k = key
    def _next(self):
        self._k, sub = jax.random.split(self._k)
        return sub
    def normal(self, shape):
        return jax.random.normal(self._next(), shape, dtype=jnp.bfloat16)
    def randint(self, lo, hi, shape):
        return jax.random.randint(self._next(), shape, lo, hi, dtype=jnp.int32)
    def uniform(self, shape, lo=0.0, hi=1.0):
        return jax.random.uniform(self._next(), shape, jnp.bfloat16, lo, hi)
    def permutation(self, n):
        return jax.random.permutation(self._next(), n)


kernel_name = 'parallel_sum__sliding_local_dilated__glu_gated_bilinear__prompt'

def setup_inputs():
    _rng = _Rng(jax.random.key(int.from_bytes(__import__("os").urandom(4), "little")))
    _w = (lambda a: (lambda t: t.astype(jnp.bfloat16) if jnp.issubdtype(t.dtype, jnp.floating) else t)(jnp.asarray(a)))
    def _A_setup():
        B, S, D = 1, 2048, 1024
        return {
            "x": _w((lambda *s: _rng.normal(s) * 0.05)(B, S, D)),
            "wqkv": _w((lambda *s: _rng.normal(s) * 0.05)(D, 3 * D)),
            "wo": _w((lambda *s: _rng.normal(s) * 0.05)(D, D)),
        }
    _A_in = _A_setup()

    def _B_setup():
        B, S, D, F = 1, 2048, 1024, 3584
        return {
            "x": _w((lambda *s: _rng.normal(s) * 0.05)(B, S, D)),
            "w_gate": _w((lambda *s: _rng.normal(s) * 0.05)(D, F) * (D ** -0.5)),
            "w_up": _w((lambda *s: _rng.normal(s) * 0.05)(D, F) * (D ** -0.5)),
            "w_down": _w((lambda *s: _rng.normal(s) * 0.05)(F, D) * (F ** -0.5)),
        }
    _B_in = _B_setup()

    return {
        "A_x": _A_in["x"],
        "A_wqkv": _A_in["wqkv"],
        "A_wo": _A_in["wo"],
        "B_x": _B_in["x"],
        "B_w_gate": _B_in["w_gate"],
        "B_w_up": _B_in["w_up"],
        "B_w_down": _B_in["w_down"],
    }

def reference(A_x, A_wqkv, A_wo, B_x, B_w_gate, B_w_up, B_w_down):
    def _A_ref(x, wqkv, wo):
        B, S, D = x.shape
        H = 32; Dh = D // H
        W, dil = 8, 2
        qkv = (lambda x, *d: x.transpose(*d))((x @ wqkv).reshape(B, S, 3, H, Dh), 2, 0, 3, 1, 4)
        q, k, v = qkv[0], qkv[1], qkv[2]
        scale = Dh ** -0.5
        pos = jnp.arange(S)
        off = jnp.arange(W) * dil
        idx = pos[:, None] - off[None, :]
        mask = idx >= 0
        idx_c = jnp.where(mask, idx, 0).reshape(-1)
        kg = k[:, :, idx_c, :].reshape(B, H, S, W, Dh)
        vg = v[:, :, idx_c, :].reshape(B, H, S, W, Dh)
        logits = jnp.einsum("bhsd,bhswd->bhsw", q, kg) * scale
        logits = jnp.where(mask[None, None, :, :], logits, -1e9)
        attn = _softmax(logits, axis=-1)
        o = jnp.einsum("bhsw,bhswd->bhsd", attn, vg)
        return (lambda x, *d: x.transpose(*d))(o, 0, 2, 1, 3).reshape(B, S, D) @ wo

    def _B_ref(x, w_gate, w_up, w_down):
        g = jnp.einsum("bsd,df->bsf", x, w_gate)
        u = jnp.einsum("bsd,df->bsf", x, w_up)
        h = g * u
        return jnp.einsum("bsf,fd->bsd", h, w_down)

    x = A_x
    xn = _layernorm(x, axis=-1)
    return x + _A_ref(xn, A_wqkv, A_wo) + _B_ref(xn, B_w_gate, B_w_up, B_w_down)
```

```python
import jax
import jax.numpy as jnp
from jax import lax
from jax.experimental import pallas as pl
from jax.experimental.pallas import tpu as pltpu

bf = jnp.bfloat16
f32 = jnp.float32
u32 = jnp.uint32

S, D, F = 2048, 1024, 3584
WIN = 8
NP = 49
HB = S // 4
KB = D // 4
TF = 512
TB = TF // 4
NCH = F // TF
RS = 256
MPAD = 8
PADW = 8
QW = 256
EPS = 1e-5
C2 = float(32 ** -0.5 * 1.4426950408889634)
NATT = 10

A_T = [[(1, (0, 0)), (1, (1, 1))], [(1, (1, 0)), (1, (1, 1))], [(1, (0, 0))], [(1, (1, 1))],
       [(1, (0, 0)), (1, (0, 1))], [(1, (1, 0)), (-1, (0, 0))], [(1, (0, 1)), (-1, (1, 1))]]
B_T = [[(1, (0, 0)), (1, (1, 1))], [(1, (0, 0))], [(1, (0, 1)), (-1, (1, 1))], [(1, (1, 0)), (-1, (0, 0))],
       [(1, (1, 1))], [(1, (0, 0)), (1, (0, 1))], [(1, (1, 0)), (1, (1, 1))]]
C_T = {(0, 0): [(1, 0), (1, 3), (-1, 4), (1, 6)], (0, 1): [(1, 2), (1, 4)],
       (1, 0): [(1, 1), (1, 3)], (1, 1): [(1, 0), (-1, 1), (1, 2), (1, 5)]}
POS = ((0, 0), (0, 1), (1, 0), (1, 1))


def _comb(terms):
    acc = None
    for s, v in terms:
        if acc is None:
            acc = v if s > 0 else -v
        else:
            acc = acc + v if s > 0 else acc - v
    return acc


def _dot(a, b):
    return jnp.dot(a, b, preferred_element_type=f32)


def _pk(v):
    return pltpu.bitcast(v.astype(bf), u32)


def _up(w):
    return pltpu.bitcast(w, bf)


def _unpk(w):
    return pltpu.bitcast(w, bf).astype(f32)


def _as_f32(w):
    return lax.bitcast_convert_type(w, f32)


def _as_u32(v):
    return lax.bitcast_convert_type(v, u32)


def _mult(x, m):
    return x if isinstance(x, int) else pl.multiple_of(x, m)


def _opcomb(load, table, I, emit):
    sub = {(r, c): _comb([(s, load(q[0] * 2 + r, q[1] * 2 + c)) for s, q in table[I]])
           for r in range(2) for c in range(2)}
    for J, t2 in enumerate(table):
        emit(I * 7 + J, _pk(_comb([(s, sub[q]) for s, q in t2])))


def _opcomb_job(load, table, emit):
    return [(lambda I=I: _opcomb(load, table, I, emit)) for I in range(7)]


def _outpos(load, pos):
    inner = [_comb([(s, load(I * 7 + J)) for s, J in C_T[pos]]) for I in range(7)]
    return {q: _comb([(s, inner[I]) for s, I in terms]) for q, terms in C_T.items()}


def _perm8(v):
    lane = lax.broadcasted_iota(jnp.int32, v[0].shape, 1)
    v = list(v)
    for cb, lb in ((2, 4), (1, 3), (0, 2)):
        sh = 1 << lb
        hi = (lane & sh) != 0
        out = [None] * 8
        for c in range(8):
            if c & (1 << cb):
                continue
            x, y = v[c], v[c | (1 << cb)]
            out[c] = jnp.where(hi, pltpu.roll(y, sh, 1), x)
            out[c | (1 << cb)] = jnp.where(hi, y, pltpu.roll(x, 128 - sh, 1))
        v = out
    return v


def _sum4(x, lane):
    x = x + jnp.where((lane & 1) != 0, pltpu.roll(x, 1, 1), pltpu.roll(x, 127, 1))
    x = x + jnp.where((lane & 2) != 0, pltpu.roll(x, 2, 1), pltpu.roll(x, 126, 1))
    return x


def _mix(a, b):
    if not b:
        return list(a)
    if not a:
        return list(b)
    out, n, m, k = [], len(a), len(b), 0
    for i, t in enumerate(a):
        out.append(t)
        tgt = (i + 1) * m // n
        while k < tgt:
            out.append(b[k])
            k += 1
    return out


def _flat(jobs):
    return [t for j in jobs for t in j]


def _weave(mx, jobs):
    vp = _flat(jobs)
    tot = sum(c for _, c in mx)
    n, k, acc = len(vp), 0, 0
    for t, c in mx:
        t()
        acc += c
        tgt = acc * n // tot
        while k < tgt:
            vp[k]()
            k += 1
    while k < n:
        vp[k]()
        k += 1


def _kernel(one_ref, x_hbm, wqkv_hbm, wo_hbm, wg_hbm, wu_hbm, wd_hbm, out_hbm,
            xr, xn, T, wst, R0, qp, kp, vp, gst, ust, dst, B0, B1, Bd0, Bd1, M, H, hst, acc,
            sem_x, sem_w, sem_g, sem_u, sem_d, sem_o):
    Bs, Bds = (B0, B1), (Bd0, Bd1)

    def block(mx, jobs, name="blk"):
        with jax.named_scope(name):
            @pl.when(one_ref[0] > 0)
            def _():
                _weave(mx(), jobs())

    def x_copy(r):
        return pltpu.make_async_copy(x_hbm.at[pl.ds(r * 256, 256), :], xr.at[pl.ds(r * 256, 256), :], sem_x.at[r])

    def w_copy(j, slot):
        return pltpu.make_async_copy(wqkv_hbm.at[:, pl.ds(_mult(j * QW, QW), QW)], wst.at[slot], sem_w.at[slot])

    def g_copy(j, par):
        return pltpu.make_async_copy(wg_hbm.at[:, pl.ds(_mult(j * TF, TF), TF)], gst.at[par], sem_g.at[par])

    def u_copy(j, par):
        return pltpu.make_async_copy(wu_hbm.at[:, pl.ds(_mult(j * TF, TF), TF)], ust.at[par], sem_u.at[par])

    def d_copy(j, par):
        return pltpu.make_async_copy(wd_hbm.at[pl.ds(_mult(j * TF, TF), TF), :], dst.at[par], sem_d.at[par])

    def wo_copies():
        return (pltpu.make_async_copy(wo_hbm.at[:, pl.ds(0, TF)], gst.at[1], sem_g.at[1]),
                pltpu.make_async_copy(wo_hbm.at[:, pl.ds(TF, TF)], ust.at[1], sem_u.at[1]))

    def out_copy(s, a, hh, nh):
        rows = RS // nh
        r0 = a * HB + s * RS + hh * rows
        k = (s * 4 + a) * nh + hh
        return pltpu.make_async_copy(xr.at[pl.ds(r0, rows), :], out_hbm.at[pl.ds(r0, rows), :], sem_o.at[k])

    def ln_job(g):
        st = {}
        ld = lambda c: xr[pl.ds(g * 16, 16), pl.ds(c * 128, 128)].astype(f32)

        def t_mean():
            a = ld(0)
            for c in range(1, 8):
                a = a + ld(c)
            st['m'] = jnp.sum(a, axis=1, keepdims=True) * (1.0 / D)

        def t_var():
            a = None
            for c in range(8):
                dlt = ld(c) - st['m']
                a = dlt * dlt if a is None else a + dlt * dlt
            st['r'] = lax.rsqrt(jnp.sum(a, axis=1, keepdims=True) * (1.0 / D) + EPS)

        def t_norm():
            for c in range(8):
                xn[pl.ds(g * 8, 8), pl.ds(c * 128, 128)] = _pk((ld(c) - st['m']) * st['r'])
        return [t_mean, t_var, t_norm]

    def t_job(pos_idx):
        g = pos_idx // 2
        n = pos_idx % 2
        w0 = _mult(g * 8, 8)
        l0 = _mult(n * 128, 128)

        def load(i, j):
            return _unpk(xn[pl.ds(_mult(i * 256 + w0, 8), 8), pl.ds(_mult(j * KB + l0, 128), 128)])

        def emit(p, v):
            T[p, pl.ds(w0, 8), pl.ds(l0, 128)] = v
        return _opcomb_job(load, A_T, emit)

    def b_job(par_src, Bref, g, half):
        w_ref = (gst, ust)[half]

        def load(i, q):
            return w_ref[par_src, pl.ds(i * KB + g * 16, 16), pl.ds(q * TB, TB)].astype(f32)

        def emit(p, v):
            Bref[p, pl.ds(g * 8, 8), pl.ds(half * TB, TB)] = v
        return _opcomb_job(load, B_T, emit)

    def bd_job(par_src, Bref, g, n):
        def load(i, q):
            return dst[par_src, pl.ds(i * TB + g * 16, 16), pl.ds(q * KB + n * 128, 128)].astype(f32)

        def emit(p, v):
            Bref[p, pl.ds(g * 8, 8), pl.ds(n * 128, 128)] = v
        return _opcomb_job(load, B_T, emit)

    def b_jobs(par, lo=0, hi=KB // 16):
        return [b_job(par, Bs[par], g, h) for g in range(lo, hi) for h in range(2)]

    def bd_jobs(par, lo=0, hi=TB // 16):
        return [bd_job(par, Bds[par], g, n) for g in range(lo, hi) for n in range(2)]

    def raw_store(m, c, w, val):
        if m == 1:
            acc[c, w // 512, pl.ds(_mult(w % 512, 8), 8), :] = _as_f32(val)
        else:
            R0[c, pl.ds(_mult(w, 8), 8), :] = val

    def raw_load(m, c, w):
        if m == 1:
            return _as_u32(acc[c, w // 512, pl.ds(_mult(w % 512, 8), 8), :])
        return R0[c, pl.ds(_mult(w, 8), 8), :]

    def perm_job(m, grp):
        dstp = (qp, kp, vp)[m]

        def t():
            w = grp * 8
            r = _perm8([raw_load(m, c, w) for c in range(8)])
            for c in range(8):
                dstp[c, pl.ds(_mult(PADW + w, 8), 8), :] = r[c]
        return [t]

    def attn_job(grp):
        st = {}
        b = _mult(grp * 8, 8)

        def half(v, h):
            return _unpk(v)[h * 8:(h + 1) * 8]

        def qk(h, cs):
            def t():
                for c in cs:
                    qv = half(qp[c, pl.ds(_mult(b + PADW, 8), 8), :], h)
                    for w in range(WIN):
                        kv = half(kp[c, pl.ds(b + (PADW - w), 8), :], h)
                        st[(h, w)] = qv * kv if c == 0 else st[(h, w)] + qv * kv
            return t

        def sm(h):
            def t():
                lane = lax.broadcasted_iota(jnp.int32, (8, 128), 1)
                row = lax.broadcasted_iota(jnp.int32, (8, 128), 0) + (grp * 16 + h * 8)
                ls = []
                for w in range(WIN):
                    a = _sum4(st[(h, w)], lane)
                    if w > 0:
                        a = jnp.where(row >= 2 * w, a, -1e30)
                    ls.append(a)
                m = ls[0]
                for w in range(1, WIN):
                    m = jnp.maximum(m, ls[w])
                e = [jnp.exp2((l - m) * C2) for l in ls]
                den = e[0]
                for w in range(1, WIN):
                    den = den + e[w]
                inv = 1.0 / den
                st[('p', h)] = [x * inv for x in e]
            return t

        def pv(c):
            def t():
                o0 = o1 = None
                for w in range(WIN):
                    vv = _unpk(vp[c, pl.ds(b + (PADW - w), 8), :])
                    a0 = st[('p', 0)][w] * vv[0:8]
                    a1 = st[('p', 1)][w] * vv[8:16]
                    o0 = a0 if o0 is None else o0 + a0
                    o1 = a1 if o1 is None else o1 + a1
                R0[c, pl.ds(b, 8), :] = _pk(jnp.concatenate([o0, o1], axis=0))
            return t
        return ([qk(0, (c, c + 1)) for c in range(0, 8, 2)] + [qk(1, (c, c + 1)) for c in range(0, 8, 2)]
                + [sm(0), sm(1)] + [pv(c) for c in range(8)])

    def unperm_job(grp):
        def t():
            b = _mult(grp * 8, 8)
            r = _perm8([R0[c, pl.ds(b, 8), :] for c in range(8)])
            for c in range(8):
                xn[pl.ds(b, 8), pl.ds(c * 128, 128)] = r[c]
        return [t]

    def comb_job(s, g):
        sl = g % 4
        job = []
        for hf in range(2):
            for pos in POS:
                def t(hf=hf, pos=pos):
                    r = pl.ds(g * 16 + hf * 8, 8)
                    gg = _outpos(lambda p: M[s, p, 0, r, :], pos)
                    uu = _outpos(lambda p: M[s, p, 1, r, :], pos)
                    for q in gg:
                        hst[sl, (q[0] * 2 + pos[0]) * 4 + q[1] * 2 + pos[1], pl.ds(hf * 8, 8), :] = gg[q] * uu[q]
                job.append(t)

        def emit(p, v):
            H[s, p, pl.ds(g * 8, 8), :] = v
        return job + _opcomb_job(lambda i, j: hst[sl, i * 4 + j, pl.ds(0, 16), :], A_T, emit)

    def comb_jobs(s):
        return [comb_job(s, g) for g in range(RS // 16)]

    def zero_job(p):
        def t():
            for c in range(2):
                acc[p, c, pl.ds(0, HB), :] = jnp.zeros((HB, 128), f32)
        return [t]

    def final_job(s, g, n):
        job = []
        for pos in POS:
            def t(pos=pos):
                o = [_outpos(lambda p: acc[p, n, pl.ds(s * RS + g * 16 + hf * 8, 8), :], pos) for hf in range(2)]
                for q in o[0]:
                    a = q[0] * 2 + pos[0]
                    ch = (q[1] * 2 + pos[1]) * 2 + n
                    pln = a * 8 + ch
                    rows = pl.ds(a * HB + s * RS + g * 16, 16)
                    cols = pl.ds(ch * 128, 128)
                    ffn = jnp.concatenate([o[0][q], o[1][q]], axis=0)
                    att = M[s, pln // 2, pln % 2, pl.ds(g * 16, 16), :]
                    xr[rows, cols] = (xr[rows, cols].astype(f32) + att + ffn).astype(bf)
            job.append(t)
        return job

    def qkv_tasks(m, slot, cbase, pieces):
        out = []
        for r in pieces:
            for ct in range(QW // 128):
                def t(r=r, ct=ct):
                    res = _dot(_up(xn[pl.ds(r * 64, 64), :]), wst[slot, :, pl.ds(ct * 128, 128)])
                    for k in range(8):
                        raw_store(m, cbase + ct, r * 64 + k * 8, _pk(res[k * 16:(k + 1) * 16]))
                out.append((t, 256))
        return out

    def mm1_tasks(s, Bref):
        out = []
        for p in range(NP):
            for h in range(4):
                def t(p=p, h=h):
                    r = _dot(_up(T[p, pl.ds(s * 128 + h * 32, 32), :]), _up(Bref[p]))
                    for c in range(2):
                        M[s, p, c, pl.ds(h * 64, 64), :] = r[:, c * 128:(c + 1) * 128]
                out.append((t, 64))
        return out

    def mm2_tasks(s, Bref):
        out = []
        for p in range(NP):
            for h in range(2):
                def t(p=p, h=h):
                    r = _dot(_up(H[s, p, pl.ds(h * 64, 64), :]), _up(Bref[p]))
                    for c in range(2):
                        acc[p, c, pl.ds(s * RS + h * 128, 128), :] += r[:, c * 128:(c + 1) * 128]
                out.append((t, 64))
        return out

    def wo_tasks(s):
        out = []
        for a in range(4):
            for hh in range(2):
                for ch in range(8):
                    def t(a=a, hh=hh, ch=ch):
                        w_ref = (gst, ust)[ch // 4]
                        res = _dot(_up(xn[pl.ds(a * 256 + s * 128 + hh * 64, 64), :]),
                                   w_ref[1, :, pl.ds((ch % 4) * 128, 128)])
                        pln = a * 8 + ch
                        M[s, pln // 2, pln % 2, pl.ds(hh * 128, 128), :] = res
                    out.append((t, 256))
        return out

    for r in range(8):
        x_copy(r).start()
    w_copy(0, 0).start()
    w_copy(1, 1).start()
    g_copy(0, 0).start()
    u_copy(0, 0).start()
    d_copy(0, 0).start()
    for c in range(8):
        kp[c, pl.ds(0, PADW), :] = jnp.zeros((PADW, 128), u32)
        vp[c, pl.ds(0, PADW), :] = jnp.zeros((PADW, 128), u32)

    x_copy(0).wait()
    block(lambda: [(lambda: None, 1)], lambda: [ln_job(g) for g in range(16)], 'ln0')
    w_copy(0, 0).wait()
    for r in range(8):
        if r + 1 < 8:
            x_copy(r + 1).wait()
        block(lambda r=r: qkv_tasks(0, 0, 0, (2 * r, 2 * r + 1)),
              lambda r=r: [ln_job((r + 1) * 16 + g) for g in range(16)] if r + 1 < 8 else [], 'q0')

    def qkv_block(j, m, jobs):
        slot = j % 2
        w_copy(j, slot).wait()

        @pl.when(j + 1 < 12)
        def _():
            w_copy(j + 1, 1 - slot).start()
        with jax.named_scope('qkv%d' % m):
            _weave(qkv_tasks(m, slot, (j % 4) * 2, range(16)), jobs)

    def q_body(j, c):
        qkv_block(j, 0, [t_job(jnp.minimum((j - 1) * 22 + a, 63)) for a in range(22)])
        return c
    lax.fori_loop(1, 4, q_body, 0)

    g_copy(0, 0).wait()
    u_copy(0, 0).wait()
    d_copy(0, 0).wait()
    g_copy(1, 1).start()
    u_copy(1, 1).start()

    def k_body(j, c):
        qkv_block(j, 1, [perm_job(0, (j - 4) * 32 + a) for a in range(32)])
        return c
    lax.fori_loop(4, 8, k_body, 0)

    def v_body(j, c):
        qkv_block(j, 2, [perm_job(1, (j - 8) * 32 + a) for a in range(32)])
        return c
    lax.fori_loop(8, 11, v_body, 0)
    w_copy(11, 1).wait()
    block(lambda: qkv_tasks(2, 1, 6, range(16)),
          lambda: _mix(b_jobs(0) + bd_jobs(0), [perm_job(1, 96 + a) for a in range(32)]), 'vlast')

    g_copy(1, 1).wait()
    u_copy(1, 1).wait()
    d_copy(1, 1).start()
    g_copy(2, 0).start()
    u_copy(2, 0).start()
    block(lambda: mm1_tasks(0, B0),
          lambda: _mix([perm_job(2, a) for a in range(128)],
                       b_jobs(1, 0, 8) + [zero_job(p) for p in range(25)]), 'f00')
    block(lambda: mm1_tasks(1, B0),
          lambda: _mix(_mix(comb_jobs(0), b_jobs(1, 8, 16) + [zero_job(p) for p in range(25, NP)]),
                       [attn_job(a) for a in range(NATT)]), 'f01')

    def slot(j, par, s):
        u = 2 * (j - 1) + s + 1
        if s == 0:
            d_copy(j, par).wait()
            g_copy(jnp.minimum(j + 1, NCH - 1), 1 - par).wait()
            u_copy(jnp.minimum(j + 1, NCH - 1), 1 - par).wait()

            @pl.when(j + 1 < NCH)
            def _():
                d_copy(j + 1, 1 - par).start()

            @pl.when(j + 2 < NCH)
            def _():
                g_copy(j + 2, par).start()
                u_copy(j + 2, par).start()
            if par == 1:
                @pl.when(j + 2 == NCH)
                def _():
                    for cp in wo_copies():
                        cp.start()

        def jobs():
            base = _mix(comb_jobs(1 - s), b_jobs(1 - par, 8 * s, 8 * s + 8) + bd_jobs(par, 4 * s, 4 * s + 4))
            att = []
            for a in range(NATT):
                att.append(attn_job(jnp.minimum(u * NATT + a, 127)))
                att.append(unperm_job(jnp.minimum((u - 1) * NATT + a, 127)))
            n0 = max(1, len(base) // 10)
            return base[:n0] + _mix(base[n0:-n0], att) + base[-n0:]
        block(lambda: _mix(mm1_tasks(s, Bs[par]), mm2_tasks(s, Bds[1 - par])), jobs, 'slot%d%d' % (par, s))

    def steady(it, c):
        j = 2 * it + 1
        slot(j, 1, 0)
        slot(j, 1, 1)
        slot(j + 1, 0, 0)
        slot(j + 1, 0, 1)
        return c
    lax.fori_loop(0, 3, steady, 0)

    block(lambda: _mix(wo_tasks(0), mm2_tasks(0, Bd0)),
          lambda: _mix(comb_jobs(1), [unperm_job(g) for g in range(12 * NATT, 128)]), 'e1')
    block(lambda: _mix(wo_tasks(1), mm2_tasks(1, Bd0)),
          lambda: [final_job(0, g, n) for g in range(RS // 16) for n in range(2)], 'e2')
    for a in range(4):
        out_copy(0, a, 0, 1).start()
    block(lambda: [(lambda: None, 1)],
          lambda: [final_job(1, g, n) for g in range(RS // 16) for n in range(2)], 'e3')
    for a in range(4):
        out_copy(1, a, 0, 1).start()
    for s in range(2):
        for a in range(4):
            out_copy(s, a, 0, 1).wait()


@jax.jit
def pallas_parallel_sum__sliding_local_dilated__glu_gated_bilinear__prompt_kernel(
    A_x: jax.Array,
    A_wqkv: jax.Array,
    A_wo: jax.Array,
    B_x: jax.Array,
    B_w_gate: jax.Array,
    B_w_up: jax.Array,
    B_w_down: jax.Array,
):
    del B_x
    x = A_x.reshape(S, D)
    hbm = pl.BlockSpec(memory_space=pl.ANY)
    dma = pltpu.SemaphoreType.DMA
    out = pl.pallas_call(
        _kernel,
        grid=(1,),
        in_specs=[pl.BlockSpec(memory_space=pltpu.SMEM)] + [hbm] * 6,
        out_specs=hbm,
        out_shape=jax.ShapeDtypeStruct((S, D), bf),
        scratch_shapes=[
            pltpu.VMEM((S, D), bf),
            pltpu.VMEM((S // 2, D), u32),
            pltpu.VMEM((NP, HB // 2, KB), u32),
            pltpu.VMEM((2, D, QW), bf),
            pltpu.VMEM((8, S // 2 + PADW, 128), u32),
            pltpu.VMEM((8, S // 2 + PADW, 128), u32),
            pltpu.VMEM((8, S // 2 + PADW, 128), u32),
            pltpu.VMEM((8, S // 2 + PADW, 128), u32),
            pltpu.VMEM((2, D, TF), bf),
            pltpu.VMEM((2, D, TF), bf),
            pltpu.VMEM((2, TF, D), bf),
            pltpu.VMEM((NP, KB // 2, 2 * TB), u32),
            pltpu.VMEM((NP, KB // 2, 2 * TB), u32),
            pltpu.VMEM((NP, TB // 2, KB), u32),
            pltpu.VMEM((NP, TB // 2, KB), u32),
            pltpu.VMEM((2, NP, 2, RS + MPAD, 128), f32),
            pltpu.VMEM((2, NP, RS // 2, TB), u32),
            pltpu.VMEM((4, 16, 24, 128), f32),
            pltpu.VMEM((NP, 2, HB + MPAD, 128), f32),
            dma((8,)), dma((2,)), dma((2,)), dma((2,)), dma((2,)), dma((8,)),
        ],
        compiler_params=pltpu.CompilerParams(
            dimension_semantics=("arbitrary",), vmem_limit_bytes=127 * 1024 * 1024),
        name="fused_attn_ffn",
    )(jnp.ones((1,), jnp.int32), x, A_wqkv, A_wo, B_w_gate, B_w_up, B_w_down)
    return out.reshape(1, S, D)
```

```python
import jax
import jax.numpy as jnp
from jax import lax
from jax.experimental import pallas as pl
from jax.experimental.pallas import tpu as pltpu

bf = jnp.bfloat16
f32 = jnp.float32
u32 = jnp.uint32

S, D, F = 2048, 1024, 3584
WIN = 8
NP = 49
HB = S // 4
KB = D // 4
TF = 512
TB = TF // 4
NCH = F // TF
RS = 128
NSUB = HB // RS
NT = NCH * NSUB
MPAD = 8
PADW = 8
QW = 256
EPS = 1e-5
C2 = float(32 ** -0.5 * 1.4426950408889634)
NATT = 5

A_T = [[(1, (0, 0)), (1, (1, 1))], [(1, (1, 0)), (1, (1, 1))], [(1, (0, 0))], [(1, (1, 1))],
       [(1, (0, 0)), (1, (0, 1))], [(1, (1, 0)), (-1, (0, 0))], [(1, (0, 1)), (-1, (1, 1))]]
B_T = [[(1, (0, 0)), (1, (1, 1))], [(1, (0, 0))], [(1, (0, 1)), (-1, (1, 1))], [(1, (1, 0)), (-1, (0, 0))],
       [(1, (1, 1))], [(1, (0, 0)), (1, (0, 1))], [(1, (1, 0)), (1, (1, 1))]]
C_T = {(0, 0): [(1, 0), (1, 3), (-1, 4), (1, 6)], (0, 1): [(1, 2), (1, 4)],
       (1, 0): [(1, 1), (1, 3)], (1, 1): [(1, 0), (-1, 1), (1, 2), (1, 5)]}
POS = ((0, 0), (0, 1), (1, 0), (1, 1))


def _comb(terms):
    acc = None
    for s, v in terms:
        if acc is None:
            acc = v if s > 0 else -v
        else:
            acc = acc + v if s > 0 else acc - v
    return acc


def _dot(a, b):
    return jnp.dot(a, b, preferred_element_type=f32)


def _pk(v):
    return pltpu.bitcast(v.astype(bf), u32)


def _up(w):
    return pltpu.bitcast(w, bf)


def _unpk(w):
    return pltpu.bitcast(w, bf).astype(f32)


def _as_f32(w):
    return lax.bitcast_convert_type(w, f32)


def _as_u32(v):
    return lax.bitcast_convert_type(v, u32)


def _mult(x, m):
    return x if isinstance(x, int) else pl.multiple_of(x, m)


def _opcomb(load, table, I, emit):
    sub = {(r, c): _comb([(s, load(q[0] * 2 + r, q[1] * 2 + c)) for s, q in table[I]])
           for r in range(2) for c in range(2)}
    for J, t2 in enumerate(table):
        emit(I * 7 + J, _pk(_comb([(s, sub[q]) for s, q in t2])))


def _opcomb_job(load, table, emit):
    return [(lambda I=I: _opcomb(load, table, I, emit)) for I in range(7)]


def _outpos(load, pos):
    inner = [_comb([(s, load(I * 7 + J)) for s, J in C_T[pos]]) for I in range(7)]
    return {q: _comb([(s, inner[I]) for s, I in terms]) for q, terms in C_T.items()}


def _perm8(v):
    lane = lax.broadcasted_iota(jnp.int32, v[0].shape, 1)
    v = list(v)
    for cb, lb in ((2, 4), (1, 3), (0, 2)):
        sh = 1 << lb
        hi = (lane & sh) != 0
        out = [None] * 8
        for c in range(8):
            if c & (1 << cb):
                continue
            x, y = v[c], v[c | (1 << cb)]
            out[c] = jnp.where(hi, pltpu.roll(y, sh, 1), x)
            out[c | (1 << cb)] = jnp.where(hi, y, pltpu.roll(x, 128 - sh, 1))
        v = out
    return v


def _sum4(x, lane):
    x = x + jnp.where((lane & 1) != 0, pltpu.roll(x, 1, 1), pltpu.roll(x, 127, 1))
    x = x + jnp.where((lane & 2) != 0, pltpu.roll(x, 2, 1), pltpu.roll(x, 126, 1))
    return x


def _mix(a, b):
    if not b:
        return list(a)
    if not a:
        return list(b)
    out, n, m, k = [], len(a), len(b), 0
    for i, t in enumerate(a):
        out.append(t)
        tgt = (i + 1) * m // n
        while k < tgt:
            out.append(b[k])
            k += 1
    return out


def _flat(jobs):
    return [t for j in jobs for t in j]


def _weave(mx, jobs):
    vp = _flat(jobs)
    tot = sum(c for _, c in mx)
    n, k, acc = len(vp), 0, 0
    for t, c in mx:
        t()
        acc += c
        tgt = acc * n // tot
        while k < tgt:
            vp[k]()
            k += 1
    while k < n:
        vp[k]()
        k += 1


def _kernel(one_ref, x_hbm, wqkv_hbm, wo_hbm, wg_hbm, wu_hbm, wd_hbm, out_hbm,
            xr, xn, T, wst, R, P, gst, ust, dst, B, Bd, M, H, hst, ost, acc,
            sem_x, sem_w, sem_g, sem_u, sem_d, sem_o):

    def block(mx, jobs, name="blk"):
        with jax.named_scope(name):
            @pl.when(one_ref[0] > 0)
            def _():
                _weave(mx(), jobs())

    def x_copy(r):
        rows = pl.ds(_mult(r * 256, 256), 256)
        return pltpu.make_async_copy(x_hbm.at[rows, :], xr.at[rows, :], sem_x.at[r])

    def w_copy(j, slot):
        return pltpu.make_async_copy(wqkv_hbm.at[:, pl.ds(_mult(j * QW, QW), QW)], wst.at[slot], sem_w.at[slot])

    def gu_copies(j, par):
        cols = pl.ds(_mult(j * TF, TF), TF)
        return (pltpu.make_async_copy(wg_hbm.at[:, cols], gst.at[par], sem_g.at[par]),
                pltpu.make_async_copy(wu_hbm.at[:, cols], ust.at[par], sem_u.at[par]))

    def d_copy(j, par):
        return pltpu.make_async_copy(wd_hbm.at[pl.ds(_mult(j * TF, TF), TF), :], dst.at[par], sem_d.at[par])

    def wo_copies():
        return (pltpu.make_async_copy(wo_hbm.at[:, pl.ds(0, TF)], gst.at[1], sem_g.at[1]),
                pltpu.make_async_copy(wo_hbm.at[:, pl.ds(TF, TF)], ust.at[1], sem_u.at[1]))

    def out_copy(i, a):
        par = i % 2
        return pltpu.make_async_copy(dst.at[par, pl.ds(a * RS, RS), :],
                                     out_hbm.at[pl.ds(_mult(a * HB + i * RS, RS), RS), :], sem_o.at[par * 4 + a])

    def start(cps):
        for cp in cps:
            cp.start()

    def wait(cps):
        for cp in cps:
            cp.wait()

    def ln_job(g):
        st = {}
        rows = pl.ds(_mult(g * 16, 16), 16)
        ld = lambda c: xr[rows, pl.ds(c * 128, 128)].astype(f32)

        def t_mean():
            a = ld(0)
            for c in range(1, 8):
                a = a + ld(c)
            st['m'] = jnp.sum(a, axis=1, keepdims=True) * (1.0 / D)

        def t_var():
            a = None
            for c in range(8):
                dlt = ld(c) - st['m']
                a = dlt * dlt if a is None else a + dlt * dlt
            st['r'] = lax.rsqrt(jnp.sum(a, axis=1, keepdims=True) * (1.0 / D) + EPS)

        def t_norm():
            for c in range(8):
                xn[pl.ds(_mult(g * 8, 8), 8), pl.ds(c * 128, 128)] = _pk((ld(c) - st['m']) * st['r'])
        return [t_mean, t_var, t_norm]

    def t_job(pos_idx):
        w0 = _mult((pos_idx // 2) * 8, 8)
        l0 = _mult((pos_idx % 2) * 128, 128)

        def load(i, j):
            return _unpk(xn[pl.ds(_mult(i * 256 + w0, 8), 8), pl.ds(_mult(j * KB + l0, 128), 128)])

        def emit(p, v):
            T[p, pl.ds(w0, 8), pl.ds(l0, 128)] = v
        return _opcomb_job(load, A_T, emit)

    def b_job(par, g, half):
        w_ref = (gst, ust)[half]

        def load(i, q):
            return w_ref[par, pl.ds(_mult(i * KB + g * 16, 16), 16), pl.ds(q * TB, TB)].astype(f32)

        def emit(p, v):
            B[par, p, pl.ds(_mult(g * 8, 8), 8), pl.ds(half * TB, TB)] = v
        return _opcomb_job(load, B_T, emit)

    def bd_job(par, g, n):
        def load(i, q):
            return dst[par, pl.ds(_mult(i * TB + g * 16, 16), 16), pl.ds(q * KB + n * 128, 128)].astype(f32)

        def emit(p, v):
            Bd[par, p, pl.ds(_mult(g * 8, 8), 8), pl.ds(n * 128, 128)] = v
        return _opcomb_job(load, B_T, emit)

    def b_jobs(par, k):
        return [b_job(par, 4 * k + g, h) for g in range(4) for h in range(2)]

    def bd_jobs(par, k):
        return [bd_job(par, 2 * k + g, n) for g in range(2) for n in range(2)]

    def perm_job(m, grp):
        def t():
            w = _mult(grp * 8, 8)
            r = _perm8([R[m % 2, c, pl.ds(w, 8), :] for c in range(8)])
            for c in range(8):
                P[m, c, pl.ds(_mult(PADW + w, 8), 8), :] = r[c]
        return [t]

    def attn_job(grp, sl):
        b = _mult(grp * 8, 8)
        job = []
        for h in range(2):
            st = {}
            half = lambda v, h=h: _unpk(v)[h * 8:(h + 1) * 8]

            def qk(cs, st=st, half=half):
                def t():
                    for c in cs:
                        qv = half(P[0, c, pl.ds(_mult(b + PADW, 8), 8), :])
                        for w in range(WIN):
                            kv = half(P[1, c, pl.ds(b + (PADW - w), 8), :])
                            st[w] = qv * kv if c == 0 else st[w] + qv * kv
                return t

            def sm(st=st, h=h):
                lane = lax.broadcasted_iota(jnp.int32, (8, 128), 1)
                row = lax.broadcasted_iota(jnp.int32, (8, 128), 0) + (grp * 16 + h * 8)
                ls = []
                for w in range(WIN):
                    a = _sum4(st[w], lane)
                    if w > 0:
                        a = jnp.where(row >= 2 * w, a, -1e30)
                    ls.append(a)
                m = ls[0]
                for w in range(1, WIN):
                    m = jnp.maximum(m, ls[w])
                e = [jnp.exp2((l - m) * C2) for l in ls]
                den = e[0]
                for w in range(1, WIN):
                    den = den + e[w]
                inv = 1.0 / den
                st['p'] = [x * inv for x in e]

            def pv(cs, st=st, half=half, h=h):
                def t():
                    for c in cs:
                        o = None
                        for w in range(WIN):
                            a = st['p'][w] * half(P[2, c, pl.ds(b + (PADW - w), 8), :])
                            o = a if o is None else o + a
                        ost[sl, c, pl.ds(h * 8, 8), :] = o
                return t
            job += [qk((c, c + 1)) for c in range(0, 8, 2)] + [sm] + [pv((c, c + 1)) for c in range(0, 8, 2)]

        def fin():
            r = _perm8([_pk(ost[sl, c, pl.ds(0, 16), :]) for c in range(8)])
            for c in range(8):
                xn[pl.ds(b, 8), pl.ds(c * 128, 128)] = r[c]
        return job + [fin]

    def comb_job(mp, g):
        sl = g % 4
        job = []
        for hf in range(2):
            for pos in POS:
                def t(hf=hf, pos=pos):
                    r = pl.ds(g * 16 + hf * 8, 8)
                    gg = _outpos(lambda p: M[mp, p, 0, r, :], pos)
                    uu = _outpos(lambda p: M[mp, p, 1, r, :], pos)
                    for q in gg:
                        hst[sl, (q[0] * 2 + pos[0]) * 4 + q[1] * 2 + pos[1], pl.ds(hf * 8, 8), :] = gg[q] * uu[q]
                job.append(t)

        def emit(p, v):
            H[mp, p, pl.ds(g * 8, 8), :] = v
        return job + _opcomb_job(lambda i, j: hst[sl, i * 4 + j, pl.ds(0, 16), :], A_T, emit)

    def comb_jobs(mp):
        return [comb_job(mp, g) for g in range(RS // 16)]

    def zero_job(p):
        def t():
            for c in range(2):
                acc[p, c, pl.ds(0, HB), :] = jnp.zeros((HB, 128), f32)
        return [t]

    def final_job(i, g, n):
        job = []
        par = i % 2
        for pos in POS:
            def t(pos=pos):
                r0 = _mult(i * RS + g * 16, 16)
                o = [_outpos(lambda p: acc[p, n, pl.ds(r0 + hf * 8, 8), :], pos) for hf in range(2)]
                for q in o[0]:
                    a = q[0] * 2 + pos[0]
                    ch = (q[1] * 2 + pos[1]) * 2 + n
                    pln = a * 8 + ch
                    cols = pl.ds(ch * 128, 128)
                    ffn = jnp.concatenate([o[0][q], o[1][q]], axis=0)
                    att = M[par, pln // 2, pln % 2, pl.ds(g * 16, 16), :]
                    res = xr[pl.ds(_mult(a * HB + r0, 16), 16), cols].astype(f32) + att + ffn
                    dst[par, pl.ds(a * RS + g * 16, 16), cols] = res.astype(bf)
            job.append(t)
        return job

    def final_jobs(i):
        return [final_job(i, g, n) for g in range(RS // 16) for n in range(2)]

    def qkv_tasks(m, slot, cbase, pieces):
        out = []
        for r in pieces:
            for ct in range(QW // 128):
                def t(r=r, ct=ct):
                    res = _dot(_up(xn[pl.ds(_mult(r * 64, 64), 64), :]), wst[slot, :, pl.ds(ct * 128, 128)])
                    for k in range(8):
                        R[m % 2, cbase + ct, pl.ds(_mult(r * 64 + k * 8, 8), 8), :] = _pk(res[k * 16:(k + 1) * 16])
                out.append((t, 256))
        return out

    def mm1_tasks(mp, s, par):
        out = []
        for p in range(NP):
            for h in range(RS // 64):
                def t(p=p, h=h):
                    r = _dot(_up(T[p, pl.ds(_mult(s * (RS // 2) + h * 32, 32), 32), :]), _up(B[par, p]))
                    for c in range(2):
                        M[mp, p, c, pl.ds(h * 64, 64), :] = r[:, c * 128:(c + 1) * 128]
                out.append((t, 64))
        return out

    def mm2_tasks(mp, s, par):
        out = []
        for p in range(NP):
            def t(p=p):
                r = _dot(_up(H[mp, p]), _up(Bd[par, p]))
                for c in range(2):
                    acc[p, c, pl.ds(_mult(s * RS, RS), RS), :] += r[:, c * 128:(c + 1) * 128]
            out.append((t, 64))
        return out

    def wo_tasks(i):
        out = []
        for a in range(4):
            for ch in range(8):
                def t(a=a, ch=ch):
                    w_ref = (gst, ust)[ch // 4]
                    res = _dot(_up(xn[pl.ds(_mult(a * 256 + i * 64, 64), 64), :]),
                               w_ref[1, :, pl.ds((ch % 4) * 128, 128)])
                    pln = a * 8 + ch
                    M[i % 2, pln // 2, pln % 2, pl.ds(0, RS), :] = res
                out.append((t, 256))
        return out

    nothing = lambda: [(lambda: None, 1)]

    x_copy(0).start()
    w_copy(0, 0).start()
    for c in range(8):
        P[1, c, pl.ds(0, PADW), :] = jnp.zeros((PADW, 128), u32)
        P[2, c, pl.ds(0, PADW), :] = jnp.zeros((PADW, 128), u32)
    x_copy(0).wait()
    x_copy(1).start()
    x_copy(2).start()
    block(nothing, lambda: [ln_job(g) for g in range(16)], 'ln0')
    w_copy(0, 0).wait()

    def p0_body(r, c):
        @pl.when(r + 3 < 8)
        def _():
            x_copy(r + 3).start()

        @pl.when(r == 4)
        def _():
            w_copy(1, 1).start()

        @pl.when(r + 1 < 8)
        def _():
            x_copy(r + 1).wait()
        with jax.named_scope('q0'):
            for t, _ in qkv_tasks(0, 0, 0, (2 * r, 2 * r + 1)):
                t()
            rn = jnp.minimum(r + 1, 7)
            for t in _flat([ln_job(rn * 16 + g) for g in range(16)]):
                t()
        return c
    lax.fori_loop(0, 8, p0_body, 0)

    start(gu_copies(0, 0))
    d_copy(0, 0).start()
    start(gu_copies(1, 1))
    d_copy(1, 1).start()

    def qkv_block(j, m, jobs):
        slot = j % 2
        w_copy(j, slot).wait()

        @pl.when(j + 1 < 12)
        def _():
            w_copy(j + 1, 1 - slot).start()
        with jax.named_scope('qkv'):
            _weave(qkv_tasks(m, slot, (j % 4) * 2, range(16)), jobs)

    def q_body(j, c):
        qkv_block(j, 0, [t_job(jnp.minimum((j - 1) * 22 + a, 63)) for a in range(22)])
        return c
    lax.fori_loop(1, 4, q_body, 0)

    wait(gu_copies(0, 0))
    d_copy(0, 0).wait()

    def kv_body(j, c):
        i = j - 4
        m = j // 4
        extra = ([b_job(0, 2 * i + g, h) for g in range(2) for h in range(2)]
                 + [bd_job(0, i // 2, i % 2)]
                 + [zero_job(jnp.minimum(i * 7 + a, NP - 1)) for a in range(7)])
        qkv_block(j, m, _mix([perm_job(m - 1, (i % 4) * 32 + a) for a in range(32)], extra))
        return c
    lax.fori_loop(4, 12, kv_body, 0)

    wait(gu_copies(1, 1))
    start(gu_copies(2, 0))
    block(lambda: mm1_tasks(0, 0, 0),
          lambda: _mix([perm_job(2, a) for a in range(32)], b_jobs(1, 0) + bd_jobs(0, 2)), 'f0')
    block(lambda: mm1_tasks(1, 1, 0),
          lambda: _mix(_mix(comb_jobs(0), b_jobs(1, 1) + bd_jobs(0, 3)),
                       [perm_job(2, 32 + a) for a in range(32)]), 'f1')

    def slot(t, mp):
        j = t // 4
        s = t % 4
        par = j % 2
        if mp == 0:
            @pl.when(jnp.logical_and(s == 0, j > 0))
            def _():
                wait(gu_copies(jnp.minimum(j + 1, NCH - 1), 1 - par))

                @pl.when(j + 2 < NCH)
                def _():
                    start(gu_copies(j + 2, par))

                @pl.when(j + 2 == NCH)
                def _():
                    start(wo_copies())

            @pl.when(jnp.logical_and(s == 2, j + 1 < NCH))
            def _():
                d_copy(j + 1, 1 - par).wait()

                @pl.when(j + 2 < NCH)
                def _():
                    d_copy(j + 2, par).start()
        jd = (t + 2) // 4
        kd = (t + 2) % 4
        u = t - 2

        def jobs():
            base = _mix(comb_jobs(1 - mp), b_jobs(1 - par, s) + bd_jobs(jd % 2, kd))
            att = []
            for a in range(NATT):
                att.append(attn_job(jnp.minimum(u * NATT + a, 127), a % 4))
                att.append(perm_job(2, jnp.minimum(64 + u * NATT + a, 127)))
            n0 = max(1, len(base) // 10)
            return base[:n0] + _mix(base[n0:-n0], att) + base[-n0:]
        block(lambda: _mix(mm1_tasks(mp, s, par), mm2_tasks(mp, (t - 2) % 4, ((t - 2) // 4) % 2)), jobs,
              'slot%d' % mp)

    def steady(it, c):
        slot(2 * it + 2, 0)
        slot(2 * it + 3, 1)
        return c
    lax.fori_loop(0, (NT - 2) // 2, steady, 0)

    block(lambda: mm2_tasks(0, 2, 0), lambda: comb_jobs(1), 'e0')
    block(lambda: _mix(wo_tasks(0), mm2_tasks(1, 3, 0)), lambda: [], 'e1')

    def wo_body(i, c):
        @pl.when(i >= 3)
        def _():
            wait([out_copy(i - 3, a) for a in range(4)])
        with jax.named_scope('wo'):
            _weave(wo_tasks(i), final_jobs(i - 1))
        start([out_copy(i - 1, a) for a in range(4)])
        return c
    lax.fori_loop(1, 4, wo_body, 0)
    wait([out_copy(1, a) for a in range(4)])
    block(nothing, lambda: final_jobs(3), 'e3')
    start([out_copy(3, a) for a in range(4)])
    wait([out_copy(2, a) for a in range(4)])
    wait([out_copy(3, a) for a in range(4)])


@jax.jit
def pallas_parallel_sum__sliding_local_dilated__glu_gated_bilinear__prompt_kernel(
    A_x: jax.Array,
    A_wqkv: jax.Array,
    A_wo: jax.Array,
    B_x: jax.Array,
    B_w_gate: jax.Array,
    B_w_up: jax.Array,
    B_w_down: jax.Array,
):
    del B_x
    x = A_x.reshape(S, D)
    hbm = pl.BlockSpec(memory_space=pl.ANY)
    dma = pltpu.SemaphoreType.DMA
    out = pl.pallas_call(
        _kernel,
        grid=(1,),
        in_specs=[pl.BlockSpec(memory_space=pltpu.SMEM)] + [hbm] * 6,
        out_specs=hbm,
        out_shape=jax.ShapeDtypeStruct((S, D), bf),
        scratch_shapes=[
            pltpu.VMEM((S, D), bf),
            pltpu.VMEM((S // 2, D), u32),
            pltpu.VMEM((NP, HB // 2, KB), u32),
            pltpu.VMEM((2, D, QW), bf),
            pltpu.VMEM((2, 8, S // 2 + PADW, 128), u32),
            pltpu.VMEM((3, 8, S // 2 + PADW, 128), u32),
            pltpu.VMEM((2, D, TF), bf),
            pltpu.VMEM((2, D, TF), bf),
            pltpu.VMEM((2, TF, D), bf),
            pltpu.VMEM((2, NP, KB // 2, 2 * TB), u32),
            pltpu.VMEM((2, NP, TB // 2, KB), u32),
            pltpu.VMEM((2, NP, 2, RS + MPAD, 128), f32),
            pltpu.VMEM((2, NP, RS // 2, TB), u32),
            pltpu.VMEM((4, 16, 24, 128), f32),
            pltpu.VMEM((4, 8, 24, 128), f32),
            pltpu.VMEM((NP, 2, HB + MPAD, 128), f32),
            dma((8,)), dma((2,)), dma((2,)), dma((2,)), dma((2,)), dma((8,)),
        ],
        compiler_params=pltpu.CompilerParams(
            dimension_semantics=("arbitrary",), vmem_limit_bytes=127 * 1024 * 1024),
        name="fused_attn_ffn",
    )(jnp.ones((1,), jnp.int32), x, A_wqkv, A_wo, B_w_gate, B_w_up, B_w_down)
    return out.reshape(1, S, D)
```

```python
import jax
import jax.numpy as jnp
from jax import lax
from jax.experimental import pallas as pl
from jax.experimental.pallas import tpu as pltpu

bf = jnp.bfloat16
f32 = jnp.float32
u32 = jnp.uint32

S, D, F = 2048, 1024, 3584
WIN = 8
NP = 49
HB = S // 4
KB = D // 4
TF = 512
TB = TF // 4
NCH = F // TF
RS = 128
NSUB = HB // RS
NT = NCH * NSUB
MPAD = 8
PADW = 8
QW = 256
EPS = 1e-5
C2 = float(32 ** -0.5 * 1.4426950408889634)
NATT = 5
NATT0 = 1

A_T = [[(1, (0, 0)), (1, (1, 1))], [(1, (1, 0)), (1, (1, 1))], [(1, (0, 0))], [(1, (1, 1))],
       [(1, (0, 0)), (1, (0, 1))], [(1, (1, 0)), (-1, (0, 0))], [(1, (0, 1)), (-1, (1, 1))]]
B_T = [[(1, (0, 0)), (1, (1, 1))], [(1, (0, 0))], [(1, (0, 1)), (-1, (1, 1))], [(1, (1, 0)), (-1, (0, 0))],
       [(1, (1, 1))], [(1, (0, 0)), (1, (0, 1))], [(1, (1, 0)), (1, (1, 1))]]
C_T = {(0, 0): [(1, 0), (1, 3), (-1, 4), (1, 6)], (0, 1): [(1, 2), (1, 4)],
       (1, 0): [(1, 1), (1, 3)], (1, 1): [(1, 0), (-1, 1), (1, 2), (1, 5)]}
POS = ((0, 0), (0, 1), (1, 0), (1, 1))


def _comb(terms):
    acc = None
    for s, v in terms:
        if acc is None:
            acc = v if s > 0 else -v
        else:
            acc = acc + v if s > 0 else acc - v
    return acc


def _dot(a, b):
    return jnp.dot(a, b, preferred_element_type=f32)


def _pk(v):
    return pltpu.bitcast(v.astype(bf), u32)


def _up(w):
    return pltpu.bitcast(w, bf)


def _unpk(w):
    return pltpu.bitcast(w, bf).astype(f32)


def _as_f32(w):
    return lax.bitcast_convert_type(w, f32)


def _as_u32(v):
    return lax.bitcast_convert_type(v, u32)


def _mult(x, m):
    return x if isinstance(x, int) else pl.multiple_of(x, m)


def _opcomb(load, table, I, emit):
    sub = {(r, c): _comb([(s, load(q[0] * 2 + r, q[1] * 2 + c)) for s, q in table[I]])
           for r in range(2) for c in range(2)}
    for J, t2 in enumerate(table):
        emit(I * 7 + J, _pk(_comb([(s, sub[q]) for s, q in t2])))


def _opcomb_job(load, table, emit):
    return [(lambda I=I: _opcomb(load, table, I, emit)) for I in range(7)]


def _outpos(load, pos):
    inner = [_comb([(s, load(I * 7 + J)) for s, J in C_T[pos]]) for I in range(7)]
    return {q: _comb([(s, inner[I]) for s, I in terms]) for q, terms in C_T.items()}


def _perm8(v):
    lane = lax.broadcasted_iota(jnp.int32, v[0].shape, 1)
    v = list(v)
    for cb, lb in ((2, 4), (1, 3), (0, 2)):
        sh = 1 << lb
        hi = (lane & sh) != 0
        out = [None] * 8
        for c in range(8):
            if c & (1 << cb):
                continue
            x, y = v[c], v[c | (1 << cb)]
            out[c] = jnp.where(hi, pltpu.roll(y, sh, 1), x)
            out[c | (1 << cb)] = jnp.where(hi, y, pltpu.roll(x, 128 - sh, 1))
        v = out
    return v


def _sum4(x, lane):
    x = x + jnp.where((lane & 1) != 0, pltpu.roll(x, 1, 1), pltpu.roll(x, 127, 1))
    x = x + jnp.where((lane & 2) != 0, pltpu.roll(x, 2, 1), pltpu.roll(x, 126, 1))
    return x


def _mix(a, b):
    if not b:
        return list(a)
    if not a:
        return list(b)
    out, n, m, k = [], len(a), len(b), 0
    for i, t in enumerate(a):
        out.append(t)
        tgt = (i + 1) * m // n
        while k < tgt:
            out.append(b[k])
            k += 1
    return out


def _flat(jobs):
    return [t for j in jobs for t in j]


def _weave(mx, jobs):
    vp = _flat(jobs)
    tot = sum(c for _, c in mx)
    n, k, acc = len(vp), 0, 0
    for t, c in mx:
        t()
        acc += c
        tgt = acc * n // tot
        while k < tgt:
            vp[k]()
            k += 1
    while k < n:
        vp[k]()
        k += 1


def _kernel(one_ref, x_hbm, wqkv_hbm, wo_hbm, wg_hbm, wu_hbm, wd_hbm, out_hbm,
            xr, xn, T, wst, wqr, wqp, R, P, gst, ust, dst, B, Bd, M, H, hst, ost, acc,
            sem_x, sem_w, sem_q, sem_g, sem_u, sem_d, sem_o):

    def block(mx, jobs, name="blk"):
        with jax.named_scope(name):
            @pl.when(one_ref[0] > 0)
            def _():
                _weave(mx(), jobs())

    def x_copy(r):
        rows = pl.ds(_mult(r * 256, 256), 256)
        return pltpu.make_async_copy(x_hbm.at[rows, :], xr.at[rows, :], sem_x.at[r])

    def w_copy(j, slot):
        col = (2 - j // 4) * D + (j % 4) * QW
        return pltpu.make_async_copy(wqkv_hbm.at[:, pl.ds(_mult(col, QW), QW)], wst.at[slot], sem_w.at[slot])

    def wq_copy():
        return pltpu.make_async_copy(wqkv_hbm.at[:, pl.ds(0, D)], wqr, sem_q.at[0])

    def gu_copies(j, par):
        cols = pl.ds(_mult(j * TF, TF), TF)
        return (pltpu.make_async_copy(wg_hbm.at[:, cols], gst.at[par], sem_g.at[par]),
                pltpu.make_async_copy(wu_hbm.at[:, cols], ust.at[par], sem_u.at[par]))

    def d_copy(j, par):
        return pltpu.make_async_copy(wd_hbm.at[pl.ds(_mult(j * TF, TF), TF), :], dst.at[par], sem_d.at[par])

    def wo_copies():
        return (pltpu.make_async_copy(wo_hbm.at[:, pl.ds(0, TF)], gst.at[1], sem_g.at[1]),
                pltpu.make_async_copy(wo_hbm.at[:, pl.ds(TF, TF)], ust.at[1], sem_u.at[1]))

    def out_copy(i, a):
        par = i % 2
        return pltpu.make_async_copy(dst.at[par, pl.ds(a * RS, RS), :],
                                     out_hbm.at[pl.ds(_mult(a * HB + i * RS, RS), RS), :], sem_o.at[par * 4 + a])

    def start(cps):
        for cp in cps:
            cp.start()

    def wait(cps):
        for cp in cps:
            cp.wait()

    def ln_job(g):
        def t():
            v = [xr[pl.ds(g * 16, 16), pl.ds(c * 128, 128)].astype(f32) for c in range(8)]
            a = v[0]
            for c in range(1, 8):
                a = a + v[c]
            mean = jnp.sum(a, axis=1, keepdims=True) * (1.0 / D)
            v = [x - mean for x in v]
            a = v[0] * v[0]
            for c in range(1, 8):
                a = a + v[c] * v[c]
            r = lax.rsqrt(jnp.sum(a, axis=1, keepdims=True) * (1.0 / D) + EPS)
            for c in range(8):
                xn[pl.ds(g * 8, 8), pl.ds(c * 128, 128)] = _pk(v[c] * r)
        return [t]

    def ln_jobs(r):
        return [ln_job(r * 16 + g) for g in range(16)]

    def t_job(pos_idx):
        w0 = _mult((pos_idx // 2) * 8, 8)
        l0 = _mult((pos_idx % 2) * 128, 128)

        def load(i, j):
            return _unpk(xn[pl.ds(_mult(i * 256 + w0, 8), 8), pl.ds(_mult(j * KB + l0, 128), 128)])

        def emit(p, v):
            T[p, pl.ds(w0, 8), pl.ds(l0, 128)] = v
        return _opcomb_job(load, A_T, emit)

    def b_job(par, g, half):
        w_ref = (gst, ust)[half]

        def load(i, q):
            return w_ref[par, pl.ds(_mult(i * KB + g * 16, 16), 16), pl.ds(q * TB, TB)].astype(f32)

        def emit(p, v):
            B[par, p, pl.ds(_mult(g * 8, 8), 8), pl.ds(half * TB, TB)] = v
        return _opcomb_job(load, B_T, emit)

    def bd_job(par, g, n):
        def load(i, q):
            return dst[par, pl.ds(_mult(i * TB + g * 16, 16), 16), pl.ds(q * KB + n * 128, 128)].astype(f32)

        def emit(p, v):
            Bd[par, p, pl.ds(_mult(g * 8, 8), 8), pl.ds(n * 128, 128)] = v
        return _opcomb_job(load, B_T, emit)

    def b_jobs(par, k):
        return [b_job(par, 4 * k + g, h) for g in range(4) for h in range(2)]

    def bd_jobs(par, k):
        return [bd_job(par, 2 * k + g, n) for g in range(2) for n in range(2)]

    def perm_job(m, grp):
        def t():
            w = _mult(grp * 8, 8)
            r = _perm8([R[2 - m, c, pl.ds(w, 8), :] for c in range(8)])
            for c in range(8):
                P[m, c, pl.ds(_mult(PADW + w, 8), 8), :] = r[c]
        return [t]

    def wq_job(grp):
        def t():
            rows = pl.ds(_mult(grp * 16, 16), 16)
            r = _perm8([pltpu.bitcast(wqr[rows, pl.ds(c * 128, 128)], u32) for c in range(8)])
            for c in range(8):
                wqp[pl.ds(_mult(grp * 8, 8), 8), pl.ds(c * 128, 128)] = r[c]
        return [t]

    def attn_job(grp, sl):
        b = _mult(grp * 8, 8)
        job = []
        for h in range(2):
            st = {}
            half = lambda v, h=h: _unpk(v)[h * 8:(h + 1) * 8]

            def qk(cs, st=st, half=half):
                def t():
                    for c in cs:
                        qv = half(P[0, c, pl.ds(_mult(b + PADW, 8), 8), :])
                        for w in range(WIN):
                            kv = half(P[1, c, pl.ds(b + (PADW - w), 8), :])
                            st[w] = qv * kv if c == 0 else st[w] + qv * kv
                return t

            def sm(st=st, h=h):
                lane = lax.broadcasted_iota(jnp.int32, (8, 128), 1)
                row = lax.broadcasted_iota(jnp.int32, (8, 128), 0) + (grp * 16 + h * 8)
                ls = []
                for w in range(WIN):
                    a = _sum4(st[w], lane)
                    if w > 0:
                        a = jnp.where(row >= 2 * w, a, -1e30)
                    ls.append(a)
                m = ls[0]
                for w in range(1, WIN):
                    m = jnp.maximum(m, ls[w])
                e = [jnp.exp2((l - m) * C2) for l in ls]
                den = e[0]
                for w in range(1, WIN):
                    den = den + e[w]
                inv = 1.0 / den
                st['p'] = [x * inv for x in e]

            def pv(cs, st=st, half=half, h=h):
                def t():
                    for c in cs:
                        o = None
                        for w in range(WIN):
                            a = st['p'][w] * half(P[2, c, pl.ds(b + (PADW - w), 8), :])
                            o = a if o is None else o + a
                        ost[sl, c, pl.ds(h * 8, 8), :] = o
                return t
            job += [qk((0, 1, 2, 3)), qk((4, 5, 6, 7)), sm, pv((0, 1, 2, 3)), pv((4, 5, 6, 7))]

        def fin():
            r = _perm8([_pk(ost[sl, c, pl.ds(0, 16), :]) for c in range(8)])
            for c in range(8):
                xn[pl.ds(b, 8), pl.ds(c * 128, 128)] = r[c]
        return job + [fin]

    def comb_job(mp, g):
        sl = g % 4
        job = []
        for hf in range(2):
            for pos in POS:
                def t(hf=hf, pos=pos):
                    r = pl.ds(g * 16 + hf * 8, 8)
                    gg = _outpos(lambda p: M[mp, p, 0, r, :], pos)
                    uu = _outpos(lambda p: M[mp, p, 1, r, :], pos)
                    for q in gg:
                        hst[sl, (q[0] * 2 + pos[0]) * 4 + q[1] * 2 + pos[1], pl.ds(hf * 8, 8), :] = gg[q] * uu[q]
                job.append(t)

        def emit(p, v):
            H[mp, p, pl.ds(g * 8, 8), :] = v
        return job + _opcomb_job(lambda i, j: hst[sl, i * 4 + j, pl.ds(0, 16), :], A_T, emit)

    def comb_jobs(mp):
        return [comb_job(mp, g) for g in range(RS // 16)]

    def zero_job(p):
        def t():
            for c in range(2):
                acc[p, c, pl.ds(0, HB), :] = jnp.zeros((HB, 128), f32)
        return [t]

    def final_job(i, g, n):
        job = []
        par = i % 2
        for pos in POS:
            def t(pos=pos):
                r0 = _mult(i * RS + g * 16, 16)
                o = [_outpos(lambda p: acc[p, n, pl.ds(r0 + hf * 8, 8), :], pos) for hf in range(2)]
                for q in o[0]:
                    a = q[0] * 2 + pos[0]
                    ch = (q[1] * 2 + pos[1]) * 2 + n
                    pln = a * 8 + ch
                    cols = pl.ds(ch * 128, 128)
                    ffn = jnp.concatenate([o[0][q], o[1][q]], axis=0)
                    att = M[par, pln // 2, pln % 2, pl.ds(g * 16, 16), :]
                    res = xr[pl.ds(_mult(a * HB + r0, 16), 16), cols].astype(f32) + att + ffn
                    dst[par, pl.ds(a * RS + g * 16, 16), cols] = res.astype(bf)
            job.append(t)
        return job

    def final_jobs(i):
        return [final_job(i, g, n) for g in range(RS // 16) for n in range(2)]

    def kv_tasks(m, slot, cbase, pieces):
        out = []
        for r in pieces:
            for ct in range(QW // 128):
                def t(r=r, ct=ct):
                    res = _dot(_up(xn[pl.ds(_mult(r * 64, 64), 64), :]), wst[slot, :, pl.ds(ct * 128, 128)])
                    for k in range(8):
                        R[2 - m, cbase + ct, pl.ds(_mult(r * 64 + k * 8, 8), 8), :] = _pk(res[k * 16:(k + 1) * 16])
                out.append((t, 256))
        return out

    def q_tasks(cbase):
        out = []
        for r in range(16):
            for ct in range(QW // 128):
                def t(r=r, ct=ct):
                    res = _dot(_up(xn[pl.ds(r * 64, 64), :]),
                               _up(wqp[:, pl.ds(_mult((cbase + ct) * 128, 128), 128)]))
                    for k in range(8):
                        P[0, cbase + ct, pl.ds(PADW + r * 64 + k * 8, 8), :] = _pk(res[k * 16:(k + 1) * 16])
                out.append((t, 256))
        return out

    def mm1_tasks(mp, s, par):
        out = []
        for p in range(NP):
            def t(p=p):
                r = _dot(_up(T[p, pl.ds(_mult(s * (RS // 2), RS // 2), RS // 2), :]), _up(B[par, p]))
                for c in range(2):
                    M[mp, p, c, pl.ds(0, RS), :] = r[:, c * 128:(c + 1) * 128]
            out.append((t, 128))
        return out

    def mm2_tasks(mp, s, par):
        out = []
        for p in range(NP):
            def t(p=p):
                r = _dot(_up(H[mp, p]), _up(Bd[par, p]))
                for c in range(2):
                    acc[p, c, pl.ds(_mult(s * RS, RS), RS), :] += r[:, c * 128:(c + 1) * 128]
            out.append((t, 64))
        return out

    def wo_tasks(i):
        out = []
        for a in range(4):
            for ch in range(8):
                def t(a=a, ch=ch):
                    w_ref = (gst, ust)[ch // 4]
                    res = _dot(_up(xn[pl.ds(_mult(a * 256 + i * 64, 64), 64), :]),
                               w_ref[1, :, pl.ds((ch % 4) * 128, 128)])
                    pln = a * 8 + ch
                    M[i % 2, pln // 2, pln % 2, pl.ds(0, RS), :] = res
                out.append((t, 256))
        return out

    nothing = lambda: [(lambda: None, 1)]

    x_copy(0).start()
    w_copy(0, 0).start()
    for c in range(8):
        P[1, c, pl.ds(0, PADW), :] = jnp.zeros((PADW, 128), u32)
        P[2, c, pl.ds(0, PADW), :] = jnp.zeros((PADW, 128), u32)
    x_copy(0).wait()
    w_copy(1, 1).start()
    x_copy(1).start()
    block(nothing, lambda: ln_jobs(0), 'ln0')
    w_copy(0, 0).wait()

    for r in range(8):
        if r + 2 < 8:
            x_copy(r + 2).start()
        if r == 0:
            block(lambda: kv_tasks(2, 0, 0, (0, 1)), lambda: [], 'p0')
            w_copy(1, 1).wait()
        if r == 5:
            w_copy(2, 2).start()
            wq_copy().start()
        if r + 1 < 8:
            x_copy(r + 1).wait()
        block(lambda r=r: (kv_tasks(2, 0, 0, (2 * r, 2 * r + 1)) if r > 0 else [])
              + kv_tasks(2, 1, 2, (2 * r, 2 * r + 1)),
              lambda r=r: ln_jobs(r + 1) if r + 1 < 8 else [], 'p0')

    def kv_block(j, m, after_start, jobs, name):
        slot = j % 3
        w_copy(j, slot).wait()

        @pl.when(j + 1 < 8)
        def _():
            w_copy(j + 1, (j + 1) % 3).start()
        after_start()
        with jax.named_scope(name):
            _weave(kv_tasks(m, slot, (j % 4) * 2, range(16)), jobs)

    def v_body(j, c):
        def dmas():
            @pl.when(j == 2)
            def _():
                start(gu_copies(0, 0))

            @pl.when(j == 3)
            def _():
                d_copy(0, 0).start()
                d_copy(1, 1).start()
        kv_block(j, 2, dmas, _mix([wq_job((j - 2) * 32 + a) for a in range(32)],
                                  [t_job((j - 2) * 8 + a) for a in range(8)]), 'v')
        return c
    wq_copy().wait()
    lax.fori_loop(2, 4, v_body, 0)

    def k_body(j, c):
        def dmas():
            @pl.when(j == 4)
            def _():
                start(gu_copies(1, 1))
        i = j - 4
        kv_block(j, 1, dmas, _mix([perm_job(2, i * 32 + a) for a in range(32)],
                                  [t_job(16 + i * 12 + a) for a in range(12)]), 'k')
        return c
    lax.fori_loop(4, 8, k_body, 0)

    wait(gu_copies(0, 0))
    d_copy(0, 0).wait()

    def q_body(i, c):
        extra = ([b_job(0, 4 * i + g, h) for g in range(4) for h in range(2)]
                 + [bd_job(0, i, n) for n in range(2)]
                 + [zero_job(jnp.minimum(i * 13 + a, NP - 1)) for a in range(13)])
        with jax.named_scope('q'):
            _weave(q_tasks(i * 2), _mix([perm_job(1, i * 32 + a) for a in range(32)], extra))
        return c
    lax.fori_loop(0, 4, q_body, 0)

    wait(gu_copies(1, 1))
    start(gu_copies(2, 0))
    block(lambda: mm1_tasks(0, 0, 0),
          lambda: _mix([attn_job(a, a % 4) for a in range(NATT0)], b_jobs(1, 0) + bd_jobs(0, 2)), 'f0')
    block(lambda: mm1_tasks(1, 1, 0),
          lambda: _mix(_mix(comb_jobs(0), b_jobs(1, 1) + bd_jobs(0, 3)),
                       [attn_job(NATT0 + a, a % 4) for a in range(NATT0)]), 'f1')

    def slot(t, mp):
        j = t // 4
        s = t % 4
        par = j % 2
        if mp == 0:
            @pl.when(jnp.logical_and(s == 0, j > 0))
            def _():
                wait(gu_copies(jnp.minimum(j + 1, NCH - 1), 1 - par))

                @pl.when(j + 2 < NCH)
                def _():
                    start(gu_copies(j + 2, par))

                @pl.when(j + 2 == NCH)
                def _():
                    start(wo_copies())

            @pl.when(jnp.logical_and(s == 2, j + 1 < NCH))
            def _():
                d_copy(j + 1, 1 - par).wait()

                @pl.when(j + 2 < NCH)
                def _():
                    d_copy(j + 2, par).start()
        jd = (t + 2) // 4
        kd = (t + 2) % 4
        u = t - 2

        def jobs():
            base = _mix(comb_jobs(1 - mp), b_jobs(1 - par, s) + bd_jobs(jd % 2, kd))
            att = []
            for a in range(NATT):
                att.append(attn_job(jnp.minimum(2 * NATT0 + u * NATT + a, 127), a % 4))
            n0 = max(1, len(base) // 10)
            return base[:n0] + _mix(base[n0:-n0], att) + base[-n0:]
        block(lambda: _mix(mm1_tasks(mp, s, par), mm2_tasks(mp, (t - 2) % 4, ((t - 2) // 4) % 2)), jobs,
              'slot%d' % mp)

    def steady(it, c):
        slot(2 * it + 2, 0)
        slot(2 * it + 3, 1)
        return c
    lax.fori_loop(0, (NT - 2) // 2, steady, 0)

    block(lambda: mm2_tasks(0, 2, 0), lambda: comb_jobs(1), 'e0')
    block(lambda: _mix(wo_tasks(0), mm2_tasks(1, 3, 0)), lambda: [], 'e1')

    def wo_body(i, c):
        @pl.when(i >= 3)
        def _():
            wait([out_copy(i - 3, a) for a in range(4)])
        with jax.named_scope('wo'):
            _weave(wo_tasks(i), final_jobs(i - 1))
        start([out_copy(i - 1, a) for a in range(4)])
        return c
    lax.fori_loop(1, 4, wo_body, 0)
    wait([out_copy(1, a) for a in range(4)])
    block(nothing, lambda: final_jobs(3), 'e3')
    start([out_copy(3, a) for a in range(4)])
    wait([out_copy(2, a) for a in range(4)])
    wait([out_copy(3, a) for a in range(4)])


@jax.jit
def pallas_parallel_sum__sliding_local_dilated__glu_gated_bilinear__prompt_kernel(
    A_x: jax.Array,
    A_wqkv: jax.Array,
    A_wo: jax.Array,
    B_x: jax.Array,
    B_w_gate: jax.Array,
    B_w_up: jax.Array,
    B_w_down: jax.Array,
):
    del B_x
    x = A_x.reshape(S, D)
    hbm = pl.BlockSpec(memory_space=pl.ANY)
    dma = pltpu.SemaphoreType.DMA
    out = pl.pallas_call(
        _kernel,
        grid=(1,),
        in_specs=[pl.BlockSpec(memory_space=pltpu.SMEM)] + [hbm] * 6,
        out_specs=hbm,
        out_shape=jax.ShapeDtypeStruct((S, D), bf),
        scratch_shapes=[
            pltpu.VMEM((S, D), bf),
            pltpu.VMEM((S // 2, D), u32),
            pltpu.VMEM((NP, HB // 2, KB), u32),
            pltpu.VMEM((3, D, QW), bf),
            pltpu.VMEM((D, D), bf),
            pltpu.VMEM((D // 2, D), u32),
            pltpu.VMEM((2, 8, S // 2 + PADW, 128), u32),
            pltpu.VMEM((3, 8, S // 2 + PADW, 128), u32),
            pltpu.VMEM((2, D, TF), bf),
            pltpu.VMEM((2, D, TF), bf),
            pltpu.VMEM((2, TF, D), bf),
            pltpu.VMEM((2, NP, KB // 2, 2 * TB), u32),
            pltpu.VMEM((2, NP, TB // 2, KB), u32),
            pltpu.VMEM((2, NP, 2, RS + MPAD, 128), f32),
            pltpu.VMEM((2, NP, RS // 2, TB), u32),
            pltpu.VMEM((4, 16, 24, 128), f32),
            pltpu.VMEM((4, 8, 24, 128), f32),
            pltpu.VMEM((NP, 2, HB + MPAD, 128), f32),
            dma((8,)), dma((3,)), dma((1,)), dma((2,)), dma((2,)), dma((2,)), dma((8,)),
        ],
        compiler_params=pltpu.CompilerParams(
            dimension_semantics=("arbitrary",), vmem_limit_bytes=127 * 1024 * 1024),
        name="fused_attn_ffn",
    )(jnp.ones((1,), jnp.int32), x, A_wqkv, A_wo, B_w_gate, B_w_up, B_w_down)
    return out.reshape(1, S, D)
```

```python
import jax
import jax.numpy as jnp
from jax import lax
from jax.experimental import pallas as pl
from jax.experimental.pallas import tpu as pltpu

bf = jnp.bfloat16
f32 = jnp.float32
u32 = jnp.uint32

S, D, F = 2048, 1024, 3584
WIN = 8
NP = 49
HB = S // 4
KB = D // 4
TF = 512
TB = TF // 4
NCH = F // TF
RS = 128
NSUB = HB // RS
NT = NCH * NSUB
MPAD = 8
PADW = 8
QW = 256
EPS = 1e-5
C2 = float(32 ** -0.5 * 1.4426950408889634)
NATT = 5
NATT0 = 1

A_T = [[(1, (0, 0)), (1, (1, 1))], [(1, (1, 0)), (1, (1, 1))], [(1, (0, 0))], [(1, (1, 1))],
       [(1, (0, 0)), (1, (0, 1))], [(1, (1, 0)), (-1, (0, 0))], [(1, (0, 1)), (-1, (1, 1))]]
B_T = [[(1, (0, 0)), (1, (1, 1))], [(1, (0, 0))], [(1, (0, 1)), (-1, (1, 1))], [(1, (1, 0)), (-1, (0, 0))],
       [(1, (1, 1))], [(1, (0, 0)), (1, (0, 1))], [(1, (1, 0)), (1, (1, 1))]]
C_T = {(0, 0): [(1, 0), (1, 3), (-1, 4), (1, 6)], (0, 1): [(1, 2), (1, 4)],
       (1, 0): [(1, 1), (1, 3)], (1, 1): [(1, 0), (-1, 1), (1, 2), (1, 5)]}
POS = ((0, 0), (0, 1), (1, 0), (1, 1))


def _comb(terms):
    acc = None
    for s, v in terms:
        if acc is None:
            acc = v if s > 0 else -v
        else:
            acc = acc + v if s > 0 else acc - v
    return acc


def _dot(a, b):
    return jnp.dot(a, b, preferred_element_type=f32)


def _pk(v):
    return pltpu.bitcast(v.astype(bf), u32)


def _up(w):
    return pltpu.bitcast(w, bf)


def _unpk(w):
    return pltpu.bitcast(w, bf).astype(f32)


def _as_f32(w):
    return lax.bitcast_convert_type(w, f32)


def _as_u32(v):
    return lax.bitcast_convert_type(v, u32)


def _mult(x, m):
    return x if isinstance(x, int) else pl.multiple_of(x, m)


def _opcomb(load, table, I, emit):
    sub = {(r, c): _comb([(s, load(q[0] * 2 + r, q[1] * 2 + c)) for s, q in table[I]])
           for r in range(2) for c in range(2)}
    for J, t2 in enumerate(table):
        emit(I * 7 + J, _pk(_comb([(s, sub[q]) for s, q in t2])))


def _opcomb_job(load, table, emit):
    return [(lambda I=I: _opcomb(load, table, I, emit)) for I in range(7)]


def _outpos(load, pos):
    inner = [_comb([(s, load(I * 7 + J)) for s, J in C_T[pos]]) for I in range(7)]
    return {q: _comb([(s, inner[I]) for s, I in terms]) for q, terms in C_T.items()}


def _perm8(v):
    lane = lax.broadcasted_iota(jnp.int32, v[0].shape, 1)
    v = list(v)
    for cb, lb in ((2, 4), (1, 3), (0, 2)):
        sh = 1 << lb
        hi = (lane & sh) != 0
        out = [None] * 8
        for c in range(8):
            if c & (1 << cb):
                continue
            x, y = v[c], v[c | (1 << cb)]
            out[c] = jnp.where(hi, pltpu.roll(y, sh, 1), x)
            out[c | (1 << cb)] = jnp.where(hi, y, pltpu.roll(x, 128 - sh, 1))
        v = out
    return v


def _sum4(x, lane):
    x = x + jnp.where((lane & 1) != 0, pltpu.roll(x, 1, 1), pltpu.roll(x, 127, 1))
    x = x + jnp.where((lane & 2) != 0, pltpu.roll(x, 2, 1), pltpu.roll(x, 126, 1))
    return x


def _mix(a, b):
    if not b:
        return list(a)
    if not a:
        return list(b)
    out, n, m, k = [], len(a), len(b), 0
    for i, t in enumerate(a):
        out.append(t)
        tgt = (i + 1) * m // n
        while k < tgt:
            out.append(b[k])
            k += 1
    return out


def _flat(jobs):
    return [t for j in jobs for t in j]


def _weave(mx, jobs):
    vp = _flat(jobs)
    tot = sum(c for _, c in mx)
    n, k, acc = len(vp), 0, 0
    for t, c in mx:
        t()
        acc += c
        tgt = acc * n // tot
        while k < tgt:
            vp[k]()
            k += 1
    while k < n:
        vp[k]()
        k += 1


def _kernel(one_ref, x_hbm, wqkv_hbm, wo_hbm, wg_hbm, wu_hbm, wd_hbm, out_hbm,
            xr, xn, T, wst, wqr, wqp, R, P, gst, ust, dst, B, Bd, M, H, hst, ost, acc,
            sem_x, sem_w, sem_q, sem_g, sem_u, sem_d, sem_o):

    def block(mx, jobs, name="blk"):
        with jax.named_scope(name):
            @pl.when(one_ref[0] > 0)
            def _():
                _weave(mx(), jobs())

    def x_copy(r):
        rows = pl.ds(_mult(r * 256, 256), 256)
        return pltpu.make_async_copy(x_hbm.at[rows, :], xr.at[rows, :], sem_x.at[r])

    def w_copy(j, slot):
        col = (2 - j // 4) * D + (j % 4) * QW
        return pltpu.make_async_copy(wqkv_hbm.at[:, pl.ds(_mult(col, QW), QW)], wst.at[slot], sem_w.at[slot])

    def wq_copy():
        return pltpu.make_async_copy(wqkv_hbm.at[:, pl.ds(0, D)], wqr, sem_q.at[0])

    def gu_copies(j, par):
        cols = pl.ds(_mult(j * TF, TF), TF)
        return (pltpu.make_async_copy(wg_hbm.at[:, cols], gst.at[par], sem_g.at[par]),
                pltpu.make_async_copy(wu_hbm.at[:, cols], ust.at[par], sem_u.at[par]))

    def d_copy(j, par):
        return pltpu.make_async_copy(wd_hbm.at[pl.ds(_mult(j * TF, TF), TF), :], dst.at[par], sem_d.at[par])

    def wo_copies():
        return (pltpu.make_async_copy(wo_hbm.at[:, pl.ds(0, TF)], gst.at[1], sem_g.at[1]),
                pltpu.make_async_copy(wo_hbm.at[:, pl.ds(TF, TF)], ust.at[1], sem_u.at[1]))

    def out_copy(i, a):
        par = i % 2
        return pltpu.make_async_copy(dst.at[par, pl.ds(a * RS, RS), :],
                                     out_hbm.at[pl.ds(_mult(a * HB + i * RS, RS), RS), :], sem_o.at[par * 4 + a])

    def start(cps):
        for cp in cps:
            cp.start()

    def wait(cps):
        for cp in cps:
            cp.wait()

    def ln_job(g):
        def t():
            v = [xr[pl.ds(g * 16, 16), pl.ds(c * 128, 128)].astype(f32) for c in range(8)]
            a = v[0]
            for c in range(1, 8):
                a = a + v[c]
            mean = jnp.sum(a, axis=1, keepdims=True) * (1.0 / D)
            v = [x - mean for x in v]
            a = v[0] * v[0]
            for c in range(1, 8):
                a = a + v[c] * v[c]
            r = lax.rsqrt(jnp.sum(a, axis=1, keepdims=True) * (1.0 / D) + EPS)
            for c in range(8):
                xn[pl.ds(g * 8, 8), pl.ds(c * 128, 128)] = _pk(v[c] * r)
        return [t]

    def ln_jobs(r):
        return [ln_job(r * 16 + g) for g in range(16)]

    def t_job(pos_idx):
        w0 = _mult((pos_idx // 2) * 8, 8)
        l0 = _mult((pos_idx % 2) * 128, 128)

        def load(i, j):
            return _unpk(xn[pl.ds(_mult(i * 256 + w0, 8), 8), pl.ds(_mult(j * KB + l0, 128), 128)])

        def emit(p, v):
            T[p, pl.ds(w0, 8), pl.ds(l0, 128)] = v
        return _opcomb_job(load, A_T, emit)

    def b_job(par, g, half):
        w_ref = (gst, ust)[half]

        def load(i, q):
            return w_ref[par, pl.ds(_mult(i * KB + g * 16, 16), 16), pl.ds(q * TB, TB)].astype(f32)

        def emit(p, v):
            B[par, p, pl.ds(_mult(g * 8, 8), 8), pl.ds(half * TB, TB)] = v
        return _opcomb_job(load, B_T, emit)

    def bd_job(par, g, n):
        def load(i, q):
            return dst[par, pl.ds(_mult(i * TB + g * 16, 16), 16), pl.ds(q * KB + n * 128, 128)].astype(f32)

        def emit(p, v):
            Bd[par, p, pl.ds(_mult(g * 8, 8), 8), pl.ds(n * 128, 128)] = v
        return _opcomb_job(load, B_T, emit)

    def b_jobs(par, k):
        return [b_job(par, 4 * k + g, h) for g in range(4) for h in range(2)]

    def bd_jobs(par, k):
        return [bd_job(par, 2 * k + g, n) for g in range(2) for n in range(2)]

    def perm_job(m, grp):
        def t():
            w = _mult(grp * 8, 8)
            r = _perm8([R[2 - m, c, pl.ds(w, 8), :] for c in range(8)])
            for c in range(8):
                P[m, c, pl.ds(_mult(PADW + w, 8), 8), :] = r[c]
        return [t]

    def wq_job(grp):
        def t():
            rows = pl.ds(_mult(grp * 16, 16), 16)
            r = _perm8([pltpu.bitcast(wqr[rows, pl.ds(c * 128, 128)], u32) for c in range(8)])
            for c in range(8):
                wqp[pl.ds(_mult(grp * 8, 8), 8), pl.ds(c * 128, 128)] = r[c]
        return [t]

    def attn_job(grp, sl):
        b = _mult(grp * 8, 8)
        job = []
        for h in range(2):
            st = {}
            half = lambda v, h=h: _unpk(v)[h * 8:(h + 1) * 8]

            def qk(cs, st=st, half=half):
                def t():
                    for c in cs:
                        qv = half(P[0, c, pl.ds(_mult(b + PADW, 8), 8), :])
                        for w in range(WIN):
                            kv = half(P[1, c, pl.ds(b + (PADW - w), 8), :])
                            st[w] = qv * kv if c == 0 else st[w] + qv * kv
                return t

            def sm(st=st, h=h):
                lane = lax.broadcasted_iota(jnp.int32, (8, 128), 1)
                row = lax.broadcasted_iota(jnp.int32, (8, 128), 0) + (grp * 16 + h * 8)
                ls = []
                for w in range(WIN):
                    a = _sum4(st[w], lane)
                    if w > 0:
                        a = jnp.where(row >= 2 * w, a, -1e30)
                    ls.append(a)
                m = ls[0]
                for w in range(1, WIN):
                    m = jnp.maximum(m, ls[w])
                e = [jnp.exp2((l - m) * C2) for l in ls]
                den = e[0]
                for w in range(1, WIN):
                    den = den + e[w]
                inv = 1.0 / den
                st['p'] = [x * inv for x in e]

            def pv(cs, st=st, half=half, h=h):
                def t():
                    for c in cs:
                        o = None
                        for w in range(WIN):
                            a = st['p'][w] * half(P[2, c, pl.ds(b + (PADW - w), 8), :])
                            o = a if o is None else o + a
                        ost[sl, c, pl.ds(h * 8, 8), :] = o
                return t
            job += [qk((0, 1, 2, 3)), qk((4, 5, 6, 7)), sm, pv((0, 1, 2, 3)), pv((4, 5, 6, 7))]

        def fin():
            r = _perm8([_pk(ost[sl, c, pl.ds(0, 16), :]) for c in range(8)])
            for c in range(8):
                xn[pl.ds(b, 8), pl.ds(c * 128, 128)] = r[c]
        return job + [fin]

    def comb_job(mp, g):
        sl = g % 4
        job = []
        for hf in range(2):
            for pos in POS:
                def t(hf=hf, pos=pos):
                    r = pl.ds(g * 16 + hf * 8, 8)
                    gg = _outpos(lambda p: M[mp, p, 0, r, :], pos)
                    uu = _outpos(lambda p: M[mp, p, 1, r, :], pos)
                    for q in gg:
                        hst[sl, (q[0] * 2 + pos[0]) * 4 + q[1] * 2 + pos[1], pl.ds(hf * 8, 8), :] = gg[q] * uu[q]
                job.append(t)

        def emit(p, v):
            H[mp, p, pl.ds(g * 8, 8), :] = v
        return job + _opcomb_job(lambda i, j: hst[sl, i * 4 + j, pl.ds(0, 16), :], A_T, emit)

    def comb_jobs(mp):
        return [comb_job(mp, g) for g in range(RS // 16)]

    def zero_job(p):
        def t():
            for c in range(2):
                acc[p, c, pl.ds(0, HB), :] = jnp.zeros((HB, 128), f32)
        return [t]

    def final_job(i, g, n):
        job = []
        par = i % 2
        for pos in POS:
            def t(pos=pos):
                r0 = _mult(i * RS + g * 16, 16)
                o = [_outpos(lambda p: acc[p, n, pl.ds(r0 + hf * 8, 8), :], pos) for hf in range(2)]
                for q in o[0]:
                    a = q[0] * 2 + pos[0]
                    ch = (q[1] * 2 + pos[1]) * 2 + n
                    pln = a * 8 + ch
                    cols = pl.ds(ch * 128, 128)
                    ffn = jnp.concatenate([o[0][q], o[1][q]], axis=0)
                    att = M[par, pln // 2, pln % 2, pl.ds(g * 16, 16), :]
                    res = xr[pl.ds(_mult(a * HB + r0, 16), 16), cols].astype(f32) + att + ffn
                    dst[par, pl.ds(a * RS + g * 16, 16), cols] = res.astype(bf)
            job.append(t)
        return job

    def final_jobs(i):
        return [final_job(i, g, n) for g in range(RS // 16) for n in range(2)]

    def kv_tasks(m, slot, cbase, pieces):
        out = []
        for r in pieces:
            for ct in range(QW // 128):
                def t(r=r, ct=ct):
                    res = _dot(_up(xn[pl.ds(_mult(r * 64, 64), 64), :]), wst[slot, :, pl.ds(ct * 128, 128)])
                    for k in range(8):
                        R[2 - m, cbase + ct, pl.ds(_mult(r * 64 + k * 8, 8), 8), :] = _pk(res[k * 16:(k + 1) * 16])
                out.append((t, 256))
        return out

    def q_tasks(cbase):
        out = []
        for r in range(16):
            for ct in range(QW // 128):
                def t(r=r, ct=ct):
                    res = _dot(_up(xn[pl.ds(r * 64, 64), :]),
                               _up(wqp[:, pl.ds(_mult((cbase + ct) * 128, 128), 128)]))
                    for k in range(8):
                        P[0, cbase + ct, pl.ds(PADW + r * 64 + k * 8, 8), :] = _pk(res[k * 16:(k + 1) * 16])
                out.append((t, 256))
        return out

    def mm1_tasks(mp, s, par):
        out = []
        for p in range(NP):
            def t(p=p):
                r = _dot(_up(T[p, pl.ds(_mult(s * (RS // 2), RS // 2), RS // 2), :]), _up(B[par, p]))
                for c in range(2):
                    M[mp, p, c, pl.ds(0, RS), :] = r[:, c * 128:(c + 1) * 128]
            out.append((t, 128))
        return out

    def mm2_tasks(mp, s, par):
        out = []
        for p in range(NP):
            def t(p=p):
                r = _dot(_up(H[mp, p]), _up(Bd[par, p]))
                for c in range(2):
                    acc[p, c, pl.ds(_mult(s * RS, RS), RS), :] += r[:, c * 128:(c + 1) * 128]
            out.append((t, 64))
        return out

    def wo_tasks(i):
        out = []
        for a in range(4):
            for ch in range(8):
                def t(a=a, ch=ch):
                    w_ref = (gst, ust)[ch // 4]
                    res = _dot(_up(xn[pl.ds(_mult(a * 256 + i * 64, 64), 64), :]),
                               w_ref[1, :, pl.ds((ch % 4) * 128, 128)])
                    pln = a * 8 + ch
                    M[i % 2, pln // 2, pln % 2, pl.ds(0, RS), :] = res
                out.append((t, 256))
        return out

    nothing = lambda: [(lambda: None, 1)]

    x_copy(0).start()
    w_copy(0, 0).start()
    for c in range(8):
        P[1, c, pl.ds(0, PADW), :] = jnp.zeros((PADW, 128), u32)
        P[2, c, pl.ds(0, PADW), :] = jnp.zeros((PADW, 128), u32)
    x_copy(0).wait()
    w_copy(1, 1).start()
    x_copy(1).start()
    block(nothing, lambda: ln_jobs(0), 'ln0')
    w_copy(0, 0).wait()

    for r in range(8):
        if r + 2 < 8:
            x_copy(r + 2).start()
        if r == 0:
            block(lambda: kv_tasks(2, 0, 0, (0, 1)), lambda: [], 'p0')
            w_copy(1, 1).wait()
        if r == 5:
            w_copy(2, 2).start()
            wq_copy().start()
        if r + 1 < 8:
            x_copy(r + 1).wait()
        block(lambda r=r: (kv_tasks(2, 0, 0, (2 * r, 2 * r + 1)) if r > 0 else [])
              + kv_tasks(2, 1, 2, (2 * r, 2 * r + 1)),
              lambda r=r: ln_jobs(r + 1) if r + 1 < 8 else [], 'p0')

    def kv_block(j, m, after_start, jobs, name):
        slot = j % 3
        w_copy(j, slot).wait()

        @pl.when(j + 1 < 8)
        def _():
            w_copy(j + 1, (j + 1) % 3).start()
        after_start()
        block(lambda: kv_tasks(m, slot, (j % 4) * 2, range(16)), jobs, name)

    def v_body(j, c):
        def dmas():
            @pl.when(j == 2)
            def _():
                start(gu_copies(0, 0))

            @pl.when(j == 3)
            def _():
                d_copy(0, 0).start()
                d_copy(1, 1).start()
        kv_block(j, 2, dmas, lambda: _mix([wq_job((j - 2) * 32 + a) for a in range(32)],
                                          [t_job((j - 2) * 8 + a) for a in range(8)]), 'v')
        return c
    wq_copy().wait()
    lax.fori_loop(2, 4, v_body, 0)

    def k_body(j, c):
        def dmas():
            @pl.when(j == 4)
            def _():
                start(gu_copies(1, 1))
        i = j - 4
        kv_block(j, 1, dmas, lambda: _mix([perm_job(2, i * 32 + a) for a in range(32)],
                                          [t_job(16 + i * 12 + a) for a in range(12)]), 'k')
        return c
    lax.fori_loop(4, 8, k_body, 0)

    wait(gu_copies(0, 0))
    d_copy(0, 0).wait()

    def q_body(i, c):
        def jobs():
            extra = ([b_job(0, 4 * i + g, h) for g in range(4) for h in range(2)]
                     + [bd_job(0, i, n) for n in range(2)]
                     + [zero_job(jnp.minimum(i * 13 + a, NP - 1)) for a in range(13)])
            return _mix([perm_job(1, i * 32 + a) for a in range(32)], extra)
        block(lambda: q_tasks(i * 2), jobs, 'q')
        return c
    lax.fori_loop(0, 4, q_body, 0)

    wait(gu_copies(1, 1))
    start(gu_copies(2, 0))
    block(lambda: mm1_tasks(0, 0, 0),
          lambda: _mix([attn_job(a, a % 4) for a in range(NATT0)], b_jobs(1, 0) + bd_jobs(0, 2)), 'f0')
    block(lambda: mm1_tasks(1, 1, 0),
          lambda: _mix(_mix(comb_jobs(0), b_jobs(1, 1) + bd_jobs(0, 3)),
                       [attn_job(NATT0 + a, a % 4) for a in range(NATT0)]), 'f1')

    def slot(t, mp):
        j = t // 4
        s = t % 4
        par = j % 2
        if mp == 0:
            @pl.when(jnp.logical_and(s == 0, j > 0))
            def _():
                wait(gu_copies(jnp.minimum(j + 1, NCH - 1), 1 - par))

                @pl.when(j + 2 < NCH)
                def _():
                    start(gu_copies(j + 2, par))

                @pl.when(j + 2 == NCH)
                def _():
                    start(wo_copies())

            @pl.when(jnp.logical_and(s == 2, j + 1 < NCH))
            def _():
                d_copy(j + 1, 1 - par).wait()

                @pl.when(j + 2 < NCH)
                def _():
                    d_copy(j + 2, par).start()
        jd = (t + 2) // 4
        kd = (t + 2) % 4
        u = t - 2

        def jobs():
            base = _mix(comb_jobs(1 - mp), b_jobs(1 - par, s) + bd_jobs(jd % 2, kd))
            att = []
            for a in range(NATT):
                att.append(attn_job(jnp.minimum(2 * NATT0 + u * NATT + a, 127), a % 4))
            n0 = max(1, len(base) // 10)
            return base[:n0] + _mix(base[n0:-n0], att) + base[-n0:]
        block(lambda: _mix(mm1_tasks(mp, s, par), mm2_tasks(mp, (t - 2) % 4, ((t - 2) // 4) % 2)), jobs,
              'slot%d' % mp)

    def steady(it, c):
        slot(2 * it + 2, 0)
        slot(2 * it + 3, 1)
        return c
    lax.fori_loop(0, (NT - 2) // 2, steady, 0)

    block(lambda: mm2_tasks(0, 2, 0), lambda: comb_jobs(1), 'e0')
    block(lambda: _mix(wo_tasks(0), mm2_tasks(1, 3, 0)), lambda: [], 'e1')

    def wo_body(i, c):
        @pl.when(i >= 3)
        def _():
            wait([out_copy(i - 3, a) for a in range(4)])
        block(lambda: wo_tasks(i), lambda: final_jobs(i - 1), 'wo')
        start([out_copy(i - 1, a) for a in range(4)])
        return c
    lax.fori_loop(1, 4, wo_body, 0)
    wait([out_copy(1, a) for a in range(4)])
    block(nothing, lambda: final_jobs(3), 'e3')
    start([out_copy(3, a) for a in range(4)])
    wait([out_copy(2, a) for a in range(4)])
    wait([out_copy(3, a) for a in range(4)])


@jax.jit
def pallas_parallel_sum__sliding_local_dilated__glu_gated_bilinear__prompt_kernel(
    A_x: jax.Array,
    A_wqkv: jax.Array,
    A_wo: jax.Array,
    B_x: jax.Array,
    B_w_gate: jax.Array,
    B_w_up: jax.Array,
    B_w_down: jax.Array,
):
    del B_x
    x = A_x.reshape(S, D)
    hbm = pl.BlockSpec(memory_space=pl.ANY)
    dma = pltpu.SemaphoreType.DMA
    out = pl.pallas_call(
        _kernel,
        grid=(1,),
        in_specs=[pl.BlockSpec(memory_space=pltpu.SMEM)] + [hbm] * 6,
        out_specs=hbm,
        out_shape=jax.ShapeDtypeStruct((S, D), bf),
        scratch_shapes=[
            pltpu.VMEM((S, D), bf),
            pltpu.VMEM((S // 2, D), u32),
            pltpu.VMEM((NP, HB // 2, KB), u32),
            pltpu.VMEM((3, D, QW), bf),
            pltpu.VMEM((D, D), bf),
            pltpu.VMEM((D // 2, D), u32),
            pltpu.VMEM((2, 8, S // 2 + PADW, 128), u32),
            pltpu.VMEM((3, 8, S // 2 + PADW, 128), u32),
            pltpu.VMEM((2, D, TF), bf),
            pltpu.VMEM((2, D, TF), bf),
            pltpu.VMEM((2, TF, D), bf),
            pltpu.VMEM((2, NP, KB // 2, 2 * TB), u32),
            pltpu.VMEM((2, NP, TB // 2, KB), u32),
            pltpu.VMEM((2, NP, 2, RS + MPAD, 128), f32),
            pltpu.VMEM((2, NP, RS // 2, TB), u32),
            pltpu.VMEM((4, 16, 24, 128), f32),
            pltpu.VMEM((4, 8, 24, 128), f32),
            pltpu.VMEM((NP, 2, HB + MPAD, 128), f32),
            dma((8,)), dma((3,)), dma((1,)), dma((2,)), dma((2,)), dma((2,)), dma((8,)),
        ],
        compiler_params=pltpu.CompilerParams(
            dimension_semantics=("arbitrary",), vmem_limit_bytes=127 * 1024 * 1024),
        name="fused_attn_ffn",
    )(jnp.ones((1,), jnp.int32), x, A_wqkv, A_wo, B_w_gate, B_w_up, B_w_down)
    return out.reshape(1, S, D)
```

```python
import jax
import jax.numpy as jnp
from jax import lax
from jax.experimental import pallas as pl
from jax.experimental.pallas import tpu as pltpu

bf = jnp.bfloat16
f32 = jnp.float32
u32 = jnp.uint32

S, D, F = 2048, 1024, 3584
WIN = 8
NP = 49
HB = S // 4
KB = D // 4
TF = 512
TB = TF // 4
NCH = F // TF
RS = 128
NSUB = HB // RS
NT = NCH * NSUB
MPAD = 8
PADW = 8
QW = 256
EPS = 1e-5
C2 = float(32 ** -0.5 * 1.4426950408889634)
NATT = 5
NATT0 = 1

A_T = [[(1, (0, 0)), (1, (1, 1))], [(1, (1, 0)), (1, (1, 1))], [(1, (0, 0))], [(1, (1, 1))],
       [(1, (0, 0)), (1, (0, 1))], [(1, (1, 0)), (-1, (0, 0))], [(1, (0, 1)), (-1, (1, 1))]]
B_T = [[(1, (0, 0)), (1, (1, 1))], [(1, (0, 0))], [(1, (0, 1)), (-1, (1, 1))], [(1, (1, 0)), (-1, (0, 0))],
       [(1, (1, 1))], [(1, (0, 0)), (1, (0, 1))], [(1, (1, 0)), (1, (1, 1))]]
C_T = {(0, 0): [(1, 0), (1, 3), (-1, 4), (1, 6)], (0, 1): [(1, 2), (1, 4)],
       (1, 0): [(1, 1), (1, 3)], (1, 1): [(1, 0), (-1, 1), (1, 2), (1, 5)]}
POS = ((0, 0), (0, 1), (1, 0), (1, 1))


def _comb(terms):
    acc = None
    for s, v in terms:
        if acc is None:
            acc = v if s > 0 else -v
        else:
            acc = acc + v if s > 0 else acc - v
    return acc


def _dot(a, b):
    return jnp.dot(a, b, preferred_element_type=f32)


def _pk(v):
    return pltpu.bitcast(v.astype(bf), u32)


def _up(w):
    return pltpu.bitcast(w, bf)


def _unpk(w):
    return pltpu.bitcast(w, bf).astype(f32)


def _as_f32(w):
    return lax.bitcast_convert_type(w, f32)


def _as_u32(v):
    return lax.bitcast_convert_type(v, u32)


def _mult(x, m):
    return x if isinstance(x, int) else pl.multiple_of(x, m)


def _opcomb(load, table, I, emit, raw):
    sub = {(r, c): _comb([(s, load(q[0] * 2 + r, q[1] * 2 + c)) for s, q in table[I]])
           for r in range(2) for c in range(2)}
    for J, t2 in enumerate(table):
        if raw is not None and len(table[I]) == 1 and len(t2) == 1:
            qo, qi = table[I][0][1], t2[0][1]
            emit(I * 7 + J, raw(qo[0] * 2 + qi[0], qo[1] * 2 + qi[1]))
        else:
            emit(I * 7 + J, _pk(_comb([(s, sub[q]) for s, q in t2])))


def _opcomb_job(load, table, emit, raw=None):
    return [(lambda I=I: _opcomb(load, table, I, emit, raw)) for I in range(7)]


def _outpos(load, pos):
    inner = [_comb([(s, load(I * 7 + J)) for s, J in C_T[pos]]) for I in range(7)]
    return {q: _comb([(s, inner[I]) for s, I in terms]) for q, terms in C_T.items()}


def _perm8(v):
    lane = lax.broadcasted_iota(jnp.int32, v[0].shape, 1)
    v = list(v)
    for cb, lb in ((2, 4), (1, 3), (0, 2)):
        sh = 1 << lb
        hi = (lane & sh) != 0
        out = [None] * 8
        for c in range(8):
            if c & (1 << cb):
                continue
            x, y = v[c], v[c | (1 << cb)]
            out[c] = jnp.where(hi, pltpu.roll(y, sh, 1), x)
            out[c | (1 << cb)] = jnp.where(hi, y, pltpu.roll(x, 128 - sh, 1))
        v = out
    return v


def _sum4(x, lane):
    x = x + jnp.where((lane & 1) != 0, pltpu.roll(x, 1, 1), pltpu.roll(x, 127, 1))
    x = x + jnp.where((lane & 2) != 0, pltpu.roll(x, 2, 1), pltpu.roll(x, 126, 1))
    return x


def _mix(a, b):
    if not b:
        return list(a)
    if not a:
        return list(b)
    out, n, m, k = [], len(a), len(b), 0
    for i, t in enumerate(a):
        out.append(t)
        tgt = (i + 1) * m // n
        while k < tgt:
            out.append(b[k])
            k += 1
    return out


def _flat(jobs):
    return [t for j in jobs for t in j]


def _weave(mx, jobs):
    vp = _flat(jobs)
    tot = sum(c for _, c in mx)
    n, k, acc = len(vp), 0, 0
    for t, c in mx:
        t()
        acc += c
        tgt = acc * n // tot
        while k < tgt:
            vp[k]()
            k += 1
    while k < n:
        vp[k]()
        k += 1


def _kernel(one_ref, x_hbm, wqkv_hbm, wo_hbm, wg_hbm, wu_hbm, wd_hbm, out_hbm,
            xr, xn, T, wst, wqr, wqp, R, P, gst, ust, dst, B, Bd, M, H, hst, ost, acc,
            sem_x, sem_w, sem_q, sem_g, sem_u, sem_d, sem_o):

    def block(mx, jobs, name="blk"):
        with jax.named_scope(name):
            @pl.when(one_ref[0] > 0)
            def _():
                _weave(mx(), jobs())

    def x_copy(r):
        rows = pl.ds(_mult(r * 256, 256), 256)
        return pltpu.make_async_copy(x_hbm.at[rows, :], xr.at[rows, :], sem_x.at[r])

    def w_copy(j, slot):
        col = (2 - j // 4) * D + (j % 4) * QW
        return pltpu.make_async_copy(wqkv_hbm.at[:, pl.ds(_mult(col, QW), QW)], wst.at[slot], sem_w.at[slot])

    def wq_copy():
        return pltpu.make_async_copy(wqkv_hbm.at[:, pl.ds(0, D)], wqr, sem_q.at[0])

    def gu_copies(j, par):
        cols = pl.ds(_mult(j * TF, TF), TF)
        return (pltpu.make_async_copy(wg_hbm.at[:, cols], gst.at[par], sem_g.at[par]),
                pltpu.make_async_copy(wu_hbm.at[:, cols], ust.at[par], sem_u.at[par]))

    def d_copy(j, par):
        return pltpu.make_async_copy(wd_hbm.at[pl.ds(_mult(j * TF, TF), TF), :], dst.at[par], sem_d.at[par])

    def wo_copies():
        return (pltpu.make_async_copy(wo_hbm.at[:, pl.ds(0, TF)], gst.at[1], sem_g.at[1]),
                pltpu.make_async_copy(wo_hbm.at[:, pl.ds(TF, TF)], ust.at[1], sem_u.at[1]))

    def out_copy(i, a):
        par = i % 2
        return pltpu.make_async_copy(dst.at[par, pl.ds(a * RS, RS), :],
                                     out_hbm.at[pl.ds(_mult(a * HB + i * RS, RS), RS), :], sem_o.at[par * 4 + a])

    def last_copy(a, h):
        rows = RS // 2
        return pltpu.make_async_copy(dst.at[1, pl.ds(a * RS + h * rows, rows), :],
                                     out_hbm.at[pl.ds(a * HB + 3 * RS + h * rows, rows), :], sem_o.at[8 + h * 4 + a])

    def start(cps):
        for cp in cps:
            cp.start()

    def wait(cps):
        for cp in cps:
            cp.wait()

    def ln_job(g):
        def t():
            v = [xr[pl.ds(g * 16, 16), pl.ds(c * 128, 128)].astype(f32) for c in range(8)]
            a = v[0]
            for c in range(1, 8):
                a = a + v[c]
            mean = jnp.sum(a, axis=1, keepdims=True) * (1.0 / D)
            v = [x - mean for x in v]
            a = v[0] * v[0]
            for c in range(1, 8):
                a = a + v[c] * v[c]
            r = lax.rsqrt(jnp.sum(a, axis=1, keepdims=True) * (1.0 / D) + EPS)
            for c in range(8):
                xn[pl.ds(g * 8, 8), pl.ds(c * 128, 128)] = _pk(v[c] * r)
        return [t]

    def ln_jobs(r):
        return [ln_job(r * 16 + g) for g in range(16)]

    def t_job(pos_idx):
        w0 = _mult((pos_idx // 2) * 8, 8)
        l0 = _mult((pos_idx % 2) * 128, 128)

        def raw(i, j):
            return xn[pl.ds(_mult(i * 256 + w0, 8), 8), pl.ds(_mult(j * KB + l0, 128), 128)]

        def emit(p, v):
            T[p, pl.ds(w0, 8), pl.ds(l0, 128)] = v
        return _opcomb_job(lambda i, j: _unpk(raw(i, j)), A_T, emit, raw)

    def b_job(par, g, half):
        w_ref = (gst, ust)[half]

        def src(i, q):
            return w_ref[par, pl.ds(_mult(i * KB + g * 16, 16), 16), pl.ds(q * TB, TB)]

        def emit(p, v):
            B[par, p, pl.ds(_mult(g * 8, 8), 8), pl.ds(half * TB, TB)] = v
        return _opcomb_job(lambda i, q: src(i, q).astype(f32), B_T, emit,
                           lambda i, q: pltpu.bitcast(src(i, q), u32))

    def bd_job(par, g, n):
        def src(i, q):
            return dst[par, pl.ds(_mult(i * TB + g * 16, 16), 16), pl.ds(q * KB + n * 128, 128)]

        def emit(p, v):
            Bd[par, p, pl.ds(_mult(g * 8, 8), 8), pl.ds(n * 128, 128)] = v
        return _opcomb_job(lambda i, q: src(i, q).astype(f32), B_T, emit,
                           lambda i, q: pltpu.bitcast(src(i, q), u32))

    def b_jobs(par, k):
        return [b_job(par, 4 * k + g, h) for g in range(4) for h in range(2)]

    def bd_jobs(par, k):
        return [bd_job(par, 2 * k + g, n) for g in range(2) for n in range(2)]

    def perm_job(m, grp):
        def t():
            w = _mult(grp * 8, 8)
            r = _perm8([R[2 - m, c, pl.ds(w, 8), :] for c in range(8)])
            for c in range(8):
                P[m, c, pl.ds(_mult(PADW + w, 8), 8), :] = r[c]
        return [t]

    def wq_job(grp):
        def t():
            rows = pl.ds(_mult(grp * 16, 16), 16)
            r = _perm8([pltpu.bitcast(wqr[rows, pl.ds(c * 128, 128)], u32) for c in range(8)])
            for c in range(8):
                wqp[pl.ds(_mult(grp * 8, 8), 8), pl.ds(c * 128, 128)] = r[c]
        return [t]

    def attn_job(grp, sl):
        b = _mult(grp * 8, 8)
        job = []
        for h in range(2):
            st = {}
            half = lambda v, h=h: _unpk(v)[h * 8:(h + 1) * 8]

            def qk(cs, st=st, half=half):
                def t():
                    for c in cs:
                        qv = half(P[0, c, pl.ds(_mult(b + PADW, 8), 8), :])
                        for w in range(WIN):
                            kv = half(P[1, c, pl.ds(b + (PADW - w), 8), :])
                            st[w] = qv * kv if c == 0 else st[w] + qv * kv
                return t

            def sm(st=st, h=h):
                lane = lax.broadcasted_iota(jnp.int32, (8, 128), 1)
                row = lax.broadcasted_iota(jnp.int32, (8, 128), 0) + (grp * 16 + h * 8)
                ls = []
                for w in range(WIN):
                    a = _sum4(st[w], lane)
                    if w > 0:
                        a = jnp.where(row >= 2 * w, a, -1e30)
                    ls.append(a)
                m = ls[0]
                for w in range(1, WIN):
                    m = jnp.maximum(m, ls[w])
                e = [jnp.exp2((l - m) * C2) for l in ls]
                den = e[0]
                for w in range(1, WIN):
                    den = den + e[w]
                inv = 1.0 / den
                st['p'] = [x * inv for x in e]

            def pv(cs, st=st, half=half, h=h):
                def t():
                    for c in cs:
                        o = None
                        for w in range(WIN):
                            a = st['p'][w] * half(P[2, c, pl.ds(b + (PADW - w), 8), :])
                            o = a if o is None else o + a
                        ost[sl, c, pl.ds(h * 8, 8), :] = o
                return t
            job += [qk((0, 1, 2, 3)), qk((4, 5, 6, 7)), sm, pv((0, 1, 2, 3)), pv((4, 5, 6, 7))]

        def fin():
            r = _perm8([_pk(ost[sl, c, pl.ds(0, 16), :]) for c in range(8)])
            for c in range(8):
                xn[pl.ds(b, 8), pl.ds(c * 128, 128)] = r[c]
        return job + [fin]

    def comb_job(mp, g):
        sl = g % 4
        job = []
        for hf in range(2):
            for pos in POS:
                def t(hf=hf, pos=pos):
                    r = pl.ds(g * 16 + hf * 8, 8)
                    gg = _outpos(lambda p: M[mp, p, 0, r, :], pos)
                    uu = _outpos(lambda p: M[mp, p, 1, r, :], pos)
                    for q in gg:
                        hst[sl, (q[0] * 2 + pos[0]) * 4 + q[1] * 2 + pos[1], pl.ds(hf * 8, 8), :] = gg[q] * uu[q]
                job.append(t)

        def emit(p, v):
            H[mp, p, pl.ds(g * 8, 8), :] = v
        return job + _opcomb_job(lambda i, j: hst[sl, i * 4 + j, pl.ds(0, 16), :], A_T, emit)

    def comb_jobs(mp):
        return [comb_job(mp, g) for g in range(RS // 16)]

    def zero_job(p):
        def t():
            for c in range(2):
                acc[p, c, pl.ds(0, HB), :] = jnp.zeros((HB, 128), f32)
        return [t]

    def final_job(i, g, n):
        job = []
        par = i % 2
        for pos in POS:
            def t(pos=pos):
                r0 = _mult(i * RS + g * 16, 16)
                o = [_outpos(lambda p: acc[p, n, pl.ds(r0 + hf * 8, 8), :], pos) for hf in range(2)]
                for q in o[0]:
                    a = q[0] * 2 + pos[0]
                    ch = (q[1] * 2 + pos[1]) * 2 + n
                    pln = a * 8 + ch
                    cols = pl.ds(ch * 128, 128)
                    ffn = jnp.concatenate([o[0][q], o[1][q]], axis=0)
                    att = M[par, pln // 2, pln % 2, pl.ds(g * 16, 16), :]
                    res = xr[pl.ds(_mult(a * HB + r0, 16), 16), cols].astype(f32) + att + ffn
                    dst[par, pl.ds(a * RS + g * 16, 16), cols] = res.astype(bf)
            job.append(t)
        return job

    def final_jobs(i):
        return [final_job(i, g, n) for g in range(RS // 16) for n in range(2)]

    def kv_tasks(m, slot, cbase, pieces):
        out = []
        for r in pieces:
            for ct in range(QW // 128):
                def t(r=r, ct=ct):
                    res = _dot(_up(xn[pl.ds(_mult(r * 64, 64), 64), :]), wst[slot, :, pl.ds(ct * 128, 128)])
                    for k in range(8):
                        R[2 - m, cbase + ct, pl.ds(_mult(r * 64 + k * 8, 8), 8), :] = _pk(res[k * 16:(k + 1) * 16])
                out.append((t, 256))
        return out

    def q_tasks(cbase):
        out = []
        for r in range(16):
            for ct in range(QW // 128):
                def t(r=r, ct=ct):
                    res = _dot(_up(xn[pl.ds(r * 64, 64), :]),
                               _up(wqp[:, pl.ds(_mult((cbase + ct) * 128, 128), 128)]))
                    for k in range(8):
                        P[0, cbase + ct, pl.ds(PADW + r * 64 + k * 8, 8), :] = _pk(res[k * 16:(k + 1) * 16])
                out.append((t, 256))
        return out

    def mm1_tasks(mp, s, par):
        out = []
        for p in range(NP):
            def t(p=p):
                r = _dot(_up(T[p, pl.ds(_mult(s * (RS // 2), RS // 2), RS // 2), :]), _up(B[par, p]))
                for c in range(2):
                    M[mp, p, c, pl.ds(0, RS), :] = r[:, c * 128:(c + 1) * 128]
            out.append((t, 128))
        return out

    def mm2_tasks(mp, s, par):
        out = []
        for p in range(NP):
            def t(p=p):
                r = _dot(_up(H[mp, p]), _up(Bd[par, p]))
                for c in range(2):
                    acc[p, c, pl.ds(_mult(s * RS, RS), RS), :] += r[:, c * 128:(c + 1) * 128]
            out.append((t, 64))
        return out

    def wo_tasks(i):
        out = []
        for a in range(4):
            for ch in range(8):
                def t(a=a, ch=ch):
                    w_ref = (gst, ust)[ch // 4]
                    res = _dot(_up(xn[pl.ds(_mult(a * 256 + i * 64, 64), 64), :]),
                               w_ref[1, :, pl.ds((ch % 4) * 128, 128)])
                    pln = a * 8 + ch
                    M[i % 2, pln // 2, pln % 2, pl.ds(0, RS), :] = res
                out.append((t, 256))
        return out

    nothing = lambda: [(lambda: None, 1)]

    x_copy(0).start()
    w_copy(0, 0).start()
    for c in range(8):
        P[1, c, pl.ds(0, PADW), :] = jnp.zeros((PADW, 128), u32)
        P[2, c, pl.ds(0, PADW), :] = jnp.zeros((PADW, 128), u32)
    x_copy(0).wait()
    w_copy(1, 1).start()
    x_copy(1).start()
    block(nothing, lambda: ln_jobs(0), 'ln0')
    w_copy(0, 0).wait()

    for r in range(8):
        if r + 2 < 8:
            x_copy(r + 2).start()
        if r == 0:
            block(lambda: kv_tasks(2, 0, 0, (0, 1)), lambda: [], 'p0')
            w_copy(1, 1).wait()
        if r == 5:
            w_copy(2, 2).start()
            wq_copy().start()
        if r + 1 < 8:
            x_copy(r + 1).wait()
        block(lambda r=r: (kv_tasks(2, 0, 0, (2 * r, 2 * r + 1)) if r > 0 else [])
              + kv_tasks(2, 1, 2, (2 * r, 2 * r + 1)),
              lambda r=r: ln_jobs(r + 1) if r + 1 < 8 else [], 'p0')

    def kv_block(j, m, after_start, jobs, name):
        slot = j % 3
        w_copy(j, slot).wait()

        @pl.when(j + 1 < 8)
        def _():
            w_copy(j + 1, (j + 1) % 3).start()
        after_start()
        block(lambda: kv_tasks(m, slot, (j % 4) * 2, range(16)), jobs, name)

    def v_body(j, c):
        def dmas():
            @pl.when(j == 2)
            def _():
                start(gu_copies(0, 0))

            @pl.when(j == 3)
            def _():
                d_copy(0, 0).start()
                d_copy(1, 1).start()
        kv_block(j, 2, dmas, lambda: _mix([wq_job((j - 2) * 32 + a) for a in range(32)],
                                          [t_job((j - 2) * 8 + a) for a in range(8)]), 'v')
        return c
    wq_copy().wait()
    lax.fori_loop(2, 4, v_body, 0)

    def k_body(j, c):
        def dmas():
            @pl.when(j == 4)
            def _():
                start(gu_copies(1, 1))
        i = j - 4
        kv_block(j, 1, dmas, lambda: _mix([perm_job(2, i * 32 + a) for a in range(32)],
                                          [t_job(16 + i * 12 + a) for a in range(12)]), 'k')
        return c
    lax.fori_loop(4, 8, k_body, 0)

    wait(gu_copies(0, 0))
    d_copy(0, 0).wait()

    def q_body(i, c):
        def jobs():
            extra = ([b_job(0, 4 * i + g, h) for g in range(4) for h in range(2)]
                     + [bd_job(0, i, n) for n in range(2)]
                     + [zero_job(jnp.minimum(i * 13 + a, NP - 1)) for a in range(13)])
            return _mix([perm_job(1, i * 32 + a) for a in range(32)], extra)
        block(lambda: q_tasks(i * 2), jobs, 'q')
        return c
    lax.fori_loop(0, 4, q_body, 0)

    wait(gu_copies(1, 1))
    start(gu_copies(2, 0))
    block(lambda: mm1_tasks(0, 0, 0),
          lambda: _mix([attn_job(a, a % 4) for a in range(NATT0)], b_jobs(1, 0) + bd_jobs(0, 2)), 'f0')
    block(lambda: mm1_tasks(1, 1, 0),
          lambda: _mix(_mix(comb_jobs(0), b_jobs(1, 1) + bd_jobs(0, 3)),
                       [attn_job(NATT0 + a, a % 4) for a in range(NATT0)]), 'f1')

    def slot(t, mp):
        j = t // 4
        s = t % 4
        par = j % 2
        if mp == 0:
            @pl.when(jnp.logical_and(s == 0, j > 0))
            def _():
                wait(gu_copies(jnp.minimum(j + 1, NCH - 1), 1 - par))

                @pl.when(j + 2 < NCH)
                def _():
                    start(gu_copies(j + 2, par))

                @pl.when(j + 2 == NCH)
                def _():
                    start(wo_copies())

            @pl.when(jnp.logical_and(s == 2, j + 1 < NCH))
            def _():
                d_copy(j + 1, 1 - par).wait()

                @pl.when(j + 2 < NCH)
                def _():
                    d_copy(j + 2, par).start()
        jd = (t + 2) // 4
        kd = (t + 2) % 4
        u = t - 2

        def jobs():
            base = _mix(comb_jobs(1 - mp), b_jobs(1 - par, s) + bd_jobs(jd % 2, kd))
            att = []
            for a in range(NATT):
                att.append(attn_job(jnp.minimum(2 * NATT0 + u * NATT + a, 127), a % 4))
            n0 = max(1, len(base) // 10)
            return base[:n0] + _mix(base[n0:-n0], att) + base[-n0:]
        block(lambda: _mix(mm1_tasks(mp, s, par), mm2_tasks(mp, (t - 2) % 4, ((t - 2) // 4) % 2)), jobs,
              'slot%d' % mp)

    def steady(it, c):
        slot(2 * it + 2, 0)
        slot(2 * it + 3, 1)
        return c
    lax.fori_loop(0, (NT - 2) // 2, steady, 0)

    block(lambda: mm2_tasks(0, 2, 0), lambda: comb_jobs(1), 'e0')
    block(lambda: _mix(wo_tasks(0), mm2_tasks(1, 3, 0)), lambda: [], 'e1')

    def wo_body(i, c):
        @pl.when(i >= 3)
        def _():
            wait([out_copy(i - 3, a) for a in range(4)])
        block(lambda: wo_tasks(i), lambda: final_jobs(i - 1), 'wo')
        start([out_copy(i - 1, a) for a in range(4)])
        return c
    lax.fori_loop(1, 4, wo_body, 0)
    wait([out_copy(1, a) for a in range(4)])
    for h in range(2):
        block(nothing, lambda h=h: [final_job(3, g, n) for g in range(4 * h, 4 * h + 4) for n in range(2)], 'e3')
        start([last_copy(a, h) for a in range(4)])
    wait([out_copy(2, a) for a in range(4)])
    wait([last_copy(a, h) for h in range(2) for a in range(4)])


@jax.jit
def pallas_parallel_sum__sliding_local_dilated__glu_gated_bilinear__prompt_kernel(
    A_x: jax.Array,
    A_wqkv: jax.Array,
    A_wo: jax.Array,
    B_x: jax.Array,
    B_w_gate: jax.Array,
    B_w_up: jax.Array,
    B_w_down: jax.Array,
):
    del B_x
    x = A_x.reshape(S, D)
    hbm = pl.BlockSpec(memory_space=pl.ANY)
    dma = pltpu.SemaphoreType.DMA
    out = pl.pallas_call(
        _kernel,
        grid=(1,),
        in_specs=[pl.BlockSpec(memory_space=pltpu.SMEM)] + [hbm] * 6,
        out_specs=hbm,
        out_shape=jax.ShapeDtypeStruct((S, D), bf),
        scratch_shapes=[
            pltpu.VMEM((S, D), bf),
            pltpu.VMEM((S // 2, D), u32),
            pltpu.VMEM((NP, HB // 2, KB), u32),
            pltpu.VMEM((3, D, QW), bf),
            pltpu.VMEM((D, D), bf),
            pltpu.VMEM((D // 2, D), u32),
            pltpu.VMEM((2, 8, S // 2 + PADW, 128), u32),
            pltpu.VMEM((3, 8, S // 2 + PADW, 128), u32),
            pltpu.VMEM((2, D, TF), bf),
            pltpu.VMEM((2, D, TF), bf),
            pltpu.VMEM((2, TF, D), bf),
            pltpu.VMEM((2, NP, KB // 2, 2 * TB), u32),
            pltpu.VMEM((2, NP, TB // 2, KB), u32),
            pltpu.VMEM((2, NP, 2, RS + MPAD, 128), f32),
            pltpu.VMEM((2, NP, RS // 2, TB), u32),
            pltpu.VMEM((4, 16, 24, 128), f32),
            pltpu.VMEM((4, 8, 24, 128), f32),
            pltpu.VMEM((NP, 2, HB + MPAD, 128), f32),
            dma((8,)), dma((3,)), dma((1,)), dma((2,)), dma((2,)), dma((2,)), dma((16,)),
        ],
        compiler_params=pltpu.CompilerParams(
            dimension_semantics=("arbitrary",), vmem_limit_bytes=127 * 1024 * 1024,
            disable_bounds_checks=True),
        name="fused_attn_ffn",
    )(jnp.ones((1,), jnp.int32), x, A_wqkv, A_wo, B_w_gate, B_w_up, B_w_down)
    return out.reshape(1, S, D)
```

```python
import jax
import jax.numpy as jnp
from jax import lax
from jax.experimental import pallas as pl
from jax.experimental.pallas import tpu as pltpu

bf = jnp.bfloat16
f32 = jnp.float32
u32 = jnp.uint32

S, D, F = 2048, 1024, 3584
WIN = 8
NP = 49
HB = S // 4
KB = D // 4
TF = 512
TB = TF // 4
NCH = F // TF
RS = 128
NSUB = HB // RS
NT = NCH * NSUB
MPAD = 8
PADW = 8
QW = 256
EPS = 1e-5
C2 = float(32 ** -0.5 * 1.4426950408889634)
NATT = 5
NATT0 = 1

A_T = [[(1, (0, 0)), (1, (1, 1))], [(1, (1, 0)), (1, (1, 1))], [(1, (0, 0))], [(1, (1, 1))],
       [(1, (0, 0)), (1, (0, 1))], [(1, (1, 0)), (-1, (0, 0))], [(1, (0, 1)), (-1, (1, 1))]]
B_T = [[(1, (0, 0)), (1, (1, 1))], [(1, (0, 0))], [(1, (0, 1)), (-1, (1, 1))], [(1, (1, 0)), (-1, (0, 0))],
       [(1, (1, 1))], [(1, (0, 0)), (1, (0, 1))], [(1, (1, 0)), (1, (1, 1))]]
C_T = {(0, 0): [(1, 0), (1, 3), (-1, 4), (1, 6)], (0, 1): [(1, 2), (1, 4)],
       (1, 0): [(1, 1), (1, 3)], (1, 1): [(1, 0), (-1, 1), (1, 2), (1, 5)]}
POS = ((0, 0), (0, 1), (1, 0), (1, 1))


def _comb(terms):
    acc = None
    for s, v in terms:
        if acc is None:
            acc = v if s > 0 else -v
        else:
            acc = acc + v if s > 0 else acc - v
    return acc


def _dot(a, b):
    return jnp.dot(a, b, preferred_element_type=f32)


def _pk(v):
    return pltpu.bitcast(v.astype(bf), u32)


def _up(w):
    return pltpu.bitcast(w, bf)


def _unpk(w):
    return pltpu.bitcast(w, bf).astype(f32)


def _as_f32(w):
    return lax.bitcast_convert_type(w, f32)


def _as_u32(v):
    return lax.bitcast_convert_type(v, u32)


def _mult(x, m):
    return x if isinstance(x, int) else pl.multiple_of(x, m)


def _opcomb(load, table, I, emit, raw):
    sub = {(r, c): _comb([(s, load(q[0] * 2 + r, q[1] * 2 + c)) for s, q in table[I]])
           for r in range(2) for c in range(2)}
    for J, t2 in enumerate(table):
        if raw is not None and len(table[I]) == 1 and len(t2) == 1:
            qo, qi = table[I][0][1], t2[0][1]
            emit(I * 7 + J, raw(qo[0] * 2 + qi[0], qo[1] * 2 + qi[1]))
        else:
            emit(I * 7 + J, _pk(_comb([(s, sub[q]) for s, q in t2])))


def _opcomb_job(load, table, emit, raw=None):
    return [(lambda I=I: _opcomb(load, table, I, emit, raw)) for I in range(7)]


def _outpos(load, pos):
    inner = [_comb([(s, load(I * 7 + J)) for s, J in C_T[pos]]) for I in range(7)]
    return {q: _comb([(s, inner[I]) for s, I in terms]) for q, terms in C_T.items()}


def _perm8(v):
    lane = lax.broadcasted_iota(jnp.int32, v[0].shape, 1)
    v = list(v)
    for cb, lb in ((2, 4), (1, 3), (0, 2)):
        sh = 1 << lb
        hi = (lane & sh) != 0
        out = [None] * 8
        for c in range(8):
            if c & (1 << cb):
                continue
            x, y = v[c], v[c | (1 << cb)]
            out[c] = jnp.where(hi, pltpu.roll(y, sh, 1), x)
            out[c | (1 << cb)] = jnp.where(hi, y, pltpu.roll(x, 128 - sh, 1))
        v = out
    return v


def _sum4(x, lane):
    x = x + jnp.where((lane & 1) != 0, pltpu.roll(x, 1, 1), pltpu.roll(x, 127, 1))
    x = x + jnp.where((lane & 2) != 0, pltpu.roll(x, 2, 1), pltpu.roll(x, 126, 1))
    return x


def _mix(a, b):
    if not b:
        return list(a)
    if not a:
        return list(b)
    out, n, m, k = [], len(a), len(b), 0
    for i, t in enumerate(a):
        out.append(t)
        tgt = (i + 1) * m // n
        while k < tgt:
            out.append(b[k])
            k += 1
    return out


def _flat(jobs):
    return [t for j in jobs for t in j]


def _weave(mx, jobs):
    vp = _flat(jobs)
    tot = sum(c for _, c in mx)
    n, k, acc = len(vp), 0, 0
    for t, c in mx:
        t()
        acc += c
        tgt = acc * n // tot
        while k < tgt:
            vp[k]()
            k += 1
    while k < n:
        vp[k]()
        k += 1


def _kernel(one_ref, x_hbm, wqkv_hbm, wo_hbm, wg_hbm, wu_hbm, wd_hbm, out_hbm,
            xr, xn, T, wst, wqr, wqp, R, P, gst, ust, dst, B, Bd, M, H, hst, ost, acc,
            sem_x, sem_w, sem_q, sem_g, sem_u, sem_d, sem_o):

    def block(mx, jobs, name="blk"):
        with jax.named_scope(name):
            @pl.when(one_ref[0] > 0)
            def _():
                _weave(mx(), jobs())

    def x_copy(r):
        rows = pl.ds(_mult(r * 256, 256), 256)
        return pltpu.make_async_copy(x_hbm.at[rows, :], xr.at[rows, :], sem_x.at[r])

    def w_copy(j, slot):
        col = (2 - j // 4) * D + (j % 4) * QW
        return pltpu.make_async_copy(wqkv_hbm.at[:, pl.ds(_mult(col, QW), QW)], wst.at[slot], sem_w.at[slot])

    def wq_copy():
        return pltpu.make_async_copy(wqkv_hbm.at[:, pl.ds(0, D)], wqr, sem_q.at[0])

    def gu_copies(j, par):
        cols = pl.ds(_mult(j * TF, TF), TF)
        return (pltpu.make_async_copy(wg_hbm.at[:, cols], gst.at[par], sem_g.at[par]),
                pltpu.make_async_copy(wu_hbm.at[:, cols], ust.at[par], sem_u.at[par]))

    def d_copy(j, par):
        return pltpu.make_async_copy(wd_hbm.at[pl.ds(_mult(j * TF, TF), TF), :], dst.at[par], sem_d.at[par])

    def wo_copies():
        return (pltpu.make_async_copy(wo_hbm.at[:, pl.ds(0, TF)], gst.at[1], sem_g.at[1]),
                pltpu.make_async_copy(wo_hbm.at[:, pl.ds(TF, TF)], ust.at[1], sem_u.at[1]))

    def out_copy(i, a):
        par = i % 2
        return pltpu.make_async_copy(dst.at[par, pl.ds(a * RS, RS), :],
                                     out_hbm.at[pl.ds(_mult(a * HB + i * RS, RS), RS), :], sem_o.at[par * 4 + a])

    def last_copy(a, h):
        rows = RS // 2
        return pltpu.make_async_copy(dst.at[1, pl.ds(a * RS + h * rows, rows), :],
                                     out_hbm.at[pl.ds(a * HB + 3 * RS + h * rows, rows), :], sem_o.at[8 + h * 4 + a])

    def start(cps):
        for cp in cps:
            cp.start()

    def wait(cps):
        for cp in cps:
            cp.wait()

    def ln_job(g):
        def t():
            v = [xr[pl.ds(g * 16, 16), pl.ds(c * 128, 128)].astype(f32) for c in range(8)]
            a = v[0]
            for c in range(1, 8):
                a = a + v[c]
            mean = jnp.sum(a, axis=1, keepdims=True) * (1.0 / D)
            v = [x - mean for x in v]
            a = v[0] * v[0]
            for c in range(1, 8):
                a = a + v[c] * v[c]
            r = lax.rsqrt(jnp.sum(a, axis=1, keepdims=True) * (1.0 / D) + EPS)
            for c in range(8):
                xn[pl.ds(g * 8, 8), pl.ds(c * 128, 128)] = _pk(v[c] * r)
        return [t]

    def ln_jobs(r):
        return [ln_job(r * 16 + g) for g in range(16)]

    def t_job(pos_idx):
        w0 = _mult((pos_idx // 2) * 8, 8)
        l0 = _mult((pos_idx % 2) * 128, 128)

        def raw(i, j):
            return xn[pl.ds(_mult(i * 256 + w0, 8), 8), pl.ds(_mult(j * KB + l0, 128), 128)]

        def emit(p, v):
            T[p, pl.ds(w0, 8), pl.ds(l0, 128)] = v
        return _opcomb_job(lambda i, j: _unpk(raw(i, j)), A_T, emit, raw)

    def b_job(par, g, half):
        w_ref = (gst, ust)[half]

        def src(i, q):
            return w_ref[par, pl.ds(_mult(i * KB + g * 16, 16), 16), pl.ds(q * TB, TB)]

        def emit(p, v):
            B[par, p, pl.ds(_mult(g * 8, 8), 8), pl.ds(half * TB, TB)] = v
        return _opcomb_job(lambda i, q: src(i, q).astype(f32), B_T, emit,
                           lambda i, q: pltpu.bitcast(src(i, q), u32))

    def bd_job(par, g, n):
        def src(i, q):
            return dst[par, pl.ds(_mult(i * TB + g * 16, 16), 16), pl.ds(q * KB + n * 128, 128)]

        def emit(p, v):
            Bd[par, p, pl.ds(_mult(g * 8, 8), 8), pl.ds(n * 128, 128)] = v
        return _opcomb_job(lambda i, q: src(i, q).astype(f32), B_T, emit,
                           lambda i, q: pltpu.bitcast(src(i, q), u32))

    def b_jobs(par, k):
        return [b_job(par, 4 * k + g, h) for g in range(4) for h in range(2)]

    def bd_jobs(par, k):
        return [bd_job(par, 2 * k + g, n) for g in range(2) for n in range(2)]

    def perm_job(m, pair):
        def t():
            w = _mult(pair * 16, 16)
            r = _perm8([R[2 - m, c, pl.ds(w, 16), :] for c in range(8)])
            for c in range(8):
                P[m, c, pl.ds(_mult(PADW + w, 8), 16), :] = r[c]
        return [t]

    def wq_job(pair):
        def t():
            rows = pl.ds(_mult(pair * 32, 32), 32)
            r = _perm8([pltpu.bitcast(wqr[rows, pl.ds(c * 128, 128)], u32) for c in range(8)])
            for c in range(8):
                wqp[pl.ds(_mult(pair * 16, 16), 16), pl.ds(c * 128, 128)] = r[c]
        return [t]

    def attn_job(grp, sl):
        b = _mult(grp * 8, 8)
        job = []
        for h in range(2):
            st = {}
            half = lambda v, h=h: _unpk(v)[h * 8:(h + 1) * 8]

            def qk(cs, st=st, half=half):
                def t():
                    for c in cs:
                        qv = half(P[0, c, pl.ds(_mult(b + PADW, 8), 8), :])
                        for w in range(WIN):
                            kv = half(P[1, c, pl.ds(b + (PADW - w), 8), :])
                            st[w] = qv * kv if c == 0 else st[w] + qv * kv
                return t

            def sm(st=st, h=h):
                lane = lax.broadcasted_iota(jnp.int32, (8, 128), 1)
                row = lax.broadcasted_iota(jnp.int32, (8, 128), 0) + (grp * 16 + h * 8)
                ls = []
                for w in range(WIN):
                    a = _sum4(st[w], lane)
                    if w > 0:
                        a = jnp.where(row >= 2 * w, a, -1e30)
                    ls.append(a)
                m = ls[0]
                for w in range(1, WIN):
                    m = jnp.maximum(m, ls[w])
                e = [jnp.exp2((l - m) * C2) for l in ls]
                den = e[0]
                for w in range(1, WIN):
                    den = den + e[w]
                inv = 1.0 / den
                st['p'] = [x * inv for x in e]

            def pv(cs, st=st, half=half, h=h):
                def t():
                    for c in cs:
                        o = None
                        for w in range(WIN):
                            a = st['p'][w] * half(P[2, c, pl.ds(b + (PADW - w), 8), :])
                            o = a if o is None else o + a
                        ost[sl, c, pl.ds(h * 8, 8), :] = o
                return t
            job += [qk((0, 1, 2, 3)), qk((4, 5, 6, 7)), sm, pv((0, 1, 2, 3)), pv((4, 5, 6, 7))]

        def fin():
            r = _perm8([_pk(ost[sl, c, pl.ds(0, 16), :]) for c in range(8)])
            for c in range(8):
                xn[pl.ds(b, 8), pl.ds(c * 128, 128)] = r[c]
        return job + [fin]

    def comb_job(mp, g):
        sl = g % 4
        job = []
        for hf in range(2):
            for pos in POS:
                def t(hf=hf, pos=pos):
                    r = pl.ds(g * 16 + hf * 8, 8)
                    gg = _outpos(lambda p: M[mp, p, 0, r, :], pos)
                    uu = _outpos(lambda p: M[mp, p, 1, r, :], pos)
                    for q in gg:
                        hst[sl, (q[0] * 2 + pos[0]) * 4 + q[1] * 2 + pos[1], pl.ds(hf * 8, 8), :] = gg[q] * uu[q]
                job.append(t)

        def emit(p, v):
            H[mp, p, pl.ds(g * 8, 8), :] = v
        return job + _opcomb_job(lambda i, j: hst[sl, i * 4 + j, pl.ds(0, 16), :], A_T, emit)

    def comb_jobs(mp):
        return [comb_job(mp, g) for g in range(RS // 16)]

    def zero_job(p):
        def t():
            for c in range(2):
                acc[p, c, pl.ds(0, HB), :] = jnp.zeros((HB, 128), f32)
        return [t]

    def final_job(i, g, n):
        job = []
        par = i % 2
        for pos in POS:
            def t(pos=pos):
                r0 = _mult(i * RS + g * 16, 16)
                o = [_outpos(lambda p: acc[p, n, pl.ds(r0 + hf * 8, 8), :], pos) for hf in range(2)]
                for q in o[0]:
                    a = q[0] * 2 + pos[0]
                    ch = (q[1] * 2 + pos[1]) * 2 + n
                    pln = a * 8 + ch
                    cols = pl.ds(ch * 128, 128)
                    ffn = jnp.concatenate([o[0][q], o[1][q]], axis=0)
                    att = M[par, pln // 2, pln % 2, pl.ds(g * 16, 16), :]
                    res = xr[pl.ds(_mult(a * HB + r0, 16), 16), cols].astype(f32) + att + ffn
                    dst[par, pl.ds(a * RS + g * 16, 16), cols] = res.astype(bf)
            job.append(t)
        return job

    def final_jobs(i):
        return [final_job(i, g, n) for g in range(RS // 16) for n in range(2)]

    def kv_tasks(m, slot, cbase, pieces):
        out = []
        for r in pieces:
            for ct in range(QW // 128):
                def t(r=r, ct=ct):
                    res = _dot(_up(xn[pl.ds(_mult(r * 64, 64), 64), :]), wst[slot, :, pl.ds(ct * 128, 128)])
                    for k in range(8):
                        R[2 - m, cbase + ct, pl.ds(_mult(r * 64 + k * 8, 8), 8), :] = _pk(res[k * 16:(k + 1) * 16])
                out.append((t, 256))
        return out

    def q_tasks(cbase):
        out = []
        for r in range(16):
            for ct in range(QW // 128):
                def t(r=r, ct=ct):
                    res = _dot(_up(xn[pl.ds(r * 64, 64), :]),
                               _up(wqp[:, pl.ds(_mult((cbase + ct) * 128, 128), 128)]))
                    for k in range(8):
                        P[0, cbase + ct, pl.ds(PADW + r * 64 + k * 8, 8), :] = _pk(res[k * 16:(k + 1) * 16])
                out.append((t, 256))
        return out

    def mm1_tasks(mp, s, par):
        out = []
        for p in range(NP):
            def t(p=p):
                r = _dot(_up(T[p, pl.ds(_mult(s * (RS // 2), RS // 2), RS // 2), :]), _up(B[par, p]))
                for c in range(2):
                    M[mp, p, c, pl.ds(0, RS), :] = r[:, c * 128:(c + 1) * 128]
            out.append((t, 128))
        return out

    def mm2_tasks(mp, s, par):
        out = []
        for p in range(NP):
            def t(p=p):
                r = _dot(_up(H[mp, p]), _up(Bd[par, p]))
                for c in range(2):
                    acc[p, c, pl.ds(_mult(s * RS, RS), RS), :] += r[:, c * 128:(c + 1) * 128]
            out.append((t, 64))
        return out

    def wo_tasks(i):
        out = []
        for a in range(4):
            for ch in range(8):
                def t(a=a, ch=ch):
                    w_ref = (gst, ust)[ch // 4]
                    res = _dot(_up(xn[pl.ds(_mult(a * 256 + i * 64, 64), 64), :]),
                               w_ref[1, :, pl.ds((ch % 4) * 128, 128)])
                    pln = a * 8 + ch
                    M[i % 2, pln // 2, pln % 2, pl.ds(0, RS), :] = res
                out.append((t, 256))
        return out

    nothing = lambda: [(lambda: None, 1)]

    x_copy(0).start()
    w_copy(0, 0).start()
    for c in range(8):
        P[1, c, pl.ds(0, PADW), :] = jnp.zeros((PADW, 128), u32)
        P[2, c, pl.ds(0, PADW), :] = jnp.zeros((PADW, 128), u32)
    x_copy(0).wait()
    w_copy(1, 1).start()
    x_copy(1).start()
    block(nothing, lambda: ln_jobs(0), 'ln0')
    w_copy(0, 0).wait()

    def v01(pieces):
        rp = [2 * r + h for r in pieces for h in range(2)]
        return kv_tasks(2, 0, 0, rp) + kv_tasks(2, 1, 2, rp)

    block(lambda: kv_tasks(2, 0, 0, (0, 1)), lambda: [], 'p0')
    w_copy(1, 1).wait()
    x_copy(2).start()
    x_copy(1).wait()
    block(lambda: kv_tasks(2, 1, 2, (0, 1)), lambda: ln_jobs(1), 'p0')
    x_copy(3).start()
    x_copy(4).start()
    x_copy(2).wait()
    block(lambda: v01((1,)), lambda: ln_jobs(2), 'p0')
    x_copy(5).start()
    x_copy(6).start()
    x_copy(3).wait()
    x_copy(4).wait()
    block(lambda: v01((2,)), lambda: ln_jobs(3) + ln_jobs(4), 'p0')
    x_copy(7).start()
    w_copy(2, 2).start()
    x_copy(5).wait()
    x_copy(6).wait()
    block(lambda: v01((3, 4)), lambda: ln_jobs(5) + ln_jobs(6), 'p0')
    wq_copy().start()
    x_copy(7).wait()
    block(lambda: v01((5, 6)), lambda: ln_jobs(7), 'p0')
    block(lambda: v01((7,)), lambda: [], 'p0')

    def kv_block(j, m, after_start, jobs, name):
        slot = j % 3
        w_copy(j, slot).wait()

        @pl.when(j + 1 < 8)
        def _():
            w_copy(j + 1, (j + 1) % 3).start()
        after_start()
        block(lambda: kv_tasks(m, slot, (j % 4) * 2, range(16)), jobs, name)

    def v_body(j, c):
        def dmas():
            @pl.when(j == 2)
            def _():
                start(gu_copies(0, 0))

            @pl.when(j == 3)
            def _():
                d_copy(0, 0).start()
                d_copy(1, 1).start()
        kv_block(j, 2, dmas, lambda: [wq_job((j - 2) * 16 + a) for a in range(16)], 'v')
        return c
    wq_copy().wait()
    lax.fori_loop(2, 4, v_body, 0)

    def k_body(j, c):
        def dmas():
            @pl.when(j == 4)
            def _():
                start(gu_copies(1, 1))
        i = j - 4
        kv_block(j, 1, dmas, lambda: _mix([perm_job(2, i * 16 + a) for a in range(16)],
                                          [t_job(i * 12 + a) for a in range(12)]), 'k')
        return c
    lax.fori_loop(4, 8, k_body, 0)

    wait(gu_copies(0, 0))
    d_copy(0, 0).wait()

    def q_body(i, c):
        def jobs():
            extra = ([b_job(0, 4 * i + g, h) for g in range(4) for h in range(2)]
                     + [bd_job(0, i, n) for n in range(2)]
                     + [zero_job(jnp.minimum(i * 13 + a, NP - 1)) for a in range(13)])
            return _mix([perm_job(1, i * 16 + a) for a in range(16)], extra)
        block(lambda: q_tasks(i * 2), jobs, 'q')
        return c
    lax.fori_loop(0, 4, q_body, 0)

    wait(gu_copies(1, 1))
    start(gu_copies(2, 0))
    block(lambda: mm1_tasks(0, 0, 0),
          lambda: _mix(b_jobs(1, 0) + bd_jobs(0, 2) + [t_job(48 + a) for a in range(8)],
                       [attn_job(a, a % 4) for a in range(NATT0)]), 'f0')
    block(lambda: mm1_tasks(1, 1, 0),
          lambda: _mix(_mix(comb_jobs(0), b_jobs(1, 1) + bd_jobs(0, 3) + [t_job(56 + a) for a in range(8)]),
                       [attn_job(NATT0 + a, a % 4) for a in range(NATT0)]), 'f1')

    def slot(t, mp):
        j = t // 4
        s = t % 4
        par = j % 2
        if mp == 0:
            @pl.when(jnp.logical_and(s == 0, j > 0))
            def _():
                wait(gu_copies(jnp.minimum(j + 1, NCH - 1), 1 - par))

                @pl.when(j + 2 < NCH)
                def _():
                    start(gu_copies(j + 2, par))

                @pl.when(j + 2 == NCH)
                def _():
                    start(wo_copies())

            @pl.when(jnp.logical_and(s == 2, j + 1 < NCH))
            def _():
                d_copy(j + 1, 1 - par).wait()

                @pl.when(j + 2 < NCH)
                def _():
                    d_copy(j + 2, par).start()
        jd = (t + 2) // 4
        kd = (t + 2) % 4
        u = t - 2

        def jobs():
            base = _mix(comb_jobs(1 - mp), b_jobs(1 - par, s) + bd_jobs(jd % 2, kd))
            att = []
            for a in range(NATT):
                att.append(attn_job(jnp.minimum(2 * NATT0 + u * NATT + a, 127), a % 4))
            n0 = max(1, len(base) // 10)
            return base[:n0] + _mix(base[n0:-n0], att) + base[-n0:]
        block(lambda: _mix(mm1_tasks(mp, s, par), mm2_tasks(mp, (t - 2) % 4, ((t - 2) // 4) % 2)), jobs,
              'slot%d' % mp)

    def steady(it, c):
        slot(2 * it + 2, 0)
        slot(2 * it + 3, 1)
        return c
    lax.fori_loop(0, (NT - 2) // 2, steady, 0)

    block(lambda: mm2_tasks(0, 2, 0), lambda: comb_jobs(1), 'e0')
    block(lambda: _mix(wo_tasks(0), mm2_tasks(1, 3, 0)), lambda: [], 'e1')

    def wo_body(i, c):
        @pl.when(i >= 3)
        def _():
            wait([out_copy(i - 3, a) for a in range(4)])
        def jobs():
            kick = [lambda: start([out_copy(i - 1, a) for a in range(4)])]
            return final_jobs(i - 1) + [kick] + [[lambda: None] * 40]
        block(lambda: wo_tasks(i), jobs, 'wo')
        return c
    lax.fori_loop(1, 4, wo_body, 0)
    wait([out_copy(1, a) for a in range(4)])
    for h in range(2):
        block(nothing, lambda h=h: [final_job(3, g, n) for g in range(4 * h, 4 * h + 4) for n in range(2)], 'e3')
        start([last_copy(a, h) for a in range(4)])
    wait([out_copy(2, a) for a in range(4)])
    wait([last_copy(a, h) for h in range(2) for a in range(4)])


@jax.jit
def pallas_parallel_sum__sliding_local_dilated__glu_gated_bilinear__prompt_kernel(
    A_x: jax.Array,
    A_wqkv: jax.Array,
    A_wo: jax.Array,
    B_x: jax.Array,
    B_w_gate: jax.Array,
    B_w_up: jax.Array,
    B_w_down: jax.Array,
):
    del B_x
    x = A_x.reshape(S, D)
    hbm = pl.BlockSpec(memory_space=pl.ANY)
    dma = pltpu.SemaphoreType.DMA
    out = pl.pallas_call(
        _kernel,
        grid=(1,),
        in_specs=[pl.BlockSpec(memory_space=pltpu.SMEM)] + [hbm] * 6,
        out_specs=hbm,
        out_shape=jax.ShapeDtypeStruct((S, D), bf),
        scratch_shapes=[
            pltpu.VMEM((S, D), bf),
            pltpu.VMEM((S // 2, D), u32),
            pltpu.VMEM((NP, HB // 2, KB), u32),
            pltpu.VMEM((3, D, QW), bf),
            pltpu.VMEM((D, D), bf),
            pltpu.VMEM((D // 2, D), u32),
            pltpu.VMEM((2, 8, S // 2 + PADW, 128), u32),
            pltpu.VMEM((3, 8, S // 2 + PADW, 128), u32),
            pltpu.VMEM((2, D, TF), bf),
            pltpu.VMEM((2, D, TF), bf),
            pltpu.VMEM((2, TF, D), bf),
            pltpu.VMEM((2, NP, KB // 2, 2 * TB), u32),
            pltpu.VMEM((2, NP, TB // 2, KB), u32),
            pltpu.VMEM((2, NP, 2, RS + MPAD, 128), f32),
            pltpu.VMEM((2, NP, RS // 2, TB), u32),
            pltpu.VMEM((4, 16, 24, 128), f32),
            pltpu.VMEM((4, 8, 24, 128), f32),
            pltpu.VMEM((NP, 2, HB + MPAD, 128), f32),
            dma((8,)), dma((3,)), dma((1,)), dma((2,)), dma((2,)), dma((2,)), dma((16,)),
        ],
        compiler_params=pltpu.CompilerParams(
            dimension_semantics=("arbitrary",), vmem_limit_bytes=127 * 1024 * 1024,
            disable_bounds_checks=True),
        name="fused_attn_ffn",
    )(jnp.ones((1,), jnp.int32), x, A_wqkv, A_wo, B_w_gate, B_w_up, B_w_down)
    return out.reshape(1, S, D)
```

```python
import jax
import jax.numpy as jnp
from jax import lax
from jax.experimental import pallas as pl
from jax.experimental.pallas import tpu as pltpu

bf = jnp.bfloat16
f32 = jnp.float32
u32 = jnp.uint32

S, D, F = 2048, 1024, 3584
WIN = 8
NP = 49
HB = S // 4
KB = D // 4
TF = 512
TB = TF // 4
NCH = F // TF
RS = 128
NSUB = HB // RS
NT = NCH * NSUB
MPAD = 8
PADW = 8
QW = 256
EPS = 1e-5
C2 = float(32 ** -0.5 * 1.4426950408889634)
NATT = 5
NATT0 = 1

A_T = [[(1, (0, 0)), (1, (1, 1))], [(1, (1, 0)), (1, (1, 1))], [(1, (0, 0))], [(1, (1, 1))],
       [(1, (0, 0)), (1, (0, 1))], [(1, (1, 0)), (-1, (0, 0))], [(1, (0, 1)), (-1, (1, 1))]]
B_T = [[(1, (0, 0)), (1, (1, 1))], [(1, (0, 0))], [(1, (0, 1)), (-1, (1, 1))], [(1, (1, 0)), (-1, (0, 0))],
       [(1, (1, 1))], [(1, (0, 0)), (1, (0, 1))], [(1, (1, 0)), (1, (1, 1))]]
C_T = {(0, 0): [(1, 0), (1, 3), (-1, 4), (1, 6)], (0, 1): [(1, 2), (1, 4)],
       (1, 0): [(1, 1), (1, 3)], (1, 1): [(1, 0), (-1, 1), (1, 2), (1, 5)]}
POS = ((0, 0), (0, 1), (1, 0), (1, 1))


def _comb(terms):
    acc = None
    for s, v in terms:
        if acc is None:
            acc = v if s > 0 else -v
        else:
            acc = acc + v if s > 0 else acc - v
    return acc


def _dot(a, b):
    return jnp.dot(a, b, preferred_element_type=f32)


def _pk(v):
    return pltpu.bitcast(v.astype(bf), u32)


def _up(w):
    return pltpu.bitcast(w, bf)


def _unpk(w):
    return pltpu.bitcast(w, bf).astype(f32)


def _as_f32(w):
    return lax.bitcast_convert_type(w, f32)


def _as_u32(v):
    return lax.bitcast_convert_type(v, u32)


def _mult(x, m):
    return x if isinstance(x, int) else pl.multiple_of(x, m)


def _opcomb(load, table, I, emit, raw):
    sub = {(r, c): _comb([(s, load(q[0] * 2 + r, q[1] * 2 + c)) for s, q in table[I]])
           for r in range(2) for c in range(2)}
    for J, t2 in enumerate(table):
        if raw is not None and len(table[I]) == 1 and len(t2) == 1:
            qo, qi = table[I][0][1], t2[0][1]
            emit(I * 7 + J, raw(qo[0] * 2 + qi[0], qo[1] * 2 + qi[1]))
        else:
            emit(I * 7 + J, _pk(_comb([(s, sub[q]) for s, q in t2])))


def _opcomb_job(load, table, emit, raw=None):
    return [(lambda I=I: _opcomb(load, table, I, emit, raw)) for I in range(7)]


def _outpos(load, pos):
    inner = [_comb([(s, load(I * 7 + J)) for s, J in C_T[pos]]) for I in range(7)]
    return {q: _comb([(s, inner[I]) for s, I in terms]) for q, terms in C_T.items()}


def _perm8(v):
    lane = lax.broadcasted_iota(jnp.int32, v[0].shape, 1)
    v = list(v)
    for cb, lb in ((2, 4), (1, 3), (0, 2)):
        sh = 1 << lb
        hi = (lane & sh) != 0
        out = [None] * 8
        for c in range(8):
            if c & (1 << cb):
                continue
            x, y = v[c], v[c | (1 << cb)]
            out[c] = jnp.where(hi, pltpu.roll(y, sh, 1), x)
            out[c | (1 << cb)] = jnp.where(hi, y, pltpu.roll(x, 128 - sh, 1))
        v = out
    return v


def _sum4(x, lane):
    x = x + jnp.where((lane & 1) != 0, pltpu.roll(x, 1, 1), pltpu.roll(x, 127, 1))
    x = x + jnp.where((lane & 2) != 0, pltpu.roll(x, 2, 1), pltpu.roll(x, 126, 1))
    return x


def _mix(a, b):
    if not b:
        return list(a)
    if not a:
        return list(b)
    out, n, m, k = [], len(a), len(b), 0
    for i, t in enumerate(a):
        out.append(t)
        tgt = (i + 1) * m // n
        while k < tgt:
            out.append(b[k])
            k += 1
    return out


def _flat(jobs):
    return [t for j in jobs for t in j]


def _weave(mx, jobs):
    vp = _flat(jobs)
    tot = sum(c for _, c in mx)
    n, k, acc = len(vp), 0, 0
    for t, c in mx:
        t()
        acc += c
        tgt = acc * n // tot
        while k < tgt:
            vp[k]()
            k += 1
    while k < n:
        vp[k]()
        k += 1


def _kernel(one_ref, x_hbm, wqkv_hbm, wo_hbm, wg_hbm, wu_hbm, wd_hbm, out_hbm,
            xr, xn, T, wst, wqr, wqp, R, P, gst, ust, dst, B, Bd, M, H, hst, ost, acc,
            sem_x, sem_w, sem_q, sem_g, sem_u, sem_d, sem_o):

    def block(mx, jobs, name="blk"):
        with jax.named_scope(name):
            @pl.when(one_ref[0] > 0)
            def _():
                _weave(mx(), jobs())

    def x_copy(r):
        rows = pl.ds(_mult(r * 256, 256), 256)
        return pltpu.make_async_copy(x_hbm.at[rows, :], xr.at[rows, :], sem_x.at[r])

    def w_copy(j, slot):
        col = (2 - j // 4) * D + (j % 4) * QW
        return pltpu.make_async_copy(wqkv_hbm.at[:, pl.ds(_mult(col, QW), QW)], wst.at[slot], sem_w.at[slot])

    def wq_copy():
        return pltpu.make_async_copy(wqkv_hbm.at[:, pl.ds(0, D)], wqr, sem_q.at[0])

    def gu_copies(j, par):
        cols = pl.ds(_mult(j * TF, TF), TF)
        return (pltpu.make_async_copy(wg_hbm.at[:, cols], gst.at[par], sem_g.at[par]),
                pltpu.make_async_copy(wu_hbm.at[:, cols], ust.at[par], sem_u.at[par]))

    def d_copy(j, par):
        return pltpu.make_async_copy(wd_hbm.at[pl.ds(_mult(j * TF, TF), TF), :], dst.at[par], sem_d.at[par])

    def wo_copies():
        return (pltpu.make_async_copy(wo_hbm.at[:, pl.ds(0, TF)], gst.at[1], sem_g.at[1]),
                pltpu.make_async_copy(wo_hbm.at[:, pl.ds(TF, TF)], ust.at[1], sem_u.at[1]))

    def out_copy(i, a):
        par = i % 2
        return pltpu.make_async_copy(dst.at[par, pl.ds(a * RS, RS), :],
                                     out_hbm.at[pl.ds(_mult(a * HB + i * RS, RS), RS), :], sem_o.at[par * 4 + a])

    def last_copy(a, h):
        rows = RS // 2
        return pltpu.make_async_copy(dst.at[1, pl.ds(a * RS + h * rows, rows), :],
                                     out_hbm.at[pl.ds(a * HB + 3 * RS + h * rows, rows), :], sem_o.at[8 + h * 4 + a])

    def start(cps):
        for cp in cps:
            cp.start()

    def wait(cps):
        for cp in cps:
            cp.wait()

    def ln_job(g):
        def t():
            v = [xr[pl.ds(g * 16, 16), pl.ds(c * 128, 128)].astype(f32) for c in range(8)]
            a = v[0]
            for c in range(1, 8):
                a = a + v[c]
            mean = jnp.sum(a, axis=1, keepdims=True) * (1.0 / D)
            v = [x - mean for x in v]
            a = v[0] * v[0]
            for c in range(1, 8):
                a = a + v[c] * v[c]
            r = lax.rsqrt(jnp.sum(a, axis=1, keepdims=True) * (1.0 / D) + EPS)
            for c in range(8):
                xn[pl.ds(g * 8, 8), pl.ds(c * 128, 128)] = _pk(v[c] * r)
        return [t]

    def ln_jobs(r):
        return [ln_job(r * 16 + g) for g in range(16)]

    def t_job(pos_idx):
        w0 = _mult((pos_idx // 2) * 8, 8)
        l0 = _mult((pos_idx % 2) * 128, 128)

        def raw(i, j):
            return xn[pl.ds(_mult(i * 256 + w0, 8), 8), pl.ds(_mult(j * KB + l0, 128), 128)]

        def emit(p, v):
            T[p, pl.ds(w0, 8), pl.ds(l0, 128)] = v
        return _opcomb_job(lambda i, j: _unpk(raw(i, j)), A_T, emit, raw)

    def b_job(par, g, half):
        w_ref = (gst, ust)[half]

        def src(i, q):
            return w_ref[par, pl.ds(_mult(i * KB + g * 16, 16), 16), pl.ds(q * TB, TB)]

        def emit(p, v):
            B[par, p, pl.ds(_mult(g * 8, 8), 8), pl.ds(half * TB, TB)] = v
        return _opcomb_job(lambda i, q: src(i, q).astype(f32), B_T, emit,
                           lambda i, q: pltpu.bitcast(src(i, q), u32))

    def bd_job(par, g, n):
        def src(i, q):
            return dst[par, pl.ds(_mult(i * TB + g * 16, 16), 16), pl.ds(q * KB + n * 128, 128)]

        def emit(p, v):
            Bd[par, p, pl.ds(_mult(g * 8, 8), 8), pl.ds(n * 128, 128)] = v
        return _opcomb_job(lambda i, q: src(i, q).astype(f32), B_T, emit,
                           lambda i, q: pltpu.bitcast(src(i, q), u32))

    def b_jobs(par, k):
        return [b_job(par, 4 * k + g, h) for g in range(4) for h in range(2)]

    def bd_jobs(par, k):
        return [bd_job(par, 2 * k + g, n) for g in range(2) for n in range(2)]

    def perm_job(m, pair):
        def t():
            w = _mult(pair * 16, 16)
            r = _perm8([R[2 - m, c, pl.ds(w, 16), :] for c in range(8)])
            for c in range(8):
                P[m, c, pl.ds(_mult(PADW + w, 8), 16), :] = r[c]
        return [t]

    def wq_job(pair):
        def t():
            rows = pl.ds(_mult(pair * 32, 32), 32)
            r = _perm8([pltpu.bitcast(wqr[rows, pl.ds(c * 128, 128)], u32) for c in range(8)])
            for c in range(8):
                wqp[pl.ds(_mult(pair * 16, 16), 16), pl.ds(c * 128, 128)] = r[c]
        return [t]

    def attn_job(grp, sl):
        b = _mult(grp * 8, 8)
        job = []
        for h in range(2):
            st = {}
            half = lambda v, h=h: _unpk(v)[h * 8:(h + 1) * 8]

            def qk(cs, st=st, half=half):
                def t():
                    for c in cs:
                        qv = half(P[0, c, pl.ds(_mult(b + PADW, 8), 8), :])
                        for w in range(WIN):
                            kv = half(P[1, c, pl.ds(b + (PADW - w), 8), :])
                            st[w] = qv * kv if c == 0 else st[w] + qv * kv
                return t

            def sm(st=st, h=h):
                lane = lax.broadcasted_iota(jnp.int32, (8, 128), 1)
                row = lax.broadcasted_iota(jnp.int32, (8, 128), 0) + (grp * 16 + h * 8)
                ls = []
                for w in range(WIN):
                    a = _sum4(st[w], lane)
                    if w > 0:
                        a = jnp.where(row >= 2 * w, a, -1e30)
                    ls.append(a)
                m = ls[0]
                for w in range(1, WIN):
                    m = jnp.maximum(m, ls[w])
                e = [jnp.exp2((l - m) * C2) for l in ls]
                den = e[0]
                for w in range(1, WIN):
                    den = den + e[w]
                inv = 1.0 / den
                st['p'] = [x * inv for x in e]

            def pv(cs, st=st, half=half, h=h):
                def t():
                    for c in cs:
                        o = None
                        for w in range(WIN):
                            a = st['p'][w] * half(P[2, c, pl.ds(b + (PADW - w), 8), :])
                            o = a if o is None else o + a
                        ost[sl, c, pl.ds(h * 8, 8), :] = o
                return t
            job += [qk((0, 1, 2, 3)), qk((4, 5, 6, 7)), sm, pv((0, 1, 2, 3)), pv((4, 5, 6, 7))]

        def fin():
            r = _perm8([_pk(ost[sl, c, pl.ds(0, 16), :]) for c in range(8)])
            for c in range(8):
                xn[pl.ds(b, 8), pl.ds(c * 128, 128)] = r[c]
        return job + [fin]

    def comb_job(mp, g):
        sl = g % 4
        job = []
        for hf in range(2):
            for pos in POS:
                def t(hf=hf, pos=pos):
                    r = pl.ds(g * 16 + hf * 8, 8)
                    gg = _outpos(lambda p: M[mp, p, 0, r, :], pos)
                    uu = _outpos(lambda p: M[mp, p, 1, r, :], pos)
                    for q in gg:
                        hst[sl, (q[0] * 2 + pos[0]) * 4 + q[1] * 2 + pos[1], pl.ds(hf * 8, 8), :] = gg[q] * uu[q]
                job.append(t)

        def emit(p, v):
            H[mp, p, pl.ds(g * 8, 8), :] = v
        return job + _opcomb_job(lambda i, j: hst[sl, i * 4 + j, pl.ds(0, 16), :], A_T, emit)

    def comb_jobs(mp):
        return [comb_job(mp, g) for g in range(RS // 16)]

    def zero_job(p):
        def t():
            for c in range(2):
                acc[p, c, pl.ds(0, HB), :] = jnp.zeros((HB, 128), f32)
        return [t]

    def final_job(i, g, n):
        job = []
        par = i % 2
        for pos in POS:
            def t(pos=pos):
                r0 = _mult(i * RS + g * 16, 16)
                o = [_outpos(lambda p: acc[p, n, pl.ds(r0 + hf * 8, 8), :], pos) for hf in range(2)]
                for q in o[0]:
                    a = q[0] * 2 + pos[0]
                    ch = (q[1] * 2 + pos[1]) * 2 + n
                    pln = a * 8 + ch
                    cols = pl.ds(ch * 128, 128)
                    ffn = jnp.concatenate([o[0][q], o[1][q]], axis=0)
                    att = M[par, pln // 2, pln % 2, pl.ds(g * 16, 16), :]
                    res = xr[pl.ds(_mult(a * HB + r0, 16), 16), cols].astype(f32) + att + ffn
                    dst[par, pl.ds(a * RS + g * 16, 16), cols] = res.astype(bf)
            job.append(t)
        return job

    def final_jobs(i):
        return [final_job(i, g, n) for g in range(RS // 16) for n in range(2)]

    def kv_tasks(m, slot, cbase, pieces):
        out = []
        for r in pieces:
            for ct in range(QW // 128):
                def t(r=r, ct=ct):
                    res = _dot(_up(xn[pl.ds(_mult(r * 64, 64), 64), :]), wst[slot, :, pl.ds(ct * 128, 128)])
                    for k in range(8):
                        R[2 - m, cbase + ct, pl.ds(_mult(r * 64 + k * 8, 8), 8), :] = _pk(res[k * 16:(k + 1) * 16])
                out.append((t, 256))
        return out

    def q_tasks(cbase):
        out = []
        for r in range(16):
            for ct in range(QW // 128):
                def t(r=r, ct=ct):
                    res = _dot(_up(xn[pl.ds(r * 64, 64), :]),
                               _up(wqp[:, pl.ds(_mult((cbase + ct) * 128, 128), 128)]))
                    for k in range(8):
                        P[0, cbase + ct, pl.ds(PADW + r * 64 + k * 8, 8), :] = _pk(res[k * 16:(k + 1) * 16])
                out.append((t, 256))
        return out

    def mm1_tasks(mp, s, par):
        out = []
        for p in range(NP):
            for c in range(2):
                def t(p=p, c=c):
                    M[mp, p, c, pl.ds(0, RS), :] = _dot(
                        _up(T[p, pl.ds(_mult(s * (RS // 2), RS // 2), RS // 2), :]),
                        _up(B[par, p, :, pl.ds(c * 128, 128)]))
                out.append((t, 64))
        return out

    def mm2_tasks(mp, s, par):
        out = []
        for p in range(NP):
            def t(p=p):
                r = _dot(_up(H[mp, p]), _up(Bd[par, p]))
                for c in range(2):
                    acc[p, c, pl.ds(_mult(s * RS, RS), RS), :] += r[:, c * 128:(c + 1) * 128]
            out.append((t, 64))
        return out

    def wo_tasks(i):
        out = []
        for a in range(4):
            for ch in range(8):
                def t(a=a, ch=ch):
                    w_ref = (gst, ust)[ch // 4]
                    res = _dot(_up(xn[pl.ds(_mult(a * 256 + i * 64, 64), 64), :]),
                               w_ref[1, :, pl.ds((ch % 4) * 128, 128)])
                    pln = a * 8 + ch
                    M[i % 2, pln // 2, pln % 2, pl.ds(0, RS), :] = res
                out.append((t, 256))
        return out

    nothing = lambda: [(lambda: None, 1)]

    x_copy(0).start()
    w_copy(0, 0).start()
    for c in range(8):
        P[1, c, pl.ds(0, PADW), :] = jnp.zeros((PADW, 128), u32)
        P[2, c, pl.ds(0, PADW), :] = jnp.zeros((PADW, 128), u32)
    x_copy(0).wait()
    w_copy(1, 1).start()
    x_copy(1).start()
    block(nothing, lambda: ln_jobs(0), 'ln0')
    w_copy(0, 0).wait()

    def v01(pieces):
        rp = [2 * r + h for r in pieces for h in range(2)]
        return kv_tasks(2, 0, 0, rp) + kv_tasks(2, 1, 2, rp)

    block(lambda: kv_tasks(2, 0, 0, (0, 1)), lambda: [], 'p0')
    w_copy(1, 1).wait()
    x_copy(2).start()
    x_copy(1).wait()
    block(lambda: kv_tasks(2, 1, 2, (0, 1)), lambda: ln_jobs(1), 'p0')
    x_copy(3).start()
    x_copy(4).start()
    x_copy(2).wait()
    block(lambda: v01((1,)), lambda: ln_jobs(2), 'p0')
    x_copy(5).start()
    x_copy(6).start()
    x_copy(3).wait()
    x_copy(4).wait()
    block(lambda: v01((2,)), lambda: ln_jobs(3) + ln_jobs(4), 'p0')
    x_copy(7).start()
    w_copy(2, 2).start()
    x_copy(5).wait()
    x_copy(6).wait()
    block(lambda: v01((3, 4)), lambda: ln_jobs(5) + ln_jobs(6), 'p0')
    wq_copy().start()
    x_copy(7).wait()
    block(lambda: v01((5, 6)), lambda: ln_jobs(7), 'p0')
    block(lambda: v01((7,)), lambda: [], 'p0')

    def kv_block(j, m, after_start, jobs, name):
        slot = j % 3
        w_copy(j, slot).wait()

        @pl.when(j + 1 < 8)
        def _():
            w_copy(j + 1, (j + 1) % 3).start()
        after_start()
        block(lambda: kv_tasks(m, slot, (j % 4) * 2, range(16)), jobs, name)

    def v_body(j, c):
        def dmas():
            @pl.when(j == 2)
            def _():
                start(gu_copies(0, 0))

            @pl.when(j == 3)
            def _():
                d_copy(0, 0).start()
                d_copy(1, 1).start()
        kv_block(j, 2, dmas, lambda: [wq_job((j - 2) * 16 + a) for a in range(16)], 'v')
        return c
    wq_copy().wait()
    lax.fori_loop(2, 4, v_body, 0)

    def k_body(j, c):
        def dmas():
            @pl.when(j == 4)
            def _():
                start(gu_copies(1, 1))
        i = j - 4
        kv_block(j, 1, dmas, lambda: _mix([perm_job(2, i * 16 + a) for a in range(16)],
                                          [t_job(i * 12 + a) for a in range(12)]), 'k')
        return c
    lax.fori_loop(4, 8, k_body, 0)

    wait(gu_copies(0, 0))
    d_copy(0, 0).wait()

    def q_body(i, c):
        def jobs():
            extra = ([b_job(0, 4 * i + g, h) for g in range(4) for h in range(2)]
                     + [bd_job(0, i, n) for n in range(2)])
            zero = [zero_job(jnp.minimum(i * 13 + a, NP - 1)) for a in range(13)]
            rest = _mix([perm_job(1, i * 16 + a) for a in range(16)], extra)
            return _mix(rest[:-6], zero) + rest[-6:]
        block(lambda: q_tasks(i * 2), jobs, 'q')
        return c
    lax.fori_loop(0, 4, q_body, 0)

    wait(gu_copies(1, 1))
    start(gu_copies(2, 0))
    block(lambda: mm1_tasks(0, 0, 0),
          lambda: _mix(b_jobs(1, 0) + bd_jobs(0, 2) + [t_job(48 + a) for a in range(8)],
                       [attn_job(a, a % 4) for a in range(NATT0)]), 'f0')
    block(lambda: mm1_tasks(1, 1, 0),
          lambda: _mix(_mix(comb_jobs(0), b_jobs(1, 1) + bd_jobs(0, 3) + [t_job(56 + a) for a in range(8)]),
                       [attn_job(NATT0 + a, a % 4) for a in range(NATT0)]), 'f1')

    def slot(t, mp):
        j = t // 4
        s = t % 4
        par = j % 2
        if mp == 0:
            @pl.when(jnp.logical_and(s == 0, j > 0))
            def _():
                wait(gu_copies(jnp.minimum(j + 1, NCH - 1), 1 - par))

                @pl.when(j + 2 < NCH)
                def _():
                    start(gu_copies(j + 2, par))

                @pl.when(j + 2 == NCH)
                def _():
                    start(wo_copies())

            @pl.when(jnp.logical_and(s == 2, j + 1 < NCH))
            def _():
                d_copy(j + 1, 1 - par).wait()

                @pl.when(j + 2 < NCH)
                def _():
                    d_copy(j + 2, par).start()
        jd = (t + 2) // 4
        kd = (t + 2) % 4
        u = t - 2

        def jobs():
            base = _mix(comb_jobs(1 - mp), b_jobs(1 - par, s) + bd_jobs(jd % 2, kd))
            att = []
            for a in range(NATT):
                att.append(attn_job(jnp.minimum(2 * NATT0 + u * NATT + a, 127), a % 4))
            n0 = max(1, len(base) // 10)
            return base[:n0] + _mix(base[n0:-n0], att) + base[-n0:]
        block(lambda: _mix(mm1_tasks(mp, s, par), mm2_tasks(mp, (t - 2) % 4, ((t - 2) // 4) % 2)), jobs,
              'slot%d' % mp)

    def steady(it, c):
        slot(2 * it + 2, 0)
        slot(2 * it + 3, 1)
        return c
    lax.fori_loop(0, (NT - 2) // 2, steady, 0)

    block(lambda: mm2_tasks(0, 2, 0), lambda: comb_jobs(1), 'e0')
    block(lambda: _mix(wo_tasks(0), mm2_tasks(1, 3, 0)), lambda: [], 'e1')

    def wo_body(i, c):
        @pl.when(i >= 3)
        def _():
            wait([out_copy(i - 3, a) for a in range(4)])
        def jobs():
            kick = [lambda: start([out_copy(i - 1, a) for a in range(4)])]
            return final_jobs(i - 1) + [kick] + [[lambda: None] * 40]
        block(lambda: wo_tasks(i), jobs, 'wo')
        return c
    lax.fori_loop(1, 4, wo_body, 0)
    wait([out_copy(1, a) for a in range(4)])
    for h in range(2):
        block(nothing, lambda h=h: [final_job(3, g, n) for g in range(4 * h, 4 * h + 4) for n in range(2)], 'e3')
        start([last_copy(a, h) for a in range(4)])
    wait([out_copy(2, a) for a in range(4)])
    wait([last_copy(a, h) for h in range(2) for a in range(4)])


@jax.jit
def pallas_parallel_sum__sliding_local_dilated__glu_gated_bilinear__prompt_kernel(
    A_x: jax.Array,
    A_wqkv: jax.Array,
    A_wo: jax.Array,
    B_x: jax.Array,
    B_w_gate: jax.Array,
    B_w_up: jax.Array,
    B_w_down: jax.Array,
):
    del B_x
    x = A_x.reshape(S, D)
    hbm = pl.BlockSpec(memory_space=pl.ANY)
    dma = pltpu.SemaphoreType.DMA
    out = pl.pallas_call(
        _kernel,
        grid=(1,),
        in_specs=[pl.BlockSpec(memory_space=pltpu.SMEM)] + [hbm] * 6,
        out_specs=hbm,
        out_shape=jax.ShapeDtypeStruct((S, D), bf),
        scratch_shapes=[
            pltpu.VMEM((S, D), bf),
            pltpu.VMEM((S // 2, D), u32),
            pltpu.VMEM((NP, HB // 2, KB), u32),
            pltpu.VMEM((3, D, QW), bf),
            pltpu.VMEM((D, D), bf),
            pltpu.VMEM((D // 2, D), u32),
            pltpu.VMEM((2, 8, S // 2 + PADW, 128), u32),
            pltpu.VMEM((3, 8, S // 2 + PADW, 128), u32),
            pltpu.VMEM((2, D, TF), bf),
            pltpu.VMEM((2, D, TF), bf),
            pltpu.VMEM((2, TF, D), bf),
            pltpu.VMEM((2, NP, KB // 2, 2 * TB), u32),
            pltpu.VMEM((2, NP, TB // 2, KB), u32),
            pltpu.VMEM((2, NP, 2, RS + MPAD, 128), f32),
            pltpu.VMEM((2, NP, RS // 2, TB), u32),
            pltpu.VMEM((4, 16, 24, 128), f32),
            pltpu.VMEM((4, 8, 24, 128), f32),
            pltpu.VMEM((NP, 2, HB + MPAD, 128), f32),
            dma((8,)), dma((3,)), dma((1,)), dma((2,)), dma((2,)), dma((2,)), dma((16,)),
        ],
        compiler_params=pltpu.CompilerParams(
            dimension_semantics=("arbitrary",), vmem_limit_bytes=127 * 1024 * 1024,
            disable_bounds_checks=True),
        name="fused_attn_ffn",
    )(jnp.ones((1,), jnp.int32), x, A_wqkv, A_wo, B_w_gate, B_w_up, B_w_down)
    return out.reshape(1, S, D)
```

```python
import jax
import jax.numpy as jnp
from jax import lax
from jax.experimental import pallas as pl
from jax.experimental.pallas import tpu as pltpu

bf = jnp.bfloat16
f32 = jnp.float32
u32 = jnp.uint32

S, D, F = 2048, 1024, 3584
WIN = 8
NP = 49
HB = S // 4
KB = D // 4
TF = 512
TB = TF // 4
NCH = F // TF
RS = 128
NSUB = HB // RS
NT = NCH * NSUB
MPAD = 8
PADW = 8
QW = 256
EPS = 1e-5
C2 = float(32 ** -0.5 * 1.4426950408889634)

A_T = [[(1, (0, 0)), (1, (1, 1))], [(1, (1, 0)), (1, (1, 1))], [(1, (0, 0))], [(1, (1, 1))],
       [(1, (0, 0)), (1, (0, 1))], [(1, (1, 0)), (-1, (0, 0))], [(1, (0, 1)), (-1, (1, 1))]]
B_T = [[(1, (0, 0)), (1, (1, 1))], [(1, (0, 0))], [(1, (0, 1)), (-1, (1, 1))], [(1, (1, 0)), (-1, (0, 0))],
       [(1, (1, 1))], [(1, (0, 0)), (1, (0, 1))], [(1, (1, 0)), (1, (1, 1))]]
C_T = {(0, 0): [(1, 0), (1, 3), (-1, 4), (1, 6)], (0, 1): [(1, 2), (1, 4)],
       (1, 0): [(1, 1), (1, 3)], (1, 1): [(1, 0), (-1, 1), (1, 2), (1, 5)]}
POS = ((0, 0), (0, 1), (1, 0), (1, 1))


def _comb(terms):
    acc = None
    for s, v in terms:
        if acc is None:
            acc = v if s > 0 else -v
        else:
            acc = acc + v if s > 0 else acc - v
    return acc


def _dot(a, b):
    return jnp.dot(a, b, preferred_element_type=f32)


def _pk(v):
    return pltpu.bitcast(v.astype(bf), u32)


def _up(w):
    return pltpu.bitcast(w, bf)


def _unpk(w):
    return pltpu.bitcast(w, bf).astype(f32)


def _as_f32(w):
    return lax.bitcast_convert_type(w, f32)


def _as_u32(v):
    return lax.bitcast_convert_type(v, u32)


def _mult(x, m):
    return x if isinstance(x, int) else pl.multiple_of(x, m)


def _opcomb(load, table, I, emit, raw):
    sub = {(r, c): _comb([(s, load(q[0] * 2 + r, q[1] * 2 + c)) for s, q in table[I]])
           for r in range(2) for c in range(2)}
    for J, t2 in enumerate(table):
        if raw is not None and len(table[I]) == 1 and len(t2) == 1:
            qo, qi = table[I][0][1], t2[0][1]
            emit(I * 7 + J, raw(qo[0] * 2 + qi[0], qo[1] * 2 + qi[1]))
        else:
            emit(I * 7 + J, _pk(_comb([(s, sub[q]) for s, q in t2])))


def _opcomb_job(load, table, emit, raw=None):
    return [(lambda I=I: _opcomb(load, table, I, emit, raw)) for I in range(7)]


def _outpos(load, pos):
    inner = [_comb([(s, load(I * 7 + J)) for s, J in C_T[pos]]) for I in range(7)]
    return {q: _comb([(s, inner[I]) for s, I in terms]) for q, terms in C_T.items()}


def _perm8(v):
    lane = lax.broadcasted_iota(jnp.int32, v[0].shape, 1)
    v = list(v)
    for cb, lb in ((2, 4), (1, 3), (0, 2)):
        sh = 1 << lb
        hi = (lane & sh) != 0
        out = [None] * 8
        for c in range(8):
            if c & (1 << cb):
                continue
            x, y = v[c], v[c | (1 << cb)]
            out[c] = jnp.where(hi, pltpu.roll(y, sh, 1), x)
            out[c | (1 << cb)] = jnp.where(hi, y, pltpu.roll(x, 128 - sh, 1))
        v = out
    return v


def _sum4(x, lane):
    x = x + jnp.where((lane & 1) != 0, pltpu.roll(x, 1, 1), pltpu.roll(x, 127, 1))
    x = x + jnp.where((lane & 2) != 0, pltpu.roll(x, 2, 1), pltpu.roll(x, 126, 1))
    return x


def _mix(a, b):
    if not b:
        return list(a)
    if not a:
        return list(b)
    out, n, m, k = [], len(a), len(b), 0
    for i, t in enumerate(a):
        out.append(t)
        tgt = (i + 1) * m // n
        while k < tgt:
            out.append(b[k])
            k += 1
    return out


def _flat(jobs, depth=1):
    return [t for j in jobs for t in j]


def _weave(mx, jobs):
    vp = _flat(jobs)
    tot = sum(c for _, c in mx)
    n, k, acc = len(vp), 0, 0
    for t, c in mx:
        t()
        acc += c
        tgt = acc * n // tot
        while k < tgt:
            vp[k]()
            k += 1
    while k < n:
        vp[k]()
        k += 1


def _kernel(one_ref, x_hbm, wqkv_hbm, wo_hbm, wg_hbm, wu_hbm, wd_hbm, out_hbm,
            xr, xn, T, wst, wqr, wqp, R, P, gst, ust, dst, B, Bd, M, H, hst, ost, acc,
            sem_x, sem_w, sem_q, sem_g, sem_u, sem_d, sem_o):

    def block(mx, jobs, name="blk"):
        with jax.named_scope(name):
            @pl.when(one_ref[0] > 0)
            def _():
                _weave(mx(), jobs())

    def x_copy(r):
        rows = pl.ds(_mult(r * 256, 256), 256)
        return pltpu.make_async_copy(x_hbm.at[rows, :], xr.at[rows, :], sem_x.at[r])

    def w_copy(j, slot):
        col = (2 - j // 4) * D + (j % 4) * QW
        return pltpu.make_async_copy(wqkv_hbm.at[:, pl.ds(_mult(col, QW), QW)], wst.at[slot], sem_w.at[slot])

    def wq_copy():
        return pltpu.make_async_copy(wqkv_hbm.at[:, pl.ds(0, D)], wqr, sem_q.at[0])

    def gu_copies(j, par):
        cols = pl.ds(_mult(j * TF, TF), TF)
        return (pltpu.make_async_copy(wg_hbm.at[:, cols], gst.at[par], sem_g.at[par]),
                pltpu.make_async_copy(wu_hbm.at[:, cols], ust.at[par], sem_u.at[par]))

    def d_copy(j, par):
        return pltpu.make_async_copy(wd_hbm.at[pl.ds(_mult(j * TF, TF), TF), :], dst.at[par], sem_d.at[par])

    def wo_copies():
        return (pltpu.make_async_copy(wo_hbm.at[:, pl.ds(0, TF)], gst.at[1], sem_g.at[1]),
                pltpu.make_async_copy(wo_hbm.at[:, pl.ds(TF, TF)], ust.at[1], sem_u.at[1]))

    def out_copy(i, a):
        par = i % 2
        return pltpu.make_async_copy(dst.at[par, pl.ds(a * RS, RS), :],
                                     out_hbm.at[pl.ds(_mult(a * HB + i * RS, RS), RS), :], sem_o.at[par * 4 + a])

    def last_copy(a, h):
        rows = RS // 2
        return pltpu.make_async_copy(dst.at[1, pl.ds(a * RS + h * rows, rows), :],
                                     out_hbm.at[pl.ds(a * HB + 3 * RS + h * rows, rows), :], sem_o.at[8 + h * 4 + a])

    def start(cps):
        for cp in cps:
            cp.start()

    def wait(cps):
        for cp in cps:
            cp.wait()

    def ln_job(g):
        def t():
            v = [xr[pl.ds(g * 16, 16), pl.ds(c * 128, 128)].astype(f32) for c in range(8)]
            a = v[0]
            for c in range(1, 8):
                a = a + v[c]
            mean = jnp.sum(a, axis=1, keepdims=True) * (1.0 / D)
            v = [x - mean for x in v]
            a = v[0] * v[0]
            for c in range(1, 8):
                a = a + v[c] * v[c]
            r = lax.rsqrt(jnp.sum(a, axis=1, keepdims=True) * (1.0 / D) + EPS)
            for c in range(8):
                xn[pl.ds(g * 8, 8), pl.ds(c * 128, 128)] = _pk(v[c] * r)
        return [t]

    def ln_jobs(r):
        return [ln_job(r * 16 + g) for g in range(16)]

    def t_job(pos_idx):
        w0 = _mult((pos_idx // 2) * 8, 8)
        l0 = _mult((pos_idx % 2) * 128, 128)

        def raw(i, j):
            return xn[pl.ds(_mult(i * 256 + w0, 8), 8), pl.ds(_mult(j * KB + l0, 128), 128)]

        def emit(p, v):
            T[p, pl.ds(w0, 8), pl.ds(l0, 128)] = v
        return _opcomb_job(lambda i, j: _unpk(raw(i, j)), A_T, emit, raw)

    def b_job(par, g, half):
        w_ref = (gst, ust)[half]

        def src(i, q):
            return w_ref[par, pl.ds(_mult(i * KB + g * 16, 16), 16), pl.ds(q * TB, TB)]

        def emit(p, v):
            B[par, p, pl.ds(_mult(g * 8, 8), 8), pl.ds(half * TB, TB)] = v
        return _opcomb_job(lambda i, q: src(i, q).astype(f32), B_T, emit,
                           lambda i, q: pltpu.bitcast(src(i, q), u32))

    def bd_job(par, g, n):
        def src(i, q):
            return dst[par, pl.ds(_mult(i * TB + g * 16, 16), 16), pl.ds(q * KB + n * 128, 128)]

        def emit(p, v):
            Bd[par, p, pl.ds(_mult(g * 8, 8), 8), pl.ds(n * 128, 128)] = v
        return _opcomb_job(lambda i, q: src(i, q).astype(f32), B_T, emit,
                           lambda i, q: pltpu.bitcast(src(i, q), u32))

    def b_jobs(par, k):
        return [b_job(par, 4 * k + g, h) for g in range(4) for h in range(2)]

    def bd_jobs(par, k):
        return [bd_job(par, 2 * k + g, n) for g in range(2) for n in range(2)]

    def perm_job(m, pair):
        def t():
            w = _mult(pair * 16, 16)
            r = _perm8([R[2 - m, c, pl.ds(w, 16), :] for c in range(8)])
            for c in range(8):
                P[m, c, pl.ds(_mult(PADW + w, 8), 16), :] = r[c]
        return [t]

    def wq_job(pair):
        def t():
            rows = pl.ds(_mult(pair * 32, 32), 32)
            r = _perm8([pltpu.bitcast(wqr[rows, pl.ds(c * 128, 128)], u32) for c in range(8)])
            for c in range(8):
                wqp[pl.ds(_mult(pair * 16, 16), 16), pl.ds(c * 128, 128)] = r[c]
        return [t]

    def attn_quad(n, stack=False):
        base = _mult(((n % 8) // 2) * 256 + (n // 8) * 64 + (n % 2) * 32, 32)
        return [attn_job(base, 8 * k, k, stack) for k in range(4)]

    def attn_job(base, off, sl, stack):
        b = base + off
        job = []
        for h in range(2):
            st = {}
            half = lambda v, h=h: _unpk(v)[h * 8:(h + 1) * 8]

            def qk(cs, st=st, half=half):
                def t():
                    for c in cs:
                        qv = half(P[0, c, pl.ds(base + (off + PADW), 8), :])
                        for w in range(WIN):
                            kv = half(P[1, c, pl.ds(base + (off + PADW - w), 8), :])
                            st[w] = qv * kv if c == 0 else st[w] + qv * kv
                return t

            def sm(st=st, h=h):
                lane = lax.broadcasted_iota(jnp.int32, (8, 128), 1)
                row = lax.broadcasted_iota(jnp.int32, (8, 128), 0) + (b * 2 + h * 8)
                if stack:
                    big = jnp.concatenate([st[w] for w in range(WIN)], axis=0)
                    big = _sum4(big, lax.broadcasted_iota(jnp.int32, (8 * WIN, 128), 1))
                    ls = [big[8 * w:8 * w + 8] for w in range(WIN)]
                else:
                    ls = [_sum4(st[w], lane) for w in range(WIN)]
                ls = [ls[0]] + [jnp.where(row >= 2 * w, ls[w], -1e30) for w in range(1, WIN)]
                m = ls[0]
                for w in range(1, WIN):
                    m = jnp.maximum(m, ls[w])
                e = [jnp.exp2((l - m) * C2) for l in ls]
                den = e[0]
                for w in range(1, WIN):
                    den = den + e[w]
                inv = 1.0 / den
                st['p'] = [x * inv for x in e]

            def pv(cs, st=st, half=half, h=h):
                def t():
                    for c in cs:
                        o = None
                        for w in range(WIN):
                            a = st['p'][w] * half(P[2, c, pl.ds(base + (off + PADW - w), 8), :])
                            o = a if o is None else o + a
                        ost[sl, c, pl.ds(h * 8, 8), :] = o
                return t
            job += [qk((0, 1, 2, 3)), qk((4, 5, 6, 7)), sm, pv((0, 1, 2, 3)), pv((4, 5, 6, 7))]

        def fin():
            r = _perm8([_pk(ost[sl, c, pl.ds(0, 16), :]) for c in range(8)])
            for c in range(8):
                xn[pl.ds(_mult(b, 8), 8), pl.ds(c * 128, 128)] = r[c]
        return job + [fin]

    def comb_job(mp, g):
        sl = g % 4
        job = []
        for hf in range(2):
            for pos in POS:
                def t(hf=hf, pos=pos):
                    r = pl.ds(g * 16 + hf * 8, 8)
                    gg = _outpos(lambda p: M[mp, p, 0, r, :], pos)
                    uu = _outpos(lambda p: M[mp, p, 1, r, :], pos)
                    for q in gg:
                        hst[sl, (q[0] * 2 + pos[0]) * 4 + q[1] * 2 + pos[1], pl.ds(hf * 8, 8), :] = gg[q] * uu[q]
                job.append(t)

        def emit(p, v):
            H[mp, p, pl.ds(g * 8, 8), :] = v
        return job + _opcomb_job(lambda i, j: hst[sl, i * 4 + j, pl.ds(0, 16), :], A_T, emit)

    def comb_jobs(mp):
        return [comb_job(mp, g) for g in range(RS // 16)]

    def zero_job(p):
        def t():
            for c in range(2):
                acc[p, c, pl.ds(0, HB), :] = jnp.zeros((HB, 128), f32)
        return [t]

    def final_job(i, g, n):
        job = []
        par = i % 2
        for pos in POS:
            def t(pos=pos):
                r0 = _mult(i * RS + g * 16, 16)
                o = [_outpos(lambda p: acc[p, n, pl.ds(r0 + hf * 8, 8), :], pos) for hf in range(2)]
                for q in o[0]:
                    a = q[0] * 2 + pos[0]
                    ch = (q[1] * 2 + pos[1]) * 2 + n
                    pln = a * 8 + ch
                    cols = pl.ds(ch * 128, 128)
                    ffn = jnp.concatenate([o[0][q], o[1][q]], axis=0)
                    att = M[par, pln // 2, pln % 2, pl.ds(g * 16, 16), :]
                    res = xr[pl.ds(_mult(a * HB + r0, 16), 16), cols].astype(f32) + att + ffn
                    dst[par, pl.ds(a * RS + g * 16, 16), cols] = res.astype(bf)
            job.append(t)
        return job

    def final_jobs(i):
        return [final_job(i, g, n) for g in range(RS // 16) for n in range(2)]

    def kv_tasks(m, slot, cbase, pieces):
        out = []
        for r in pieces:
            for ct in range(QW // 128):
                def t(r=r, ct=ct):
                    res = _dot(_up(xn[pl.ds(_mult(r * 64, 64), 64), :]), wst[slot, :, pl.ds(ct * 128, 128)])
                    for k in range(8):
                        R[2 - m, cbase + ct, pl.ds(_mult(r * 64 + k * 8, 8), 8), :] = _pk(res[k * 16:(k + 1) * 16])
                out.append((t, 256))
        return out

    def q_tasks(cbase):
        out = []
        for r in range(16):
            for ct in range(QW // 128):
                def t(r=r, ct=ct):
                    res = _dot(_up(xn[pl.ds(r * 64, 64), :]),
                               _up(wqp[:, pl.ds(_mult((cbase + ct) * 128, 128), 128)]))
                    for k in range(8):
                        P[0, cbase + ct, pl.ds(PADW + r * 64 + k * 8, 8), :] = _pk(res[k * 16:(k + 1) * 16])
                out.append((t, 256))
        return out

    def mm1_tasks(mp, s, par):
        out = []
        for p in range(NP):
            for c in range(2):
                def t(p=p, c=c):
                    M[mp, p, c, pl.ds(0, RS), :] = _dot(
                        _up(T[p, pl.ds(_mult(s * (RS // 2), RS // 2), RS // 2), :]),
                        _up(B[par, p, :, pl.ds(c * 128, 128)]))
                out.append((t, 64))
        return out

    def mm2_tasks(mp, s, par):
        out = []
        for p in range(NP):
            def t(p=p):
                r = _dot(_up(H[mp, p]), _up(Bd[par, p]))
                for c in range(2):
                    acc[p, c, pl.ds(_mult(s * RS, RS), RS), :] += r[:, c * 128:(c + 1) * 128]
            out.append((t, 64))
        return out

    def wo_tasks(i):
        out = []
        for a in range(4):
            for ch in range(8):
                def t(a=a, ch=ch):
                    w_ref = (gst, ust)[ch // 4]
                    res = _dot(_up(xn[pl.ds(_mult(a * 256 + i * 64, 64), 64), :]),
                               w_ref[1, :, pl.ds((ch % 4) * 128, 128)])
                    pln = a * 8 + ch
                    M[i % 2, pln // 2, pln % 2, pl.ds(0, RS), :] = res
                out.append((t, 256))
        return out

    nothing = lambda: [(lambda: None, 1)]

    x_copy(0).start()
    w_copy(0, 0).start()
    for c in range(8):
        P[1, c, pl.ds(0, PADW), :] = jnp.zeros((PADW, 128), u32)
        P[2, c, pl.ds(0, PADW), :] = jnp.zeros((PADW, 128), u32)
    x_copy(0).wait()
    w_copy(1, 1).start()
    x_copy(1).start()
    block(nothing, lambda: ln_jobs(0), 'ln0')
    w_copy(0, 0).wait()

    def v01(pieces):
        rp = [2 * r + h for r in pieces for h in range(2)]
        return kv_tasks(2, 0, 0, rp) + kv_tasks(2, 1, 2, rp)

    block(lambda: kv_tasks(2, 0, 0, (0, 1)), lambda: [], 'p0')
    w_copy(1, 1).wait()
    x_copy(2).start()
    x_copy(1).wait()
    block(lambda: kv_tasks(2, 1, 2, (0, 1)), lambda: ln_jobs(1), 'p0')
    x_copy(3).start()
    x_copy(4).start()
    x_copy(2).wait()
    block(lambda: v01((1,)), lambda: ln_jobs(2), 'p0')
    x_copy(5).start()
    x_copy(6).start()
    x_copy(3).wait()
    x_copy(4).wait()
    block(lambda: v01((2,)), lambda: ln_jobs(3) + ln_jobs(4), 'p0')
    x_copy(7).start()
    w_copy(2, 2).start()
    x_copy(5).wait()
    x_copy(6).wait()
    block(lambda: v01((3, 4)), lambda: ln_jobs(5) + ln_jobs(6), 'p0')
    wq_copy().start()
    x_copy(7).wait()
    block(lambda: v01((5, 6)), lambda: ln_jobs(7), 'p0')
    block(lambda: v01((7,)), lambda: [], 'p0')

    def kv_block(j, m, after_start, jobs, name):
        slot = j % 3
        w_copy(j, slot).wait()

        @pl.when(j + 1 < 8)
        def _():
            w_copy(j + 1, (j + 1) % 3).start()
        after_start()
        block(lambda: kv_tasks(m, slot, (j % 4) * 2, range(16)), jobs, name)

    def v_body(j, c):
        def dmas():
            @pl.when(j == 2)
            def _():
                start(gu_copies(0, 0))

            @pl.when(j == 3)
            def _():
                d_copy(0, 0).start()
                d_copy(1, 1).start()
        kv_block(j, 2, dmas, lambda: [wq_job((j - 2) * 16 + a) for a in range(16)], 'v')
        return c
    wq_copy().wait()
    lax.fori_loop(2, 4, v_body, 0)

    def k_body(j, c):
        def dmas():
            @pl.when(j == 4)
            def _():
                start(gu_copies(1, 1))
        i = j - 4
        kv_block(j, 1, dmas, lambda: _mix([perm_job(2, i * 16 + a) for a in range(16)],
                                          [t_job(i * 12 + a) for a in range(12)]), 'k')
        return c
    lax.fori_loop(4, 8, k_body, 0)

    wait(gu_copies(0, 0))
    d_copy(0, 0).wait()

    def q_body(i, c):
        def jobs():
            extra = ([b_job(0, 4 * i + g, h) for g in range(4) for h in range(2)]
                     + [bd_job(0, i, n) for n in range(2)])
            zero = [zero_job(jnp.minimum(i * 13 + a, NP - 1)) for a in range(13)]
            rest = _mix([perm_job(1, i * 16 + a) for a in range(16)], extra)
            return _mix(rest[:-6], zero) + rest[-6:]
        block(lambda: q_tasks(i * 2), jobs, 'q')
        return c
    lax.fori_loop(0, 4, q_body, 0)

    wait(gu_copies(1, 1))
    start(gu_copies(2, 0))
    block(lambda: mm1_tasks(0, 0, 0),
          lambda: _mix(b_jobs(1, 0) + bd_jobs(0, 2) + [t_job(48 + a) for a in range(8)],
                       attn_quad(0, True)), 'f0')
    block(lambda: mm1_tasks(1, 1, 0),
          lambda: _mix(_mix(comb_jobs(0), b_jobs(1, 1) + bd_jobs(0, 3) + [t_job(56 + a) for a in range(8)]),
                       attn_quad(1, True)), 'f1')

    def slot(t, mp):
        j = t // 4
        s = t % 4
        par = j % 2
        if mp == 0:
            @pl.when(jnp.logical_and(s == 0, j > 0))
            def _():
                wait(gu_copies(jnp.minimum(j + 1, NCH - 1), 1 - par))

                @pl.when(j + 2 < NCH)
                def _():
                    start(gu_copies(j + 2, par))

                @pl.when(j + 2 == NCH)
                def _():
                    start(wo_copies())

            @pl.when(jnp.logical_and(s == 2, j + 1 < NCH))
            def _():
                d_copy(j + 1, 1 - par).wait()

                @pl.when(j + 2 < NCH)
                def _():
                    d_copy(j + 2, par).start()
        jd = (t + 2) // 4
        kd = (t + 2) % 4
        u = t - 2

        def jobs():
            base = _mix(comb_jobs(1 - mp), b_jobs(1 - par, s) + bd_jobs(jd % 2, kd))
            att = attn_quad(u + 2)
            n0 = max(1, len(base) // 10)
            return base[:n0] + _mix(base[n0:-n0], att) + base[-n0:]
        block(lambda: _mix(mm1_tasks(mp, s, par), mm2_tasks(mp, (t - 2) % 4, ((t - 2) // 4) % 2)), jobs,
              'slot%d' % mp)

    def steady(it, c):
        slot(2 * it + 2, 0)
        slot(2 * it + 3, 1)
        return c
    lax.fori_loop(0, (NT - 2) // 2, steady, 0)

    block(lambda: mm2_tasks(0, 2, 0), lambda: _mix(comb_jobs(1), attn_quad(28, True)), 'e0')
    block(lambda: _mix(wo_tasks(0), mm2_tasks(1, 3, 0)),
          lambda: _flat([attn_quad(n, True) for n in range(29, 32)], 1) + [[lambda: None] * 20], 'e1')

    def wo_body(i, c):
        @pl.when(i >= 3)
        def _():
            wait([out_copy(i - 3, a) for a in range(4)])
        def jobs():
            kick = [lambda: start([out_copy(i - 1, a) for a in range(4)])]
            return final_jobs(i - 1) + [kick] + [[lambda: None] * 40]
        block(lambda: wo_tasks(i), jobs, 'wo')
        return c
    lax.fori_loop(1, 4, wo_body, 0)
    wait([out_copy(1, a) for a in range(4)])
    for h in range(2):
        block(nothing, lambda h=h: [final_job(3, g, n) for g in range(4 * h, 4 * h + 4) for n in range(2)], 'e3')
        start([last_copy(a, h) for a in range(4)])
    wait([out_copy(2, a) for a in range(4)])
    wait([last_copy(a, h) for h in range(2) for a in range(4)])


@jax.jit
def pallas_parallel_sum__sliding_local_dilated__glu_gated_bilinear__prompt_kernel(
    A_x: jax.Array,
    A_wqkv: jax.Array,
    A_wo: jax.Array,
    B_x: jax.Array,
    B_w_gate: jax.Array,
    B_w_up: jax.Array,
    B_w_down: jax.Array,
):
    del B_x
    x = A_x.reshape(S, D)
    hbm = pl.BlockSpec(memory_space=pl.ANY)
    dma = pltpu.SemaphoreType.DMA
    out = pl.pallas_call(
        _kernel,
        grid=(1,),
        in_specs=[pl.BlockSpec(memory_space=pltpu.SMEM)] + [hbm] * 6,
        out_specs=hbm,
        out_shape=jax.ShapeDtypeStruct((S, D), bf),
        scratch_shapes=[
            pltpu.VMEM((S, D), bf),
            pltpu.VMEM((S // 2, D), u32),
            pltpu.VMEM((NP, HB // 2, KB), u32),
            pltpu.VMEM((3, D, QW), bf),
            pltpu.VMEM((D, D), bf),
            pltpu.VMEM((D // 2, D), u32),
            pltpu.VMEM((2, 8, S // 2 + PADW, 128), u32),
            pltpu.VMEM((3, 8, S // 2 + PADW, 128), u32),
            pltpu.VMEM((2, D, TF), bf),
            pltpu.VMEM((2, D, TF), bf),
            pltpu.VMEM((2, TF, D), bf),
            pltpu.VMEM((2, NP, KB // 2, 2 * TB), u32),
            pltpu.VMEM((2, NP, TB // 2, KB), u32),
            pltpu.VMEM((2, NP, 2, RS + MPAD, 128), f32),
            pltpu.VMEM((2, NP, RS // 2, TB), u32),
            pltpu.VMEM((4, 16, 24, 128), f32),
            pltpu.VMEM((4, 8, 24, 128), f32),
            pltpu.VMEM((NP, 2, HB + MPAD, 128), f32),
            dma((8,)), dma((3,)), dma((1,)), dma((2,)), dma((2,)), dma((2,)), dma((16,)),
        ],
        compiler_params=pltpu.CompilerParams(
            dimension_semantics=("arbitrary",), vmem_limit_bytes=127 * 1024 * 1024,
            disable_bounds_checks=True),
        name="fused_attn_ffn",
    )(jnp.ones((1,), jnp.int32), x, A_wqkv, A_wo, B_w_gate, B_w_up, B_w_down)
    return out.reshape(1, S, D)
```

```python
import jax
import jax.numpy as jnp
from jax import lax
from jax.experimental import pallas as pl
from jax.experimental.pallas import tpu as pltpu

bf = jnp.bfloat16
f32 = jnp.float32
u32 = jnp.uint32

S, D, F = 2048, 1024, 3584
WIN = 8
NP = 49
HB = S // 4
KB = D // 4
TF = 512
TB = TF // 4
NCH = F // TF
RS = 128
NSUB = HB // RS
NT = NCH * NSUB
MPAD = 8
PADW = 8
QW = 256
EPS = 1e-5
C2 = float(32 ** -0.5 * 1.4426950408889634)

A_T = [[(1, (0, 0)), (1, (1, 1))], [(1, (1, 0)), (1, (1, 1))], [(1, (0, 0))], [(1, (1, 1))],
       [(1, (0, 0)), (1, (0, 1))], [(1, (1, 0)), (-1, (0, 0))], [(1, (0, 1)), (-1, (1, 1))]]
B_T = [[(1, (0, 0)), (1, (1, 1))], [(1, (0, 0))], [(1, (0, 1)), (-1, (1, 1))], [(1, (1, 0)), (-1, (0, 0))],
       [(1, (1, 1))], [(1, (0, 0)), (1, (0, 1))], [(1, (1, 0)), (1, (1, 1))]]
C_T = {(0, 0): [(1, 0), (1, 3), (-1, 4), (1, 6)], (0, 1): [(1, 2), (1, 4)],
       (1, 0): [(1, 1), (1, 3)], (1, 1): [(1, 0), (-1, 1), (1, 2), (1, 5)]}
POS = ((0, 0), (0, 1), (1, 0), (1, 1))


def _comb(terms):
    acc = None
    for s, v in terms:
        if acc is None:
            acc = v if s > 0 else -v
        else:
            acc = acc + v if s > 0 else acc - v
    return acc


def _dot(a, b):
    return jnp.dot(a, b, preferred_element_type=f32)


def _pk(v):
    return pltpu.bitcast(v.astype(bf), u32)


def _up(w):
    return pltpu.bitcast(w, bf)


def _unpk(w):
    return pltpu.bitcast(w, bf).astype(f32)


def _as_f32(w):
    return lax.bitcast_convert_type(w, f32)


def _as_u32(v):
    return lax.bitcast_convert_type(v, u32)


def _mult(x, m):
    return x if isinstance(x, int) else pl.multiple_of(x, m)


def _opcomb(load, table, I, emit, raw):
    sub = {(r, c): _comb([(s, load(q[0] * 2 + r, q[1] * 2 + c)) for s, q in table[I]])
           for r in range(2) for c in range(2)}
    for J, t2 in enumerate(table):
        if raw is not None and len(table[I]) == 1 and len(t2) == 1:
            qo, qi = table[I][0][1], t2[0][1]
            emit(I * 7 + J, raw(qo[0] * 2 + qi[0], qo[1] * 2 + qi[1]))
        else:
            emit(I * 7 + J, _pk(_comb([(s, sub[q]) for s, q in t2])))


def _opcomb_job(load, table, emit, raw=None):
    return [(lambda I=I: _opcomb(load, table, I, emit, raw)) for I in range(7)]


def _outpos(load, pos):
    inner = [_comb([(s, load(I * 7 + J)) for s, J in C_T[pos]]) for I in range(7)]
    return {q: _comb([(s, inner[I]) for s, I in terms]) for q, terms in C_T.items()}


def _perm8(v):
    lane = lax.broadcasted_iota(jnp.int32, v[0].shape, 1)
    v = list(v)
    for cb, lb in ((2, 4), (1, 3), (0, 2)):
        sh = 1 << lb
        hi = (lane & sh) != 0
        out = [None] * 8
        for c in range(8):
            if c & (1 << cb):
                continue
            x, y = v[c], v[c | (1 << cb)]
            out[c] = jnp.where(hi, pltpu.roll(y, sh, 1), x)
            out[c | (1 << cb)] = jnp.where(hi, y, pltpu.roll(x, 128 - sh, 1))
        v = out
    return v


def _sum4(x, lane):
    x = x + jnp.where((lane & 1) != 0, pltpu.roll(x, 1, 1), pltpu.roll(x, 127, 1))
    x = x + jnp.where((lane & 2) != 0, pltpu.roll(x, 2, 1), pltpu.roll(x, 126, 1))
    return x


def _mix(a, b):
    if not b:
        return list(a)
    if not a:
        return list(b)
    out, n, m, k = [], len(a), len(b), 0
    for i, t in enumerate(a):
        out.append(t)
        tgt = (i + 1) * m // n
        while k < tgt:
            out.append(b[k])
            k += 1
    return out


def _flat(jobs, depth=1):
    return [t for j in jobs for t in j]


def _weave(mx, jobs, woff=0):
    vp = _flat(jobs)
    tot = sum(c for _, c in mx)
    n, k, acc = len(vp), 0, 0
    for t, c in mx:
        t()
        acc += c
        tgt = min(n, acc * n // tot + woff)
        while k < tgt:
            vp[k]()
            k += 1
    while k < n:
        vp[k]()
        k += 1


def _kernel(one_ref, x_hbm, wqkv_hbm, wo_hbm, wg_hbm, wu_hbm, wd_hbm, out_hbm,
            xr, xn, T, wst, wqr, wqp, R, P, gst, ust, dst, B, Bd, M, H, hst, ost, acc,
            sem_x, sem_w, sem_q, sem_g, sem_u, sem_d, sem_o):

    def block(mx, jobs, name="blk", woff=0):
        with jax.named_scope(name):
            @pl.when(one_ref[0] > 0)
            def _():
                _weave(mx(), jobs(), woff)

    def x_copy(r):
        rows = pl.ds(_mult(r * 256, 256), 256)
        return pltpu.make_async_copy(x_hbm.at[rows, :], xr.at[rows, :], sem_x.at[r])

    def w_copy(j, slot):
        col = (2 - j // 4) * D + (j % 4) * QW
        return pltpu.make_async_copy(wqkv_hbm.at[:, pl.ds(_mult(col, QW), QW)], wst.at[slot], sem_w.at[slot])

    def wq_copy():
        return pltpu.make_async_copy(wqkv_hbm.at[:, pl.ds(0, D)], wqr, sem_q.at[0])

    def gu_copies(j, par):
        cols = pl.ds(_mult(j * TF, TF), TF)
        return (pltpu.make_async_copy(wg_hbm.at[:, cols], gst.at[par], sem_g.at[par]),
                pltpu.make_async_copy(wu_hbm.at[:, cols], ust.at[par], sem_u.at[par]))

    def d_copy(j, par):
        return pltpu.make_async_copy(wd_hbm.at[pl.ds(_mult(j * TF, TF), TF), :], dst.at[par], sem_d.at[par])

    def wo_copies():
        return (pltpu.make_async_copy(wo_hbm.at[:, pl.ds(0, TF)], gst.at[1], sem_g.at[1]),
                pltpu.make_async_copy(wo_hbm.at[:, pl.ds(TF, TF)], ust.at[1], sem_u.at[1]))

    def out_copy(i, a):
        par = i % 2
        return pltpu.make_async_copy(dst.at[par, pl.ds(a * RS, RS), :],
                                     out_hbm.at[pl.ds(_mult(a * HB + i * RS, RS), RS), :], sem_o.at[par * 4 + a])

    def last_copy(a, h):
        rows = RS // 2
        return pltpu.make_async_copy(dst.at[1, pl.ds(a * RS + h * rows, rows), :],
                                     out_hbm.at[pl.ds(a * HB + 3 * RS + h * rows, rows), :], sem_o.at[8 + h * 4 + a])

    def start(cps):
        for cp in cps:
            cp.start()

    def wait(cps):
        for cp in cps:
            cp.wait()

    def ln_job(g):
        def t():
            v = [xr[pl.ds(g * 16, 16), pl.ds(c * 128, 128)].astype(f32) for c in range(8)]
            a = v[0]
            for c in range(1, 8):
                a = a + v[c]
            mean = jnp.sum(a, axis=1, keepdims=True) * (1.0 / D)
            v = [x - mean for x in v]
            a = v[0] * v[0]
            for c in range(1, 8):
                a = a + v[c] * v[c]
            r = lax.rsqrt(jnp.sum(a, axis=1, keepdims=True) * (1.0 / D) + EPS)
            for c in range(8):
                xn[pl.ds(g * 8, 8), pl.ds(c * 128, 128)] = _pk(v[c] * r)
        return [t]

    def ln_jobs(r):
        return [ln_job(r * 16 + g) for g in range(16)]

    def t_job(pos_idx):
        w0 = _mult((pos_idx // 2) * 8, 8)
        l0 = _mult((pos_idx % 2) * 128, 128)

        def raw(i, j):
            return xn[pl.ds(_mult(i * 256 + w0, 8), 8), pl.ds(_mult(j * KB + l0, 128), 128)]

        def emit(p, v):
            T[p, pl.ds(w0, 8), pl.ds(l0, 128)] = v
        return _opcomb_job(lambda i, j: _unpk(raw(i, j)), A_T, emit, raw)

    def b_job(par, g, half):
        w_ref = (gst, ust)[half]

        def src(i, q):
            return w_ref[par, pl.ds(_mult(i * KB + g * 16, 16), 16), pl.ds(q * TB, TB)]

        def emit(p, v):
            B[par, p, pl.ds(_mult(g * 8, 8), 8), pl.ds(half * TB, TB)] = v
        return _opcomb_job(lambda i, q: src(i, q).astype(f32), B_T, emit,
                           lambda i, q: pltpu.bitcast(src(i, q), u32))

    def bd_job(par, g, n):
        def src(i, q):
            return dst[par, pl.ds(_mult(i * TB + g * 16, 16), 16), pl.ds(q * KB + n * 128, 128)]

        def emit(p, v):
            Bd[par, p, pl.ds(_mult(g * 8, 8), 8), pl.ds(n * 128, 128)] = v
        return _opcomb_job(lambda i, q: src(i, q).astype(f32), B_T, emit,
                           lambda i, q: pltpu.bitcast(src(i, q), u32))

    def b_jobs(par, k):
        return [b_job(par, 4 * k + g, h) for g in range(4) for h in range(2)]

    def bd_jobs(par, k):
        return [bd_job(par, 2 * k + g, n) for g in range(2) for n in range(2)]

    def perm_job(m, pair):
        def t():
            w = _mult(pair * 16, 16)
            r = _perm8([R[2 - m, c, pl.ds(w, 16), :] for c in range(8)])
            for c in range(8):
                P[m, c, pl.ds(_mult(PADW + w, 8), 16), :] = r[c]
        return [t]

    def wq_job(pair):
        def t():
            rows = pl.ds(_mult(pair * 32, 32), 32)
            r = _perm8([pltpu.bitcast(wqr[rows, pl.ds(c * 128, 128)], u32) for c in range(8)])
            for c in range(8):
                wqp[pl.ds(_mult(pair * 16, 16), 16), pl.ds(c * 128, 128)] = r[c]
        return [t]

    def attn_quad(n, stack=False):
        base = _mult(((n % 8) // 2) * 256 + (n // 8) * 64 + (n % 2) * 32, 32)
        return [attn_job(base, 8 * k, k, stack) for k in range(4)]

    def attn_job(base, off, sl, stack):
        b = base + off
        job = []
        for h in range(2):
            st = {}
            half = lambda v, h=h: _unpk(v)[h * 8:(h + 1) * 8]

            def qk(cs, st=st, half=half):
                def t():
                    for c in cs:
                        qv = half(P[0, c, pl.ds(base + (off + PADW), 8), :])
                        for w in range(WIN):
                            kv = half(P[1, c, pl.ds(base + (off + PADW - w), 8), :])
                            st[w] = qv * kv if c == 0 else st[w] + qv * kv
                return t

            def sm(st=st, h=h):
                lane = lax.broadcasted_iota(jnp.int32, (8, 128), 1)
                row = lax.broadcasted_iota(jnp.int32, (8, 128), 0) + (b * 2 + h * 8)
                if stack:
                    big = jnp.concatenate([st[w] for w in range(WIN)], axis=0)
                    big = _sum4(big, lax.broadcasted_iota(jnp.int32, (8 * WIN, 128), 1))
                    ls = [big[8 * w:8 * w + 8] for w in range(WIN)]
                else:
                    ls = [_sum4(st[w], lane) for w in range(WIN)]
                ls = [ls[0]] + [jnp.where(row >= 2 * w, ls[w], -1e30) for w in range(1, WIN)]
                m = ls[0]
                for w in range(1, WIN):
                    m = jnp.maximum(m, ls[w])
                e = [jnp.exp2((l - m) * C2) for l in ls]
                den = e[0]
                for w in range(1, WIN):
                    den = den + e[w]
                inv = 1.0 / den
                st['p'] = [x * inv for x in e]

            def pv(cs, st=st, half=half, h=h):
                def t():
                    for c in cs:
                        o = None
                        for w in range(WIN):
                            a = st['p'][w] * half(P[2, c, pl.ds(base + (off + PADW - w), 8), :])
                            o = a if o is None else o + a
                        ost[sl, c, pl.ds(h * 8, 8), :] = o
                return t
            ag = 4 if stack else 2
            job += ([qk(tuple(range(c, c + ag))) for c in range(0, 8, ag)] + [sm]
                    + [pv(tuple(range(c, c + ag))) for c in range(0, 8, ag)])

        def fin():
            r = _perm8([_pk(ost[sl, c, pl.ds(0, 16), :]) for c in range(8)])
            for c in range(8):
                xn[pl.ds(_mult(b, 8), 8), pl.ds(c * 128, 128)] = r[c]
        return job + [fin]

    def comb_job(mp, g):
        sl = g % 4
        job = []
        for hf in range(2):
            for pos in POS:
                def t(hf=hf, pos=pos):
                    r = pl.ds(g * 16 + hf * 8, 8)
                    gg = _outpos(lambda p: M[mp, p, 0, r, :], pos)
                    uu = _outpos(lambda p: M[mp, p, 1, r, :], pos)
                    for q in gg:
                        hst[sl, (q[0] * 2 + pos[0]) * 4 + q[1] * 2 + pos[1], pl.ds(hf * 8, 8), :] = gg[q] * uu[q]
                job.append(t)

        def emit(p, v):
            H[mp, p, pl.ds(g * 8, 8), :] = v
        return job + _opcomb_job(lambda i, j: hst[sl, i * 4 + j, pl.ds(0, 16), :], A_T, emit)

    def comb_jobs(mp):
        return [comb_job(mp, g) for g in range(RS // 16)]

    def zero_job(p):
        def t():
            for c in range(2):
                acc[p, c, pl.ds(0, HB), :] = jnp.zeros((HB, 128), f32)
        return [t]

    def final_job(i, g, n):
        job = []
        par = i % 2
        for pos in POS:
            def t(pos=pos):
                r0 = _mult(i * RS + g * 16, 16)
                o = [_outpos(lambda p: acc[p, n, pl.ds(r0 + hf * 8, 8), :], pos) for hf in range(2)]
                for q in o[0]:
                    a = q[0] * 2 + pos[0]
                    ch = (q[1] * 2 + pos[1]) * 2 + n
                    pln = a * 8 + ch
                    cols = pl.ds(ch * 128, 128)
                    ffn = jnp.concatenate([o[0][q], o[1][q]], axis=0)
                    att = M[par, pln // 2, pln % 2, pl.ds(g * 16, 16), :]
                    res = xr[pl.ds(_mult(a * HB + r0, 16), 16), cols].astype(f32) + att + ffn
                    dst[par, pl.ds(a * RS + g * 16, 16), cols] = res.astype(bf)
            job.append(t)
        return job

    def final_jobs(i):
        return [final_job(i, g, n) for g in range(RS // 16) for n in range(2)]

    def kv_tasks(m, slot, cbase, pieces):
        out = []
        for r in pieces:
            for ct in range(QW // 128):
                def t(r=r, ct=ct):
                    res = _dot(_up(xn[pl.ds(_mult(r * 64, 64), 64), :]), wst[slot, :, pl.ds(ct * 128, 128)])
                    for k in range(8):
                        R[2 - m, cbase + ct, pl.ds(_mult(r * 64 + k * 8, 8), 8), :] = _pk(res[k * 16:(k + 1) * 16])
                out.append((t, 256))
        return out

    def q_tasks(cbase):
        out = []
        for r in range(16):
            for ct in range(QW // 128):
                def t(r=r, ct=ct):
                    res = _dot(_up(xn[pl.ds(r * 64, 64), :]),
                               _up(wqp[:, pl.ds(_mult((cbase + ct) * 128, 128), 128)]))
                    for k in range(8):
                        P[0, cbase + ct, pl.ds(PADW + r * 64 + k * 8, 8), :] = _pk(res[k * 16:(k + 1) * 16])
                out.append((t, 256))
        return out

    def mm1_tasks(mp, s, par):
        out = []
        for p in range(NP):
            for c in range(2):
                def t(p=p, c=c):
                    M[mp, p, c, pl.ds(0, RS), :] = _dot(
                        _up(T[p, pl.ds(_mult(s * (RS // 2), RS // 2), RS // 2), :]),
                        _up(B[par, p, :, pl.ds(c * 128, 128)]))
                out.append((t, 64))
        return out

    def mm2_tasks(mp, s, par):
        out = []
        for p in range(NP):
            def t(p=p):
                r = _dot(_up(H[mp, p]), _up(Bd[par, p]))
                for c in range(2):
                    acc[p, c, pl.ds(_mult(s * RS, RS), RS), :] += r[:, c * 128:(c + 1) * 128]
            out.append((t, 64))
        return out

    def wo_tasks(i):
        out = []
        for a in range(4):
            for ch in range(8):
                def t(a=a, ch=ch):
                    w_ref = (gst, ust)[ch // 4]
                    res = _dot(_up(xn[pl.ds(_mult(a * 256 + i * 64, 64), 64), :]),
                               w_ref[1, :, pl.ds((ch % 4) * 128, 128)])
                    pln = a * 8 + ch
                    M[i % 2, pln // 2, pln % 2, pl.ds(0, RS), :] = res
                out.append((t, 256))
        return out

    nothing = lambda: [(lambda: None, 1)]

    x_copy(0).start()
    w_copy(0, 0).start()
    for c in range(8):
        P[1, c, pl.ds(0, PADW), :] = jnp.zeros((PADW, 128), u32)
        P[2, c, pl.ds(0, PADW), :] = jnp.zeros((PADW, 128), u32)
    x_copy(0).wait()
    w_copy(1, 1).start()
    x_copy(1).start()
    block(nothing, lambda: ln_jobs(0), 'ln0')
    w_copy(0, 0).wait()

    def v01(pieces):
        rp = [2 * r + h for r in pieces for h in range(2)]
        return kv_tasks(2, 0, 0, rp) + kv_tasks(2, 1, 2, rp)

    block(lambda: kv_tasks(2, 0, 0, (0, 1)), lambda: [], 'p0')
    w_copy(1, 1).wait()
    x_copy(2).start()
    x_copy(1).wait()
    block(lambda: kv_tasks(2, 1, 2, (0, 1)), lambda: ln_jobs(1), 'p0')
    x_copy(3).start()
    x_copy(4).start()
    x_copy(2).wait()
    block(lambda: v01((1,)), lambda: ln_jobs(2), 'p0')
    x_copy(5).start()
    x_copy(6).start()
    x_copy(3).wait()
    x_copy(4).wait()
    block(lambda: v01((2,)), lambda: ln_jobs(3) + ln_jobs(4), 'p0')
    x_copy(7).start()
    w_copy(2, 2).start()
    x_copy(5).wait()
    x_copy(6).wait()
    block(lambda: v01((3, 4)), lambda: ln_jobs(5) + ln_jobs(6), 'p0')
    wq_copy().start()
    x_copy(7).wait()
    block(lambda: v01((5, 6)), lambda: ln_jobs(7), 'p0')
    block(lambda: v01((7,)), lambda: [], 'p0')

    def kv_block(j, m, after_start, jobs, name):
        slot = j % 3
        w_copy(j, slot).wait()

        @pl.when(j + 1 < 8)
        def _():
            w_copy(j + 1, (j + 1) % 3).start()
        after_start()
        block(lambda: kv_tasks(m, slot, (j % 4) * 2, range(16)), jobs, name)

    def v_body(j, c):
        def dmas():
            @pl.when(j == 2)
            def _():
                start(gu_copies(0, 0))

            @pl.when(j == 3)
            def _():
                d_copy(0, 0).start()
                d_copy(1, 1).start()
        kv_block(j, 2, dmas, lambda: [wq_job((j - 2) * 16 + a) for a in range(16)], 'v')
        return c
    wq_copy().wait()
    lax.fori_loop(2, 4, v_body, 0)

    def k_body(j, c):
        def dmas():
            @pl.when(j == 4)
            def _():
                start(gu_copies(1, 1))
        i = j - 4
        kv_block(j, 1, dmas, lambda: _mix([perm_job(2, i * 16 + a) for a in range(16)],
                                          [t_job(i * 12 + a) for a in range(12)]), 'k')
        return c
    lax.fori_loop(4, 8, k_body, 0)

    wait(gu_copies(0, 0))
    d_copy(0, 0).wait()

    def q_body(i, c):
        def jobs():
            extra = ([b_job(0, 4 * i + g, h) for g in range(4) for h in range(2)]
                     + [bd_job(0, i, n) for n in range(2)]
                     + [t_job(48 + 4 * i + a) for a in range(4)])
            zero = [zero_job(jnp.minimum(i * 13 + a, NP - 1)) for a in range(13)]
            rest = _mix([perm_job(1, i * 16 + a) for a in range(16)], extra)
            return _mix(rest[:-6], zero) + rest[-6:]
        block(lambda: q_tasks(i * 2), jobs, 'q')
        return c
    lax.fori_loop(0, 4, q_body, 0)

    wait(gu_copies(1, 1))
    start(gu_copies(2, 0))
    block(lambda: mm1_tasks(0, 0, 0),
          lambda: _mix(b_jobs(1, 0) + bd_jobs(0, 2), attn_quad(0, True) + attn_quad(1, True)), 'f0')
    block(lambda: mm1_tasks(1, 1, 0),
          lambda: _mix(_mix(comb_jobs(0), b_jobs(1, 1) + bd_jobs(0, 3)), attn_quad(28, True)), 'f1')

    def slot(t, mp):
        j = t // 4
        s = t % 4
        par = j % 2
        if mp == 0:
            @pl.when(jnp.logical_and(s == 0, j > 0))
            def _():
                wait(gu_copies(jnp.minimum(j + 1, NCH - 1), 1 - par))

                @pl.when(j + 2 < NCH)
                def _():
                    start(gu_copies(j + 2, par))

                @pl.when(j + 2 == NCH)
                def _():
                    start(wo_copies())

            @pl.when(jnp.logical_and(s == 2, j + 1 < NCH))
            def _():
                d_copy(j + 1, 1 - par).wait()

                @pl.when(j + 2 < NCH)
                def _():
                    d_copy(j + 2, par).start()
        jd = (t + 2) // 4
        kd = (t + 2) % 4
        u = t - 2

        def jobs():
            base = _mix(comb_jobs(1 - mp), b_jobs(1 - par, s) + bd_jobs(jd % 2, kd))
            att = attn_quad(u + 2)
            n0 = max(1, len(base) // 10)
            return base[:n0] + _mix(base[n0:-n0], att) + base[-n0:]
        block(lambda: mm1_tasks(mp, s, par) + mm2_tasks(mp, (t - 2) % 4, ((t - 2) // 4) % 2), jobs,
              'slot%d' % mp, 3)

    def steady(it, c):
        slot(2 * it + 2, 0)
        slot(2 * it + 3, 1)
        return c
    lax.fori_loop(0, (NT - 2) // 2, steady, 0)

    block(lambda: mm2_tasks(0, 2, 0), lambda: comb_jobs(1), 'e0')
    block(lambda: _mix(wo_tasks(0), mm2_tasks(1, 3, 0)),
          lambda: _flat([attn_quad(n, True) for n in range(29, 32)], 1) + [[lambda: None] * 20], 'e1')

    def wo_body(i, c):
        @pl.when(i >= 3)
        def _():
            wait([out_copy(i - 3, a) for a in range(4)])
        def jobs():
            kick = [lambda: start([out_copy(i - 1, a) for a in range(4)])]
            return final_jobs(i - 1) + [kick] + [[lambda: None] * 40]
        block(lambda: wo_tasks(i), jobs, 'wo')
        return c
    lax.fori_loop(1, 4, wo_body, 0)
    wait([out_copy(1, a) for a in range(4)])
    for h in range(2):
        block(nothing, lambda h=h: [final_job(3, g, n) for g in range(4 * h, 4 * h + 4) for n in range(2)], 'e3')
        start([last_copy(a, h) for a in range(4)])
    wait([out_copy(2, a) for a in range(4)])
    wait([last_copy(a, h) for h in range(2) for a in range(4)])


@jax.jit
def pallas_parallel_sum__sliding_local_dilated__glu_gated_bilinear__prompt_kernel(
    A_x: jax.Array,
    A_wqkv: jax.Array,
    A_wo: jax.Array,
    B_x: jax.Array,
    B_w_gate: jax.Array,
    B_w_up: jax.Array,
    B_w_down: jax.Array,
):
    del B_x
    x = A_x.reshape(S, D)
    hbm = pl.BlockSpec(memory_space=pl.ANY)
    dma = pltpu.SemaphoreType.DMA
    out = pl.pallas_call(
        _kernel,
        grid=(1,),
        in_specs=[pl.BlockSpec(memory_space=pltpu.SMEM)] + [hbm] * 6,
        out_specs=hbm,
        out_shape=jax.ShapeDtypeStruct((S, D), bf),
        scratch_shapes=[
            pltpu.VMEM((S, D), bf),
            pltpu.VMEM((S // 2, D), u32),
            pltpu.VMEM((NP, HB // 2, KB), u32),
            pltpu.VMEM((3, D, QW), bf),
            pltpu.VMEM((D, D), bf),
            pltpu.VMEM((D // 2, D), u32),
            pltpu.VMEM((2, 8, S // 2 + PADW, 128), u32),
            pltpu.VMEM((3, 8, S // 2 + PADW, 128), u32),
            pltpu.VMEM((2, D, TF), bf),
            pltpu.VMEM((2, D, TF), bf),
            pltpu.VMEM((2, TF, D), bf),
            pltpu.VMEM((2, NP, KB // 2, 2 * TB), u32),
            pltpu.VMEM((2, NP, TB // 2, KB), u32),
            pltpu.VMEM((2, NP, 2, RS + MPAD, 128), f32),
            pltpu.VMEM((2, NP, RS // 2, TB), u32),
            pltpu.VMEM((4, 16, 24, 128), f32),
            pltpu.VMEM((4, 8, 24, 128), f32),
            pltpu.VMEM((NP, 2, HB + MPAD, 128), f32),
            dma((8,)), dma((3,)), dma((1,)), dma((2,)), dma((2,)), dma((2,)), dma((16,)),
        ],
        compiler_params=pltpu.CompilerParams(
            dimension_semantics=("arbitrary",), vmem_limit_bytes=127 * 1024 * 1024,
            disable_bounds_checks=True),
        name="fused_attn_ffn",
    )(jnp.ones((1,), jnp.int32), x, A_wqkv, A_wo, B_w_gate, B_w_up, B_w_down)
    return out.reshape(1, S, D)
```

```python
import jax
import jax.numpy as jnp
from jax import lax
from jax.experimental import pallas as pl
from jax.experimental.pallas import tpu as pltpu

bf = jnp.bfloat16
f32 = jnp.float32
u32 = jnp.uint32

S, D, F = 2048, 1024, 3584
WIN = 8
NP = 49
HB = S // 4
KB = D // 4
TF = 512
TB = TF // 4
NCH = F // TF
RS = 128
NSUB = HB // RS
NT = NCH * NSUB
MPAD = 8
PADW = 8
QW = 256
EPS = 1e-5
C2 = float(32 ** -0.5 * 1.4426950408889634)

A_T = [[(1, (0, 0)), (1, (1, 1))], [(1, (1, 0)), (1, (1, 1))], [(1, (0, 0))], [(1, (1, 1))],
       [(1, (0, 0)), (1, (0, 1))], [(1, (1, 0)), (-1, (0, 0))], [(1, (0, 1)), (-1, (1, 1))]]
B_T = [[(1, (0, 0)), (1, (1, 1))], [(1, (0, 0))], [(1, (0, 1)), (-1, (1, 1))], [(1, (1, 0)), (-1, (0, 0))],
       [(1, (1, 1))], [(1, (0, 0)), (1, (0, 1))], [(1, (1, 0)), (1, (1, 1))]]
C_T = {(0, 0): [(1, 0), (1, 3), (-1, 4), (1, 6)], (0, 1): [(1, 2), (1, 4)],
       (1, 0): [(1, 1), (1, 3)], (1, 1): [(1, 0), (-1, 1), (1, 2), (1, 5)]}
POS = ((0, 0), (0, 1), (1, 0), (1, 1))


def _comb(terms):
    acc = None
    for s, v in terms:
        if acc is None:
            acc = v if s > 0 else -v
        else:
            acc = acc + v if s > 0 else acc - v
    return acc


def _dot(a, b):
    return jnp.dot(a, b, preferred_element_type=f32)


def _pk(v):
    return pltpu.bitcast(v.astype(bf), u32)


def _up(w):
    return pltpu.bitcast(w, bf)


def _unpk(w):
    return pltpu.bitcast(w, bf).astype(f32)


def _as_f32(w):
    return lax.bitcast_convert_type(w, f32)


def _as_u32(v):
    return lax.bitcast_convert_type(v, u32)


def _mult(x, m):
    return x if isinstance(x, int) else pl.multiple_of(x, m)


def _opcomb(load, table, I, emit, raw):
    sub = {(r, c): _comb([(s, load(q[0] * 2 + r, q[1] * 2 + c)) for s, q in table[I]])
           for r in range(2) for c in range(2)}
    for J, t2 in enumerate(table):
        if raw is not None and len(table[I]) == 1 and len(t2) == 1:
            qo, qi = table[I][0][1], t2[0][1]
            emit(I * 7 + J, raw(qo[0] * 2 + qi[0], qo[1] * 2 + qi[1]))
        else:
            emit(I * 7 + J, _pk(_comb([(s, sub[q]) for s, q in t2])))


def _opcomb_job(load, table, emit, raw=None):
    return [(lambda I=I: _opcomb(load, table, I, emit, raw)) for I in range(7)]


def _outpos(load, pos):
    inner = [_comb([(s, load(I * 7 + J)) for s, J in C_T[pos]]) for I in range(7)]
    return {q: _comb([(s, inner[I]) for s, I in terms]) for q, terms in C_T.items()}


def _perm8(v):
    lane = lax.broadcasted_iota(jnp.int32, v[0].shape, 1)
    v = list(v)
    for cb, lb in ((2, 4), (1, 3), (0, 2)):
        sh = 1 << lb
        hi = (lane & sh) != 0
        out = [None] * 8
        for c in range(8):
            if c & (1 << cb):
                continue
            x, y = v[c], v[c | (1 << cb)]
            out[c] = jnp.where(hi, pltpu.roll(y, sh, 1), x)
            out[c | (1 << cb)] = jnp.where(hi, y, pltpu.roll(x, 128 - sh, 1))
        v = out
    return v


def _sum4(x, lane):
    x = x + jnp.where((lane & 1) != 0, pltpu.roll(x, 1, 1), pltpu.roll(x, 127, 1))
    x = x + jnp.where((lane & 2) != 0, pltpu.roll(x, 2, 1), pltpu.roll(x, 126, 1))
    return x


def _mix(a, b):
    if not b:
        return list(a)
    if not a:
        return list(b)
    out, n, m, k = [], len(a), len(b), 0
    for i, t in enumerate(a):
        out.append(t)
        tgt = (i + 1) * m // n
        while k < tgt:
            out.append(b[k])
            k += 1
    return out


def _flat(jobs, depth=1):
    return [t for j in jobs for t in j]


def _weave(mx, jobs, woff=0):
    vp = _flat(jobs)
    tot = sum(c for _, c in mx)
    n, k, acc = len(vp), 0, 0
    for t, c in mx:
        t()
        acc += c
        tgt = min(n, acc * n // tot + woff)
        while k < tgt:
            vp[k]()
            k += 1
    while k < n:
        vp[k]()
        k += 1


def _kernel(one_ref, x_hbm, wqkv_hbm, wo_hbm, wg_hbm, wu_hbm, wd_hbm, out_hbm,
            xr, xn, T, wst, wqr, wqp, R, P, gst, ust, dst, B, Bd, M, H, hst, ost, acc,
            sem_x, sem_w, sem_q, sem_g, sem_u, sem_d, sem_o):

    def block(mx, jobs, name="blk", woff=0):
        with jax.named_scope(name):
            @pl.when(one_ref[0] > 0)
            def _():
                _weave(mx(), jobs(), woff)

    def x_copy(r):
        rows = pl.ds(_mult(r * 256, 256), 256)
        return pltpu.make_async_copy(x_hbm.at[rows, :], xr.at[rows, :], sem_x.at[r])

    def w_copy(j, slot):
        col = (2 - j // 4) * D + (j % 4) * QW
        return pltpu.make_async_copy(wqkv_hbm.at[:, pl.ds(_mult(col, QW), QW)], wst.at[slot], sem_w.at[slot])

    def wq_copy():
        return pltpu.make_async_copy(wqkv_hbm.at[:, pl.ds(0, D)], wqr, sem_q.at[0])

    def gu_copies(j, par):
        cols = pl.ds(_mult(j * TF, TF), TF)
        return (pltpu.make_async_copy(wg_hbm.at[:, cols], gst.at[par], sem_g.at[par]),
                pltpu.make_async_copy(wu_hbm.at[:, cols], ust.at[par], sem_u.at[par]))

    def d_copy(j, par):
        return pltpu.make_async_copy(wd_hbm.at[pl.ds(_mult(j * TF, TF), TF), :], dst.at[par], sem_d.at[par])

    def wo_copies():
        return (pltpu.make_async_copy(wo_hbm.at[:, pl.ds(0, TF)], gst.at[1], sem_g.at[1]),
                pltpu.make_async_copy(wo_hbm.at[:, pl.ds(TF, TF)], ust.at[1], sem_u.at[1]))

    def out_copy(i, a):
        par = i % 2
        return pltpu.make_async_copy(dst.at[par, pl.ds(a * RS, RS), :],
                                     out_hbm.at[pl.ds(_mult(a * HB + i * RS, RS), RS), :], sem_o.at[par * 4 + a])

    def last_copy(a, h):
        rows = RS // 2
        return pltpu.make_async_copy(dst.at[1, pl.ds(a * RS + h * rows, rows), :],
                                     out_hbm.at[pl.ds(a * HB + 3 * RS + h * rows, rows), :], sem_o.at[8 + h * 4 + a])

    def start(cps):
        for cp in cps:
            cp.start()

    def wait(cps):
        for cp in cps:
            cp.wait()

    def ln_job(g):
        def t():
            v = [xr[pl.ds(g * 16, 16), pl.ds(c * 128, 128)].astype(f32) for c in range(8)]
            a = v[0]
            for c in range(1, 8):
                a = a + v[c]
            mean = jnp.sum(a, axis=1, keepdims=True) * (1.0 / D)
            v = [x - mean for x in v]
            a = v[0] * v[0]
            for c in range(1, 8):
                a = a + v[c] * v[c]
            r = lax.rsqrt(jnp.sum(a, axis=1, keepdims=True) * (1.0 / D) + EPS)
            for c in range(8):
                xn[pl.ds(g * 8, 8), pl.ds(c * 128, 128)] = _pk(v[c] * r)
        return [t]

    def ln_jobs(r):
        return [ln_job(r * 16 + g) for g in range(16)]

    def t_job(pos_idx):
        w0 = _mult((pos_idx // 2) * 8, 8)
        l0 = _mult((pos_idx % 2) * 128, 128)

        def raw(i, j):
            return xn[pl.ds(_mult(i * 256 + w0, 8), 8), pl.ds(_mult(j * KB + l0, 128), 128)]

        def emit(p, v):
            T[p, pl.ds(w0, 8), pl.ds(l0, 128)] = v
        return _opcomb_job(lambda i, j: _unpk(raw(i, j)), A_T, emit, raw)

    def b_job(par, g, half):
        w_ref = (gst, ust)[half]

        def src(i, q):
            return w_ref[par, pl.ds(_mult(i * KB + g * 16, 16), 16), pl.ds(q * TB, TB)]

        def emit(p, v):
            B[par, p, pl.ds(_mult(g * 8, 8), 8), pl.ds(half * TB, TB)] = v
        return _opcomb_job(lambda i, q: src(i, q).astype(f32), B_T, emit,
                           lambda i, q: pltpu.bitcast(src(i, q), u32))

    def bd_job(par, g, n):
        def src(i, q):
            return dst[par, pl.ds(_mult(i * TB + g * 16, 16), 16), pl.ds(q * KB + n * 128, 128)]

        def emit(p, v):
            Bd[par, p, pl.ds(_mult(g * 8, 8), 8), pl.ds(n * 128, 128)] = v
        return _opcomb_job(lambda i, q: src(i, q).astype(f32), B_T, emit,
                           lambda i, q: pltpu.bitcast(src(i, q), u32))

    def b_jobs(par, k):
        return [b_job(par, 4 * k + g, h) for g in range(4) for h in range(2)]

    def bd_jobs(par, k):
        return [bd_job(par, 2 * k + g, n) for g in range(2) for n in range(2)]

    def perm_job(m, pair):
        def t():
            w = _mult(pair * 16, 16)
            r = _perm8([R[2 - m, c, pl.ds(w, 16), :] for c in range(8)])
            for c in range(8):
                P[m, c, pl.ds(_mult(PADW + w, 8), 16), :] = r[c]
        return [t]

    def wq_job(pair):
        def t():
            rows = pl.ds(_mult(pair * 32, 32), 32)
            r = _perm8([pltpu.bitcast(wqr[rows, pl.ds(c * 128, 128)], u32) for c in range(8)])
            for c in range(8):
                wqp[pl.ds(_mult(pair * 16, 16), 16), pl.ds(c * 128, 128)] = r[c]
        return [t]

    def attn_quad(n, stack=False):
        base = _mult(((n % 8) // 2) * 256 + (n // 8) * 64 + (n % 2) * 32, 32)
        return [attn_job(base, 8 * k, k, stack) for k in range(4)]

    def attn_job(base, off, sl, stack):
        b = base + off
        job = []
        for h in range(2):
            st = {}
            half = lambda v, h=h: _unpk(v)[h * 8:(h + 1) * 8]

            def qk(cs, st=st, half=half):
                def t():
                    for c in cs:
                        qv = half(P[0, c, pl.ds(base + (off + PADW), 8), :])
                        for w in range(WIN):
                            kv = half(P[1, c, pl.ds(base + (off + PADW - w), 8), :])
                            st[w] = qv * kv if c == 0 else st[w] + qv * kv
                return t

            def sm(st=st, h=h):
                lane = lax.broadcasted_iota(jnp.int32, (8, 128), 1)
                row = lax.broadcasted_iota(jnp.int32, (8, 128), 0) + (b * 2 + h * 8)
                if stack:
                    big = jnp.concatenate([st[w] for w in range(WIN)], axis=0)
                    big = _sum4(big, lax.broadcasted_iota(jnp.int32, (8 * WIN, 128), 1))
                    ls = [big[8 * w:8 * w + 8] for w in range(WIN)]
                else:
                    ls = [_sum4(st[w], lane) for w in range(WIN)]
                ls = [ls[0]] + [jnp.where(row >= 2 * w, ls[w], -1e30) for w in range(1, WIN)]
                m = ls[0]
                for w in range(1, WIN):
                    m = jnp.maximum(m, ls[w])
                e = [jnp.exp2((l - m) * C2) for l in ls]
                den = e[0]
                for w in range(1, WIN):
                    den = den + e[w]
                inv = 1.0 / den
                st['p'] = [x * inv for x in e]

            def pv(cs, st=st, half=half, h=h):
                def t():
                    for c in cs:
                        o = None
                        for w in range(WIN):
                            a = st['p'][w] * half(P[2, c, pl.ds(base + (off + PADW - w), 8), :])
                            o = a if o is None else o + a
                        ost[sl, c, pl.ds(h * 8, 8), :] = o
                return t
            ag = 4 if stack else 2
            job += ([qk(tuple(range(c, c + ag))) for c in range(0, 8, ag)] + [sm]
                    + [pv(tuple(range(c, c + ag))) for c in range(0, 8, ag)])

        def fin():
            r = _perm8([_pk(ost[sl, c, pl.ds(0, 16), :]) for c in range(8)])
            for c in range(8):
                xn[pl.ds(_mult(b, 8), 8), pl.ds(c * 128, 128)] = r[c]
        return job + [fin]

    def comb_job(mp, g):
        sl = g % 4
        job = []
        for hf in range(2):
            for pos in POS:
                def t(hf=hf, pos=pos):
                    r = pl.ds(g * 16 + hf * 8, 8)
                    gg = _outpos(lambda p: M[mp, p, 0, r, :], pos)
                    uu = _outpos(lambda p: M[mp, p, 1, r, :], pos)
                    for q in gg:
                        hst[sl, (q[0] * 2 + pos[0]) * 4 + q[1] * 2 + pos[1], pl.ds(hf * 8, 8), :] = gg[q] * uu[q]
                job.append(t)

        def emit(p, v):
            H[mp, p, pl.ds(g * 8, 8), :] = v
        return job + _opcomb_job(lambda i, j: hst[sl, i * 4 + j, pl.ds(0, 16), :], A_T, emit)

    def comb_jobs(mp):
        return [comb_job(mp, g) for g in range(RS // 16)]

    def zero_job(p):
        def t():
            for c in range(2):
                acc[p, c, pl.ds(0, HB), :] = jnp.zeros((HB, 128), f32)
        return [t]

    def final_job(i, g, n):
        job = []
        par = i % 2
        for pos in POS:
            def t(pos=pos):
                r0 = _mult(i * RS + g * 16, 16)
                o = [_outpos(lambda p: acc[p, n, pl.ds(r0 + hf * 8, 8), :], pos) for hf in range(2)]
                for q in o[0]:
                    a = q[0] * 2 + pos[0]
                    ch = (q[1] * 2 + pos[1]) * 2 + n
                    pln = a * 8 + ch
                    cols = pl.ds(ch * 128, 128)
                    ffn = jnp.concatenate([o[0][q], o[1][q]], axis=0)
                    att = M[par, pln // 2, pln % 2, pl.ds(g * 16, 16), :]
                    res = xr[pl.ds(_mult(a * HB + r0, 16), 16), cols].astype(f32) + att + ffn
                    dst[par, pl.ds(a * RS + g * 16, 16), cols] = res.astype(bf)
            job.append(t)
        return job

    def final_jobs(i):
        return [final_job(i, g, n) for g in range(RS // 16) for n in range(2)]

    def kv_tasks(m, slot, cbase, pieces):
        out = []
        for r in pieces:
            for ct in range(QW // 128):
                def t(r=r, ct=ct):
                    res = _dot(_up(xn[pl.ds(_mult(r * 64, 64), 64), :]), wst[slot, :, pl.ds(ct * 128, 128)])
                    for k in range(8):
                        R[2 - m, cbase + ct, pl.ds(_mult(r * 64 + k * 8, 8), 8), :] = _pk(res[k * 16:(k + 1) * 16])
                out.append((t, 256))
        return out

    def q_tasks(cbase):
        out = []
        for r in range(16):
            for ct in range(QW // 128):
                def t(r=r, ct=ct):
                    res = _dot(_up(xn[pl.ds(r * 64, 64), :]),
                               _up(wqp[:, pl.ds(_mult((cbase + ct) * 128, 128), 128)]))
                    for k in range(8):
                        P[0, cbase + ct, pl.ds(PADW + r * 64 + k * 8, 8), :] = _pk(res[k * 16:(k + 1) * 16])
                out.append((t, 256))
        return out

    def mm1_tasks(mp, s, par):
        out = []
        for p in range(NP):
            for c in range(2):
                def t(p=p, c=c):
                    M[mp, p, c, pl.ds(0, RS), :] = _dot(
                        _up(T[p, pl.ds(_mult(s * (RS // 2), RS // 2), RS // 2), :]),
                        _up(B[par, p, :, pl.ds(c * 128, 128)]))
                out.append((t, 64))
        return out

    def mm2_tasks(mp, s, par):
        out = []
        for p in range(NP):
            def t(p=p):
                r = _dot(_up(H[mp, p]), _up(Bd[par, p]))
                for c in range(2):
                    acc[p, c, pl.ds(_mult(s * RS, RS), RS), :] += r[:, c * 128:(c + 1) * 128]
            out.append((t, 64))
        return out

    def wo_tasks(i):
        out = []
        for a in range(4):
            for ch in range(8):
                def t(a=a, ch=ch):
                    w_ref = (gst, ust)[ch // 4]
                    res = _dot(_up(xn[pl.ds(_mult(a * 256 + i * 64, 64), 64), :]),
                               w_ref[1, :, pl.ds((ch % 4) * 128, 128)])
                    pln = a * 8 + ch
                    M[i % 2, pln // 2, pln % 2, pl.ds(0, RS), :] = res
                out.append((t, 256))
        return out

    nothing = lambda: [(lambda: None, 1)]

    x_copy(0).start()
    w_copy(0, 0).start()
    for c in range(8):
        P[1, c, pl.ds(0, PADW), :] = jnp.zeros((PADW, 128), u32)
        P[2, c, pl.ds(0, PADW), :] = jnp.zeros((PADW, 128), u32)
    x_copy(0).wait()
    w_copy(1, 1).start()
    x_copy(1).start()
    block(nothing, lambda: ln_jobs(0), 'ln0')
    w_copy(0, 0).wait()

    def v01(pieces):
        rp = [2 * r + h for r in pieces for h in range(2)]
        return kv_tasks(2, 0, 0, rp) + kv_tasks(2, 1, 2, rp)

    block(lambda: kv_tasks(2, 0, 0, (0, 1)), lambda: [], 'p0')
    w_copy(1, 1).wait()
    x_copy(2).start()
    x_copy(1).wait()
    block(lambda: kv_tasks(2, 1, 2, (0, 1)), lambda: ln_jobs(1), 'p0')
    x_copy(3).start()
    x_copy(4).start()
    x_copy(2).wait()
    block(lambda: v01((1,)), lambda: ln_jobs(2), 'p0')
    x_copy(5).start()
    x_copy(6).start()
    x_copy(3).wait()
    x_copy(4).wait()
    block(lambda: v01((2,)), lambda: ln_jobs(3) + ln_jobs(4), 'p0')
    x_copy(7).start()
    w_copy(2, 2).start()
    x_copy(5).wait()
    x_copy(6).wait()
    block(lambda: v01((3, 4)), lambda: ln_jobs(5) + ln_jobs(6), 'p0')
    wq_copy().start()
    x_copy(7).wait()
    block(lambda: v01((5, 6)), lambda: ln_jobs(7), 'p0')
    block(lambda: v01((7,)), lambda: [], 'p0')

    def kv_block(j, m, after_start, jobs, name, woff=0):
        slot = j % 3
        w_copy(j, slot).wait()

        @pl.when(j + 1 < 8)
        def _():
            w_copy(j + 1, (j + 1) % 3).start()
        after_start()
        block(lambda: kv_tasks(m, slot, (j % 4) * 2, range(16)), jobs, name, woff)

    def v_body(j, c):
        def dmas():
            @pl.when(j == 2)
            def _():
                start(gu_copies(0, 0))

            @pl.when(j == 3)
            def _():
                d_copy(0, 0).start()
                d_copy(1, 1).start()
        kv_block(j, 2, dmas, lambda: [wq_job((j - 2) * 16 + a) for a in range(16)], 'v')
        return c
    wq_copy().wait()
    lax.fori_loop(2, 4, v_body, 0)

    def k_body(j, c):
        def dmas():
            @pl.when(j == 4)
            def _():
                start(gu_copies(1, 1))
        i = j - 4
        kv_block(j, 1, dmas, lambda: _mix([perm_job(2, i * 16 + a) for a in range(16)],
                                          [t_job(i * 12 + a) for a in range(12)]), 'k', 2)
        return c
    lax.fori_loop(4, 8, k_body, 0)

    wait(gu_copies(0, 0))
    d_copy(0, 0).wait()

    def q_body(i, c):
        def jobs():
            extra = ([b_job(0, 4 * i + g, h) for g in range(4) for h in range(2)]
                     + [bd_job(0, i, n) for n in range(2)]
                     + [t_job(48 + 4 * i + a) for a in range(4)])
            zero = [zero_job(jnp.minimum(i * 13 + a, NP - 1)) for a in range(13)]
            rest = _mix([perm_job(1, i * 16 + a) for a in range(16)], extra)
            return _mix(rest[:-6], zero) + rest[-6:]
        block(lambda: q_tasks(i * 2), jobs, 'q', 2)
        return c
    lax.fori_loop(0, 4, q_body, 0)

    wait(gu_copies(1, 1))
    start(gu_copies(2, 0))
    block(lambda: mm1_tasks(0, 0, 0),
          lambda: _mix(b_jobs(1, 0) + bd_jobs(0, 2), attn_quad(0, True) + attn_quad(1, True)), 'f0')
    block(lambda: mm1_tasks(1, 1, 0),
          lambda: _mix(_mix(comb_jobs(0), b_jobs(1, 1) + bd_jobs(0, 3)), attn_quad(28, True)), 'f1', 3)

    def slot(t, mp):
        j = t // 4
        s = t % 4
        par = j % 2
        if mp == 0:
            @pl.when(jnp.logical_and(s == 0, j > 0))
            def _():
                wait(gu_copies(jnp.minimum(j + 1, NCH - 1), 1 - par))

                @pl.when(j + 2 < NCH)
                def _():
                    start(gu_copies(j + 2, par))

                @pl.when(j + 2 == NCH)
                def _():
                    start(wo_copies())

            @pl.when(jnp.logical_and(s == 2, j + 1 < NCH))
            def _():
                d_copy(j + 1, 1 - par).wait()

                @pl.when(j + 2 < NCH)
                def _():
                    d_copy(j + 2, par).start()
        jd = (t + 2) // 4
        kd = (t + 2) % 4
        u = t - 2

        def jobs():
            base = _mix(comb_jobs(1 - mp), b_jobs(1 - par, s) + bd_jobs(jd % 2, kd))
            att = attn_quad(u + 2)
            n0 = max(1, len(base) // 10)
            return base[:n0] + _mix(base[n0:-n0], att) + base[-n0:]
        block(lambda: mm1_tasks(mp, s, par) + mm2_tasks(mp, (t - 2) % 4, ((t - 2) // 4) % 2), jobs,
              'slot%d' % mp, 3)

    def steady(it, c):
        slot(2 * it + 2, 0)
        slot(2 * it + 3, 1)
        return c
    lax.fori_loop(0, (NT - 2) // 2, steady, 0)

    block(lambda: mm2_tasks(0, 2, 0), lambda: comb_jobs(1), 'e0')
    block(lambda: _mix(wo_tasks(0), mm2_tasks(1, 3, 0)),
          lambda: _flat([attn_quad(n, True) for n in range(29, 32)], 1) + [[lambda: None] * 20], 'e1')

    def wo_body(i, c):
        @pl.when(i >= 3)
        def _():
            wait([out_copy(i - 3, a) for a in range(4)])
        def jobs():
            kick = [lambda: start([out_copy(i - 1, a) for a in range(4)])]
            return final_jobs(i - 1) + [kick] + [[lambda: None] * 40]
        block(lambda: wo_tasks(i), jobs, 'wo')
        return c
    lax.fori_loop(1, 4, wo_body, 0)
    wait([out_copy(1, a) for a in range(4)])
    for h in range(2):
        block(nothing, lambda h=h: [final_job(3, g, n) for g in range(4 * h, 4 * h + 4) for n in range(2)], 'e3')
        start([last_copy(a, h) for a in range(4)])
    wait([out_copy(2, a) for a in range(4)])
    wait([last_copy(a, h) for h in range(2) for a in range(4)])


@jax.jit
def pallas_parallel_sum__sliding_local_dilated__glu_gated_bilinear__prompt_kernel(
    A_x: jax.Array,
    A_wqkv: jax.Array,
    A_wo: jax.Array,
    B_x: jax.Array,
    B_w_gate: jax.Array,
    B_w_up: jax.Array,
    B_w_down: jax.Array,
):
    del B_x
    x = A_x.reshape(S, D)
    hbm = pl.BlockSpec(memory_space=pl.ANY)
    dma = pltpu.SemaphoreType.DMA
    out = pl.pallas_call(
        _kernel,
        grid=(1,),
        in_specs=[pl.BlockSpec(memory_space=pltpu.SMEM)] + [hbm] * 6,
        out_specs=hbm,
        out_shape=jax.ShapeDtypeStruct((S, D), bf),
        scratch_shapes=[
            pltpu.VMEM((S, D), bf),
            pltpu.VMEM((S // 2, D), u32),
            pltpu.VMEM((NP, HB // 2, KB), u32),
            pltpu.VMEM((3, D, QW), bf),
            pltpu.VMEM((D, D), bf),
            pltpu.VMEM((D // 2, D), u32),
            pltpu.VMEM((2, 8, S // 2 + PADW, 128), u32),
            pltpu.VMEM((3, 8, S // 2 + PADW, 128), u32),
            pltpu.VMEM((2, D, TF), bf),
            pltpu.VMEM((2, D, TF), bf),
            pltpu.VMEM((2, TF, D), bf),
            pltpu.VMEM((2, NP, KB // 2, 2 * TB), u32),
            pltpu.VMEM((2, NP, TB // 2, KB), u32),
            pltpu.VMEM((2, NP, 2, RS + MPAD, 128), f32),
            pltpu.VMEM((2, NP, RS // 2, TB), u32),
            pltpu.VMEM((4, 16, 24, 128), f32),
            pltpu.VMEM((4, 8, 24, 128), f32),
            pltpu.VMEM((NP, 2, HB + MPAD, 128), f32),
            dma((8,)), dma((3,)), dma((1,)), dma((2,)), dma((2,)), dma((2,)), dma((16,)),
        ],
        compiler_params=pltpu.CompilerParams(
            dimension_semantics=("arbitrary",), vmem_limit_bytes=127 * 1024 * 1024,
            disable_bounds_checks=True),
        name="fused_attn_ffn",
    )(jnp.ones((1,), jnp.int32), x, A_wqkv, A_wo, B_w_gate, B_w_up, B_w_down)
    return out.reshape(1, S, D)
```

```python
import jax
import jax.numpy as jnp
from jax import lax
from jax.experimental import pallas as pl
from jax.experimental.pallas import tpu as pltpu

bf = jnp.bfloat16
f32 = jnp.float32
u32 = jnp.uint32

S, D, F = 2048, 1024, 3584
WIN = 8
NP = 49
HB = S // 4
KB = D // 4
TF = 512
TB = TF // 4
NCH = F // TF
RS = 128
NSUB = HB // RS
NT = NCH * NSUB
MPAD = 8
PADW = 8
PADR = 16
QW = 256
EPS = 1e-5
C2 = float(32 ** -0.5 * 1.4426950408889634)

A_T = [[(1, (0, 0)), (1, (1, 1))], [(1, (1, 0)), (1, (1, 1))], [(1, (0, 0))], [(1, (1, 1))],
       [(1, (0, 0)), (1, (0, 1))], [(1, (1, 0)), (-1, (0, 0))], [(1, (0, 1)), (-1, (1, 1))]]
B_T = [[(1, (0, 0)), (1, (1, 1))], [(1, (0, 0))], [(1, (0, 1)), (-1, (1, 1))], [(1, (1, 0)), (-1, (0, 0))],
       [(1, (1, 1))], [(1, (0, 0)), (1, (0, 1))], [(1, (1, 0)), (1, (1, 1))]]
C_T = {(0, 0): [(1, 0), (1, 3), (-1, 4), (1, 6)], (0, 1): [(1, 2), (1, 4)],
       (1, 0): [(1, 1), (1, 3)], (1, 1): [(1, 0), (-1, 1), (1, 2), (1, 5)]}
POS = ((0, 0), (0, 1), (1, 0), (1, 1))


def _comb(terms):
    acc = None
    for s, v in terms:
        if acc is None:
            acc = v if s > 0 else -v
        else:
            acc = acc + v if s > 0 else acc - v
    return acc


def _dot(a, b):
    return jnp.dot(a, b, preferred_element_type=f32)


def _pk(v):
    return pltpu.bitcast(v.astype(bf), u32)


def _up(w):
    return pltpu.bitcast(w, bf)


def _unpk(w):
    return pltpu.bitcast(w, bf).astype(f32)


def _as_f32(w):
    return lax.bitcast_convert_type(w, f32)


def _as_u32(v):
    return lax.bitcast_convert_type(v, u32)


def _mult(x, m):
    return x if isinstance(x, int) else pl.multiple_of(x, m)


def _opcomb(load, table, I, emit, raw):
    sub = {(r, c): _comb([(s, load(q[0] * 2 + r, q[1] * 2 + c)) for s, q in table[I]])
           for r in range(2) for c in range(2)}
    for J, t2 in enumerate(table):
        if raw is not None and len(table[I]) == 1 and len(t2) == 1:
            qo, qi = table[I][0][1], t2[0][1]
            emit(I * 7 + J, raw(qo[0] * 2 + qi[0], qo[1] * 2 + qi[1]))
        else:
            emit(I * 7 + J, _pk(_comb([(s, sub[q]) for s, q in t2])))


def _opcomb_job(load, table, emit, raw=None):
    return [(lambda I=I: _opcomb(load, table, I, emit, raw)) for I in range(7)]


def _outpos(load, pos):
    inner = [_comb([(s, load(I * 7 + J)) for s, J in C_T[pos]]) for I in range(7)]
    return {q: _comb([(s, inner[I]) for s, I in terms]) for q, terms in C_T.items()}


def _perm8(v):
    lane = lax.broadcasted_iota(jnp.int32, v[0].shape, 1)
    v = list(v)
    for cb, lb in ((2, 4), (1, 3), (0, 2)):
        sh = 1 << lb
        hi = (lane & sh) != 0
        out = [None] * 8
        for c in range(8):
            if c & (1 << cb):
                continue
            x, y = v[c], v[c | (1 << cb)]
            out[c] = jnp.where(hi, pltpu.roll(y, sh, 1), x)
            out[c | (1 << cb)] = jnp.where(hi, y, pltpu.roll(x, 128 - sh, 1))
        v = out
    return v


def _sum4(x, lane):
    x = x + jnp.where((lane & 1) != 0, pltpu.roll(x, 1, 1), pltpu.roll(x, 127, 1))
    x = x + jnp.where((lane & 2) != 0, pltpu.roll(x, 2, 1), pltpu.roll(x, 126, 1))
    return x


def _mix(a, b):
    if not b:
        return list(a)
    if not a:
        return list(b)
    out, n, m, k = [], len(a), len(b), 0
    for i, t in enumerate(a):
        out.append(t)
        tgt = (i + 1) * m // n
        while k < tgt:
            out.append(b[k])
            k += 1
    return out


def _flat(jobs, depth=1):
    return [t for j in jobs for t in j]


def _weave(mx, jobs, woff=0):
    vp = _flat(jobs)
    tot = sum(c for _, c in mx)
    n, k, acc = len(vp), 0, 0
    for t, c in mx:
        t()
        acc += c
        tgt = min(n, acc * n // tot + woff)
        while k < tgt:
            vp[k]()
            k += 1
    while k < n:
        vp[k]()
        k += 1


def _kernel(one_ref, x_hbm, wqkv_hbm, wo_hbm, wg_hbm, wu_hbm, wd_hbm, out_hbm,
            xr, xn, T, wst, wqr, wqp, R, QP, KF, VF, gst, ust, dst, B, Bd, M, H, hst, ost, acc,
            sem_x, sem_w, sem_q, sem_g, sem_u, sem_d, sem_o):

    def block(mx, jobs, name="blk", woff=0):
        with jax.named_scope(name):
            @pl.when(one_ref[0] > 0)
            def _():
                _weave(mx(), jobs(), woff)

    def x_copy(r):
        rows = pl.ds(_mult(r * 256, 256), 256)
        return pltpu.make_async_copy(x_hbm.at[rows, :], xr.at[rows, :], sem_x.at[r])

    def w_copy(j, slot):
        col = (2 - j // 4) * D + (j % 4) * QW
        return pltpu.make_async_copy(wqkv_hbm.at[:, pl.ds(_mult(col, QW), QW)], wst.at[slot], sem_w.at[slot])

    def wq_copy():
        return pltpu.make_async_copy(wqkv_hbm.at[:, pl.ds(0, D)], wqr, sem_q.at[0])

    def gu_copies(j, par):
        cols = pl.ds(_mult(j * TF, TF), TF)
        return (pltpu.make_async_copy(wg_hbm.at[:, cols], gst.at[par], sem_g.at[par]),
                pltpu.make_async_copy(wu_hbm.at[:, cols], ust.at[par], sem_u.at[par]))

    def d_copy(j, par):
        return pltpu.make_async_copy(wd_hbm.at[pl.ds(_mult(j * TF, TF), TF), :], dst.at[par], sem_d.at[par])

    def wo_copies():
        return (pltpu.make_async_copy(wo_hbm.at[:, pl.ds(0, TF)], gst.at[1], sem_g.at[1]),
                pltpu.make_async_copy(wo_hbm.at[:, pl.ds(TF, TF)], ust.at[1], sem_u.at[1]))

    def out_copy(i, a):
        par = i % 2
        return pltpu.make_async_copy(dst.at[par, pl.ds(a * RS, RS), :],
                                     out_hbm.at[pl.ds(_mult(a * HB + i * RS, RS), RS), :], sem_o.at[par * 4 + a])

    def last_copy(a, h):
        rows = RS // 2
        return pltpu.make_async_copy(dst.at[1, pl.ds(a * RS + h * rows, rows), :],
                                     out_hbm.at[pl.ds(a * HB + 3 * RS + h * rows, rows), :], sem_o.at[8 + h * 4 + a])

    def start(cps):
        for cp in cps:
            cp.start()

    def wait(cps):
        for cp in cps:
            cp.wait()

    def ln_job(g):
        def t():
            v = [xr[pl.ds(g * 16, 16), pl.ds(c * 128, 128)].astype(f32) for c in range(8)]
            a = v[0]
            for c in range(1, 8):
                a = a + v[c]
            mean = jnp.sum(a, axis=1, keepdims=True) * (1.0 / D)
            v = [x - mean for x in v]
            a = v[0] * v[0]
            for c in range(1, 8):
                a = a + v[c] * v[c]
            r = lax.rsqrt(jnp.sum(a, axis=1, keepdims=True) * (1.0 / D) + EPS)
            for c in range(8):
                xn[pl.ds(g * 8, 8), pl.ds(c * 128, 128)] = _pk(v[c] * r)
        return [t]

    def ln_jobs(r):
        return [ln_job(r * 16 + g) for g in range(16)]

    def t_job(pos_idx):
        w0 = _mult((pos_idx // 2) * 8, 8)
        l0 = _mult((pos_idx % 2) * 128, 128)

        def raw(i, j):
            return xn[pl.ds(_mult(i * 256 + w0, 8), 8), pl.ds(_mult(j * KB + l0, 128), 128)]

        def emit(p, v):
            T[p, pl.ds(w0, 8), pl.ds(l0, 128)] = v
        return _opcomb_job(lambda i, j: _unpk(raw(i, j)), A_T, emit, raw)

    def b_job(par, g, half):
        w_ref = (gst, ust)[half]

        def src(i, q):
            return w_ref[par, pl.ds(_mult(i * KB + g * 16, 16), 16), pl.ds(q * TB, TB)]

        def emit(p, v):
            B[par, p, pl.ds(_mult(g * 8, 8), 8), pl.ds(half * TB, TB)] = v
        return _opcomb_job(lambda i, q: src(i, q).astype(f32), B_T, emit,
                           lambda i, q: pltpu.bitcast(src(i, q), u32))

    def bd_job(par, g, n):
        def src(i, q):
            return dst[par, pl.ds(_mult(i * TB + g * 16, 16), 16), pl.ds(q * KB + n * 128, 128)]

        def emit(p, v):
            Bd[par, p, pl.ds(_mult(g * 8, 8), 8), pl.ds(n * 128, 128)] = v
        return _opcomb_job(lambda i, q: src(i, q).astype(f32), B_T, emit,
                           lambda i, q: pltpu.bitcast(src(i, q), u32))

    def b_jobs(par, k):
        return [b_job(par, 4 * k + g, h) for g in range(4) for h in range(2)]

    def bd_jobs(par, k):
        return [bd_job(par, 2 * k + g, n) for g in range(2) for n in range(2)]

    def perm_job(m, pair):
        dstp = (None, KF, VF)[m]

        def t():
            w = _mult(pair * 16, 16)
            r = _perm8([R[2 - m, c, pl.ds(w, 16), :] for c in range(8)])
            for c in range(8):
                dstp[c, pl.ds(_mult(PADR + pair * 32, 16), 32), :] = _unpk(r[c])
        return [t]

    def wq_job(pair):
        def t():
            rows = pl.ds(_mult(pair * 32, 32), 32)
            r = _perm8([pltpu.bitcast(wqr[rows, pl.ds(c * 128, 128)], u32) for c in range(8)])
            for c in range(8):
                wqp[pl.ds(_mult(pair * 16, 16), 16), pl.ds(c * 128, 128)] = r[c]
        return [t]

    def attn_quad(n, stack=False):
        base = _mult(((n % 8) // 2) * 256 + (n // 8) * 64 + (n % 2) * 32, 32)
        return [attn_job(base, 8 * k, k, stack) for k in range(4)]

    def attn_job(base, off, sl, stack):
        b = base + off
        rbase = _mult(base * 2, 64)
        job = []
        for h in range(2):
            st = {}
            half = lambda v, h=h: _unpk(v)[h * 8:(h + 1) * 8]

            def qk(cs, st=st, half=half, h=h):
                def t():
                    for c in cs:
                        qv = half(QP[c, pl.ds(base + off, 8), :])
                        for w in range(WIN):
                            kv = KF[c, pl.ds(rbase + (2 * off + 8 * h + PADR - 2 * w), 8), :]
                            st[w] = qv * kv if c == 0 else st[w] + qv * kv
                return t

            def sm(st=st, h=h):
                lane = lax.broadcasted_iota(jnp.int32, (8, 128), 1)
                row = lax.broadcasted_iota(jnp.int32, (8, 128), 0) + (b * 2 + h * 8)
                if stack:
                    big = jnp.concatenate([st[w] for w in range(WIN)], axis=0)
                    big = _sum4(big, lax.broadcasted_iota(jnp.int32, (8 * WIN, 128), 1))
                    ls = [big[8 * w:8 * w + 8] for w in range(WIN)]
                else:
                    ls = [_sum4(st[w], lane) for w in range(WIN)]
                ls = [ls[0]] + [jnp.where(row >= 2 * w, ls[w], -1e30) for w in range(1, WIN)]
                m = ls[0]
                for w in range(1, WIN):
                    m = jnp.maximum(m, ls[w])
                e = [jnp.exp2((l - m) * C2) for l in ls]
                den = e[0]
                for w in range(1, WIN):
                    den = den + e[w]
                inv = 1.0 / den
                st['p'] = [x * inv for x in e]

            def pv(cs, st=st, half=half, h=h):
                def t():
                    for c in cs:
                        o = None
                        for w in range(WIN):
                            a = st['p'][w] * VF[c, pl.ds(rbase + (2 * off + 8 * h + PADR - 2 * w), 8), :]
                            o = a if o is None else o + a
                        ost[sl, c, pl.ds(h * 8, 8), :] = o
                return t
            job += [qk((0, 1, 2, 3)), qk((4, 5, 6, 7)), sm, pv((0, 1, 2, 3)), pv((4, 5, 6, 7))]

        def fin():
            r = _perm8([_pk(ost[sl, c, pl.ds(0, 16), :]) for c in range(8)])
            for c in range(8):
                xn[pl.ds(_mult(b, 8), 8), pl.ds(c * 128, 128)] = r[c]
        return job + [fin]

    def comb_job(mp, g):
        sl = g % 4
        job = []
        for hf in range(2):
            for pos in POS:
                def t(hf=hf, pos=pos):
                    r = pl.ds(g * 16 + hf * 8, 8)
                    gg = _outpos(lambda p: M[mp, p, 0, r, :], pos)
                    uu = _outpos(lambda p: M[mp, p, 1, r, :], pos)
                    for q in gg:
                        hst[sl, (q[0] * 2 + pos[0]) * 4 + q[1] * 2 + pos[1], pl.ds(hf * 8, 8), :] = gg[q] * uu[q]
                job.append(t)

        def emit(p, v):
            H[mp, p, pl.ds(g * 8, 8), :] = v
        return job + _opcomb_job(lambda i, j: hst[sl, i * 4 + j, pl.ds(0, 16), :], A_T, emit)

    def comb_jobs(mp):
        return [comb_job(mp, g) for g in range(RS // 16)]

    def zero_job(p):
        def t():
            for c in range(2):
                acc[p, c, pl.ds(0, HB), :] = jnp.zeros((HB, 128), f32)
        return [t]

    def final_job(i, g, n):
        job = []
        par = i % 2
        for pos in POS:
            def t(pos=pos):
                r0 = _mult(i * RS + g * 16, 16)
                o = [_outpos(lambda p: acc[p, n, pl.ds(r0 + hf * 8, 8), :], pos) for hf in range(2)]
                for q in o[0]:
                    a = q[0] * 2 + pos[0]
                    ch = (q[1] * 2 + pos[1]) * 2 + n
                    pln = a * 8 + ch
                    cols = pl.ds(ch * 128, 128)
                    ffn = jnp.concatenate([o[0][q], o[1][q]], axis=0)
                    att = M[par, pln // 2, pln % 2, pl.ds(g * 16, 16), :]
                    res = xr[pl.ds(_mult(a * HB + r0, 16), 16), cols].astype(f32) + att + ffn
                    dst[par, pl.ds(a * RS + g * 16, 16), cols] = res.astype(bf)
            job.append(t)
        return job

    def final_jobs(i):
        return [final_job(i, g, n) for g in range(RS // 16) for n in range(2)]

    def kv_tasks(m, slot, cbase, pieces):
        out = []
        for r in pieces:
            for ct in range(QW // 128):
                def t(r=r, ct=ct):
                    res = _dot(_up(xn[pl.ds(_mult(r * 64, 64), 64), :]), wst[slot, :, pl.ds(ct * 128, 128)])
                    for k in range(8):
                        R[2 - m, cbase + ct, pl.ds(_mult(r * 64 + k * 8, 8), 8), :] = _pk(res[k * 16:(k + 1) * 16])
                out.append((t, 256))
        return out

    def q_tasks(cbase):
        out = []
        for r in range(16):
            for ct in range(QW // 128):
                def t(r=r, ct=ct):
                    res = _dot(_up(xn[pl.ds(r * 64, 64), :]),
                               _up(wqp[:, pl.ds(_mult((cbase + ct) * 128, 128), 128)]))
                    for k in range(8):
                        QP[cbase + ct, pl.ds(r * 64 + k * 8, 8), :] = _pk(res[k * 16:(k + 1) * 16])
                out.append((t, 256))
        return out

    def mm1_tasks(mp, s, par):
        out = []
        for p in range(NP):
            for c in range(2):
                def t(p=p, c=c):
                    M[mp, p, c, pl.ds(0, RS), :] = _dot(
                        _up(T[p, pl.ds(_mult(s * (RS // 2), RS // 2), RS // 2), :]),
                        _up(B[par, p, :, pl.ds(c * 128, 128)]))
                out.append((t, 64))
        return out

    def mm2_tasks(mp, s, par):
        out = []
        for p in range(NP):
            def t(p=p):
                r = _dot(_up(H[mp, p]), _up(Bd[par, p]))
                for c in range(2):
                    acc[p, c, pl.ds(_mult(s * RS, RS), RS), :] += r[:, c * 128:(c + 1) * 128]
            out.append((t, 64))
        return out

    def wo_tasks(i):
        out = []
        for a in range(4):
            for ch in range(8):
                def t(a=a, ch=ch):
                    w_ref = (gst, ust)[ch // 4]
                    res = _dot(_up(xn[pl.ds(_mult(a * 256 + i * 64, 64), 64), :]),
                               w_ref[1, :, pl.ds((ch % 4) * 128, 128)])
                    pln = a * 8 + ch
                    M[i % 2, pln // 2, pln % 2, pl.ds(0, RS), :] = res
                out.append((t, 256))
        return out

    nothing = lambda: [(lambda: None, 1)]

    x_copy(0).start()
    w_copy(0, 0).start()
    for c in range(8):
        KF[c, pl.ds(0, PADR), :] = jnp.zeros((PADR, 128), f32)
        VF[c, pl.ds(0, PADR), :] = jnp.zeros((PADR, 128), f32)
    x_copy(0).wait()
    w_copy(1, 1).start()
    x_copy(1).start()
    block(nothing, lambda: ln_jobs(0), 'ln0')
    w_copy(0, 0).wait()

    def v01(pieces):
        rp = [2 * r + h for r in pieces for h in range(2)]
        return kv_tasks(2, 0, 0, rp) + kv_tasks(2, 1, 2, rp)

    block(lambda: kv_tasks(2, 0, 0, (0, 1)), lambda: [], 'p0')
    w_copy(1, 1).wait()
    x_copy(2).start()
    x_copy(1).wait()
    block(lambda: kv_tasks(2, 1, 2, (0, 1)), lambda: ln_jobs(1), 'p0')
    x_copy(3).start()
    x_copy(4).start()
    x_copy(2).wait()
    block(lambda: v01((1,)), lambda: ln_jobs(2), 'p0')
    x_copy(5).start()
    x_copy(6).start()
    x_copy(3).wait()
    x_copy(4).wait()
    block(lambda: v01((2,)), lambda: ln_jobs(3) + ln_jobs(4), 'p0')
    x_copy(7).start()
    w_copy(2, 2).start()
    x_copy(5).wait()
    x_copy(6).wait()
    block(lambda: v01((3, 4)), lambda: ln_jobs(5) + ln_jobs(6), 'p0')
    wq_copy().start()
    x_copy(7).wait()
    block(lambda: v01((5, 6)), lambda: ln_jobs(7), 'p0')
    block(lambda: v01((7,)), lambda: [], 'p0')

    def kv_block(j, m, after_start, jobs, name, woff=0):
        slot = j % 3
        w_copy(j, slot).wait()

        @pl.when(j + 1 < 8)
        def _():
            w_copy(j + 1, (j + 1) % 3).start()
        after_start()
        block(lambda: kv_tasks(m, slot, (j % 4) * 2, range(16)), jobs, name, woff)

    def v_body(j, c):
        def dmas():
            @pl.when(j == 2)
            def _():
                start(gu_copies(0, 0))

            @pl.when(j == 3)
            def _():
                d_copy(0, 0).start()
                d_copy(1, 1).start()
        kv_block(j, 2, dmas, lambda: [wq_job((j - 2) * 16 + a) for a in range(16)], 'v')
        return c
    wq_copy().wait()
    lax.fori_loop(2, 4, v_body, 0)

    def k_body(j, c):
        def dmas():
            @pl.when(j == 4)
            def _():
                start(gu_copies(1, 1))
        i = j - 4
        kv_block(j, 1, dmas, lambda: _mix([perm_job(2, i * 16 + a) for a in range(16)],
                                          [t_job(i * 12 + a) for a in range(12)]), 'k', 2)
        return c
    lax.fori_loop(4, 8, k_body, 0)

    wait(gu_copies(0, 0))
    d_copy(0, 0).wait()

    def q_body(i, c):
        def jobs():
            extra = ([b_job(0, 4 * i + g, h) for g in range(4) for h in range(2)]
                     + [bd_job(0, i, n) for n in range(2)]
                     + [t_job(48 + 4 * i + a) for a in range(4)])
            zero = [zero_job(jnp.minimum(i * 13 + a, NP - 1)) for a in range(13)]
            rest = _mix([perm_job(1, i * 16 + a) for a in range(16)], extra)
            return _mix(rest[:-6], zero) + rest[-6:]
        block(lambda: q_tasks(i * 2), jobs, 'q', 2)
        return c
    lax.fori_loop(0, 4, q_body, 0)

    wait(gu_copies(1, 1))
    start(gu_copies(2, 0))
    block(lambda: mm1_tasks(0, 0, 0),
          lambda: _mix(b_jobs(1, 0) + bd_jobs(0, 2), attn_quad(0, True) + attn_quad(1, True)), 'f0')
    block(lambda: mm1_tasks(1, 1, 0),
          lambda: _mix(_mix(comb_jobs(0), b_jobs(1, 1) + bd_jobs(0, 3)), attn_quad(28, True)), 'f1', 3)

    def slot(t, mp):
        j = t // 4
        s = t % 4
        par = j % 2
        if mp == 0:
            @pl.when(jnp.logical_and(s == 0, j > 0))
            def _():
                wait(gu_copies(jnp.minimum(j + 1, NCH - 1), 1 - par))

                @pl.when(j + 2 < NCH)
                def _():
                    start(gu_copies(j + 2, par))

                @pl.when(j + 2 == NCH)
                def _():
                    start(wo_copies())

            @pl.when(jnp.logical_and(s == 2, j + 1 < NCH))
            def _():
                d_copy(j + 1, 1 - par).wait()

                @pl.when(j + 2 < NCH)
                def _():
                    d_copy(j + 2, par).start()
        jd = (t + 2) // 4
        kd = (t + 2) % 4
        u = t - 2

        def jobs():
            base = _mix(comb_jobs(1 - mp), b_jobs(1 - par, s) + bd_jobs(jd % 2, kd))
            att = attn_quad(u + 2)
            n0 = max(1, len(base) // 10)
            return base[:n0] + _mix(base[n0:-n0], att) + base[-n0:]
        block(lambda: mm1_tasks(mp, s, par) + mm2_tasks(mp, (t - 2) % 4, ((t - 2) // 4) % 2), jobs,
              'slot%d' % mp, 3)

    def steady(it, c):
        slot(2 * it + 2, 0)
        slot(2 * it + 3, 1)
        return c
    lax.fori_loop(0, (NT - 2) // 2, steady, 0)

    block(lambda: mm2_tasks(0, 2, 0), lambda: comb_jobs(1), 'e0')
    block(lambda: _mix(wo_tasks(0), mm2_tasks(1, 3, 0)),
          lambda: _flat([attn_quad(n, True) for n in range(29, 32)], 1) + [[lambda: None] * 20], 'e1')

    def wo_body(i, c):
        @pl.when(i >= 3)
        def _():
            wait([out_copy(i - 3, a) for a in range(4)])
        block(lambda: wo_tasks(i)[:20], lambda: final_jobs(i - 1), 'wo')
        start([out_copy(i - 1, a) for a in range(4)])
        block(lambda: wo_tasks(i)[20:], lambda: [], 'wo')
        return c
    lax.fori_loop(1, 4, wo_body, 0)
    wait([out_copy(1, a) for a in range(4)])
    for h in range(2):
        block(nothing, lambda h=h: [final_job(3, g, n) for g in range(4 * h, 4 * h + 4) for n in range(2)], 'e3')
        start([last_copy(a, h) for a in range(4)])
    wait([out_copy(2, a) for a in range(4)])
    wait([last_copy(a, h) for h in range(2) for a in range(4)])


@jax.jit
def pallas_parallel_sum__sliding_local_dilated__glu_gated_bilinear__prompt_kernel(
    A_x: jax.Array,
    A_wqkv: jax.Array,
    A_wo: jax.Array,
    B_x: jax.Array,
    B_w_gate: jax.Array,
    B_w_up: jax.Array,
    B_w_down: jax.Array,
):
    del B_x
    x = A_x.reshape(S, D)
    hbm = pl.BlockSpec(memory_space=pl.ANY)
    dma = pltpu.SemaphoreType.DMA
    out = pl.pallas_call(
        _kernel,
        grid=(1,),
        in_specs=[pl.BlockSpec(memory_space=pltpu.SMEM)] + [hbm] * 6,
        out_specs=hbm,
        out_shape=jax.ShapeDtypeStruct((S, D), bf),
        scratch_shapes=[
            pltpu.VMEM((S, D), bf),
            pltpu.VMEM((S // 2, D), u32),
            pltpu.VMEM((NP, HB // 2, KB), u32),
            pltpu.VMEM((3, D, QW), bf),
            pltpu.VMEM((D, D), bf),
            pltpu.VMEM((D // 2, D), u32),
            pltpu.VMEM((2, 8, S // 2 + PADW, 128), u32),
            pltpu.VMEM((8, S // 2 + PADW, 128), u32),
            pltpu.VMEM((8, S + PADR + 8, 128), f32),
            pltpu.VMEM((8, S + PADR + 8, 128), f32),
            pltpu.VMEM((2, D, TF), bf),
            pltpu.VMEM((2, D, TF), bf),
            pltpu.VMEM((2, TF, D), bf),
            pltpu.VMEM((2, NP, KB // 2, 2 * TB), u32),
            pltpu.VMEM((2, NP, TB // 2, KB), u32),
            pltpu.VMEM((2, NP, 2, RS + MPAD, 128), f32),
            pltpu.VMEM((2, NP, RS // 2, TB), u32),
            pltpu.VMEM((4, 16, 24, 128), f32),
            pltpu.VMEM((4, 8, 24, 128), f32),
            pltpu.VMEM((NP, 2, HB + MPAD, 128), f32),
            dma((8,)), dma((3,)), dma((1,)), dma((2,)), dma((2,)), dma((2,)), dma((16,)),
        ],
        compiler_params=pltpu.CompilerParams(
            dimension_semantics=("arbitrary",), vmem_limit_bytes=127 * 1024 * 1024,
            disable_bounds_checks=True),
        name="fused_attn_ffn",
    )(jnp.ones((1,), jnp.int32), x, A_wqkv, A_wo, B_w_gate, B_w_up, B_w_down)
    return out.reshape(1, S, D)
```

```python
import jax
import jax.numpy as jnp
from jax import lax
from jax.experimental import pallas as pl
from jax.experimental.pallas import tpu as pltpu

bf = jnp.bfloat16
f32 = jnp.float32
u32 = jnp.uint32

S, D, F = 2048, 1024, 3584
WIN = 8
NP = 49
HB = S // 4
KB = D // 4
TF = 512
TB = TF // 4
NCH = F // TF
RS = 128
NSUB = HB // RS
NT = NCH * NSUB
MPAD = 8
PADW = 8
PADR = 16
QW = 256
EPS = 1e-5
C2 = float(32 ** -0.5 * 1.4426950408889634)

A_T = [[(1, (0, 0)), (1, (1, 1))], [(1, (1, 0)), (1, (1, 1))], [(1, (0, 0))], [(1, (1, 1))],
       [(1, (0, 0)), (1, (0, 1))], [(1, (1, 0)), (-1, (0, 0))], [(1, (0, 1)), (-1, (1, 1))]]
B_T = [[(1, (0, 0)), (1, (1, 1))], [(1, (0, 0))], [(1, (0, 1)), (-1, (1, 1))], [(1, (1, 0)), (-1, (0, 0))],
       [(1, (1, 1))], [(1, (0, 0)), (1, (0, 1))], [(1, (1, 0)), (1, (1, 1))]]
C_T = {(0, 0): [(1, 0), (1, 3), (-1, 4), (1, 6)], (0, 1): [(1, 2), (1, 4)],
       (1, 0): [(1, 1), (1, 3)], (1, 1): [(1, 0), (-1, 1), (1, 2), (1, 5)]}
POS = ((0, 0), (0, 1), (1, 0), (1, 1))


def _comb(terms):
    acc = None
    for s, v in terms:
        if acc is None:
            acc = v if s > 0 else -v
        else:
            acc = acc + v if s > 0 else acc - v
    return acc


def _dot(a, b):
    return jnp.dot(a, b, preferred_element_type=f32)


def _pk(v):
    return pltpu.bitcast(v.astype(bf), u32)


def _up(w):
    return pltpu.bitcast(w, bf)


def _unpk(w):
    return pltpu.bitcast(w, bf).astype(f32)


def _as_f32(w):
    return lax.bitcast_convert_type(w, f32)


def _as_u32(v):
    return lax.bitcast_convert_type(v, u32)


def _mult(x, m):
    return x if isinstance(x, int) else pl.multiple_of(x, m)


def _opcomb(load, table, I, emit, raw):
    sub = {(r, c): _comb([(s, load(q[0] * 2 + r, q[1] * 2 + c)) for s, q in table[I]])
           for r in range(2) for c in range(2)}
    for J, t2 in enumerate(table):
        if raw is not None and len(table[I]) == 1 and len(t2) == 1:
            qo, qi = table[I][0][1], t2[0][1]
            emit(I * 7 + J, raw(qo[0] * 2 + qi[0], qo[1] * 2 + qi[1]))
        else:
            emit(I * 7 + J, _pk(_comb([(s, sub[q]) for s, q in t2])))


def _opcomb_job(load, table, emit, raw=None):
    return [(lambda I=I: _opcomb(load, table, I, emit, raw)) for I in range(7)]


def _outpos(load, pos):
    inner = [_comb([(s, load(I * 7 + J)) for s, J in C_T[pos]]) for I in range(7)]
    return {q: _comb([(s, inner[I]) for s, I in terms]) for q, terms in C_T.items()}


def _perm8(v):
    lane = lax.broadcasted_iota(jnp.int32, v[0].shape, 1)
    v = list(v)
    for cb, lb in ((2, 4), (1, 3), (0, 2)):
        sh = 1 << lb
        hi = (lane & sh) != 0
        out = [None] * 8
        for c in range(8):
            if c & (1 << cb):
                continue
            x, y = v[c], v[c | (1 << cb)]
            out[c] = jnp.where(hi, pltpu.roll(y, sh, 1), x)
            out[c | (1 << cb)] = jnp.where(hi, y, pltpu.roll(x, 128 - sh, 1))
        v = out
    return v


def _sum4(x, lane):
    x = x + jnp.where((lane & 1) != 0, pltpu.roll(x, 1, 1), pltpu.roll(x, 127, 1))
    x = x + jnp.where((lane & 2) != 0, pltpu.roll(x, 2, 1), pltpu.roll(x, 126, 1))
    return x


def _mix(a, b):
    if not b:
        return list(a)
    if not a:
        return list(b)
    out, n, m, k = [], len(a), len(b), 0
    for i, t in enumerate(a):
        out.append(t)
        tgt = (i + 1) * m // n
        while k < tgt:
            out.append(b[k])
            k += 1
    return out


def _flat(jobs, depth=1):
    return [t for j in jobs for t in j]


def _weave(mx, jobs, woff=0):
    vp = _flat(jobs)
    tot = sum(c for _, c in mx)
    n, k, acc = len(vp), 0, 0
    for t, c in mx:
        t()
        acc += c
        tgt = min(n, acc * n // tot + woff)
        while k < tgt:
            vp[k]()
            k += 1
    while k < n:
        vp[k]()
        k += 1


def _kernel(one_ref, x_hbm, wqkv_hbm, wo_hbm, wg_hbm, wu_hbm, wd_hbm, out_hbm,
            xr, xn, T, wst, wqr, wqp, R, QP, KF, VF, gst, ust, dst, B, Bd, M, H, hst, ost, acc,
            sem_x, sem_w, sem_q, sem_g, sem_u, sem_d, sem_o):

    def block(mx, jobs, name="blk", woff=0):
        with jax.named_scope(name):
            @pl.when(one_ref[0] > 0)
            def _():
                _weave(mx(), jobs(), woff)

    def x_copy(r):
        rows = pl.ds(_mult(r * 256, 256), 256)
        return pltpu.make_async_copy(x_hbm.at[rows, :], xr.at[rows, :], sem_x.at[r])

    def w_copy(j, slot):
        col = (2 - j // 4) * D + (j % 4) * QW
        return pltpu.make_async_copy(wqkv_hbm.at[:, pl.ds(_mult(col, QW), QW)], wst.at[slot], sem_w.at[slot])

    def wq_copy():
        return pltpu.make_async_copy(wqkv_hbm.at[:, pl.ds(0, D)], wqr, sem_q.at[0])

    def gu_copies(j, par):
        cols = pl.ds(_mult(j * TF, TF), TF)
        return (pltpu.make_async_copy(wg_hbm.at[:, cols], gst.at[par], sem_g.at[par]),
                pltpu.make_async_copy(wu_hbm.at[:, cols], ust.at[par], sem_u.at[par]))

    def d_copy(j, par):
        return pltpu.make_async_copy(wd_hbm.at[pl.ds(_mult(j * TF, TF), TF), :], dst.at[par], sem_d.at[par])

    def wo_copies():
        return (pltpu.make_async_copy(wo_hbm.at[:, pl.ds(0, TF)], gst.at[1], sem_g.at[1]),
                pltpu.make_async_copy(wo_hbm.at[:, pl.ds(TF, TF)], ust.at[1], sem_u.at[1]))

    def out_copy(i, a):
        par = i % 2
        return pltpu.make_async_copy(dst.at[par, pl.ds(a * RS, RS), :],
                                     out_hbm.at[pl.ds(_mult(a * HB + i * RS, RS), RS), :], sem_o.at[par * 4 + a])

    def last_copy(a, h):
        rows = RS // 2
        return pltpu.make_async_copy(dst.at[1, pl.ds(a * RS + h * rows, rows), :],
                                     out_hbm.at[pl.ds(a * HB + 3 * RS + h * rows, rows), :], sem_o.at[8 + h * 4 + a])

    def start(cps):
        for cp in cps:
            cp.start()

    def wait(cps):
        for cp in cps:
            cp.wait()

    def ln_job(g):
        def t():
            v = [xr[pl.ds(g * 16, 16), pl.ds(c * 128, 128)].astype(f32) for c in range(8)]
            a = v[0]
            for c in range(1, 8):
                a = a + v[c]
            mean = jnp.sum(a, axis=1, keepdims=True) * (1.0 / D)
            v = [x - mean for x in v]
            a = v[0] * v[0]
            for c in range(1, 8):
                a = a + v[c] * v[c]
            r = lax.rsqrt(jnp.sum(a, axis=1, keepdims=True) * (1.0 / D) + EPS)
            for c in range(8):
                xn[pl.ds(g * 8, 8), pl.ds(c * 128, 128)] = _pk(v[c] * r)
        return [t]

    def ln_jobs(r):
        return [ln_job(r * 16 + g) for g in range(16)]

    def t_job(wb, pos):
        w0 = _mult(wb, 16) + (pos // 2) * 8
        l0 = (pos % 2) * 128

        def raw(i, j):
            return xn[pl.ds(w0 + i * 256, 8), pl.ds(j * KB + l0, 128)]

        def emit(p, v):
            T[p, pl.ds(w0, 8), pl.ds(l0, 128)] = v
        return _opcomb_job(lambda i, j: _unpk(raw(i, j)), A_T, emit, raw)

    def b_job(par, k, g, half):
        w_ref = (gst, ust)[half]

        def src(i, q):
            return w_ref[par, pl.ds(_mult(k * 64, 64) + (i * KB + g * 16), 16), pl.ds(q * TB, TB)]

        def emit(p, v):
            B[par, p, pl.ds(_mult(k * 32, 32) + g * 8, 8), pl.ds(half * TB, TB)] = v
        return _opcomb_job(lambda i, q: src(i, q).astype(f32), B_T, emit,
                           lambda i, q: pltpu.bitcast(src(i, q), u32))

    def bd_job(par, gb, g, n):
        def src(i, q):
            return dst[par, pl.ds(_mult(gb, 16) + (i * TB + g * 16), 16), pl.ds(q * KB + n * 128, 128)]

        def emit(p, v):
            Bd[par, p, pl.ds(_mult(gb // 2, 8) + g * 8, 8), pl.ds(n * 128, 128)] = v
        return _opcomb_job(lambda i, q: src(i, q).astype(f32), B_T, emit,
                           lambda i, q: pltpu.bitcast(src(i, q), u32))

    def b_jobs(par, k):
        return [b_job(par, k, g, h) for g in range(4) for h in range(2)]

    def bd_jobs(par, k):
        return [bd_job(par, k * 32, g, n) for g in range(2) for n in range(2)]

    def perm_job(m, i, a):
        dstp = (None, KF, VF)[m]

        def t():
            r = _perm8([R[2 - m, c, pl.ds(_mult(i * 256, 256) + a * 16, 16), :] for c in range(8)])
            for c in range(8):
                dstp[c, pl.ds(_mult(i * 512, 512) + (PADR + a * 32), 32), :] = _unpk(r[c])
        return [t]

    def wq_job(i, a):
        def t():
            rows = pl.ds(_mult(i * 512, 512) + a * 32, 32)
            r = _perm8([pltpu.bitcast(wqr[rows, pl.ds(c * 128, 128)], u32) for c in range(8)])
            for c in range(8):
                wqp[pl.ds(_mult(i * 256, 256) + a * 16, 16), pl.ds(c * 128, 128)] = r[c]
        return [t]

    def attn_quad(n, stack=False):
        base = _mult(((n % 8) // 2) * 256 + (n // 8) * 64 + (n % 2) * 32, 32)
        return [attn_job(base, 8 * k, k, stack) for k in range(4)]

    def attn_job(base, off, sl, stack):
        b = base + off
        rbase = _mult(base * 2, 64)
        job = []
        for h in range(2):
            st = {}
            half = lambda v, h=h: _unpk(v)[h * 8:(h + 1) * 8]

            def qk(cs, st=st, half=half, h=h):
                def t():
                    for c in cs:
                        qv = half(QP[c, pl.ds(base + off, 8), :])
                        for w in range(WIN):
                            kv = KF[c, pl.ds(rbase + (2 * off + 8 * h + PADR - 2 * w), 8), :]
                            st[w] = qv * kv if c == 0 else st[w] + qv * kv
                return t

            def sm(st=st, h=h):
                lane = lax.broadcasted_iota(jnp.int32, (8, 128), 1)
                row = lax.broadcasted_iota(jnp.int32, (8, 128), 0) + (b * 2 + h * 8)
                if stack:
                    big = jnp.concatenate([st[w] for w in range(WIN)], axis=0)
                    big = _sum4(big, lax.broadcasted_iota(jnp.int32, (8 * WIN, 128), 1))
                    ls = [big[8 * w:8 * w + 8] for w in range(WIN)]
                else:
                    ls = [_sum4(st[w], lane) for w in range(WIN)]
                ls = [ls[0]] + [jnp.where(row >= 2 * w, ls[w], -1e30) for w in range(1, WIN)]
                m = ls[0]
                for w in range(1, WIN):
                    m = jnp.maximum(m, ls[w])
                e = [jnp.exp2((l - m) * C2) for l in ls]
                den = e[0]
                for w in range(1, WIN):
                    den = den + e[w]
                inv = 1.0 / den
                st['p'] = [x * inv for x in e]

            def pv(cs, st=st, half=half, h=h):
                def t():
                    for c in cs:
                        o = None
                        for w in range(WIN):
                            a = st['p'][w] * VF[c, pl.ds(rbase + (2 * off + 8 * h + PADR - 2 * w), 8), :]
                            o = a if o is None else o + a
                        ost[sl, c, pl.ds(h * 8, 8), :] = o
                return t
            job += [qk((0, 1, 2, 3)), qk((4, 5, 6, 7)), sm, pv((0, 1, 2, 3)), pv((4, 5, 6, 7))]

        def fin():
            r = _perm8([_pk(ost[sl, c, pl.ds(0, 16), :]) for c in range(8)])
            for c in range(8):
                xn[pl.ds(_mult(b, 8), 8), pl.ds(c * 128, 128)] = r[c]
        return job + [fin]

    def comb_job(mp, g):
        sl = g % 4
        job = []
        for hf in range(2):
            for pos in POS:
                def t(hf=hf, pos=pos):
                    r = pl.ds(g * 16 + hf * 8, 8)
                    gg = _outpos(lambda p: M[mp, p, 0, r, :], pos)
                    uu = _outpos(lambda p: M[mp, p, 1, r, :], pos)
                    for q in gg:
                        hst[sl, (q[0] * 2 + pos[0]) * 4 + q[1] * 2 + pos[1], pl.ds(hf * 8, 8), :] = gg[q] * uu[q]
                job.append(t)

        def emit(p, v):
            H[mp, p, pl.ds(g * 8, 8), :] = v
        return job + _opcomb_job(lambda i, j: hst[sl, i * 4 + j, pl.ds(0, 16), :], A_T, emit)

    def comb_jobs(mp):
        return [comb_job(mp, g) for g in range(RS // 16)]

    def zero_job(p):
        def t():
            for c in range(2):
                acc[p, c, pl.ds(0, HB), :] = jnp.zeros((HB, 128), f32)
        return [t]

    def final_job(i, g, n):
        job = []
        par = i % 2
        for pos in POS:
            def t(pos=pos):
                r0 = _mult(i * RS + g * 16, 16)
                o = [_outpos(lambda p: acc[p, n, pl.ds(r0 + hf * 8, 8), :], pos) for hf in range(2)]
                for q in o[0]:
                    a = q[0] * 2 + pos[0]
                    ch = (q[1] * 2 + pos[1]) * 2 + n
                    pln = a * 8 + ch
                    cols = pl.ds(ch * 128, 128)
                    ffn = jnp.concatenate([o[0][q], o[1][q]], axis=0)
                    att = M[par, pln // 2, pln % 2, pl.ds(g * 16, 16), :]
                    res = xr[pl.ds(_mult(a * HB + r0, 16), 16), cols].astype(f32) + att + ffn
                    dst[par, pl.ds(a * RS + g * 16, 16), cols] = res.astype(bf)
            job.append(t)
        return job

    def final_jobs(i):
        return [final_job(i, g, n) for g in range(RS // 16) for n in range(2)]

    def kv_tasks(m, slot, cbase, pieces):
        out = []
        for r in pieces:
            for ct in range(QW // 128):
                def t(r=r, ct=ct):
                    res = _dot(_up(xn[pl.ds(_mult(r * 64, 64), 64), :]), wst[slot, :, pl.ds(ct * 128, 128)])
                    for k in range(8):
                        R[2 - m, cbase + ct, pl.ds(_mult(r * 64 + k * 8, 8), 8), :] = _pk(res[k * 16:(k + 1) * 16])
                out.append((t, 256))
        return out

    def q_tasks(cbase):
        out = []
        for r in range(16):
            for ct in range(QW // 128):
                def t(r=r, ct=ct):
                    res = _dot(_up(xn[pl.ds(r * 64, 64), :]),
                               _up(wqp[:, pl.ds(_mult((cbase + ct) * 128, 128), 128)]))
                    for k in range(8):
                        QP[cbase + ct, pl.ds(r * 64 + k * 8, 8), :] = _pk(res[k * 16:(k + 1) * 16])
                out.append((t, 256))
        return out

    def mm1_tasks(mp, s, par):
        out = []
        for p in range(NP):
            for c in range(2):
                def t(p=p, c=c):
                    M[mp, p, c, pl.ds(0, RS), :] = _dot(
                        _up(T[p, pl.ds(_mult(s * (RS // 2), RS // 2), RS // 2), :]),
                        _up(B[par, p, :, pl.ds(c * 128, 128)]))
                out.append((t, 64))
        return out

    def mm2_tasks(mp, s, par):
        out = []
        for p in range(NP):
            def t(p=p):
                r = _dot(_up(H[mp, p]), _up(Bd[par, p]))
                for c in range(2):
                    acc[p, c, pl.ds(_mult(s * RS, RS), RS), :] += r[:, c * 128:(c + 1) * 128]
            out.append((t, 64))
        return out

    def wo_tasks(i):
        out = []
        for a in range(4):
            for ch in range(8):
                def t(a=a, ch=ch):
                    w_ref = (gst, ust)[ch // 4]
                    res = _dot(_up(xn[pl.ds(_mult(a * 256 + i * 64, 64), 64), :]),
                               w_ref[1, :, pl.ds((ch % 4) * 128, 128)])
                    pln = a * 8 + ch
                    M[i % 2, pln // 2, pln % 2, pl.ds(0, RS), :] = res
                out.append((t, 256))
        return out

    nothing = lambda: [(lambda: None, 1)]

    x_copy(0).start()
    w_copy(0, 0).start()
    for c in range(8):
        KF[c, pl.ds(0, PADR), :] = jnp.zeros((PADR, 128), f32)
        VF[c, pl.ds(0, PADR), :] = jnp.zeros((PADR, 128), f32)
    x_copy(0).wait()
    w_copy(1, 1).start()
    x_copy(1).start()
    block(nothing, lambda: ln_jobs(0), 'ln0')
    w_copy(0, 0).wait()

    def v01(pieces):
        rp = [2 * r + h for r in pieces for h in range(2)]
        return kv_tasks(2, 0, 0, rp) + kv_tasks(2, 1, 2, rp)

    block(lambda: kv_tasks(2, 0, 0, (0, 1)), lambda: [], 'p0')
    w_copy(1, 1).wait()
    x_copy(2).start()
    x_copy(1).wait()
    block(lambda: kv_tasks(2, 1, 2, (0, 1)), lambda: ln_jobs(1), 'p0')
    x_copy(3).start()
    x_copy(4).start()
    x_copy(2).wait()
    block(lambda: v01((1,)), lambda: ln_jobs(2), 'p0')
    x_copy(5).start()
    x_copy(6).start()
    x_copy(3).wait()
    x_copy(4).wait()
    block(lambda: v01((2,)), lambda: ln_jobs(3) + ln_jobs(4), 'p0')
    x_copy(7).start()
    w_copy(2, 2).start()
    x_copy(5).wait()
    x_copy(6).wait()
    block(lambda: v01((3, 4)), lambda: ln_jobs(5) + ln_jobs(6), 'p0')
    wq_copy().start()
    x_copy(7).wait()
    block(lambda: v01((5, 6)), lambda: ln_jobs(7), 'p0')
    block(lambda: v01((7,)), lambda: [], 'p0')

    def kv_block(j, m, after_start, jobs, name, woff=0):
        slot = j % 3
        w_copy(j, slot).wait()

        @pl.when(j + 1 < 8)
        def _():
            w_copy(j + 1, (j + 1) % 3).start()
        after_start()
        block(lambda: kv_tasks(m, slot, (j % 4) * 2, range(16)), jobs, name, woff)

    def v_body(j, c):
        def dmas():
            @pl.when(j == 2)
            def _():
                start(gu_copies(0, 0))

            @pl.when(j == 3)
            def _():
                d_copy(0, 0).start()
                d_copy(1, 1).start()
        kv_block(j, 2, dmas, lambda: [wq_job(j - 2, a) for a in range(16)], 'v')
        return c
    wq_copy().wait()
    lax.fori_loop(2, 4, v_body, 0)

    def k_body(j, c):
        def dmas():
            @pl.when(j == 4)
            def _():
                start(gu_copies(1, 1))
        i = j - 4
        kv_block(j, 1, dmas, lambda: _mix([perm_job(2, i, a) for a in range(16)],
                                          [t_job(i * 48, a) for a in range(12)]), 'k', 2)
        return c
    lax.fori_loop(4, 8, k_body, 0)

    wait(gu_copies(0, 0))
    d_copy(0, 0).wait()

    def q_body(i, c):
        def jobs():
            extra = (b_jobs(0, i)
                     + [bd_job(0, i * 16, 0, n) for n in range(2)]
                     + [t_job(192 + 16 * i, a) for a in range(4)])
            zero = [zero_job(jnp.minimum(i * 13 + a, NP - 1)) for a in range(13)]
            rest = _mix([perm_job(1, i, a) for a in range(16)], extra)
            return _mix(rest[:-6], zero) + rest[-6:]
        block(lambda: q_tasks(i * 2), jobs, 'q', 2)
        return c
    lax.fori_loop(0, 4, q_body, 0)

    wait(gu_copies(1, 1))
    start(gu_copies(2, 0))
    block(lambda: mm1_tasks(0, 0, 0),
          lambda: _mix(b_jobs(1, 0) + bd_jobs(0, 2), attn_quad(0, True) + attn_quad(1, True)), 'f0')
    block(lambda: mm1_tasks(1, 1, 0),
          lambda: _mix(_mix(comb_jobs(0), b_jobs(1, 1) + bd_jobs(0, 3)), attn_quad(28, True)), 'f1', 3)

    def slot(t, mp):
        j = t // 4
        s = t % 4
        par = j % 2
        if mp == 0:
            @pl.when(jnp.logical_and(s == 0, j > 0))
            def _():
                wait(gu_copies(jnp.minimum(j + 1, NCH - 1), 1 - par))

                @pl.when(j + 2 < NCH)
                def _():
                    start(gu_copies(j + 2, par))

                @pl.when(j + 2 == NCH)
                def _():
                    start(wo_copies())

            @pl.when(jnp.logical_and(s == 2, j + 1 < NCH))
            def _():
                d_copy(j + 1, 1 - par).wait()

                @pl.when(j + 2 < NCH)
                def _():
                    d_copy(j + 2, par).start()
        jd = (t + 2) // 4
        kd = (t + 2) % 4
        u = t - 2

        def jobs():
            base = _mix(comb_jobs(1 - mp), b_jobs(1 - par, s) + bd_jobs(jd % 2, kd))
            att = attn_quad(u + 2)
            n0 = max(1, len(base) // 10)
            return base[:n0] + _mix(base[n0:-n0], att) + base[-n0:]
        block(lambda: mm1_tasks(mp, s, par) + mm2_tasks(mp, (t - 2) % 4, ((t - 2) // 4) % 2), jobs,
              'slot%d' % mp, 3)

    def steady(it, c):
        slot(2 * it + 2, 0)
        slot(2 * it + 3, 1)
        return c
    lax.fori_loop(0, (NT - 2) // 2, steady, 0)

    block(lambda: mm2_tasks(0, 2, 0), lambda: comb_jobs(1), 'e0')
    block(lambda: _mix(wo_tasks(0), mm2_tasks(1, 3, 0)),
          lambda: _flat([attn_quad(n, True) for n in range(29, 32)], 1) + [[lambda: None] * 20], 'e1')

    def wo_body(i, c):
        @pl.when(i >= 3)
        def _():
            wait([out_copy(i - 3, a) for a in range(4)])
        block(lambda: wo_tasks(i)[:20], lambda: final_jobs(i - 1), 'wo')
        start([out_copy(i - 1, a) for a in range(4)])
        block(lambda: wo_tasks(i)[20:], lambda: [], 'wo')
        return c
    lax.fori_loop(1, 4, wo_body, 0)
    wait([out_copy(1, a) for a in range(4)])
    for h in range(2):
        block(nothing, lambda h=h: [final_job(3, g, n) for g in range(4 * h, 4 * h + 4) for n in range(2)], 'e3')
        start([last_copy(a, h) for a in range(4)])
    wait([out_copy(2, a) for a in range(4)])
    wait([last_copy(a, h) for h in range(2) for a in range(4)])


@jax.jit
def pallas_parallel_sum__sliding_local_dilated__glu_gated_bilinear__prompt_kernel(
    A_x: jax.Array,
    A_wqkv: jax.Array,
    A_wo: jax.Array,
    B_x: jax.Array,
    B_w_gate: jax.Array,
    B_w_up: jax.Array,
    B_w_down: jax.Array,
):
    del B_x
    x = A_x.reshape(S, D)
    hbm = pl.BlockSpec(memory_space=pl.ANY)
    dma = pltpu.SemaphoreType.DMA
    out = pl.pallas_call(
        _kernel,
        grid=(1,),
        in_specs=[pl.BlockSpec(memory_space=pltpu.SMEM)] + [hbm] * 6,
        out_specs=hbm,
        out_shape=jax.ShapeDtypeStruct((S, D), bf),
        scratch_shapes=[
            pltpu.VMEM((S, D), bf),
            pltpu.VMEM((S // 2, D), u32),
            pltpu.VMEM((NP, HB // 2, KB), u32),
            pltpu.VMEM((3, D, QW), bf),
            pltpu.VMEM((D, D), bf),
            pltpu.VMEM((D // 2, D), u32),
            pltpu.VMEM((2, 8, S // 2 + PADW, 128), u32),
            pltpu.VMEM((8, S // 2 + PADW, 128), u32),
            pltpu.VMEM((8, S + PADR + 8, 128), f32),
            pltpu.VMEM((8, S + PADR + 8, 128), f32),
            pltpu.VMEM((2, D, TF), bf),
            pltpu.VMEM((2, D, TF), bf),
            pltpu.VMEM((2, TF, D), bf),
            pltpu.VMEM((2, NP, KB // 2, 2 * TB), u32),
            pltpu.VMEM((2, NP, TB // 2, KB), u32),
            pltpu.VMEM((2, NP, 2, RS + MPAD, 128), f32),
            pltpu.VMEM((2, NP, RS // 2, TB), u32),
            pltpu.VMEM((4, 16, 24, 128), f32),
            pltpu.VMEM((4, 8, 24, 128), f32),
            pltpu.VMEM((NP, 2, HB + MPAD, 128), f32),
            dma((8,)), dma((3,)), dma((1,)), dma((2,)), dma((2,)), dma((2,)), dma((16,)),
        ],
        compiler_params=pltpu.CompilerParams(
            dimension_semantics=("arbitrary",), vmem_limit_bytes=127 * 1024 * 1024,
            disable_bounds_checks=True),
        name="fused_attn_ffn",
    )(jnp.ones((1,), jnp.int32), x, A_wqkv, A_wo, B_w_gate, B_w_up, B_w_down)
    return out.reshape(1, S, D)
```

```python
import jax
import jax.numpy as jnp
from jax import lax
from jax.experimental import pallas as pl
from jax.experimental.pallas import tpu as pltpu

bf = jnp.bfloat16
f32 = jnp.float32
u32 = jnp.uint32

S, D, F = 2048, 1024, 3584
WIN = 8
NP = 49
HB = S // 4
KB = D // 4
TF = 512
TB = TF // 4
NCH = F // TF
RS = 128
NSUB = HB // RS
NT = NCH * NSUB
MPAD = 8
PADW = 8
PADR = 16
QW = 256
EPS = 1e-5
C2 = float(32 ** -0.5 * 1.4426950408889634)

A_T = [[(1, (0, 0)), (1, (1, 1))], [(1, (1, 0)), (1, (1, 1))], [(1, (0, 0))], [(1, (1, 1))],
       [(1, (0, 0)), (1, (0, 1))], [(1, (1, 0)), (-1, (0, 0))], [(1, (0, 1)), (-1, (1, 1))]]
B_T = [[(1, (0, 0)), (1, (1, 1))], [(1, (0, 0))], [(1, (0, 1)), (-1, (1, 1))], [(1, (1, 0)), (-1, (0, 0))],
       [(1, (1, 1))], [(1, (0, 0)), (1, (0, 1))], [(1, (1, 0)), (1, (1, 1))]]
C_T = {(0, 0): [(1, 0), (1, 3), (-1, 4), (1, 6)], (0, 1): [(1, 2), (1, 4)],
       (1, 0): [(1, 1), (1, 3)], (1, 1): [(1, 0), (-1, 1), (1, 2), (1, 5)]}
POS = ((0, 0), (0, 1), (1, 0), (1, 1))


def _comb(terms):
    acc = None
    for s, v in terms:
        if acc is None:
            acc = v if s > 0 else -v
        else:
            acc = acc + v if s > 0 else acc - v
    return acc


def _dot(a, b):
    return jnp.dot(a, b, preferred_element_type=f32)


def _pk(v):
    return pltpu.bitcast(v.astype(bf), u32)


def _up(w):
    return pltpu.bitcast(w, bf)


def _unpk(w):
    return pltpu.bitcast(w, bf).astype(f32)


def _as_f32(w):
    return lax.bitcast_convert_type(w, f32)


def _as_u32(v):
    return lax.bitcast_convert_type(v, u32)


def _mult(x, m):
    return x if isinstance(x, int) else pl.multiple_of(x, m)


def _opcomb(load, table, I, emit, raw):
    sub = {(r, c): _comb([(s, load(q[0] * 2 + r, q[1] * 2 + c)) for s, q in table[I]])
           for r in range(2) for c in range(2)}
    for J, t2 in enumerate(table):
        if raw is not None and len(table[I]) == 1 and len(t2) == 1:
            qo, qi = table[I][0][1], t2[0][1]
            emit(I * 7 + J, raw(qo[0] * 2 + qi[0], qo[1] * 2 + qi[1]))
        else:
            emit(I * 7 + J, _pk(_comb([(s, sub[q]) for s, q in t2])))


def _opcomb_job(load, table, emit, raw=None):
    return [(lambda I=I: _opcomb(load, table, I, emit, raw)) for I in range(7)]


def _outpos(load, pos):
    inner = [_comb([(s, load(I * 7 + J)) for s, J in C_T[pos]]) for I in range(7)]
    return {q: _comb([(s, inner[I]) for s, I in terms]) for q, terms in C_T.items()}


def _perm8(v):
    lane = lax.broadcasted_iota(jnp.int32, v[0].shape, 1)
    v = list(v)
    for cb, lb in ((2, 4), (1, 3), (0, 2)):
        sh = 1 << lb
        hi = (lane & sh) != 0
        out = [None] * 8
        for c in range(8):
            if c & (1 << cb):
                continue
            x, y = v[c], v[c | (1 << cb)]
            out[c] = jnp.where(hi, pltpu.roll(y, sh, 1), x)
            out[c | (1 << cb)] = jnp.where(hi, y, pltpu.roll(x, 128 - sh, 1))
        v = out
    return v


def _sum4(x, lane):
    x = x + jnp.where((lane & 1) != 0, pltpu.roll(x, 1, 1), pltpu.roll(x, 127, 1))
    x = x + jnp.where((lane & 2) != 0, pltpu.roll(x, 2, 1), pltpu.roll(x, 126, 1))
    return x


def _mix(a, b):
    if not b:
        return list(a)
    if not a:
        return list(b)
    out, n, m, k = [], len(a), len(b), 0
    for i, t in enumerate(a):
        out.append(t)
        tgt = (i + 1) * m // n
        while k < tgt:
            out.append(b[k])
            k += 1
    return out


def _flat(jobs, depth=1):
    return [t for j in jobs for t in j]


def _weave(mx, jobs, woff=0):
    vp = _flat(jobs)
    tot = sum(c for _, c in mx)
    n, k, acc = len(vp), 0, 0
    for t, c in mx:
        t()
        acc += c
        tgt = min(n, acc * n // tot + woff)
        while k < tgt:
            vp[k]()
            k += 1
    while k < n:
        vp[k]()
        k += 1


def _kernel(one_ref, x_hbm, wqkv_hbm, wo_hbm, wg_hbm, wu_hbm, wd_hbm, out_hbm,
            xr, xn, T, wst, wqr, wqp, R, QP, KF, VF, gst, ust, dst, B, Bd, M, H, hst, ost, acc,
            sem_x, sem_w, sem_q, sem_g, sem_u, sem_d, sem_o):

    def block(mx, jobs, name="blk", woff=0):
        with jax.named_scope(name):
            @pl.when(one_ref[0] > 0)
            def _():
                _weave(mx(), jobs(), woff)

    def x_copy(r):
        rows = pl.ds(_mult(r * 256, 256), 256)
        return pltpu.make_async_copy(x_hbm.at[rows, :], xr.at[rows, :], sem_x.at[r])

    def w_copy(j, slot):
        col = (2 - j // 4) * D + (j % 4) * QW
        return pltpu.make_async_copy(wqkv_hbm.at[:, pl.ds(_mult(col, QW), QW)], wst.at[slot], sem_w.at[slot])

    def wq_copy():
        return pltpu.make_async_copy(wqkv_hbm.at[:, pl.ds(0, D)], wqr, sem_q.at[0])

    def gu_copies(j, par):
        cols = pl.ds(_mult(j * TF, TF), TF)
        return (pltpu.make_async_copy(wg_hbm.at[:, cols], gst.at[par], sem_g.at[par]),
                pltpu.make_async_copy(wu_hbm.at[:, cols], ust.at[par], sem_u.at[par]))

    def d_copy(j, par):
        return pltpu.make_async_copy(wd_hbm.at[pl.ds(_mult(j * TF, TF), TF), :], dst.at[par], sem_d.at[par])

    def wo_copies():
        return [pltpu.make_async_copy(wo_hbm.at[:, pl.ds(q * KB + h * TB, TB)],
                                      (gst, ust)[h].at[1, :, pl.ds(q * TB, TB)], (sem_g, sem_u)[h].at[1])
                for h in range(2) for q in range(4)]

    def out_copy(i, a):
        par = i % 2
        return pltpu.make_async_copy(dst.at[par, pl.ds(a * RS, RS), :],
                                     out_hbm.at[pl.ds(_mult(a * HB + i * RS, RS), RS), :], sem_o.at[par * 4 + a])

    def last_copy(a, h):
        rows = RS // 2
        return pltpu.make_async_copy(dst.at[1, pl.ds(a * RS + h * rows, rows), :],
                                     out_hbm.at[pl.ds(a * HB + 3 * RS + h * rows, rows), :], sem_o.at[8 + h * 4 + a])

    def start(cps):
        for cp in cps:
            cp.start()

    def wait(cps):
        for cp in cps:
            cp.wait()

    def ln_job(g):
        def t():
            v = [xr[pl.ds(g * 16, 16), pl.ds(c * 128, 128)].astype(f32) for c in range(8)]
            a = v[0]
            for c in range(1, 8):
                a = a + v[c]
            mean = jnp.sum(a, axis=1, keepdims=True) * (1.0 / D)
            v = [x - mean for x in v]
            a = v[0] * v[0]
            for c in range(1, 8):
                a = a + v[c] * v[c]
            r = lax.rsqrt(jnp.sum(a, axis=1, keepdims=True) * (1.0 / D) + EPS)
            for c in range(8):
                xn[pl.ds(g * 8, 8), pl.ds(c * 128, 128)] = _pk(v[c] * r)
        return [t]

    def ln_jobs(r):
        return [ln_job(r * 16 + g) for g in range(16)]

    def t_job(wb, pos):
        w0 = _mult(wb, 16) + (pos // 2) * 8
        l0 = (pos % 2) * 128

        def raw(i, j):
            return xn[pl.ds(w0 + i * 256, 8), pl.ds(j * KB + l0, 128)]

        def emit(p, v):
            T[p, pl.ds(w0, 8), pl.ds(l0, 128)] = v
        return _opcomb_job(lambda i, j: _unpk(raw(i, j)), A_T, emit, raw)

    def b_job(par, k, g, half):
        w_ref = (gst, ust)[half]

        def src(i, q):
            return w_ref[par, pl.ds(_mult(k * 64, 64) + (i * KB + g * 16), 16), pl.ds(q * TB, TB)]

        def emit(p, v):
            B[par, p, pl.ds(_mult(k * 32, 32) + g * 8, 8), pl.ds(half * TB, TB)] = v
        return _opcomb_job(lambda i, q: src(i, q).astype(f32), B_T, emit,
                           lambda i, q: pltpu.bitcast(src(i, q), u32))

    def bd_job(par, gb, g, n):
        def src(i, q):
            return dst[par, pl.ds(_mult(gb, 16) + (i * TB + g * 16), 16), pl.ds(q * KB + n * 128, 128)]

        def emit(p, v):
            Bd[par, p, pl.ds(_mult(gb // 2, 8) + g * 8, 8), pl.ds(n * 128, 128)] = v
        return _opcomb_job(lambda i, q: src(i, q).astype(f32), B_T, emit,
                           lambda i, q: pltpu.bitcast(src(i, q), u32))

    def b_jobs(par, k):
        return [b_job(par, k, g, h) for g in range(4) for h in range(2)]

    def bd_jobs(par, k):
        return [bd_job(par, k * 32, g, n) for g in range(2) for n in range(2)]

    def perm_job(m, i, a):
        dstp = (None, KF, VF)[m]

        def t():
            r = _perm8([R[2 - m, c, pl.ds(_mult(i * 256, 256) + a * 16, 16), :] for c in range(8)])
            for c in range(8):
                dstp[c, pl.ds(_mult(i * 512, 512) + (PADR + a * 32), 32), :] = _unpk(r[c])
        return [t]

    def wq_job(i, a):
        def t():
            rows = pl.ds(_mult(i * 512, 512) + a * 32, 32)
            r = _perm8([pltpu.bitcast(wqr[rows, pl.ds(c * 128, 128)], u32) for c in range(8)])
            for c in range(8):
                wqp[pl.ds(_mult(i * 256, 256) + a * 16, 16), pl.ds(c * 128, 128)] = r[c]
        return [t]

    def attn_quad(n, stack=False):
        base = _mult(((n % 8) // 2) * 256 + (n // 8) * 64 + (n % 2) * 32, 32)
        return [attn_job(base, 8 * k, k, stack) for k in range(4)]

    def attn_job(base, off, sl, stack):
        b = base + off
        rbase = _mult(base * 2, 64)
        job = []
        for h in range(2):
            st = {}
            half = lambda v, h=h: _unpk(v)[h * 8:(h + 1) * 8]

            def qk(cs, st=st, half=half, h=h):
                def t():
                    for c in cs:
                        qv = half(QP[c, pl.ds(base + off, 8), :])
                        for w in range(WIN):
                            kv = KF[c, pl.ds(rbase + (2 * off + 8 * h + PADR - 2 * w), 8), :]
                            st[w] = qv * kv if c == 0 else st[w] + qv * kv
                return t

            def sm(st=st, h=h):
                lane = lax.broadcasted_iota(jnp.int32, (8, 128), 1)
                row = lax.broadcasted_iota(jnp.int32, (8, 128), 0) + (b * 2 + h * 8)
                if stack:
                    big = jnp.concatenate([st[w] for w in range(WIN)], axis=0)
                    big = _sum4(big, lax.broadcasted_iota(jnp.int32, (8 * WIN, 128), 1))
                    ls = [big[8 * w:8 * w + 8] for w in range(WIN)]
                else:
                    ls = [_sum4(st[w], lane) for w in range(WIN)]
                ls = [ls[0]] + [jnp.where(row >= 2 * w, ls[w], -1e30) for w in range(1, WIN)]
                m = ls[0]
                for w in range(1, WIN):
                    m = jnp.maximum(m, ls[w])
                e = [jnp.exp2((l - m) * C2) for l in ls]
                den = e[0]
                for w in range(1, WIN):
                    den = den + e[w]
                inv = 1.0 / den
                st['p'] = [x * inv for x in e]

            def pv(cs, st=st, half=half, h=h):
                def t():
                    for c in cs:
                        o = None
                        for w in range(WIN):
                            a = st['p'][w] * VF[c, pl.ds(rbase + (2 * off + 8 * h + PADR - 2 * w), 8), :]
                            o = a if o is None else o + a
                        ost[sl, c, pl.ds(h * 8, 8), :] = o
                return t
            job += [qk((0, 1, 2, 3)), qk((4, 5, 6, 7)), sm, pv((0, 1, 2, 3)), pv((4, 5, 6, 7))]

        def fin():
            r = _perm8([_pk(ost[sl, c, pl.ds(0, 16), :]) for c in range(8)])
            for c in range(8):
                xn[pl.ds(_mult(b, 8), 8), pl.ds(c * 128, 128)] = r[c]
        return job + [fin]

    def comb_job(mp, g):
        sl = g % 4
        job = []
        for hf in range(2):
            for pos in POS:
                def t(hf=hf, pos=pos):
                    r = pl.ds(g * 16 + hf * 8, 8)
                    gg = _outpos(lambda p: M[mp, p, 0, r, :], pos)
                    uu = _outpos(lambda p: M[mp, p, 1, r, :], pos)
                    for q in gg:
                        hst[sl, (q[0] * 2 + pos[0]) * 4 + q[1] * 2 + pos[1], pl.ds(hf * 8, 8), :] = gg[q] * uu[q]
                job.append(t)

        def emit(p, v):
            H[mp, p, pl.ds(g * 8, 8), :] = v
        return job + _opcomb_job(lambda i, j: hst[sl, i * 4 + j, pl.ds(0, 16), :], A_T, emit)

    def comb_jobs(mp):
        return [comb_job(mp, g) for g in range(RS // 16)]

    def zero_job(p):
        def t():
            for c in range(2):
                acc[p, c, pl.ds(0, HB), :] = jnp.zeros((HB, 128), f32)
        return [t]

    def oc_job(i, g, n):
        def load(a, kb):
            return _unpk(xn[pl.ds(_mult(i * 64, 64) + (a * 256 + g * 8), 8), pl.ds(kb * KB + n * 128, 128)])

        def one(I):
            sub = {(r, c): _comb([(sg, load(q[0] * 2 + r, q[1] * 2 + c)) for sg, q in A_T[I]])
                   for r in range(2) for c in range(2)}
            for J, t2 in enumerate(A_T):
                M[i % 2, I * 7 + J, n, pl.ds(g * 16, 16), :] = _comb([(sg, sub[q]) for sg, q in t2])
        return [(lambda I=I: one(I)) for I in range(7)]

    def oc_jobs(i):
        return [oc_job(i, g, n) for g in range(RS // 16) for n in range(2)]

    def final_job(i, g, n):
        job = []
        par = i % 2
        for pos in POS:
            def t(pos=pos):
                r0 = _mult(i * RS, RS) + g * 16
                o = [_outpos(lambda p: acc[p, n, pl.ds(r0 + hf * 8, 8), :], pos) for hf in range(2)]
                for q in o[0]:
                    a = q[0] * 2 + pos[0]
                    cols = pl.ds(((q[1] * 2 + pos[1]) * 2 + n) * 128, 128)
                    res = xr[pl.ds(r0 + a * HB, 16), cols].astype(f32) + jnp.concatenate([o[0][q], o[1][q]], axis=0)
                    dst[par, pl.ds(a * RS + g * 16, 16), cols] = res.astype(bf)
            job.append(t)
        return job

    def final_jobs(i):
        return [final_job(i, g, n) for g in range(RS // 16) for n in range(2)]

    def kv_tasks(m, slot, cbase, pieces):
        out = []
        for r in pieces:
            for ct in range(QW // 128):
                def t(r=r, ct=ct):
                    res = _dot(_up(xn[pl.ds(_mult(r * 64, 64), 64), :]), wst[slot, :, pl.ds(ct * 128, 128)])
                    for k in range(8):
                        R[2 - m, cbase + ct, pl.ds(_mult(r * 64 + k * 8, 8), 8), :] = _pk(res[k * 16:(k + 1) * 16])
                out.append((t, 256))
        return out

    def q_tasks(cbase):
        out = []
        for r in range(16):
            for ct in range(QW // 128):
                def t(r=r, ct=ct):
                    res = _dot(_up(xn[pl.ds(r * 64, 64), :]),
                               _up(wqp[:, pl.ds(_mult((cbase + ct) * 128, 128), 128)]))
                    for k in range(8):
                        QP[cbase + ct, pl.ds(r * 64 + k * 8, 8), :] = _pk(res[k * 16:(k + 1) * 16])
                out.append((t, 256))
        return out

    def mm1_tasks(mp, s, par):
        out = []
        for p in range(NP):
            for c in range(2):
                def t(p=p, c=c):
                    M[mp, p, c, pl.ds(0, RS), :] = _dot(
                        _up(T[p, pl.ds(_mult(s * (RS // 2), RS // 2), RS // 2), :]),
                        _up(B[par, p, :, pl.ds(c * 128, 128)]))
                out.append((t, 64))
        return out

    def mm2_tasks(mp, s, par):
        out = []
        for p in range(NP):
            def t(p=p):
                r = _dot(_up(H[mp, p]), _up(Bd[par, p]))
                for c in range(2):
                    acc[p, c, pl.ds(_mult(s * RS, RS), RS), :] += r[:, c * 128:(c + 1) * 128]
            out.append((t, 64))
        return out

    def wo_tasks(i):
        out = []
        for p in range(NP):
            for c in range(2):
                def t(p=p, c=c):
                    lhs = jnp.concatenate([M[i % 2, p, n, pl.ds(0, RS), :] for n in range(2)], axis=1)
                    acc[p, c, pl.ds(_mult(i * RS, RS), RS), :] += lax.dot_general(
                        lhs, _up(B[1, p, :, pl.ds(c * 128, 128)]), (((1,), (0,)), ((), ())),
                        preferred_element_type=f32)
                out.append((t, 64))
        return out

    nothing = lambda: [(lambda: None, 1)]

    x_copy(0).start()
    w_copy(0, 0).start()
    for c in range(8):
        KF[c, pl.ds(0, PADR), :] = jnp.zeros((PADR, 128), f32)
        VF[c, pl.ds(0, PADR), :] = jnp.zeros((PADR, 128), f32)
    x_copy(0).wait()
    w_copy(1, 1).start()
    x_copy(1).start()
    block(nothing, lambda: ln_jobs(0), 'ln0')
    w_copy(0, 0).wait()

    def v01(pieces):
        rp = [2 * r + h for r in pieces for h in range(2)]
        return kv_tasks(2, 0, 0, rp) + kv_tasks(2, 1, 2, rp)

    block(lambda: kv_tasks(2, 0, 0, (0, 1)), lambda: [], 'p0')
    w_copy(1, 1).wait()
    x_copy(2).start()
    x_copy(1).wait()
    block(lambda: kv_tasks(2, 1, 2, (0, 1)), lambda: ln_jobs(1), 'p0')
    x_copy(3).start()
    x_copy(4).start()
    x_copy(2).wait()
    block(lambda: v01((1,)), lambda: ln_jobs(2), 'p0')
    x_copy(5).start()
    x_copy(6).start()
    x_copy(3).wait()
    x_copy(4).wait()
    block(lambda: v01((2,)), lambda: ln_jobs(3) + ln_jobs(4), 'p0')
    x_copy(7).start()
    w_copy(2, 2).start()
    x_copy(5).wait()
    x_copy(6).wait()
    block(lambda: v01((3, 4)), lambda: ln_jobs(5) + ln_jobs(6), 'p0')
    wq_copy().start()
    x_copy(7).wait()
    block(lambda: v01((5, 6)), lambda: ln_jobs(7), 'p0')
    block(lambda: v01((7,)), lambda: [], 'p0')

    def kv_block(j, m, after_start, jobs, name, woff=0):
        slot = j % 3
        w_copy(j, slot).wait()

        @pl.when(j + 1 < 8)
        def _():
            w_copy(j + 1, (j + 1) % 3).start()
        after_start()
        block(lambda: kv_tasks(m, slot, (j % 4) * 2, range(16)), jobs, name, woff)

    def v_body(j, c):
        def dmas():
            @pl.when(j == 2)
            def _():
                start(gu_copies(0, 0))

            @pl.when(j == 3)
            def _():
                d_copy(0, 0).start()
                d_copy(1, 1).start()
        kv_block(j, 2, dmas, lambda: [wq_job(j - 2, a) for a in range(16)], 'v')
        return c
    wq_copy().wait()
    lax.fori_loop(2, 4, v_body, 0)

    def k_body(j, c):
        def dmas():
            @pl.when(j == 4)
            def _():
                start(gu_copies(1, 1))
        i = j - 4
        kv_block(j, 1, dmas, lambda: _mix([perm_job(2, i, a) for a in range(16)],
                                          [t_job(i * 48, a) for a in range(12)]), 'k', 2)
        return c
    lax.fori_loop(4, 8, k_body, 0)

    wait(gu_copies(0, 0))
    d_copy(0, 0).wait()

    def q_body(i, c):
        def jobs():
            extra = (b_jobs(0, i)
                     + [bd_job(0, i * 16, 0, n) for n in range(2)]
                     + [t_job(192 + 16 * i, a) for a in range(4)])
            zero = [zero_job(jnp.minimum(i * 13 + a, NP - 1)) for a in range(13)]
            rest = _mix([perm_job(1, i, a) for a in range(16)], extra)
            return _mix(rest[:-6], zero) + rest[-6:]
        block(lambda: q_tasks(i * 2), jobs, 'q', 2)
        return c
    lax.fori_loop(0, 4, q_body, 0)

    wait(gu_copies(1, 1))
    start(gu_copies(2, 0))
    block(lambda: mm1_tasks(0, 0, 0),
          lambda: _mix(b_jobs(1, 0) + bd_jobs(0, 2), attn_quad(0, True) + attn_quad(1, True)), 'f0')
    block(lambda: mm1_tasks(1, 1, 0),
          lambda: _mix(_mix(comb_jobs(0), b_jobs(1, 1) + bd_jobs(0, 3)), _flat([attn_quad(n, True) for n in []])), 'f1', 3)

    def slot(t, mp):
        j = t // 4
        s = t % 4
        par = j % 2
        if mp == 0:
            @pl.when(jnp.logical_and(s == 0, j > 0))
            def _():
                wait(gu_copies(jnp.minimum(j + 1, NCH - 1), 1 - par))

                @pl.when(j + 2 < NCH)
                def _():
                    start(gu_copies(j + 2, par))

                @pl.when(j + 2 == NCH)
                def _():
                    start(wo_copies())

            @pl.when(jnp.logical_and(s == 2, j + 1 < NCH))
            def _():
                d_copy(j + 1, 1 - par).wait()

                @pl.when(j + 2 < NCH)
                def _():
                    d_copy(j + 2, par).start()
        jd = (t + 2) // 4
        kd = (t + 2) % 4
        u = t - 2

        def jobs():
            base = _mix(comb_jobs(1 - mp), b_jobs(1 - par, s) + bd_jobs(jd % 2, kd))
            att = attn_quad(u + 2)
            n0 = max(1, len(base) // 10)
            return base[:n0] + _mix(base[n0:-n0], att) + base[-n0:]
        block(lambda: mm1_tasks(mp, s, par) + mm2_tasks(mp, (t - 2) % 4, ((t - 2) // 4) % 2), jobs,
              'slot%d' % mp, 3)

    def steady(it, c):
        slot(2 * it + 2, 0)
        slot(2 * it + 3, 1)
        return c
    lax.fori_loop(0, (NT - 2) // 2, steady, 0)

    block(lambda: mm2_tasks(0, 2, 0), lambda: comb_jobs(1), 'e0')
    block(lambda: mm2_tasks(1, 3, 0), lambda: _mix(oc_jobs(0), _flat([attn_quad(n, True) for n in []])), 'e1')
    block(lambda: wo_tasks(0),
          lambda: _mix(oc_jobs(1), _flat([attn_quad(n, True) for n in [28, 29]])), 'wo')
    for i in range(1, 4):
        if i == 3:
            wait([out_copy(0, a) for a in range(4)])
        block(lambda i=i: wo_tasks(i),
              lambda i=i: _mix(final_jobs(i - 1) + (oc_jobs(i + 1) if i < 3 else []),
                                _flat([attn_quad(n, True) for n in ([30, 31] if i == 1 else [])])), 'wo')
        start([out_copy(i - 1, a) for a in range(4)])
    wait([out_copy(1, a) for a in range(4)])
    for h in range(2):
        block(nothing, lambda h=h: [final_job(3, g, n) for g in range(4 * h, 4 * h + 4) for n in range(2)], 'e3')
        start([last_copy(a, h) for a in range(4)])
    wait([out_copy(2, a) for a in range(4)])
    wait([last_copy(a, h) for h in range(2) for a in range(4)])


@jax.jit
def pallas_parallel_sum__sliding_local_dilated__glu_gated_bilinear__prompt_kernel(
    A_x: jax.Array,
    A_wqkv: jax.Array,
    A_wo: jax.Array,
    B_x: jax.Array,
    B_w_gate: jax.Array,
    B_w_up: jax.Array,
    B_w_down: jax.Array,
):
    del B_x
    x = A_x.reshape(S, D)
    hbm = pl.BlockSpec(memory_space=pl.ANY)
    dma = pltpu.SemaphoreType.DMA
    out = pl.pallas_call(
        _kernel,
        grid=(1,),
        in_specs=[pl.BlockSpec(memory_space=pltpu.SMEM)] + [hbm] * 6,
        out_specs=hbm,
        out_shape=jax.ShapeDtypeStruct((S, D), bf),
        scratch_shapes=[
            pltpu.VMEM((S, D), bf),
            pltpu.VMEM((S // 2, D), u32),
            pltpu.VMEM((NP, HB // 2, KB), u32),
            pltpu.VMEM((3, D, QW), bf),
            pltpu.VMEM((D, D), bf),
            pltpu.VMEM((D // 2, D), u32),
            pltpu.VMEM((2, 8, S // 2 + PADW, 128), u32),
            pltpu.VMEM((8, S // 2 + PADW, 128), u32),
            pltpu.VMEM((8, S + PADR + 8, 128), f32),
            pltpu.VMEM((8, S + PADR + 8, 128), f32),
            pltpu.VMEM((2, D, TF), bf),
            pltpu.VMEM((2, D, TF), bf),
            pltpu.VMEM((2, TF, D), bf),
            pltpu.VMEM((2, NP, KB // 2, 2 * TB), u32),
            pltpu.VMEM((2, NP, TB // 2, KB), u32),
            pltpu.VMEM((2, NP, 2, RS + MPAD, 128), f32),
            pltpu.VMEM((2, NP, RS // 2, TB), u32),
            pltpu.VMEM((4, 16, 24, 128), f32),
            pltpu.VMEM((4, 8, 24, 128), f32),
            pltpu.VMEM((NP, 2, HB + MPAD, 128), f32),
            dma((8,)), dma((3,)), dma((1,)), dma((2,)), dma((2,)), dma((2,)), dma((16,)),
        ],
        compiler_params=pltpu.CompilerParams(
            dimension_semantics=("arbitrary",), vmem_limit_bytes=127 * 1024 * 1024,
            disable_bounds_checks=True),
        name="fused_attn_ffn",
    )(jnp.ones((1,), jnp.int32), x, A_wqkv, A_wo, B_w_gate, B_w_up, B_w_down)
    return out.reshape(1, S, D)
```

```python
import jax
import jax.numpy as jnp
from jax import lax
from jax.experimental import pallas as pl
from jax.experimental.pallas import tpu as pltpu

bf = jnp.bfloat16
f32 = jnp.float32
u32 = jnp.uint32

S, D, F = 2048, 1024, 3584
WIN = 8
NP = 49
HB = S // 4
KB = D // 4
TF = 512
TB = TF // 4
NCH = F // TF
RS = 128
NSUB = HB // RS
NT = NCH * NSUB
MPAD = 8
PADW = 8
PADR = 16
QW = 256
EPS = 1e-5
C2 = float(32 ** -0.5 * 1.4426950408889634)

A_T = [[(1, (0, 0)), (1, (1, 1))], [(1, (1, 0)), (1, (1, 1))], [(1, (0, 0))], [(1, (1, 1))],
       [(1, (0, 0)), (1, (0, 1))], [(1, (1, 0)), (-1, (0, 0))], [(1, (0, 1)), (-1, (1, 1))]]
B_T = [[(1, (0, 0)), (1, (1, 1))], [(1, (0, 0))], [(1, (0, 1)), (-1, (1, 1))], [(1, (1, 0)), (-1, (0, 0))],
       [(1, (1, 1))], [(1, (0, 0)), (1, (0, 1))], [(1, (1, 0)), (1, (1, 1))]]
C_T = {(0, 0): [(1, 0), (1, 3), (-1, 4), (1, 6)], (0, 1): [(1, 2), (1, 4)],
       (1, 0): [(1, 1), (1, 3)], (1, 1): [(1, 0), (-1, 1), (1, 2), (1, 5)]}
POS = ((0, 0), (0, 1), (1, 0), (1, 1))


def _comb(terms):
    acc = None
    for s, v in terms:
        if acc is None:
            acc = v if s > 0 else -v
        else:
            acc = acc + v if s > 0 else acc - v
    return acc


def _dot(a, b):
    return jnp.dot(a, b, preferred_element_type=f32)


def _pk(v):
    return pltpu.bitcast(v.astype(bf), u32)


def _up(w):
    return pltpu.bitcast(w, bf)


def _unpk(w):
    return pltpu.bitcast(w, bf).astype(f32)


def _as_f32(w):
    return lax.bitcast_convert_type(w, f32)


def _as_u32(v):
    return lax.bitcast_convert_type(v, u32)


def _mult(x, m):
    return x if isinstance(x, int) else pl.multiple_of(x, m)


def _opcomb(load, table, I, emit, raw):
    sub = {(r, c): _comb([(s, load(q[0] * 2 + r, q[1] * 2 + c)) for s, q in table[I]])
           for r in range(2) for c in range(2)}
    for J, t2 in enumerate(table):
        if raw is not None and len(table[I]) == 1 and len(t2) == 1:
            qo, qi = table[I][0][1], t2[0][1]
            emit(I * 7 + J, raw(qo[0] * 2 + qi[0], qo[1] * 2 + qi[1]))
        else:
            emit(I * 7 + J, _pk(_comb([(s, sub[q]) for s, q in t2])))


def _opcomb_job(load, table, emit, raw=None):
    return [(lambda I=I: _opcomb(load, table, I, emit, raw)) for I in range(7)]


def _outpos(load, pos):
    inner = [_comb([(s, load(I * 7 + J)) for s, J in C_T[pos]]) for I in range(7)]
    return {q: _comb([(s, inner[I]) for s, I in terms]) for q, terms in C_T.items()}


def _perm8(v):
    lane = lax.broadcasted_iota(jnp.int32, v[0].shape, 1)
    v = list(v)
    for cb, lb in ((2, 4), (1, 3), (0, 2)):
        sh = 1 << lb
        hi = (lane & sh) != 0
        out = [None] * 8
        for c in range(8):
            if c & (1 << cb):
                continue
            x, y = v[c], v[c | (1 << cb)]
            out[c] = jnp.where(hi, pltpu.roll(y, sh, 1), x)
            out[c | (1 << cb)] = jnp.where(hi, y, pltpu.roll(x, 128 - sh, 1))
        v = out
    return v


def _sum4(x, lane):
    x = x + jnp.where((lane & 1) != 0, pltpu.roll(x, 1, 1), pltpu.roll(x, 127, 1))
    x = x + jnp.where((lane & 2) != 0, pltpu.roll(x, 2, 1), pltpu.roll(x, 126, 1))
    return x


def _mix(a, b):
    if not b:
        return list(a)
    if not a:
        return list(b)
    out, n, m, k = [], len(a), len(b), 0
    for i, t in enumerate(a):
        out.append(t)
        tgt = (i + 1) * m // n
        while k < tgt:
            out.append(b[k])
            k += 1
    return out


def _flat(jobs, depth=1):
    return [t for j in jobs for t in j]


def _weave(mx, jobs, woff=0):
    vp = _flat(jobs)
    tot = sum(c for _, c in mx)
    n, k, acc = len(vp), 0, 0
    for t, c in mx:
        t()
        acc += c
        tgt = min(n, acc * n // tot + woff)
        while k < tgt:
            vp[k]()
            k += 1
    while k < n:
        vp[k]()
        k += 1


def _kernel(one_ref, x_hbm, wqkv_hbm, wo_hbm, wg_hbm, wu_hbm, wd_hbm, out_hbm,
            xr, xn, T, wst, wqr, wqp, wvp, R, QP, KF, VF, gst, ust, dst, B, Bd, M, H, hst, ost, acc,
            sem_x, sem_w, sem_q, sem_g, sem_u, sem_d, sem_o):

    def block(mx, jobs, name="blk", woff=0):
        with jax.named_scope(name):
            @pl.when(one_ref[0] > 0)
            def _():
                _weave(mx(), jobs(), woff)

    def x_copy(r):
        rows = pl.ds(_mult(r * 256, 256), 256)
        return pltpu.make_async_copy(x_hbm.at[rows, :], xr.at[rows, :], sem_x.at[r])

    def w_copy(j, slot):
        return pltpu.make_async_copy(wqkv_hbm.at[:, pl.ds(_mult(D + j * QW, QW), QW)], wst.at[slot], sem_w.at[slot])

    def wv_copies():
        return (pltpu.make_async_copy(wqkv_hbm.at[:, pl.ds(2 * D, TF)], gst.at[1], sem_g.at[1]),
                pltpu.make_async_copy(wqkv_hbm.at[:, pl.ds(2 * D + TF, TF)], ust.at[1], sem_u.at[1]))

    def wq_copy():
        return pltpu.make_async_copy(wqkv_hbm.at[:, pl.ds(0, D)], wqr, sem_q.at[0])

    def gu_copies(j, par):
        cols = pl.ds(_mult(j * TF, TF), TF)
        return (pltpu.make_async_copy(wg_hbm.at[:, cols], gst.at[par], sem_g.at[par]),
                pltpu.make_async_copy(wu_hbm.at[:, cols], ust.at[par], sem_u.at[par]))

    def d_copy(j, par):
        return pltpu.make_async_copy(wd_hbm.at[pl.ds(_mult(j * TF, TF), TF), :], dst.at[par], sem_d.at[par])

    def wo_copies():
        return [pltpu.make_async_copy(wo_hbm.at[:, pl.ds(q * KB + h * TB, TB)],
                                      (gst, ust)[h].at[1, :, pl.ds(q * TB, TB)], (sem_g, sem_u)[h].at[1])
                for h in range(2) for q in range(4)]

    def out_copy(i, a):
        par = i % 2
        return pltpu.make_async_copy(dst.at[par, pl.ds(a * RS, RS), :],
                                     out_hbm.at[pl.ds(_mult(a * HB + i * RS, RS), RS), :], sem_o.at[par * 4 + a])

    def last_copy(a, h):
        rows = RS // 2
        return pltpu.make_async_copy(dst.at[1, pl.ds(a * RS + h * rows, rows), :],
                                     out_hbm.at[pl.ds(a * HB + 3 * RS + h * rows, rows), :], sem_o.at[8 + h * 4 + a])

    def start(cps):
        for cp in cps:
            cp.start()

    def wait(cps):
        for cp in cps:
            cp.wait()

    def ln_job(g):
        def t():
            v = [xr[pl.ds(g * 16, 16), pl.ds(c * 128, 128)].astype(f32) for c in range(8)]
            a = v[0]
            for c in range(1, 8):
                a = a + v[c]
            mean = jnp.sum(a, axis=1, keepdims=True) * (1.0 / D)
            v = [x - mean for x in v]
            a = v[0] * v[0]
            for c in range(1, 8):
                a = a + v[c] * v[c]
            r = lax.rsqrt(jnp.sum(a, axis=1, keepdims=True) * (1.0 / D) + EPS)
            for c in range(8):
                xn[pl.ds(g * 8, 8), pl.ds(c * 128, 128)] = _pk(v[c] * r)
        return [t]

    def ln_jobs(r):
        return [ln_job(r * 16 + g) for g in range(16)]

    def t_job(wb, pos):
        w0 = _mult(wb, 16) + (pos // 2) * 8
        l0 = (pos % 2) * 128

        def raw(i, j):
            return xn[pl.ds(w0 + i * 256, 8), pl.ds(j * KB + l0, 128)]

        def emit(p, v):
            T[p, pl.ds(w0, 8), pl.ds(l0, 128)] = v
        return _opcomb_job(lambda i, j: _unpk(raw(i, j)), A_T, emit, raw)

    def b_job(par, k, g, half):
        w_ref = (gst, ust)[half]

        def src(i, q):
            return w_ref[par, pl.ds(_mult(k * 64, 64) + (i * KB + g * 16), 16), pl.ds(q * TB, TB)]

        def emit(p, v):
            B[par, p, pl.ds(_mult(k * 32, 32) + g * 8, 8), pl.ds(half * TB, TB)] = v
        return _opcomb_job(lambda i, q: src(i, q).astype(f32), B_T, emit,
                           lambda i, q: pltpu.bitcast(src(i, q), u32))

    def bd_job(par, gb, g, n):
        def src(i, q):
            return dst[par, pl.ds(_mult(gb, 16) + (i * TB + g * 16), 16), pl.ds(q * KB + n * 128, 128)]

        def emit(p, v):
            Bd[par, p, pl.ds(_mult(gb // 2, 8) + g * 8, 8), pl.ds(n * 128, 128)] = v
        return _opcomb_job(lambda i, q: src(i, q).astype(f32), B_T, emit,
                           lambda i, q: pltpu.bitcast(src(i, q), u32))

    def b_jobs(par, k):
        return [b_job(par, k, g, h) for g in range(4) for h in range(2)]

    def bd_jobs(par, k):
        return [bd_job(par, k * 32, g, n) for g in range(2) for n in range(2)]

    def kperm_job(i, a):
        def t():
            r = _perm8([R[c, pl.ds(_mult(i * 256, 256) + a * 16, 16), :] for c in range(8)])
            for c in range(8):
                KF[c, pl.ds(_mult(i * 512, 512) + (PADR + a * 32), 32), :] = _unpk(r[c])
        return [t]

    def wperm_job(which, pb, a, np_=1):
        def t():
            rows = pl.ds(_mult(pb * 32, 256) + a * 32, 32 * np_)
            if which == 'q':
                src = [wqr[rows, pl.ds(c * 128, 128)] for c in range(8)]
            else:
                src = [(gst, ust)[c // 4][1, rows, pl.ds((c % 4) * 128, 128)] for c in range(8)]
            r = _perm8([pltpu.bitcast(v, u32) for v in src])
            for c in range(8):
                (wqp if which == 'q' else wvp)[pl.ds(_mult(pb * 16, 128) + a * 16, 16 * np_), pl.ds(c * 128, 128)] = r[c]
        return [t]

    def bv_job(k, g, half):
        def raw(i, q):
            return wvp[pl.ds(_mult(k * 32, 32) + (i * (KB // 2) + g * 8), 8), pl.ds((2 * q + half) * 128, 128)]

        def emit(p, v):
            B[1, p, pl.ds(_mult(k * 32, 32) + g * 8, 8), pl.ds(half * TB, TB)] = v
        return _opcomb_job(lambda i, q: _unpk(raw(i, q)), B_T, emit, raw)

    def vcomb_job(mp, s, g):
        job = []
        for hf in range(2):
            for pos in POS:
                def t(hf=hf, pos=pos):
                    for n in range(2):
                        o = _outpos(lambda p: M[mp, p, n, pl.ds(g * 16 + hf * 8, 8), :], pos)
                        for q in o:
                            a = q[0] * 2 + pos[0]
                            ch = (q[1] * 2 + pos[1]) * 2 + n
                            VF[ch, pl.ds(_mult(s * RS, RS) + (PADR + a * HB + g * 16 + hf * 8), 8), :] = o[q]
                job.append(t)
        return job

    def vcomb_jobs(mp, s):
        return [vcomb_job(mp, s, g) for g in range(RS // 16)]

    def mzero_job(p):
        def t():
            for c in range(2):
                M[1, p, c, pl.ds(0, RS), :] = jnp.zeros((RS, 128), f32)
        return [t]

    def attn_quad(n, stack=False):
        base = _mult(((n % 8) // 2) * 256 + (n // 8) * 64 + (n % 2) * 32, 32)
        return [attn_job(base, 8 * k, k, stack) for k in range(4)]

    def attn_job(base, off, sl, stack):
        b = base + off
        rbase = _mult(base * 2, 64)
        job = []
        for h in range(2):
            st = {}
            half = lambda v, h=h: _unpk(v)[h * 8:(h + 1) * 8]

            def qk(cs, st=st, half=half, h=h):
                def t():
                    for c in cs:
                        qv = half(QP[c, pl.ds(base + off, 8), :])
                        for w in range(WIN):
                            kv = KF[c, pl.ds(rbase + (2 * off + 8 * h + PADR - 2 * w), 8), :]
                            st[w] = qv * kv if c == 0 else st[w] + qv * kv
                return t

            def sm(st=st, h=h):
                lane = lax.broadcasted_iota(jnp.int32, (8, 128), 1)
                row = lax.broadcasted_iota(jnp.int32, (8, 128), 0) + (b * 2 + h * 8)
                if stack:
                    big = jnp.concatenate([st[w] for w in range(WIN)], axis=0)
                    big = _sum4(big, lax.broadcasted_iota(jnp.int32, (8 * WIN, 128), 1))
                    ls = [big[8 * w:8 * w + 8] for w in range(WIN)]
                else:
                    ls = [_sum4(st[w], lane) for w in range(WIN)]
                ls = [ls[0]] + [jnp.where(row >= 2 * w, ls[w], -1e30) for w in range(1, WIN)]
                m = ls[0]
                for w in range(1, WIN):
                    m = jnp.maximum(m, ls[w])
                e = [jnp.exp2((l - m) * C2) for l in ls]
                den = e[0]
                for w in range(1, WIN):
                    den = den + e[w]
                inv = 1.0 / den
                st['p'] = [x * inv for x in e]

            def pv(cs, st=st, half=half, h=h):
                def t():
                    for c in cs:
                        o = None
                        for w in range(WIN):
                            a = st['p'][w] * VF[c, pl.ds(rbase + (2 * off + 8 * h + PADR - 2 * w), 8), :]
                            o = a if o is None else o + a
                        ost[sl, c, pl.ds(h * 8, 8), :] = o
                return t
            job += [qk((0, 1, 2, 3)), qk((4, 5, 6, 7)), sm, pv((0, 1, 2, 3)), pv((4, 5, 6, 7))]

        def fin():
            r = _perm8([_pk(ost[sl, c, pl.ds(0, 16), :]) for c in range(8)])
            for c in range(8):
                xn[pl.ds(_mult(b, 8), 8), pl.ds(c * 128, 128)] = r[c]
        return job + [fin]

    def comb_job(mp, g):
        sl = g % 4
        job = []
        for hf in range(2):
            for pos in POS:
                def t(hf=hf, pos=pos):
                    r = pl.ds(g * 16 + hf * 8, 8)
                    gg = _outpos(lambda p: M[mp, p, 0, r, :], pos)
                    uu = _outpos(lambda p: M[mp, p, 1, r, :], pos)
                    for q in gg:
                        hst[sl, (q[0] * 2 + pos[0]) * 4 + q[1] * 2 + pos[1], pl.ds(hf * 8, 8), :] = gg[q] * uu[q]
                job.append(t)

        def emit(p, v):
            H[mp, p, pl.ds(g * 8, 8), :] = v
        return job + _opcomb_job(lambda i, j: hst[sl, i * 4 + j, pl.ds(0, 16), :], A_T, emit)

    def comb_jobs(mp):
        return [comb_job(mp, g) for g in range(RS // 16)]

    def zero_job(p):
        def t():
            for c in range(2):
                acc[p, c, pl.ds(0, HB), :] = jnp.zeros((HB, 128), f32)
        return [t]

    def oc_job(i, g, n):
        def load(a, kb):
            return _unpk(xn[pl.ds(_mult(i * 64, 64) + (a * 256 + g * 8), 8), pl.ds(kb * KB + n * 128, 128)])

        def one(I):
            sub = {(r, c): _comb([(sg, load(q[0] * 2 + r, q[1] * 2 + c)) for sg, q in A_T[I]])
                   for r in range(2) for c in range(2)}
            for J, t2 in enumerate(A_T):
                M[i % 2, I * 7 + J, n, pl.ds(g * 16, 16), :] = _comb([(sg, sub[q]) for sg, q in t2])
        return [(lambda I=I: one(I)) for I in range(7)]

    def oc_jobs(i):
        return [oc_job(i, g, n) for g in range(RS // 16) for n in range(2)]

    def final_job(i, g, n):
        job = []
        par = i % 2
        for pos in POS:
            def t(pos=pos):
                r0 = _mult(i * RS, RS) + g * 16
                o = [_outpos(lambda p: acc[p, n, pl.ds(r0 + hf * 8, 8), :], pos) for hf in range(2)]
                for q in o[0]:
                    a = q[0] * 2 + pos[0]
                    cols = pl.ds(((q[1] * 2 + pos[1]) * 2 + n) * 128, 128)
                    res = xr[pl.ds(r0 + a * HB, 16), cols].astype(f32) + jnp.concatenate([o[0][q], o[1][q]], axis=0)
                    dst[par, pl.ds(a * RS + g * 16, 16), cols] = res.astype(bf)
            job.append(t)
        return job

    def final_jobs(i):
        return [final_job(i, g, n) for g in range(RS // 16) for n in range(2)]

    def k_tasks(slot, cbase, pieces):
        out = []
        for r in pieces:
            for ct in range(QW // 128):
                def t(r=r, ct=ct):
                    res = _dot(_up(xn[pl.ds(_mult(r * 64, 64), 64), :]), wst[slot, :, pl.ds(ct * 128, 128)])
                    for k in range(8):
                        R[cbase + ct, pl.ds(_mult(r * 64 + k * 8, 8), 8), :] = _pk(res[k * 16:(k + 1) * 16])
                out.append((t, 256))
        return out

    def q_tasks(cbase):
        out = []
        for r in range(16):
            for ct in range(QW // 128):
                def t(r=r, ct=ct):
                    res = _dot(_up(xn[pl.ds(r * 64, 64), :]),
                               _up(wqp[:, pl.ds(_mult((cbase + ct) * 128, 128), 128)]))
                    for k in range(8):
                        QP[cbase + ct, pl.ds(r * 64 + k * 8, 8), :] = _pk(res[k * 16:(k + 1) * 16])
                out.append((t, 256))
        return out

    def mm1_tasks(mp, s, par):
        out = []
        for p in range(NP):
            for c in range(2):
                def t(p=p, c=c):
                    M[mp, p, c, pl.ds(0, RS), :] = _dot(
                        _up(T[p, pl.ds(_mult(s * (RS // 2), RS // 2), RS // 2), :]),
                        _up(B[par, p, :, pl.ds(c * 128, 128)]))
                out.append((t, 64))
        return out

    def mm2_tasks(mp, s, par):
        out = []
        for p in range(NP):
            def t(p=p):
                r = _dot(_up(H[mp, p]), _up(Bd[par, p]))
                for c in range(2):
                    acc[p, c, pl.ds(_mult(s * RS, RS), RS), :] += r[:, c * 128:(c + 1) * 128]
            out.append((t, 64))
        return out

    def wo_tasks(i):
        out = []
        for p in range(NP):
            for c in range(2):
                def t(p=p, c=c):
                    lhs = jnp.concatenate([M[i % 2, p, n, pl.ds(0, RS), :] for n in range(2)], axis=1)
                    acc[p, c, pl.ds(_mult(i * RS, RS), RS), :] += lax.dot_general(
                        lhs, _up(B[1, p, :, pl.ds(c * 128, 128)]), (((1,), (0,)), ((), ())),
                        preferred_element_type=f32)
                out.append((t, 64))
        return out

    nothing = lambda: [(lambda: None, 1)]

    x_copy(0).start()
    w_copy(0, 0).start()
    for c in range(8):
        KF[c, pl.ds(0, PADR), :] = jnp.zeros((PADR, 128), f32)
        VF[c, pl.ds(0, PADR), :] = jnp.zeros((PADR, 128), f32)
    x_copy(0).wait()
    w_copy(1, 1).start()
    x_copy(1).start()
    block(nothing, lambda: ln_jobs(0), 'ln0')
    w_copy(0, 0).wait()

    def k01(pieces):
        rp = [2 * r + h for r in pieces for h in range(2)]
        return k_tasks(0, 0, rp) + k_tasks(1, 2, rp)

    block(lambda: k_tasks(0, 0, (0, 1)), lambda: [], 'p0')
    w_copy(1, 1).wait()
    x_copy(2).start()
    x_copy(1).wait()
    block(lambda: k_tasks(1, 2, (0, 1)), lambda: ln_jobs(1), 'p0')
    x_copy(3).start()
    x_copy(4).start()
    x_copy(2).wait()
    block(lambda: k01((1,)), lambda: ln_jobs(2), 'p0')
    x_copy(5).start()
    x_copy(6).start()
    x_copy(3).wait()
    x_copy(4).wait()
    block(lambda: k01((2,)), lambda: ln_jobs(3) + ln_jobs(4), 'p0')
    x_copy(7).start()
    wq_copy().start()
    x_copy(5).wait()
    x_copy(6).wait()
    block(lambda: k01((3, 4)), lambda: ln_jobs(5) + ln_jobs(6), 'p0')
    w_copy(2, 2).start()
    start(wv_copies())
    x_copy(7).wait()
    wq_copy().wait()
    block(lambda: k01((5, 6)), lambda: _mix(ln_jobs(7), [wperm_job('q', 0, a, 2) for a in range(0, 10, 2)]), 'p0')
    block(lambda: k01((7,)), lambda: [wperm_job('q', 0, a, 2) for a in range(10, 16, 2)], 'p0')

    wait(wv_copies())

    def k_body(j, c):
        w_copy(j, j % 3).wait()

        @pl.when(j == 2)
        def _():
            w_copy(3, 0).start()
            start(gu_copies(0, 0))

        @pl.when(j == 3)
        def _():
            d_copy(0, 0).start()
            d_copy(1, 1).start()
        i = j - 2

        def jobs():
            perms = _mix([wperm_job('v', i * 16, a) for a in range(16)], [wperm_job('q', 16 + i * 8, a) for a in range(8)])
            extra = _mix([t_job(i * 32, a) for a in range(8)]
                         + [mzero_job(jnp.minimum(i * 25 + a, NP - 1)) for a in range(25)],
                         [zero_job(jnp.minimum(i * 25 + a, NP - 1)) for a in range(25)])
            return _mix(perms[:-4], extra) + perms[-4:]
        block(lambda: k_tasks(j % 3, j * 2, range(16)), jobs, 'k', 2)
        return c
    lax.fori_loop(2, 4, k_body, 0)
    start(gu_copies(1, 1))

    def q_body(i, c):
        def jobs():
            extra = ([bv_job(i, g, h) for g in range(4) for h in range(2)]
                     + [t_job(64 + 48 * i, a) for a in range(12)])
            return _mix([kperm_job(i, a) for a in range(16)], extra)
        block(lambda: q_tasks(i * 2), jobs, 'q', 2)
        return c
    lax.fori_loop(0, 4, q_body, 0)

    wait(gu_copies(0, 0))
    d_copy(0, 0).wait()

    def v_slot(s, mp):
        def jobs():
            return _mix(vcomb_jobs(1 - mp, jnp.maximum(s - 1, 0)), b_jobs(0, s) + bd_jobs(0, s)[:2])
        block(lambda: mm1_tasks(mp, s, 1), jobs, 'v', 3)

    def v_body(it, c):
        v_slot(2 * it, 0)
        v_slot(2 * it + 1, 1)
        return c
    lax.fori_loop(0, 2, v_body, 0)

    wait(gu_copies(1, 1))
    start(gu_copies(2, 0))
    block(lambda: mm1_tasks(0, 0, 0), lambda: _mix(vcomb_jobs(1, 3), b_jobs(1, 0) + bd_jobs(0, 0)[2:] + bd_jobs(0, 1)[2:]), 'f0', 3)
    block(lambda: mm1_tasks(1, 1, 0),
          lambda: _mix(_mix(comb_jobs(0), b_jobs(1, 1) + bd_jobs(0, 2)[2:] + bd_jobs(0, 3)[2:]), attn_quad(26, True)), 'f1', 3)

    def slot(t, mp):
        j = t // 4
        s = t % 4
        par = j % 2
        if mp == 0:
            @pl.when(jnp.logical_and(s == 0, j > 0))
            def _():
                wait(gu_copies(jnp.minimum(j + 1, NCH - 1), 1 - par))

                @pl.when(j + 2 < NCH)
                def _():
                    start(gu_copies(j + 2, par))

                @pl.when(j + 2 == NCH)
                def _():
                    start(wo_copies())

            @pl.when(jnp.logical_and(s == 2, j + 1 < NCH))
            def _():
                d_copy(j + 1, 1 - par).wait()

                @pl.when(j + 2 < NCH)
                def _():
                    d_copy(j + 2, par).start()
        jd = (t + 2) // 4
        kd = (t + 2) % 4
        u = t - 2

        def jobs():
            base = _mix(comb_jobs(1 - mp), b_jobs(1 - par, s) + bd_jobs(jd % 2, kd))
            att = attn_quad(u)
            n0 = max(1, len(base) // 10)
            return base[:n0] + _mix(base[n0:-n0], att) + base[-n0:]
        block(lambda: mm1_tasks(mp, s, par) + mm2_tasks(mp, (t - 2) % 4, ((t - 2) // 4) % 2), jobs,
              'slot%d' % mp, 3)

    def steady(it, c):
        slot(2 * it + 2, 0)
        slot(2 * it + 3, 1)
        return c
    lax.fori_loop(0, (NT - 2) // 2, steady, 0)

    block(lambda: mm2_tasks(0, 2, 0), lambda: comb_jobs(1), 'e0')
    block(lambda: mm2_tasks(1, 3, 0), lambda: _mix(oc_jobs(0), attn_quad(27, True)), 'e1')
    block(lambda: wo_tasks(0),
          lambda: _mix(oc_jobs(1), _flat([attn_quad(n, True) for n in [28, 29]])), 'wo')
    for i in range(1, 4):
        if i == 3:
            wait([out_copy(0, a) for a in range(4)])
        block(lambda i=i: wo_tasks(i),
              lambda i=i: _mix(final_jobs(i - 1) + (oc_jobs(i + 1) if i < 3 else []),
                                _flat([attn_quad(n, True) for n in ([30, 31] if i == 1 else [])])), 'wo')
        start([out_copy(i - 1, a) for a in range(4)])
    wait([out_copy(1, a) for a in range(4)])
    for h in range(2):
        block(nothing, lambda h=h: [final_job(3, g, n) for g in range(4 * h, 4 * h + 4) for n in range(2)], 'e3')
        start([last_copy(a, h) for a in range(4)])
    wait([out_copy(2, a) for a in range(4)])
    wait([last_copy(a, h) for h in range(2) for a in range(4)])


@jax.jit
def pallas_parallel_sum__sliding_local_dilated__glu_gated_bilinear__prompt_kernel(
    A_x: jax.Array,
    A_wqkv: jax.Array,
    A_wo: jax.Array,
    B_x: jax.Array,
    B_w_gate: jax.Array,
    B_w_up: jax.Array,
    B_w_down: jax.Array,
):
    del B_x
    x = A_x.reshape(S, D)
    hbm = pl.BlockSpec(memory_space=pl.ANY)
    dma = pltpu.SemaphoreType.DMA
    out = pl.pallas_call(
        _kernel,
        grid=(1,),
        in_specs=[pl.BlockSpec(memory_space=pltpu.SMEM)] + [hbm] * 6,
        out_specs=hbm,
        out_shape=jax.ShapeDtypeStruct((S, D), bf),
        scratch_shapes=[
            pltpu.VMEM((S, D), bf),
            pltpu.VMEM((S // 2, D), u32),
            pltpu.VMEM((NP, HB // 2, KB), u32),
            pltpu.VMEM((3, D, QW), bf),
            pltpu.VMEM((D, D), bf),
            pltpu.VMEM((D // 2, D), u32),
            pltpu.VMEM((D // 2, D), u32),
            pltpu.VMEM((8, S // 2 + PADW, 128), u32),
            pltpu.VMEM((8, S // 2 + PADW, 128), u32),
            pltpu.VMEM((8, S + PADR + 8, 128), f32),
            pltpu.VMEM((8, S + PADR + 8, 128), f32),
            pltpu.VMEM((2, D, TF), bf),
            pltpu.VMEM((2, D, TF), bf),
            pltpu.VMEM((2, TF, D), bf),
            pltpu.VMEM((2, NP, KB // 2, 2 * TB), u32),
            pltpu.VMEM((2, NP, TB // 2, KB), u32),
            pltpu.VMEM((2, NP, 2, RS + MPAD, 128), f32),
            pltpu.VMEM((2, NP, RS // 2, TB), u32),
            pltpu.VMEM((4, 16, 24, 128), f32),
            pltpu.VMEM((4, 8, 24, 128), f32),
            pltpu.VMEM((NP, 2, HB + MPAD, 128), f32),
            dma((8,)), dma((3,)), dma((1,)), dma((2,)), dma((2,)), dma((2,)), dma((16,)),
        ],
        compiler_params=pltpu.CompilerParams(
            dimension_semantics=("arbitrary",), vmem_limit_bytes=127 * 1024 * 1024,
            disable_bounds_checks=True),
        name="fused_attn_ffn",
    )(jnp.ones((1,), jnp.int32), x, A_wqkv, A_wo, B_w_gate, B_w_up, B_w_down)
    return out.reshape(1, S, D)
```

```python
import jax
import jax.numpy as jnp
from jax import lax
from jax.experimental import pallas as pl
from jax.experimental.pallas import tpu as pltpu

bf = jnp.bfloat16
f32 = jnp.float32
u32 = jnp.uint32

S, D, F = 2048, 1024, 3584
WIN = 8
NP = 49
HB = S // 4
KB = D // 4
TF = 512
TB = TF // 4
NCH = F // TF
RS = 128
NSUB = HB // RS
NT = NCH * NSUB
MPAD = 8
PADW = 8
PADR = 16
QW = 256
EPS = 1e-5
C2 = float(32 ** -0.5 * 1.4426950408889634)

A_T = [[(1, (0, 0)), (1, (1, 1))], [(1, (1, 0)), (1, (1, 1))], [(1, (0, 0))], [(1, (1, 1))],
       [(1, (0, 0)), (1, (0, 1))], [(1, (1, 0)), (-1, (0, 0))], [(1, (0, 1)), (-1, (1, 1))]]
B_T = [[(1, (0, 0)), (1, (1, 1))], [(1, (0, 0))], [(1, (0, 1)), (-1, (1, 1))], [(1, (1, 0)), (-1, (0, 0))],
       [(1, (1, 1))], [(1, (0, 0)), (1, (0, 1))], [(1, (1, 0)), (1, (1, 1))]]
C_T = {(0, 0): [(1, 0), (1, 3), (-1, 4), (1, 6)], (0, 1): [(1, 2), (1, 4)],
       (1, 0): [(1, 1), (1, 3)], (1, 1): [(1, 0), (-1, 1), (1, 2), (1, 5)]}
POS = ((0, 0), (0, 1), (1, 0), (1, 1))


def _comb(terms):
    acc = None
    for s, v in terms:
        if acc is None:
            acc = v if s > 0 else -v
        else:
            acc = acc + v if s > 0 else acc - v
    return acc


def _dot(a, b):
    return jnp.dot(a, b, preferred_element_type=f32)


def _pk(v):
    return pltpu.bitcast(v.astype(bf), u32)


def _up(w):
    return pltpu.bitcast(w, bf)


def _unpk(w):
    return pltpu.bitcast(w, bf).astype(f32)


def _as_f32(w):
    return lax.bitcast_convert_type(w, f32)


def _as_u32(v):
    return lax.bitcast_convert_type(v, u32)


def _mult(x, m):
    return x if isinstance(x, int) else pl.multiple_of(x, m)


def _opcomb(load, table, I, emit, raw):
    sub = {(r, c): _comb([(s, load(q[0] * 2 + r, q[1] * 2 + c)) for s, q in table[I]])
           for r in range(2) for c in range(2)}
    for J, t2 in enumerate(table):
        if raw is not None and len(table[I]) == 1 and len(t2) == 1:
            qo, qi = table[I][0][1], t2[0][1]
            emit(I * 7 + J, raw(qo[0] * 2 + qi[0], qo[1] * 2 + qi[1]))
        else:
            emit(I * 7 + J, _pk(_comb([(s, sub[q]) for s, q in t2])))


def _opcomb_job(load, table, emit, raw=None):
    return [(lambda I=I: _opcomb(load, table, I, emit, raw)) for I in range(7)]


def _outpos(load, pos):
    inner = [_comb([(s, load(I * 7 + J)) for s, J in C_T[pos]]) for I in range(7)]
    return {q: _comb([(s, inner[I]) for s, I in terms]) for q, terms in C_T.items()}


def _perm8(v):
    lane = lax.broadcasted_iota(jnp.int32, v[0].shape, 1)
    v = list(v)
    for cb, lb in ((2, 4), (1, 3), (0, 2)):
        sh = 1 << lb
        hi = (lane & sh) != 0
        out = [None] * 8
        for c in range(8):
            if c & (1 << cb):
                continue
            x, y = v[c], v[c | (1 << cb)]
            out[c] = jnp.where(hi, pltpu.roll(y, sh, 1), x)
            out[c | (1 << cb)] = jnp.where(hi, y, pltpu.roll(x, 128 - sh, 1))
        v = out
    return v


def _sum4(x, lane):
    x = x + jnp.where((lane & 1) != 0, pltpu.roll(x, 1, 1), pltpu.roll(x, 127, 1))
    x = x + jnp.where((lane & 2) != 0, pltpu.roll(x, 2, 1), pltpu.roll(x, 126, 1))
    return x


def _mix(a, b):
    if not b:
        return list(a)
    if not a:
        return list(b)
    out, n, m, k = [], len(a), len(b), 0
    for i, t in enumerate(a):
        out.append(t)
        tgt = (i + 1) * m // n
        while k < tgt:
            out.append(b[k])
            k += 1
    return out


def _flat(jobs, depth=1):
    return [t for j in jobs for t in j]


def _weave(mx, jobs, woff=0):
    vp = _flat(jobs)
    tot = sum(c for _, c in mx)
    n, k, acc = len(vp), 0, 0
    for t, c in mx:
        t()
        acc += c
        tgt = min(n, acc * n // tot + woff)
        while k < tgt:
            vp[k]()
            k += 1
    while k < n:
        vp[k]()
        k += 1


def _kernel(one_ref, x_hbm, wqkv_hbm, wo_hbm, wg_hbm, wu_hbm, wd_hbm, out_hbm,
            xr, xn, T, wst, wqr, wqp, wvp, R, QP, KF, VF, gst, ust, dst, B, Bd, M, H, hst, ost, acc,
            sem_x, sem_w, sem_q, sem_g, sem_u, sem_d, sem_o):

    def block(mx, jobs, name="blk", woff=0):
        with jax.named_scope(name):
            @pl.when(one_ref[0] > 0)
            def _():
                _weave(mx(), jobs(), woff)

    def x_copy(r):
        rows = pl.ds(_mult(r * 256, 256), 256)
        return pltpu.make_async_copy(x_hbm.at[rows, :], xr.at[rows, :], sem_x.at[r])

    def w_copy(j, slot):
        return pltpu.make_async_copy(wqkv_hbm.at[:, pl.ds(_mult(D + j * QW, QW), QW)], wst.at[slot], sem_w.at[slot])

    def wv_copies():
        return (pltpu.make_async_copy(wqkv_hbm.at[:, pl.ds(2 * D, TF)], gst.at[1], sem_g.at[1]),
                pltpu.make_async_copy(wqkv_hbm.at[:, pl.ds(2 * D + TF, TF)], ust.at[1], sem_u.at[1]))

    def wq_copy():
        return pltpu.make_async_copy(wqkv_hbm.at[:, pl.ds(0, D)], wqr, sem_q.at[0])

    def gu_copies(j, par):
        cols = pl.ds(_mult(j * TF, TF), TF)
        return (pltpu.make_async_copy(wg_hbm.at[:, cols], gst.at[par], sem_g.at[par]),
                pltpu.make_async_copy(wu_hbm.at[:, cols], ust.at[par], sem_u.at[par]))

    def d_copy(j, par):
        return pltpu.make_async_copy(wd_hbm.at[pl.ds(_mult(j * TF, TF), TF), :], dst.at[par], sem_d.at[par])

    def wo_copies():
        return [pltpu.make_async_copy(wo_hbm.at[:, pl.ds(q * KB + h * TB, TB)],
                                      (gst, ust)[h].at[1, :, pl.ds(q * TB, TB)], (sem_g, sem_u)[h].at[1])
                for h in range(2) for q in range(4)]

    def out_copy(i, a):
        par = i % 2
        return pltpu.make_async_copy(dst.at[par, pl.ds(a * RS, RS), :],
                                     out_hbm.at[pl.ds(_mult(a * HB + i * RS, RS), RS), :], sem_o.at[par * 4 + a])

    def last_copy(a, h):
        rows = RS // 2
        return pltpu.make_async_copy(dst.at[1, pl.ds(a * RS + h * rows, rows), :],
                                     out_hbm.at[pl.ds(a * HB + 3 * RS + h * rows, rows), :], sem_o.at[8 + h * 4 + a])

    def start(cps):
        for cp in cps:
            cp.start()

    def wait(cps):
        for cp in cps:
            cp.wait()

    def ln_job(g):
        def t():
            v = [xr[pl.ds(g * 16, 16), pl.ds(c * 128, 128)].astype(f32) for c in range(8)]
            a = v[0]
            for c in range(1, 8):
                a = a + v[c]
            mean = jnp.sum(a, axis=1, keepdims=True) * (1.0 / D)
            v = [x - mean for x in v]
            a = v[0] * v[0]
            for c in range(1, 8):
                a = a + v[c] * v[c]
            r = lax.rsqrt(jnp.sum(a, axis=1, keepdims=True) * (1.0 / D) + EPS)
            for c in range(8):
                xn[pl.ds(g * 8, 8), pl.ds(c * 128, 128)] = _pk(v[c] * r)
        return [t]

    def ln_jobs(r):
        return [ln_job(r * 16 + g) for g in range(16)]

    def t_job(wb, pos):
        w0 = _mult(wb, 16) + (pos // 2) * 8
        l0 = (pos % 2) * 128

        def raw(i, j):
            return xn[pl.ds(w0 + i * 256, 8), pl.ds(j * KB + l0, 128)]

        def emit(p, v):
            T[p, pl.ds(w0, 8), pl.ds(l0, 128)] = v
        return _opcomb_job(lambda i, j: _unpk(raw(i, j)), A_T, emit, raw)

    def b_job(par, k, g, half):
        w_ref = (gst, ust)[half]

        def src(i, q):
            return w_ref[par, pl.ds(_mult(k * 64, 64) + (i * KB + g * 16), 16), pl.ds(q * TB, TB)]

        def emit(p, v):
            B[par, p, pl.ds(_mult(k * 32, 32) + g * 8, 8), pl.ds(half * TB, TB)] = v
        return _opcomb_job(lambda i, q: src(i, q).astype(f32), B_T, emit,
                           lambda i, q: pltpu.bitcast(src(i, q), u32))

    def bd_job(par, gb, g, n):
        def src(i, q):
            return dst[par, pl.ds(_mult(gb, 16) + (i * TB + g * 16), 16), pl.ds(q * KB + n * 128, 128)]

        def emit(p, v):
            Bd[par, p, pl.ds(_mult(gb // 2, 8) + g * 8, 8), pl.ds(n * 128, 128)] = v
        return _opcomb_job(lambda i, q: src(i, q).astype(f32), B_T, emit,
                           lambda i, q: pltpu.bitcast(src(i, q), u32))

    def b_jobs(par, k):
        return [b_job(par, k, g, h) for g in range(4) for h in range(2)]

    def bd_jobs(par, k):
        return [bd_job(par, k * 32, g, n) for g in range(2) for n in range(2)]

    def kperm_job(i, a):
        def t():
            r = _perm8([R[c, pl.ds(_mult(i * 256, 256) + a * 16, 16), :] for c in range(8)])
            for c in range(8):
                KF[c, pl.ds(_mult(i * 512, 512) + (PADR + a * 32), 32), :] = _unpk(r[c])
        return [t]

    def wperm_job(which, pb, a, np_=1):
        def t():
            rows = pl.ds(_mult(pb * 32, 64) + a * 32, 32 * np_)
            if which == 'q':
                src = [wqr[rows, pl.ds(c * 128, 128)] for c in range(8)]
            else:
                src = [(gst, ust)[c // 4][1, rows, pl.ds((c % 4) * 128, 128)] for c in range(8)]
            r = _perm8([pltpu.bitcast(v, u32) for v in src])
            for c in range(8):
                (wqp if which == 'q' else wvp)[pl.ds(_mult(pb * 16, 32) + a * 16, 16 * np_), pl.ds(c * 128, 128)] = r[c]
        return [t]

    def bv_job(k, g, half):
        def raw(i, q):
            return wvp[pl.ds(_mult(k * 32, 32) + (i * (KB // 2) + g * 8), 8), pl.ds((2 * q + half) * 128, 128)]

        def emit(p, v):
            B[1, p, pl.ds(_mult(k * 32, 32) + g * 8, 8), pl.ds(half * TB, TB)] = v
        return _opcomb_job(lambda i, q: _unpk(raw(i, q)), B_T, emit, raw)

    def vcomb_job(mp, s, g):
        job = []
        for hf in range(2):
            for pos in POS:
                def t(hf=hf, pos=pos):
                    for n in range(2):
                        o = _outpos(lambda p: M[mp, p, n, pl.ds(g * 16 + hf * 8, 8), :], pos)
                        for q in o:
                            a = q[0] * 2 + pos[0]
                            ch = (q[1] * 2 + pos[1]) * 2 + n
                            VF[ch, pl.ds(_mult(s * RS, RS) + (PADR + a * HB + g * 16 + hf * 8), 8), :] = o[q]
                job.append(t)
        return job

    def vcomb_jobs(mp, s):
        return [vcomb_job(mp, s, g) for g in range(RS // 16)]

    def mzero_job(p):
        def t():
            for c in range(2):
                M[1, p, c, pl.ds(0, RS), :] = jnp.zeros((RS, 128), f32)
        return [t]

    def attn_quad(n, stack=False):
        base = _mult(((n % 8) // 2) * 256 + (n // 8) * 64 + (n % 2) * 32, 32)
        return [attn_job(base, 8 * k, k, stack) for k in range(4)]

    def attn_job(base, off, sl, stack):
        b = base + off
        rbase = _mult(base * 2, 64)
        job = []
        for h in range(2):
            st = {}
            half = lambda v, h=h: _unpk(v)[h * 8:(h + 1) * 8]

            def qk(cs, st=st, half=half, h=h):
                def t():
                    for c in cs:
                        qv = half(QP[c, pl.ds(base + off, 8), :])
                        for w in range(WIN):
                            kv = KF[c, pl.ds(rbase + (2 * off + 8 * h + PADR - 2 * w), 8), :]
                            st[w] = qv * kv if c == 0 else st[w] + qv * kv
                return t

            def sm(st=st, h=h):
                lane = lax.broadcasted_iota(jnp.int32, (8, 128), 1)
                row = lax.broadcasted_iota(jnp.int32, (8, 128), 0) + (b * 2 + h * 8)
                if stack:
                    big = jnp.concatenate([st[w] for w in range(WIN)], axis=0)
                    big = _sum4(big, lax.broadcasted_iota(jnp.int32, (8 * WIN, 128), 1))
                    ls = [big[8 * w:8 * w + 8] for w in range(WIN)]
                else:
                    ls = [_sum4(st[w], lane) for w in range(WIN)]
                ls = [ls[0]] + [jnp.where(row >= 2 * w, ls[w], -1e30) for w in range(1, WIN)]
                m = ls[0]
                for w in range(1, WIN):
                    m = jnp.maximum(m, ls[w])
                e = [jnp.exp2((l - m) * C2) for l in ls]
                den = e[0]
                for w in range(1, WIN):
                    den = den + e[w]
                inv = 1.0 / den
                st['p'] = [x * inv for x in e]

            def pv(cs, st=st, half=half, h=h):
                def t():
                    for c in cs:
                        o = None
                        for w in range(WIN):
                            a = st['p'][w] * VF[c, pl.ds(rbase + (2 * off + 8 * h + PADR - 2 * w), 8), :]
                            o = a if o is None else o + a
                        ost[sl, c, pl.ds(h * 8, 8), :] = o
                return t
            job += [qk((0, 1, 2, 3)), qk((4, 5, 6, 7)), sm, pv((0, 1, 2, 3)), pv((4, 5, 6, 7))]

        def fin():
            r = _perm8([_pk(ost[sl, c, pl.ds(0, 16), :]) for c in range(8)])
            for c in range(8):
                xn[pl.ds(_mult(b, 8), 8), pl.ds(c * 128, 128)] = r[c]
        return job + [fin]

    def comb_job(mp, g):
        sl = g % 4
        job = []
        for hf in range(2):
            for pos in POS:
                def t(hf=hf, pos=pos):
                    r = pl.ds(g * 16 + hf * 8, 8)
                    gg = _outpos(lambda p: M[mp, p, 0, r, :], pos)
                    uu = _outpos(lambda p: M[mp, p, 1, r, :], pos)
                    for q in gg:
                        hst[sl, (q[0] * 2 + pos[0]) * 4 + q[1] * 2 + pos[1], pl.ds(hf * 8, 8), :] = gg[q] * uu[q]
                job.append(t)

        def emit(p, v):
            H[mp, p, pl.ds(g * 8, 8), :] = v
        return job + _opcomb_job(lambda i, j: hst[sl, i * 4 + j, pl.ds(0, 16), :], A_T, emit)

    def comb_jobs(mp):
        return [comb_job(mp, g) for g in range(RS // 16)]

    def zero_job(p):
        def t():
            for c in range(2):
                acc[p, c, pl.ds(0, HB), :] = jnp.zeros((HB, 128), f32)
        return [t]

    def oc_job(i, g, n):
        def load(a, kb):
            return _unpk(xn[pl.ds(_mult(i * 64, 64) + (a * 256 + g * 8), 8), pl.ds(kb * KB + n * 128, 128)])

        def one(I):
            sub = {(r, c): _comb([(sg, load(q[0] * 2 + r, q[1] * 2 + c)) for sg, q in A_T[I]])
                   for r in range(2) for c in range(2)}
            for J, t2 in enumerate(A_T):
                M[i % 2, I * 7 + J, n, pl.ds(g * 16, 16), :] = _comb([(sg, sub[q]) for sg, q in t2])
        return [(lambda I=I: one(I)) for I in range(7)]

    def oc_jobs(i):
        return [oc_job(i, g, n) for g in range(RS // 16) for n in range(2)]

    def final_job(i, g, n):
        job = []
        par = i % 2
        for pos in POS:
            def t(pos=pos):
                r0 = _mult(i * RS, RS) + g * 16
                o = [_outpos(lambda p: acc[p, n, pl.ds(r0 + hf * 8, 8), :], pos) for hf in range(2)]
                for q in o[0]:
                    a = q[0] * 2 + pos[0]
                    cols = pl.ds(((q[1] * 2 + pos[1]) * 2 + n) * 128, 128)
                    res = xr[pl.ds(r0 + a * HB, 16), cols].astype(f32) + jnp.concatenate([o[0][q], o[1][q]], axis=0)
                    dst[par, pl.ds(a * RS + g * 16, 16), cols] = res.astype(bf)
            job.append(t)
        return job

    def final_jobs(i):
        return [final_job(i, g, n) for g in range(RS // 16) for n in range(2)]

    def k_tasks(slot, cbase, pieces):
        out = []
        for r in pieces:
            for ct in range(QW // 128):
                def t(r=r, ct=ct):
                    res = _dot(_up(xn[pl.ds(_mult(r * 64, 64), 64), :]), wst[slot, :, pl.ds(ct * 128, 128)])
                    for k in range(8):
                        R[cbase + ct, pl.ds(_mult(r * 64 + k * 8, 8), 8), :] = _pk(res[k * 16:(k + 1) * 16])
                out.append((t, 256))
        return out

    def q_tasks(cbase):
        out = []
        for r in range(16):
            for ct in range(QW // 128):
                def t(r=r, ct=ct):
                    res = _dot(_up(xn[pl.ds(r * 64, 64), :]),
                               _up(wqp[:, pl.ds(_mult((cbase + ct) * 128, 128), 128)]))
                    for k in range(8):
                        QP[cbase + ct, pl.ds(r * 64 + k * 8, 8), :] = _pk(res[k * 16:(k + 1) * 16])
                out.append((t, 256))
        return out

    def mm1_tasks(mp, s, par):
        out = []
        for p in range(NP):
            for c in range(2):
                def t(p=p, c=c):
                    M[mp, p, c, pl.ds(0, RS), :] = _dot(
                        _up(T[p, pl.ds(_mult(s * (RS // 2), RS // 2), RS // 2), :]),
                        _up(B[par, p, :, pl.ds(c * 128, 128)]))
                out.append((t, 64))
        return out

    def mm2_tasks(mp, s, par):
        out = []
        for p in range(NP):
            def t(p=p):
                r = _dot(_up(H[mp, p]), _up(Bd[par, p]))
                for c in range(2):
                    acc[p, c, pl.ds(_mult(s * RS, RS), RS), :] += r[:, c * 128:(c + 1) * 128]
            out.append((t, 64))
        return out

    def wo_tasks(i):
        out = []
        for p in range(NP):
            for c in range(2):
                def t(p=p, c=c):
                    lhs = jnp.concatenate([M[i % 2, p, n, pl.ds(0, RS), :] for n in range(2)], axis=1)
                    acc[p, c, pl.ds(_mult(i * RS, RS), RS), :] += lax.dot_general(
                        lhs, _up(B[1, p, :, pl.ds(c * 128, 128)]), (((1,), (0,)), ((), ())),
                        preferred_element_type=f32)
                out.append((t, 64))
        return out

    nothing = lambda: [(lambda: None, 1)]

    x_copy(0).start()
    w_copy(0, 0).start()
    for c in range(8):
        KF[c, pl.ds(0, PADR), :] = jnp.zeros((PADR, 128), f32)
        VF[c, pl.ds(0, PADR), :] = jnp.zeros((PADR, 128), f32)
    x_copy(0).wait()
    w_copy(1, 1).start()
    x_copy(1).start()
    block(nothing, lambda: ln_jobs(0), 'ln0')
    w_copy(0, 0).wait()

    def k01(pieces):
        rp = [2 * r + h for r in pieces for h in range(2)]
        return k_tasks(0, 0, rp) + k_tasks(1, 2, rp)

    block(lambda: k_tasks(0, 0, (0, 1)), lambda: [], 'p0')
    w_copy(1, 1).wait()
    x_copy(2).start()
    x_copy(1).wait()
    block(lambda: k_tasks(1, 2, (0, 1)), lambda: ln_jobs(1), 'p0')
    x_copy(3).start()
    x_copy(4).start()
    x_copy(2).wait()
    block(lambda: k01((1,)), lambda: ln_jobs(2), 'p0')
    x_copy(5).start()
    x_copy(6).start()
    x_copy(3).wait()
    x_copy(4).wait()
    block(lambda: k01((2,)), lambda: ln_jobs(3) + ln_jobs(4), 'p0')
    x_copy(7).start()
    wq_copy().start()
    x_copy(5).wait()
    x_copy(6).wait()
    block(lambda: k01((3, 4)), lambda: ln_jobs(5) + ln_jobs(6), 'p0')
    w_copy(2, 2).start()
    start(wv_copies())
    x_copy(7).wait()
    block(lambda: k01((5, 6)), lambda: ln_jobs(7), 'p0')
    wq_copy().wait()
    block(lambda: k01((7,)), lambda: [wperm_job('q', 0, a, 2) for a in range(0, 8, 2)], 'p0')

    wait(wv_copies())

    def k_body(j, c):
        w_copy(j, j % 3).wait()

        @pl.when(j == 2)
        def _():
            w_copy(3, 0).start()
            start(gu_copies(0, 0))

        @pl.when(j == 3)
        def _():
            d_copy(0, 0).start()
            d_copy(1, 1).start()
        i = j - 2

        def jobs():
            perms = _mix([wperm_job('v', i * 16, a) for a in range(16)], [wperm_job('q', 8 + 12 * i, a, 2) for a in range(0, 12, 2)])
            extra = _mix([t_job(i * 32, a) for a in range(8)]
                         + [mzero_job(jnp.minimum(i * 25 + a, NP - 1)) for a in range(25)],
                         [zero_job(jnp.minimum(i * 25 + a, NP - 1)) for a in range(25)])
            return _mix(perms[:-4], extra) + perms[-4:]
        block(lambda: k_tasks(j % 3, j * 2, range(16)), jobs, 'k', 2)
        return c
    lax.fori_loop(2, 4, k_body, 0)
    start(gu_copies(1, 1))

    def q_body(i, c):
        def jobs():
            extra = ([bv_job(i, g, h) for g in range(4) for h in range(2)]
                     + [t_job(64 + 48 * i, a) for a in range(12)])
            return _mix([kperm_job(i, a) for a in range(16)], extra)
        block(lambda: q_tasks(i * 2), jobs, 'q', 2)
        return c
    lax.fori_loop(0, 4, q_body, 0)

    wait(gu_copies(0, 0))
    d_copy(0, 0).wait()

    def v_slot(s, mp):
        def jobs():
            return _mix(vcomb_jobs(1 - mp, jnp.maximum(s - 1, 0)), b_jobs(0, s) + bd_jobs(0, s)[:2])
        block(lambda: mm1_tasks(mp, s, 1), jobs, 'v', 3)

    def v_body(it, c):
        v_slot(2 * it, 0)
        v_slot(2 * it + 1, 1)
        return c
    lax.fori_loop(0, 2, v_body, 0)

    wait(gu_copies(1, 1))
    start(gu_copies(2, 0))
    block(lambda: mm1_tasks(0, 0, 0), lambda: _mix(vcomb_jobs(1, 3), b_jobs(1, 0) + bd_jobs(0, 0)[2:] + bd_jobs(0, 1)[2:]), 'f0', 3)
    block(lambda: mm1_tasks(1, 1, 0),
          lambda: _mix(_mix(comb_jobs(0), b_jobs(1, 1) + bd_jobs(0, 2)[2:] + bd_jobs(0, 3)[2:]), attn_quad(26, True)), 'f1', 3)

    def slot(t, mp):
        j = t // 4
        s = t % 4
        par = j % 2
        if mp == 0:
            @pl.when(jnp.logical_and(s == 0, j > 0))
            def _():
                wait(gu_copies(jnp.minimum(j + 1, NCH - 1), 1 - par))

                @pl.when(j + 2 < NCH)
                def _():
                    start(gu_copies(j + 2, par))

                @pl.when(j + 2 == NCH)
                def _():
                    start(wo_copies())

            @pl.when(jnp.logical_and(s == 2, j + 1 < NCH))
            def _():
                d_copy(j + 1, 1 - par).wait()

                @pl.when(j + 2 < NCH)
                def _():
                    d_copy(j + 2, par).start()
        jd = (t + 2) // 4
        kd = (t + 2) % 4
        u = t - 2

        def jobs():
            base = _mix(comb_jobs(1 - mp), b_jobs(1 - par, s) + bd_jobs(jd % 2, kd))
            att = attn_quad(u)
            n0 = max(1, len(base) // 10)
            return base[:n0] + _mix(base[n0:-n0], att) + base[-n0:]
        block(lambda: mm1_tasks(mp, s, par) + mm2_tasks(mp, (t - 2) % 4, ((t - 2) // 4) % 2), jobs,
              'slot%d' % mp, 3)

    def steady(it, c):
        slot(2 * it + 2, 0)
        slot(2 * it + 3, 1)
        return c
    lax.fori_loop(0, (NT - 2) // 2, steady, 0)

    block(lambda: mm2_tasks(0, 2, 0), lambda: comb_jobs(1), 'e0')
    block(lambda: mm2_tasks(1, 3, 0), lambda: _mix(oc_jobs(0), attn_quad(27, True)), 'e1')
    block(lambda: wo_tasks(0),
          lambda: _mix(oc_jobs(1), _flat([attn_quad(n, True) for n in [28, 29]])), 'wo')
    for i in range(1, 4):
        if i == 3:
            wait([out_copy(0, a) for a in range(4)])
        block(lambda i=i: wo_tasks(i),
              lambda i=i: _mix(final_jobs(i - 1) + (oc_jobs(i + 1) if i < 3 else []),
                                _flat([attn_quad(n, True) for n in ([30, 31] if i == 1 else [])])), 'wo')
        start([out_copy(i - 1, a) for a in range(4)])
    wait([out_copy(1, a) for a in range(4)])
    for h in range(2):
        block(nothing, lambda h=h: [final_job(3, g, n) for g in range(4 * h, 4 * h + 4) for n in range(2)], 'e3')
        start([last_copy(a, h) for a in range(4)])
    wait([out_copy(2, a) for a in range(4)])
    wait([last_copy(a, h) for h in range(2) for a in range(4)])


@jax.jit
def pallas_parallel_sum__sliding_local_dilated__glu_gated_bilinear__prompt_kernel(
    A_x: jax.Array,
    A_wqkv: jax.Array,
    A_wo: jax.Array,
    B_x: jax.Array,
    B_w_gate: jax.Array,
    B_w_up: jax.Array,
    B_w_down: jax.Array,
):
    del B_x
    x = A_x.reshape(S, D)
    hbm = pl.BlockSpec(memory_space=pl.ANY)
    dma = pltpu.SemaphoreType.DMA
    out = pl.pallas_call(
        _kernel,
        grid=(1,),
        in_specs=[pl.BlockSpec(memory_space=pltpu.SMEM)] + [hbm] * 6,
        out_specs=hbm,
        out_shape=jax.ShapeDtypeStruct((S, D), bf),
        scratch_shapes=[
            pltpu.VMEM((S, D), bf),
            pltpu.VMEM((S // 2, D), u32),
            pltpu.VMEM((NP, HB // 2, KB), u32),
            pltpu.VMEM((3, D, QW), bf),
            pltpu.VMEM((D, D), bf),
            pltpu.VMEM((D // 2, D), u32),
            pltpu.VMEM((D // 2, D), u32),
            pltpu.VMEM((8, S // 2 + PADW, 128), u32),
            pltpu.VMEM((8, S // 2 + PADW, 128), u32),
            pltpu.VMEM((8, S + PADR + 8, 128), f32),
            pltpu.VMEM((8, S + PADR + 8, 128), f32),
            pltpu.VMEM((2, D, TF), bf),
            pltpu.VMEM((2, D, TF), bf),
            pltpu.VMEM((2, TF, D), bf),
            pltpu.VMEM((2, NP, KB // 2, 2 * TB), u32),
            pltpu.VMEM((2, NP, TB // 2, KB), u32),
            pltpu.VMEM((2, NP, 2, RS + MPAD, 128), f32),
            pltpu.VMEM((2, NP, RS // 2, TB), u32),
            pltpu.VMEM((4, 16, 24, 128), f32),
            pltpu.VMEM((4, 8, 24, 128), f32),
            pltpu.VMEM((NP, 2, HB + MPAD, 128), f32),
            dma((8,)), dma((3,)), dma((1,)), dma((2,)), dma((2,)), dma((2,)), dma((16,)),
        ],
        compiler_params=pltpu.CompilerParams(
            dimension_semantics=("arbitrary",), vmem_limit_bytes=127 * 1024 * 1024,
            disable_bounds_checks=True),
        name="fused_attn_ffn",
    )(jnp.ones((1,), jnp.int32), x, A_wqkv, A_wo, B_w_gate, B_w_up, B_w_down)
    return out.reshape(1, S, D)
```

```python
import jax
import jax.numpy as jnp
from jax import lax
from jax.experimental import pallas as pl
from jax.experimental.pallas import tpu as pltpu

bf = jnp.bfloat16
f32 = jnp.float32
u32 = jnp.uint32

S, D, F = 2048, 1024, 3584
WIN = 8
NP = 49
HB = S // 4
KB = D // 4
TF = 512
TB = TF // 4
NCH = F // TF
RS = 128
NSUB = HB // RS
NT = NCH * NSUB
MPAD = 8
PADW = 8
PADR = 16
QW = 256
EPS = 1e-5
C2 = float(32 ** -0.5 * 1.4426950408889634)

A_T = [[(1, (0, 0)), (1, (1, 1))], [(1, (1, 0)), (1, (1, 1))], [(1, (0, 0))], [(1, (1, 1))],
       [(1, (0, 0)), (1, (0, 1))], [(1, (1, 0)), (-1, (0, 0))], [(1, (0, 1)), (-1, (1, 1))]]
B_T = [[(1, (0, 0)), (1, (1, 1))], [(1, (0, 0))], [(1, (0, 1)), (-1, (1, 1))], [(1, (1, 0)), (-1, (0, 0))],
       [(1, (1, 1))], [(1, (0, 0)), (1, (0, 1))], [(1, (1, 0)), (1, (1, 1))]]
C_T = {(0, 0): [(1, 0), (1, 3), (-1, 4), (1, 6)], (0, 1): [(1, 2), (1, 4)],
       (1, 0): [(1, 1), (1, 3)], (1, 1): [(1, 0), (-1, 1), (1, 2), (1, 5)]}
POS = ((0, 0), (0, 1), (1, 0), (1, 1))


def _comb(terms):
    acc = None
    for s, v in terms:
        if acc is None:
            acc = v if s > 0 else -v
        else:
            acc = acc + v if s > 0 else acc - v
    return acc


def _dot(a, b):
    return jnp.dot(a, b, preferred_element_type=f32)


def _pk(v):
    return pltpu.bitcast(v.astype(bf), u32)


def _up(w):
    return pltpu.bitcast(w, bf)


def _unpk(w):
    return pltpu.bitcast(w, bf).astype(f32)


def _as_f32(w):
    return lax.bitcast_convert_type(w, f32)


def _as_u32(v):
    return lax.bitcast_convert_type(v, u32)


def _mult(x, m):
    return x if isinstance(x, int) else pl.multiple_of(x, m)


def _opcomb(load, table, I, emit, raw):
    sub = {(r, c): _comb([(s, load(q[0] * 2 + r, q[1] * 2 + c)) for s, q in table[I]])
           for r in range(2) for c in range(2)}
    for J, t2 in enumerate(table):
        if raw is not None and len(table[I]) == 1 and len(t2) == 1:
            qo, qi = table[I][0][1], t2[0][1]
            emit(I * 7 + J, raw(qo[0] * 2 + qi[0], qo[1] * 2 + qi[1]))
        else:
            emit(I * 7 + J, _pk(_comb([(s, sub[q]) for s, q in t2])))


def _opcomb_job(load, table, emit, raw=None):
    return [(lambda I=I: _opcomb(load, table, I, emit, raw)) for I in range(7)]


def _outpos(load, pos):
    inner = [_comb([(s, load(I * 7 + J)) for s, J in C_T[pos]]) for I in range(7)]
    return {q: _comb([(s, inner[I]) for s, I in terms]) for q, terms in C_T.items()}


def _perm8(v):
    lane = lax.broadcasted_iota(jnp.int32, v[0].shape, 1)
    v = list(v)
    for cb, lb in ((2, 4), (1, 3), (0, 2)):
        sh = 1 << lb
        hi = (lane & sh) != 0
        out = [None] * 8
        for c in range(8):
            if c & (1 << cb):
                continue
            x, y = v[c], v[c | (1 << cb)]
            out[c] = jnp.where(hi, pltpu.roll(y, sh, 1), x)
            out[c | (1 << cb)] = jnp.where(hi, y, pltpu.roll(x, 128 - sh, 1))
        v = out
    return v


def _sum4(x, lane):
    x = x + jnp.where((lane & 1) != 0, pltpu.roll(x, 1, 1), pltpu.roll(x, 127, 1))
    x = x + jnp.where((lane & 2) != 0, pltpu.roll(x, 2, 1), pltpu.roll(x, 126, 1))
    return x


def _mix(a, b):
    if not b:
        return list(a)
    if not a:
        return list(b)
    out, n, m, k = [], len(a), len(b), 0
    for i, t in enumerate(a):
        out.append(t)
        tgt = (i + 1) * m // n
        while k < tgt:
            out.append(b[k])
            k += 1
    return out


def _flat(jobs, depth=1):
    return [t for j in jobs for t in j]


def _weave(mx, jobs, woff=0):
    vp = _flat(jobs)
    tot = sum(c for _, c in mx)
    n, k, acc = len(vp), 0, 0
    for t, c in mx:
        t()
        acc += c
        tgt = min(n, acc * n // tot + woff)
        while k < tgt:
            vp[k]()
            k += 1
    while k < n:
        vp[k]()
        k += 1


def _kernel(one_ref, x_hbm, wqkv_hbm, wo_hbm, wg_hbm, wu_hbm, wd_hbm, out_hbm,
            xr, xn, T, wst, wqr, wqp, wvp, R, QP, KF, VF, gst, ust, dst, B, Bd, M, H, hst, ost, acc,
            sem_x, sem_w, sem_q, sem_g, sem_u, sem_d, sem_o):

    def block(mx, jobs, name="blk", woff=0):
        with jax.named_scope(name):
            @pl.when(one_ref[0] > 0)
            def _():
                _weave(mx(), jobs(), woff)

    def x_copy(r):
        rows = pl.ds(_mult(r * 256, 256), 256)
        return pltpu.make_async_copy(x_hbm.at[rows, :], xr.at[rows, :], sem_x.at[r])

    def w_copy(j, slot):
        return pltpu.make_async_copy(wqkv_hbm.at[:, pl.ds(_mult(D + j * QW, QW), QW)], wst.at[slot], sem_w.at[slot])

    def wv_copies():
        return (pltpu.make_async_copy(wqkv_hbm.at[:, pl.ds(2 * D, TF)], gst.at[1], sem_g.at[1]),
                pltpu.make_async_copy(wqkv_hbm.at[:, pl.ds(2 * D + TF, TF)], ust.at[1], sem_u.at[1]))

    def wq_copy():
        return pltpu.make_async_copy(wqkv_hbm.at[:, pl.ds(0, D)], wqr, sem_q.at[0])

    def gu_copies(j, par):
        cols = pl.ds(_mult(j * TF, TF), TF)
        return (pltpu.make_async_copy(wg_hbm.at[:, cols], gst.at[par], sem_g.at[par]),
                pltpu.make_async_copy(wu_hbm.at[:, cols], ust.at[par], sem_u.at[par]))

    def d_copy(j, par):
        return pltpu.make_async_copy(wd_hbm.at[pl.ds(_mult(j * TF, TF), TF), :], dst.at[par], sem_d.at[par])

    def wo_copies():
        return [pltpu.make_async_copy(wo_hbm.at[:, pl.ds(q * KB + h * TB, TB)],
                                      (gst, ust)[h].at[1, :, pl.ds(q * TB, TB)], (sem_g, sem_u)[h].at[1])
                for h in range(2) for q in range(4)]

    def out_copy(i, a):
        par = i % 2
        return pltpu.make_async_copy(dst.at[par, pl.ds(a * RS, RS), :],
                                     out_hbm.at[pl.ds(_mult(a * HB + i * RS, RS), RS), :], sem_o.at[par * 4 + a])

    def last_copy(a, h):
        rows = RS // 2
        return pltpu.make_async_copy(dst.at[1, pl.ds(a * RS + h * rows, rows), :],
                                     out_hbm.at[pl.ds(a * HB + 3 * RS + h * rows, rows), :], sem_o.at[8 + h * 4 + a])

    def start(cps):
        for cp in cps:
            cp.start()

    def wait(cps):
        for cp in cps:
            cp.wait()

    def ln_job(g):
        def t():
            v = [xr[pl.ds(g * 16, 16), pl.ds(c * 128, 128)].astype(f32) for c in range(8)]
            a = v[0]
            for c in range(1, 8):
                a = a + v[c]
            mean = jnp.sum(a, axis=1, keepdims=True) * (1.0 / D)
            v = [x - mean for x in v]
            a = v[0] * v[0]
            for c in range(1, 8):
                a = a + v[c] * v[c]
            r = lax.rsqrt(jnp.sum(a, axis=1, keepdims=True) * (1.0 / D) + EPS)
            for c in range(8):
                xn[pl.ds(g * 8, 8), pl.ds(c * 128, 128)] = _pk(v[c] * r)
        return [t]

    def ln_jobs(r):
        return [ln_job(r * 16 + g) for g in range(16)]

    def t_job(wb, pos):
        w0 = _mult(wb, 16) + (pos // 2) * 8
        l0 = (pos % 2) * 128

        def raw(i, j):
            return xn[pl.ds(w0 + i * 256, 8), pl.ds(j * KB + l0, 128)]

        def emit(p, v):
            T[p, pl.ds(w0, 8), pl.ds(l0, 128)] = v
        return _opcomb_job(lambda i, j: _unpk(raw(i, j)), A_T, emit, raw)

    def b_job(par, k, g, half):
        w_ref = (gst, ust)[half]

        def src(i, q):
            return w_ref[par, pl.ds(_mult(k * 64, 64) + (i * KB + g * 16), 16), pl.ds(q * TB, TB)]

        def emit(p, v):
            B[par, p, pl.ds(_mult(k * 32, 32) + g * 8, 8), pl.ds(half * TB, TB)] = v
        return _opcomb_job(lambda i, q: src(i, q).astype(f32), B_T, emit,
                           lambda i, q: pltpu.bitcast(src(i, q), u32))

    def bd_job(par, gb, g, n):
        def src(i, q):
            return dst[par, pl.ds(_mult(gb, 16) + (i * TB + g * 16), 16), pl.ds(q * KB + n * 128, 128)]

        def emit(p, v):
            Bd[par, p, pl.ds(_mult(gb // 2, 8) + g * 8, 8), pl.ds(n * 128, 128)] = v
        return _opcomb_job(lambda i, q: src(i, q).astype(f32), B_T, emit,
                           lambda i, q: pltpu.bitcast(src(i, q), u32))

    def b_jobs(par, k):
        return [b_job(par, k, g, h) for g in range(4) for h in range(2)]

    def bd_jobs(par, k):
        return [bd_job(par, k * 32, g, n) for g in range(2) for n in range(2)]

    def kperm_job(i, a):
        def t():
            r = _perm8([R[c, pl.ds(_mult(i * 256, 256) + a * 16, 16), :] for c in range(8)])
            for c in range(8):
                KF[c, pl.ds(_mult(i * 512, 512) + (PADR + a * 32), 32), :] = _unpk(r[c])
        return [t]

    def wperm_job(which, pb, a, np_=1):
        def t():
            rows = pl.ds(_mult(pb * 32, 64) + a * 32, 32 * np_)
            if which == 'q':
                src = [wqr[rows, pl.ds(c * 128, 128)] for c in range(8)]
            else:
                src = [(gst, ust)[c // 4][1, rows, pl.ds((c % 4) * 128, 128)] for c in range(8)]
            r = _perm8([pltpu.bitcast(v, u32) for v in src])
            for c in range(8):
                (wqp if which == 'q' else wvp)[pl.ds(_mult(pb * 16, 32) + a * 16, 16 * np_), pl.ds(c * 128, 128)] = r[c]
        return [t]

    def bv_job(k, g, half):
        def raw(i, q):
            return wvp[pl.ds(_mult(k * 32, 32) + (i * (KB // 2) + g * 8), 8), pl.ds((2 * q + half) * 128, 128)]

        def emit(p, v):
            B[1, p, pl.ds(_mult(k * 32, 32) + g * 8, 8), pl.ds(half * TB, TB)] = v
        return _opcomb_job(lambda i, q: _unpk(raw(i, q)), B_T, emit, raw)

    def vcomb_job(mp, s, g):
        job = []
        for hf in range(2):
            for pos in POS:
                def t(hf=hf, pos=pos):
                    for n in range(2):
                        o = _outpos(lambda p: M[mp, p, n, pl.ds(g * 16 + hf * 8, 8), :], pos)
                        for q in o:
                            a = q[0] * 2 + pos[0]
                            ch = (q[1] * 2 + pos[1]) * 2 + n
                            VF[ch, pl.ds(_mult(s * RS, RS) + (PADR + a * HB + g * 16 + hf * 8), 8), :] = o[q]
                job.append(t)
        return job

    def vcomb_jobs(mp, s):
        return [vcomb_job(mp, s, g) for g in range(RS // 16)]

    def mzero_job(p):
        def t():
            for c in range(2):
                M[1, p, c, pl.ds(0, RS), :] = jnp.zeros((RS, 128), f32)
        return [t]

    def attn_quad(n, stack=False):
        base = _mult(((n % 8) // 2) * 256 + (n // 8) * 64 + (n % 2) * 32, 32)
        return [attn_job(base, 8 * k, k, stack) for k in range(4)]

    def attn_job(base, off, sl, stack):
        b = base + off
        rbase = _mult(base * 2, 64)
        job = []
        for h in range(2):
            st = {}
            half = lambda v, h=h: _unpk(v)[h * 8:(h + 1) * 8]

            def qk(cs, st=st, half=half, h=h):
                def t():
                    for c in cs:
                        qv = half(QP[c, pl.ds(base + off, 8), :])
                        for w in range(WIN):
                            kv = KF[c, pl.ds(rbase + (2 * off + 8 * h + PADR - 2 * w), 8), :]
                            st[w] = qv * kv if c == 0 else st[w] + qv * kv
                return t

            def sm(st=st, h=h):
                lane = lax.broadcasted_iota(jnp.int32, (8, 128), 1)
                row = lax.broadcasted_iota(jnp.int32, (8, 128), 0) + (b * 2 + h * 8)
                if stack:
                    big = jnp.concatenate([st[w] for w in range(WIN)], axis=0)
                    big = _sum4(big, lax.broadcasted_iota(jnp.int32, (8 * WIN, 128), 1))
                    ls = [big[8 * w:8 * w + 8] for w in range(WIN)]
                else:
                    ls = [_sum4(st[w], lane) for w in range(WIN)]
                ls = [ls[0]] + [jnp.where(row >= 2 * w, ls[w], -1e30) for w in range(1, WIN)]
                m = ls[0]
                for w in range(1, WIN):
                    m = jnp.maximum(m, ls[w])
                e = [jnp.exp2((l - m) * C2) for l in ls]
                den = e[0]
                for w in range(1, WIN):
                    den = den + e[w]
                inv = 1.0 / den
                st['p'] = [x * inv for x in e]

            def pv(cs, st=st, half=half, h=h):
                def t():
                    for c in cs:
                        o = None
                        for w in range(WIN):
                            a = st['p'][w] * VF[c, pl.ds(rbase + (2 * off + 8 * h + PADR - 2 * w), 8), :]
                            o = a if o is None else o + a
                        ost[sl, c, pl.ds(h * 8, 8), :] = o
                return t
            job += [qk((0, 1, 2, 3)), qk((4, 5, 6, 7)), sm, pv((0, 1, 2, 3)), pv((4, 5, 6, 7))]

        def fin():
            r = _perm8([_pk(ost[sl, c, pl.ds(0, 16), :]) for c in range(8)])
            for c in range(8):
                xn[pl.ds(_mult(b, 8), 8), pl.ds(c * 128, 128)] = r[c]
        return job + [fin]

    def comb_job(mp, g):
        sl = g % 4
        job = []
        for hf in range(2):
            for pos in POS:
                def t(hf=hf, pos=pos):
                    r = pl.ds(g * 16 + hf * 8, 8)
                    gg = _outpos(lambda p: M[mp, p, 0, r, :], pos)
                    uu = _outpos(lambda p: M[mp, p, 1, r, :], pos)
                    for q in gg:
                        hst[sl, (q[0] * 2 + pos[0]) * 4 + q[1] * 2 + pos[1], pl.ds(hf * 8, 8), :] = gg[q] * uu[q]
                job.append(t)

        def emit(p, v):
            H[mp, p, pl.ds(g * 8, 8), :] = v
        return job + _opcomb_job(lambda i, j: hst[sl, i * 4 + j, pl.ds(0, 16), :], A_T, emit)

    def comb_jobs(mp):
        return [comb_job(mp, g) for g in range(RS // 16)]

    def zero_job(p):
        def t():
            for c in range(2):
                acc[p, c, pl.ds(0, HB), :] = jnp.zeros((HB, 128), f32)
        return [t]

    def oc_job(i, g, n):
        def load(a, kb):
            return _unpk(xn[pl.ds(_mult(i * 64, 64) + (a * 256 + g * 8), 8), pl.ds(kb * KB + n * 128, 128)])

        def one(I):
            sub = {(r, c): _comb([(sg, load(q[0] * 2 + r, q[1] * 2 + c)) for sg, q in A_T[I]])
                   for r in range(2) for c in range(2)}
            for J, t2 in enumerate(A_T):
                M[i % 2, I * 7 + J, n, pl.ds(g * 16, 16), :] = _comb([(sg, sub[q]) for sg, q in t2])
        return [(lambda I=I: one(I)) for I in range(7)]

    def oc_jobs(i):
        return [oc_job(i, g, n) for g in range(RS // 16) for n in range(2)]

    def final_job(i, g, n):
        job = []
        par = i % 2
        for pos in POS:
            def t(pos=pos):
                r0 = _mult(i * RS, RS) + g * 16
                o = [_outpos(lambda p: acc[p, n, pl.ds(r0 + hf * 8, 8), :], pos) for hf in range(2)]
                for q in o[0]:
                    a = q[0] * 2 + pos[0]
                    cols = pl.ds(((q[1] * 2 + pos[1]) * 2 + n) * 128, 128)
                    res = xr[pl.ds(r0 + a * HB, 16), cols].astype(f32) + jnp.concatenate([o[0][q], o[1][q]], axis=0)
                    dst[par, pl.ds(a * RS + g * 16, 16), cols] = res.astype(bf)
            job.append(t)
        return job

    def final_jobs(i):
        return [final_job(i, g, n) for g in range(RS // 16) for n in range(2)]

    def k_tasks(slot, cbase, pieces):
        out = []
        for r in pieces:
            for ct in range(QW // 128):
                def t(r=r, ct=ct):
                    res = _dot(_up(xn[pl.ds(_mult(r * 64, 64), 64), :]), wst[slot, :, pl.ds(ct * 128, 128)])
                    for k in range(8):
                        R[cbase + ct, pl.ds(_mult(r * 64 + k * 8, 8), 8), :] = _pk(res[k * 16:(k + 1) * 16])
                out.append((t, 256))
        return out

    def q_tasks(cbase):
        out = []
        for r in range(16):
            for ct in range(QW // 128):
                def t(r=r, ct=ct):
                    res = _dot(_up(xn[pl.ds(r * 64, 64), :]),
                               _up(wqp[:, pl.ds(_mult((cbase + ct) * 128, 128), 128)]))
                    for k in range(8):
                        QP[cbase + ct, pl.ds(r * 64 + k * 8, 8), :] = _pk(res[k * 16:(k + 1) * 16])
                out.append((t, 256))
        return out

    def mm1_tasks(mp, s, par):
        out = []
        for p in range(NP):
            for c in range(2):
                def t(p=p, c=c):
                    M[mp, p, c, pl.ds(0, RS), :] = _dot(
                        _up(T[p, pl.ds(_mult(s * (RS // 2), RS // 2), RS // 2), :]),
                        _up(B[par, p, :, pl.ds(c * 128, 128)]))
                out.append((t, 64))
        return out

    def mm2_tasks(mp, s, par):
        out = []
        for p in range(NP):
            def t(p=p):
                r = _dot(_up(H[mp, p]), _up(Bd[par, p]))
                for c in range(2):
                    acc[p, c, pl.ds(_mult(s * RS, RS), RS), :] += r[:, c * 128:(c + 1) * 128]
            out.append((t, 64))
        return out

    def wo_tasks(i):
        out = []
        for p in range(NP):
            for c in range(2):
                def t(p=p, c=c):
                    lhs = jnp.concatenate([M[i % 2, p, n, pl.ds(0, RS), :] for n in range(2)], axis=1)
                    acc[p, c, pl.ds(_mult(i * RS, RS), RS), :] += lax.dot_general(
                        lhs, _up(B[1, p, :, pl.ds(c * 128, 128)]), (((1,), (0,)), ((), ())),
                        preferred_element_type=f32)
                out.append((t, 64))
        return out

    nothing = lambda: [(lambda: None, 1)]

    x_copy(0).start()
    w_copy(0, 0).start()
    for c in range(8):
        KF[c, pl.ds(0, PADR), :] = jnp.zeros((PADR, 128), f32)
        VF[c, pl.ds(0, PADR), :] = jnp.zeros((PADR, 128), f32)
    x_copy(0).wait()
    w_copy(1, 1).start()
    x_copy(1).start()
    block(nothing, lambda: ln_jobs(0), 'ln0')
    w_copy(0, 0).wait()

    def k01(pieces):
        rp = [2 * r + h for r in pieces for h in range(2)]
        return k_tasks(0, 0, rp) + k_tasks(1, 2, rp)

    block(lambda: k_tasks(0, 0, (0, 1)), lambda: [], 'p0')
    w_copy(1, 1).wait()
    x_copy(2).start()
    x_copy(1).wait()
    block(lambda: k_tasks(1, 2, (0, 1)), lambda: ln_jobs(1), 'p0')
    x_copy(3).start()
    x_copy(4).start()
    x_copy(2).wait()
    block(lambda: k01((1,)), lambda: ln_jobs(2), 'p0')
    x_copy(5).start()
    x_copy(6).start()
    x_copy(3).wait()
    x_copy(4).wait()
    block(lambda: k01((2,)), lambda: ln_jobs(3) + ln_jobs(4), 'p0')
    x_copy(7).start()
    wq_copy().start()
    x_copy(5).wait()
    x_copy(6).wait()
    block(lambda: k01((3, 4)), lambda: ln_jobs(5) + ln_jobs(6), 'p0')
    w_copy(2, 2).start()
    start(wv_copies())
    x_copy(7).wait()
    block(lambda: k01((5, 6)), lambda: ln_jobs(7), 'p0')
    wq_copy().wait()
    block(lambda: k01((7,)), lambda: [wperm_job('q', 0, a, 2) for a in range(0, 8, 2)], 'p0')

    wait(wv_copies())

    def k_body(j, c):
        w_copy(j, j % 3).wait()

        @pl.when(j == 2)
        def _():
            w_copy(3, 0).start()
            start(gu_copies(0, 0))

        @pl.when(j == 3)
        def _():
            d_copy(0, 0).start()
            d_copy(1, 1).start()
        i = j - 2

        def jobs():
            perms = _mix([wperm_job('v', i * 16, a) for a in range(16)], [wperm_job('q', 8 + 12 * i, a, 2) for a in range(0, 12, 2)])
            extra = _mix([t_job(i * 32, a) for a in range(8)]
                         + [mzero_job(jnp.minimum(i * 25 + a, NP - 1)) for a in range(25)],
                         [zero_job(jnp.minimum(i * 25 + a, NP - 1)) for a in range(25)])
            return _mix(perms[:-4], extra) + perms[-4:]
        block(lambda: k_tasks(j % 3, j * 2, range(16)), jobs, 'k', 0)
        return c
    lax.fori_loop(2, 4, k_body, 0)
    start(gu_copies(1, 1))

    def q_body(i, c):
        def jobs():
            extra = ([bv_job(i, g, h) for g in range(4) for h in range(2)]
                     + [t_job(64 + 48 * i, a) for a in range(12)])
            return _mix([kperm_job(i, a) for a in range(16)], extra)
        block(lambda: q_tasks(i * 2), jobs, 'q', 2)
        return c
    lax.fori_loop(0, 4, q_body, 0)

    wait(gu_copies(0, 0))
    d_copy(0, 0).wait()

    def v_slot(s, mp):
        def jobs():
            return b_jobs(0, s) + bd_jobs(0, s)[:2] + vcomb_jobs(1 - mp, jnp.maximum(s - 1, 0))
        block(lambda: mm1_tasks(mp, s, 1), jobs, 'v', 2)

    def v_body(it, c):
        v_slot(2 * it, 0)
        v_slot(2 * it + 1, 1)
        return c
    lax.fori_loop(0, 2, v_body, 0)

    wait(gu_copies(1, 1))
    start(gu_copies(2, 0))
    block(lambda: mm1_tasks(0, 0, 0), lambda: _mix(vcomb_jobs(1, 3), b_jobs(1, 0) + bd_jobs(0, 0)[2:] + bd_jobs(0, 1)[2:]), 'f0', 0)
    block(lambda: mm1_tasks(1, 1, 0),
          lambda: _mix(_mix(comb_jobs(0), b_jobs(1, 1) + bd_jobs(0, 2)[2:] + bd_jobs(0, 3)[2:]), attn_quad(26, True)), 'f1', 3)

    def slot(t, mp):
        j = t // 4
        s = t % 4
        par = j % 2
        if mp == 0:
            @pl.when(jnp.logical_and(s == 0, j > 0))
            def _():
                wait(gu_copies(jnp.minimum(j + 1, NCH - 1), 1 - par))

                @pl.when(j + 2 < NCH)
                def _():
                    start(gu_copies(j + 2, par))

                @pl.when(j + 2 == NCH)
                def _():
                    start(wo_copies())

            @pl.when(jnp.logical_and(s == 2, j + 1 < NCH))
            def _():
                d_copy(j + 1, 1 - par).wait()

                @pl.when(j + 2 < NCH)
                def _():
                    d_copy(j + 2, par).start()
        jd = (t + 2) // 4
        kd = (t + 2) % 4
        u = t - 2

        def jobs():
            base = _mix(comb_jobs(1 - mp), b_jobs(1 - par, s) + bd_jobs(jd % 2, kd))
            att = attn_quad(u)
            n0 = max(1, len(base) // 10)
            return base[:n0] + _mix(base[n0:-n0], att) + base[-n0:]
        block(lambda: mm1_tasks(mp, s, par) + mm2_tasks(mp, (t - 2) % 4, ((t - 2) // 4) % 2), jobs,
              'slot%d' % mp, 3)

    def steady(it, c):
        slot(2 * it + 2, 0)
        slot(2 * it + 3, 1)
        return c
    lax.fori_loop(0, (NT - 2) // 2, steady, 0)

    block(lambda: mm2_tasks(0, 2, 0), lambda: comb_jobs(1), 'e0')
    block(lambda: mm2_tasks(1, 3, 0), lambda: _mix(oc_jobs(0), attn_quad(27, True)), 'e1')
    block(lambda: wo_tasks(0),
          lambda: _mix(oc_jobs(1), _flat([attn_quad(n, True) for n in [28, 29]])), 'wo')
    for i in range(1, 4):
        if i == 3:
            wait([out_copy(0, a) for a in range(4)])
        block(lambda i=i: wo_tasks(i),
              lambda i=i: _mix(final_jobs(i - 1) + (oc_jobs(i + 1) if i < 3 else []),
                                _flat([attn_quad(n, True) for n in ([30, 31] if i == 1 else [])])), 'wo')
        start([out_copy(i - 1, a) for a in range(4)])
    wait([out_copy(1, a) for a in range(4)])
    for h in range(2):
        block(nothing, lambda h=h: [final_job(3, g, n) for g in range(4 * h, 4 * h + 4) for n in range(2)], 'e3')
        start([last_copy(a, h) for a in range(4)])
    wait([out_copy(2, a) for a in range(4)])
    wait([last_copy(a, h) for h in range(2) for a in range(4)])


@jax.jit
def pallas_parallel_sum__sliding_local_dilated__glu_gated_bilinear__prompt_kernel(
    A_x: jax.Array,
    A_wqkv: jax.Array,
    A_wo: jax.Array,
    B_x: jax.Array,
    B_w_gate: jax.Array,
    B_w_up: jax.Array,
    B_w_down: jax.Array,
):
    del B_x
    x = A_x.reshape(S, D)
    hbm = pl.BlockSpec(memory_space=pl.ANY)
    dma = pltpu.SemaphoreType.DMA
    out = pl.pallas_call(
        _kernel,
        grid=(1,),
        in_specs=[pl.BlockSpec(memory_space=pltpu.SMEM)] + [hbm] * 6,
        out_specs=hbm,
        out_shape=jax.ShapeDtypeStruct((S, D), bf),
        scratch_shapes=[
            pltpu.VMEM((S, D), bf),
            pltpu.VMEM((S // 2, D), u32),
            pltpu.VMEM((NP, HB // 2, KB), u32),
            pltpu.VMEM((3, D, QW), bf),
            pltpu.VMEM((D, D), bf),
            pltpu.VMEM((D // 2, D), u32),
            pltpu.VMEM((D // 2, D), u32),
            pltpu.VMEM((8, S // 2 + PADW, 128), u32),
            pltpu.VMEM((8, S // 2 + PADW, 128), u32),
            pltpu.VMEM((8, S + PADR + 8, 128), f32),
            pltpu.VMEM((8, S + PADR + 8, 128), f32),
            pltpu.VMEM((2, D, TF), bf),
            pltpu.VMEM((2, D, TF), bf),
            pltpu.VMEM((2, TF, D), bf),
            pltpu.VMEM((2, NP, KB // 2, 2 * TB), u32),
            pltpu.VMEM((2, NP, TB // 2, KB), u32),
            pltpu.VMEM((2, NP, 2, RS + MPAD, 128), f32),
            pltpu.VMEM((2, NP, RS // 2, TB), u32),
            pltpu.VMEM((4, 16, 24, 128), f32),
            pltpu.VMEM((4, 8, 24, 128), f32),
            pltpu.VMEM((NP, 2, HB + MPAD, 128), f32),
            dma((8,)), dma((3,)), dma((1,)), dma((2,)), dma((2,)), dma((2,)), dma((16,)),
        ],
        compiler_params=pltpu.CompilerParams(
            dimension_semantics=("arbitrary",), vmem_limit_bytes=127 * 1024 * 1024,
            disable_bounds_checks=True),
        name="fused_attn_ffn",
    )(jnp.ones((1,), jnp.int32), x, A_wqkv, A_wo, B_w_gate, B_w_up, B_w_down)
    return out.reshape(1, S, D)
```

```python
import jax
import jax.numpy as jnp
from jax import lax
from jax.experimental import pallas as pl
from jax.experimental.pallas import tpu as pltpu

bf = jnp.bfloat16
f32 = jnp.float32
u32 = jnp.uint32

S, D, F = 2048, 1024, 3584
WIN = 8
NP = 49
HB = S // 4
KB = D // 4
TF = 512
TB = TF // 4
NCH = F // TF
RS = 128
NSUB = HB // RS
NT = NCH * NSUB
MPAD = 8
PADW = 8
PADR = 16
QW = 256
EPS = 1e-5
C2 = float(32 ** -0.5 * 1.4426950408889634)

A_T = [[(1, (0, 0)), (1, (1, 1))], [(1, (1, 0)), (1, (1, 1))], [(1, (0, 0))], [(1, (1, 1))],
       [(1, (0, 0)), (1, (0, 1))], [(1, (1, 0)), (-1, (0, 0))], [(1, (0, 1)), (-1, (1, 1))]]
B_T = [[(1, (0, 0)), (1, (1, 1))], [(1, (0, 0))], [(1, (0, 1)), (-1, (1, 1))], [(1, (1, 0)), (-1, (0, 0))],
       [(1, (1, 1))], [(1, (0, 0)), (1, (0, 1))], [(1, (1, 0)), (1, (1, 1))]]
C_T = {(0, 0): [(1, 0), (1, 3), (-1, 4), (1, 6)], (0, 1): [(1, 2), (1, 4)],
       (1, 0): [(1, 1), (1, 3)], (1, 1): [(1, 0), (-1, 1), (1, 2), (1, 5)]}
POS = ((0, 0), (0, 1), (1, 0), (1, 1))


def _comb(terms):
    acc = None
    for s, v in terms:
        if acc is None:
            acc = v if s > 0 else -v
        else:
            acc = acc + v if s > 0 else acc - v
    return acc


def _dot(a, b):
    return jnp.dot(a, b, preferred_element_type=f32)


def _pk(v):
    return pltpu.bitcast(v.astype(bf), u32)


def _up(w):
    return pltpu.bitcast(w, bf)


def _unpk(w):
    return pltpu.bitcast(w, bf).astype(f32)


def _as_f32(w):
    return lax.bitcast_convert_type(w, f32)


def _as_u32(v):
    return lax.bitcast_convert_type(v, u32)


def _mult(x, m):
    return x if isinstance(x, int) else pl.multiple_of(x, m)


def _opcomb(load, table, I, emit, raw):
    sub = {(r, c): _comb([(s, load(q[0] * 2 + r, q[1] * 2 + c)) for s, q in table[I]])
           for r in range(2) for c in range(2)}
    for J, t2 in enumerate(table):
        if raw is not None and len(table[I]) == 1 and len(t2) == 1:
            qo, qi = table[I][0][1], t2[0][1]
            emit(I * 7 + J, raw(qo[0] * 2 + qi[0], qo[1] * 2 + qi[1]))
        else:
            emit(I * 7 + J, _pk(_comb([(s, sub[q]) for s, q in t2])))


def _opcomb_job(load, table, emit, raw=None):
    return [(lambda I=I: _opcomb(load, table, I, emit, raw)) for I in range(7)]


def _outpos(load, pos):
    inner = [_comb([(s, load(I * 7 + J)) for s, J in C_T[pos]]) for I in range(7)]
    return {q: _comb([(s, inner[I]) for s, I in terms]) for q, terms in C_T.items()}


def _perm8(v):
    lane = lax.broadcasted_iota(jnp.int32, v[0].shape, 1)
    v = list(v)
    for cb, lb in ((2, 4), (1, 3), (0, 2)):
        sh = 1 << lb
        hi = (lane & sh) != 0
        out = [None] * 8
        for c in range(8):
            if c & (1 << cb):
                continue
            x, y = v[c], v[c | (1 << cb)]
            out[c] = jnp.where(hi, pltpu.roll(y, sh, 1), x)
            out[c | (1 << cb)] = jnp.where(hi, y, pltpu.roll(x, 128 - sh, 1))
        v = out
    return v


def _sum4(x, lane):
    x = x + jnp.where((lane & 1) != 0, pltpu.roll(x, 1, 1), pltpu.roll(x, 127, 1))
    x = x + jnp.where((lane & 2) != 0, pltpu.roll(x, 2, 1), pltpu.roll(x, 126, 1))
    return x


def _mix(a, b):
    if not b:
        return list(a)
    if not a:
        return list(b)
    out, n, m, k = [], len(a), len(b), 0
    for i, t in enumerate(a):
        out.append(t)
        tgt = (i + 1) * m // n
        while k < tgt:
            out.append(b[k])
            k += 1
    return out


def _flat(jobs, depth=1):
    return [t for j in jobs for t in j]


def _weave(mx, jobs, woff=0):
    vp = _flat(jobs)
    tot = sum(c for _, c in mx)
    n, k, acc = len(vp), 0, 0
    for t, c in mx:
        t()
        acc += c
        tgt = min(n, acc * n // tot + woff)
        while k < tgt:
            vp[k]()
            k += 1
    while k < n:
        vp[k]()
        k += 1


def _kernel(one_ref, x_hbm, wqkv_hbm, wo_hbm, wg_hbm, wu_hbm, wd_hbm, out_hbm,
            xr, xn, T, wst, wqr, wqp, wvp, R, QP, KF, VF, gst, ust, dst, B, Bd, M, H, hst, ost, acc,
            sem_x, sem_w, sem_q, sem_g, sem_u, sem_d, sem_o):

    def block(mx, jobs, name="blk", woff=0):
        with jax.named_scope(name):
            @pl.when(one_ref[0] > 0)
            def _():
                _weave(mx(), jobs(), woff)

    def x_copy(r):
        rows = pl.ds(_mult(r * 256, 256), 256)
        return pltpu.make_async_copy(x_hbm.at[rows, :], xr.at[rows, :], sem_x.at[r])

    def w_copy(j, slot):
        return pltpu.make_async_copy(wqkv_hbm.at[:, pl.ds(_mult(D + j * QW, QW), QW)], wst.at[slot], sem_w.at[slot])

    def wv_copies():
        return (pltpu.make_async_copy(wqkv_hbm.at[:, pl.ds(2 * D, TF)], gst.at[1], sem_g.at[1]),
                pltpu.make_async_copy(wqkv_hbm.at[:, pl.ds(2 * D + TF, TF)], ust.at[1], sem_u.at[1]))

    def wq_copy():
        return pltpu.make_async_copy(wqkv_hbm.at[:, pl.ds(0, D)], wqr, sem_q.at[0])

    def gu_copies(j, par):
        cols = pl.ds(_mult(j * TF, TF), TF)
        return (pltpu.make_async_copy(wg_hbm.at[:, cols], gst.at[par], sem_g.at[par]),
                pltpu.make_async_copy(wu_hbm.at[:, cols], ust.at[par], sem_u.at[par]))

    def d_copy(j, par):
        return pltpu.make_async_copy(wd_hbm.at[pl.ds(_mult(j * TF, TF), TF), :], dst.at[par], sem_d.at[par])

    def wo_copies():
        return [pltpu.make_async_copy(wo_hbm.at[:, pl.ds(q * KB + h * TB, TB)],
                                      (gst, ust)[h].at[1, :, pl.ds(q * TB, TB)], (sem_g, sem_u)[h].at[1])
                for h in range(2) for q in range(4)]

    def out_copy(i, a):
        par = i % 2
        return pltpu.make_async_copy(dst.at[par, pl.ds(a * RS, RS), :],
                                     out_hbm.at[pl.ds(_mult(a * HB + i * RS, RS), RS), :], sem_o.at[par * 4 + a])

    def last_copy(a, h):
        rows = RS // 2
        return pltpu.make_async_copy(dst.at[1, pl.ds(a * RS + h * rows, rows), :],
                                     out_hbm.at[pl.ds(a * HB + 3 * RS + h * rows, rows), :], sem_o.at[8 + h * 4 + a])

    def start(cps):
        for cp in cps:
            cp.start()

    def wait(cps):
        for cp in cps:
            cp.wait()

    def ln_job(g):
        def t():
            v = [xr[pl.ds(g * 16, 16), pl.ds(c * 128, 128)].astype(f32) for c in range(8)]
            a = v[0]
            for c in range(1, 8):
                a = a + v[c]
            mean = jnp.sum(a, axis=1, keepdims=True) * (1.0 / D)
            v = [x - mean for x in v]
            a = v[0] * v[0]
            for c in range(1, 8):
                a = a + v[c] * v[c]
            r = lax.rsqrt(jnp.sum(a, axis=1, keepdims=True) * (1.0 / D) + EPS)
            for c in range(8):
                xn[pl.ds(g * 8, 8), pl.ds(c * 128, 128)] = _pk(v[c] * r)
        return [t]

    def ln_jobs(r):
        return [ln_job(r * 16 + g) for g in range(16)]

    def t_job(wb, pos):
        w0 = _mult(wb, 16) + (pos // 2) * 8
        l0 = (pos % 2) * 128

        def raw(i, j):
            return xn[pl.ds(w0 + i * 256, 8), pl.ds(j * KB + l0, 128)]

        def emit(p, v):
            T[p, pl.ds(w0, 8), pl.ds(l0, 128)] = v
        return _opcomb_job(lambda i, j: _unpk(raw(i, j)), A_T, emit, raw)

    def b_job(par, k, g, half):
        w_ref = (gst, ust)[half]

        def src(i, q):
            return w_ref[par, pl.ds(_mult(k * 64, 64) + (i * KB + g * 16), 16), pl.ds(q * TB, TB)]

        def emit(p, v):
            B[par, p, pl.ds(_mult(k * 32, 32) + g * 8, 8), pl.ds(half * TB, TB)] = v
        return _opcomb_job(lambda i, q: src(i, q).astype(f32), B_T, emit,
                           lambda i, q: pltpu.bitcast(src(i, q), u32))

    def bd_job(par, gb, g, n):
        def src(i, q):
            return dst[par, pl.ds(_mult(gb, 16) + (i * TB + g * 16), 16), pl.ds(q * KB + n * 128, 128)]

        def emit(p, v):
            Bd[par, p, pl.ds(_mult(gb // 2, 8) + g * 8, 8), pl.ds(n * 128, 128)] = v
        return _opcomb_job(lambda i, q: src(i, q).astype(f32), B_T, emit,
                           lambda i, q: pltpu.bitcast(src(i, q), u32))

    def b_jobs(par, k):
        return [b_job(par, k, g, h) for g in range(4) for h in range(2)]

    def bd_jobs(par, k):
        return [bd_job(par, k * 32, g, n) for g in range(2) for n in range(2)]

    def kperm_job(i, a):
        def t():
            r = _perm8([R[c, pl.ds(_mult(i * 256, 256) + a * 16, 16), :] for c in range(8)])
            for c in range(8):
                KF[c, pl.ds(_mult(i * 512, 512) + (PADR + a * 32), 32), :] = _unpk(r[c])
        return [t]

    def wperm_job(which, pb, a, np_=1):
        def t():
            rows = pl.ds(_mult(pb * 32, 64) + a * 32, 32 * np_)
            if which == 'q':
                src = [wqr[rows, pl.ds(c * 128, 128)] for c in range(8)]
            else:
                src = [(gst, ust)[c // 4][1, rows, pl.ds((c % 4) * 128, 128)] for c in range(8)]
            r = _perm8([pltpu.bitcast(v, u32) for v in src])
            for c in range(8):
                (wqp if which == 'q' else wvp)[pl.ds(_mult(pb * 16, 32) + a * 16, 16 * np_), pl.ds(c * 128, 128)] = r[c]
        return [t]

    def bv_job(k, g, half):
        def raw(i, q):
            return wvp[pl.ds(_mult(k * 32, 32) + (i * (KB // 2) + g * 8), 8), pl.ds((2 * q + half) * 128, 128)]

        def emit(p, v):
            B[1, p, pl.ds(_mult(k * 32, 32) + g * 8, 8), pl.ds(half * TB, TB)] = v
        return _opcomb_job(lambda i, q: _unpk(raw(i, q)), B_T, emit, raw)

    def vcomb_job(mp, s, g):
        job = []
        for hf in range(2):
            for pos in POS:
                def t(hf=hf, pos=pos):
                    for n in range(2):
                        o = _outpos(lambda p: M[mp, p, n, pl.ds(g * 16 + hf * 8, 8), :], pos)
                        for q in o:
                            a = q[0] * 2 + pos[0]
                            ch = (q[1] * 2 + pos[1]) * 2 + n
                            VF[ch, pl.ds(_mult(s * RS, RS) + (PADR + a * HB + g * 16 + hf * 8), 8), :] = o[q]
                job.append(t)
        return job

    def vcomb_jobs(mp, s):
        return [vcomb_job(mp, s, g) for g in range(RS // 16)]

    def mzero_job(p):
        def t():
            for c in range(2):
                M[1, p, c, pl.ds(0, RS), :] = jnp.zeros((RS, 128), f32)
        return [t]

    def attn_quad(n, stack=False):
        base = _mult(((n % 8) // 2) * 256 + (n // 8) * 64 + (n % 2) * 32, 32)
        return [attn_job(base, 8 * k, k, stack) for k in range(4)]

    def attn_job(base, off, sl, stack):
        b = base + off
        rbase = _mult(base * 2, 64)
        job = []
        for h in range(2):
            st = {}
            half = lambda v, h=h: _unpk(v)[h * 8:(h + 1) * 8]

            def qk(cs, st=st, half=half, h=h):
                def t():
                    for c in cs:
                        qv = half(QP[c, pl.ds(base + off, 8), :])
                        for w in range(WIN):
                            kv = KF[c, pl.ds(rbase + (2 * off + 8 * h + PADR - 2 * w), 8), :]
                            st[w] = qv * kv if c == 0 else st[w] + qv * kv
                return t

            def sm(st=st, h=h):
                lane = lax.broadcasted_iota(jnp.int32, (8, 128), 1)
                row = lax.broadcasted_iota(jnp.int32, (8, 128), 0) + (b * 2 + h * 8)
                if stack:
                    big = jnp.concatenate([st[w] for w in range(WIN)], axis=0)
                    big = _sum4(big, lax.broadcasted_iota(jnp.int32, (8 * WIN, 128), 1))
                    ls = [big[8 * w:8 * w + 8] for w in range(WIN)]
                else:
                    ls = [_sum4(st[w], lane) for w in range(WIN)]
                ls = [ls[0]] + [jnp.where(row >= 2 * w, ls[w], -1e30) for w in range(1, WIN)]
                m = ls[0]
                for w in range(1, WIN):
                    m = jnp.maximum(m, ls[w])
                e = [jnp.exp2((l - m) * C2) for l in ls]
                den = e[0]
                for w in range(1, WIN):
                    den = den + e[w]
                inv = 1.0 / den
                st['p'] = [x * inv for x in e]

            def pv(cs, st=st, half=half, h=h):
                def t():
                    for c in cs:
                        o = None
                        for w in range(WIN):
                            a = st['p'][w] * VF[c, pl.ds(rbase + (2 * off + 8 * h + PADR - 2 * w), 8), :]
                            o = a if o is None else o + a
                        ost[sl, c, pl.ds(h * 8, 8), :] = o
                return t
            job += [qk((0, 1, 2, 3)), qk((4, 5, 6, 7)), sm, pv((0, 1, 2, 3)), pv((4, 5, 6, 7))]

        def fin():
            r = _perm8([_pk(ost[sl, c, pl.ds(0, 16), :]) for c in range(8)])
            for c in range(8):
                xn[pl.ds(_mult(b, 8), 8), pl.ds(c * 128, 128)] = r[c]
        return job + [fin]

    def comb_job(mp, g):
        sl = g % 4
        job = []
        for hf in range(2):
            for pos in POS:
                def t(hf=hf, pos=pos):
                    r = pl.ds(g * 16 + hf * 8, 8)
                    gg = _outpos(lambda p: M[mp, p, 0, r, :], pos)
                    uu = _outpos(lambda p: M[mp, p, 1, r, :], pos)
                    for q in gg:
                        hst[sl, (q[0] * 2 + pos[0]) * 4 + q[1] * 2 + pos[1], pl.ds(hf * 8, 8), :] = gg[q] * uu[q]
                job.append(t)

        def emit(p, v):
            H[mp, p, pl.ds(g * 8, 8), :] = v
        return job + _opcomb_job(lambda i, j: hst[sl, i * 4 + j, pl.ds(0, 16), :], A_T, emit)

    def comb_jobs(mp):
        return [comb_job(mp, g) for g in range(RS // 16)]

    def zero_job(p):
        def t():
            for c in range(2):
                acc[p, c, pl.ds(0, HB), :] = jnp.zeros((HB, 128), f32)
        return [t]

    def oc_job(i, g, n):
        def load(a, kb):
            return _unpk(xn[pl.ds(_mult(i * 64, 64) + (a * 256 + g * 8), 8), pl.ds(kb * KB + n * 128, 128)])

        def one(I):
            sub = {(r, c): _comb([(sg, load(q[0] * 2 + r, q[1] * 2 + c)) for sg, q in A_T[I]])
                   for r in range(2) for c in range(2)}
            for J, t2 in enumerate(A_T):
                M[i % 2, I * 7 + J, n, pl.ds(g * 16, 16), :] = _comb([(sg, sub[q]) for sg, q in t2])
        return [(lambda I=I: one(I)) for I in range(7)]

    def oc_jobs(i):
        return [oc_job(i, g, n) for g in range(RS // 16) for n in range(2)]

    def final_job(i, g, n):
        job = []
        par = i % 2
        for pos in POS:
            def t(pos=pos):
                r0 = _mult(i * RS, RS) + g * 16
                o = [_outpos(lambda p: acc[p, n, pl.ds(r0 + hf * 8, 8), :], pos) for hf in range(2)]
                for q in o[0]:
                    a = q[0] * 2 + pos[0]
                    cols = pl.ds(((q[1] * 2 + pos[1]) * 2 + n) * 128, 128)
                    res = xr[pl.ds(r0 + a * HB, 16), cols].astype(f32) + jnp.concatenate([o[0][q], o[1][q]], axis=0)
                    dst[par, pl.ds(a * RS + g * 16, 16), cols] = res.astype(bf)
            job.append(t)
        return job

    def final_jobs(i):
        return [final_job(i, g, n) for g in range(RS // 16) for n in range(2)]

    def k_tasks(slot, cbase, pieces):
        out = []
        for r in pieces:
            for ct in range(QW // 128):
                def t(r=r, ct=ct):
                    res = _dot(_up(xn[pl.ds(_mult(r * 64, 64), 64), :]), wst[slot, :, pl.ds(ct * 128, 128)])
                    for k in range(8):
                        R[cbase + ct, pl.ds(_mult(r * 64 + k * 8, 8), 8), :] = _pk(res[k * 16:(k + 1) * 16])
                out.append((t, 256))
        return out

    def q_tasks(cbase):
        out = []
        for r in range(16):
            for ct in range(QW // 128):
                def t(r=r, ct=ct):
                    res = _dot(_up(xn[pl.ds(r * 64, 64), :]),
                               _up(wqp[:, pl.ds(_mult((cbase + ct) * 128, 128), 128)]))
                    for k in range(8):
                        QP[cbase + ct, pl.ds(r * 64 + k * 8, 8), :] = _pk(res[k * 16:(k + 1) * 16])
                out.append((t, 256))
        return out

    def mm1_tasks(mp, s, par):
        out = []
        for p in range(NP):
            for c in range(2):
                def t(p=p, c=c):
                    M[mp, p, c, pl.ds(0, RS), :] = _dot(
                        _up(T[p, pl.ds(_mult(s * (RS // 2), RS // 2), RS // 2), :]),
                        _up(B[par, p, :, pl.ds(c * 128, 128)]))
                out.append((t, 64))
        return out

    def mm2_tasks(mp, s, par):
        out = []
        for p in range(NP):
            def t(p=p):
                r = _dot(_up(H[mp, p]), _up(Bd[par, p]))
                for c in range(2):
                    acc[p, c, pl.ds(_mult(s * RS, RS), RS), :] += r[:, c * 128:(c + 1) * 128]
            out.append((t, 64))
        return out

    def wo_tasks(i):
        out = []
        for p in range(NP):
            for c in range(2):
                def t(p=p, c=c):
                    lhs = jnp.concatenate([M[i % 2, p, n, pl.ds(0, RS), :] for n in range(2)], axis=1)
                    acc[p, c, pl.ds(_mult(i * RS, RS), RS), :] += lax.dot_general(
                        lhs, _up(B[1, p, :, pl.ds(c * 128, 128)]), (((1,), (0,)), ((), ())),
                        preferred_element_type=f32)
                out.append((t, 64))
        return out

    nothing = lambda: [(lambda: None, 1)]

    x_copy(0).start()
    w_copy(0, 0).start()
    for c in range(8):
        KF[c, pl.ds(0, PADR), :] = jnp.zeros((PADR, 128), f32)
        VF[c, pl.ds(0, PADR), :] = jnp.zeros((PADR, 128), f32)
    x_copy(0).wait()
    w_copy(1, 1).start()
    x_copy(1).start()
    block(nothing, lambda: ln_jobs(0), 'ln0')
    w_copy(0, 0).wait()

    def k01(pieces):
        rp = [2 * r + h for r in pieces for h in range(2)]
        return k_tasks(0, 0, rp) + k_tasks(1, 2, rp)

    block(lambda: k_tasks(0, 0, (0, 1)), lambda: [], 'p0')
    w_copy(1, 1).wait()
    x_copy(2).start()
    x_copy(1).wait()
    block(lambda: k_tasks(1, 2, (0, 1)), lambda: ln_jobs(1), 'p0')
    x_copy(3).start()
    x_copy(4).start()
    x_copy(2).wait()
    block(lambda: k01((1,)), lambda: ln_jobs(2), 'p0')
    x_copy(5).start()
    x_copy(6).start()
    x_copy(3).wait()
    x_copy(4).wait()
    block(lambda: k01((2,)), lambda: ln_jobs(3) + ln_jobs(4), 'p0')
    x_copy(7).start()
    wq_copy().start()
    x_copy(5).wait()
    x_copy(6).wait()
    block(lambda: k01((3, 4)), lambda: ln_jobs(5) + ln_jobs(6), 'p0')
    w_copy(2, 2).start()
    start(wv_copies())
    x_copy(7).wait()
    block(lambda: k01((5, 6)), lambda: ln_jobs(7), 'p0')
    wq_copy().wait()
    block(lambda: k01((7,)), lambda: [wperm_job('q', 0, a, 2) for a in range(0, 8, 2)], 'p0')

    wait(wv_copies())

    def k_body(j, c):
        w_copy(j, j % 3).wait()

        @pl.when(j == 2)
        def _():
            w_copy(3, 0).start()
            start(gu_copies(0, 0))

        @pl.when(j == 3)
        def _():
            d_copy(0, 0).start()
            d_copy(1, 1).start()
        i = j - 2

        def jobs():
            perms = _mix([wperm_job('v', i * 16, a) for a in range(16)], [wperm_job('q', 8 + 12 * i, a, 2) for a in range(0, 12, 2)])
            extra = [t_job(i * 32, a) for a in range(8)] + [mzero_job(jnp.minimum(i * 25 + a, NP - 1)) for a in range(25)]
            return _mix(perms[:-4], extra) + perms[-4:]
        block(lambda: k_tasks(j % 3, j * 2, range(16)), jobs, 'k', 0)
        return c
    lax.fori_loop(2, 4, k_body, 0)
    start(gu_copies(1, 1))

    def q_body(i, c):
        def jobs():
            extra = ([bv_job(i, g, h) for g in range(4) for h in range(2)]
                     + [t_job(64 + 48 * i, a) for a in range(12)])
            return _mix([kperm_job(i, a) for a in range(16)], extra)
        block(lambda: q_tasks(i * 2), jobs, 'q', 2)
        return c
    lax.fori_loop(0, 4, q_body, 0)

    wait(gu_copies(0, 0))
    d_copy(0, 0).wait()

    def v_slot(s, mp):
        def jobs():
            return _mix(b_jobs(0, s) + bd_jobs(0, s)[:2], [zero_job(jnp.minimum(s * 13 + a, NP - 1)) for a in range(13)]) + vcomb_jobs(1 - mp, jnp.maximum(s - 1, 0))
        block(lambda: mm1_tasks(mp, s, 1), jobs, 'v', 2)

    def v_body(it, c):
        v_slot(2 * it, 0)
        v_slot(2 * it + 1, 1)
        return c
    lax.fori_loop(0, 2, v_body, 0)

    wait(gu_copies(1, 1))
    start(gu_copies(2, 0))
    block(lambda: mm1_tasks(0, 0, 0), lambda: _mix(vcomb_jobs(1, 3), b_jobs(1, 0) + bd_jobs(0, 0)[2:] + bd_jobs(0, 1)[2:]), 'f0', 0)
    block(lambda: mm1_tasks(1, 1, 0),
          lambda: _mix(_mix(comb_jobs(0), b_jobs(1, 1) + bd_jobs(0, 2)[2:] + bd_jobs(0, 3)[2:]), attn_quad(26, True)), 'f1', 3)

    def slot(t, mp):
        j = t // 4
        s = t % 4
        par = j % 2
        if mp == 0:
            @pl.when(jnp.logical_and(s == 0, j > 0))
            def _():
                wait(gu_copies(jnp.minimum(j + 1, NCH - 1), 1 - par))

                @pl.when(j + 2 < NCH)
                def _():
                    start(gu_copies(j + 2, par))

                @pl.when(j + 2 == NCH)
                def _():
                    start(wo_copies())

            @pl.when(jnp.logical_and(s == 2, j + 1 < NCH))
            def _():
                d_copy(j + 1, 1 - par).wait()

                @pl.when(j + 2 < NCH)
                def _():
                    d_copy(j + 2, par).start()
        jd = (t + 2) // 4
        kd = (t + 2) % 4
        u = t - 2

        def jobs():
            base = _mix(comb_jobs(1 - mp), b_jobs(1 - par, s) + bd_jobs(jd % 2, kd))
            att = attn_quad(u)
            n0 = max(1, len(base) // 10)
            return base[:n0] + _mix(base[n0:-n0], att) + base[-n0:]
        block(lambda: mm1_tasks(mp, s, par) + mm2_tasks(mp, (t - 2) % 4, ((t - 2) // 4) % 2), jobs,
              'slot%d' % mp, 3)

    def steady(it, c):
        slot(2 * it + 2, 0)
        slot(2 * it + 3, 1)
        return c
    lax.fori_loop(0, (NT - 2) // 2, steady, 0)

    block(lambda: mm2_tasks(0, 2, 0), lambda: comb_jobs(1), 'e0')
    block(lambda: mm2_tasks(1, 3, 0), lambda: _mix(oc_jobs(0), attn_quad(27, True)), 'e1')
    block(lambda: wo_tasks(0),
          lambda: _mix(oc_jobs(1), _flat([attn_quad(n, True) for n in [28, 29]])), 'wo')
    for i in range(1, 4):
        if i == 3:
            wait([out_copy(0, a) for a in range(4)])
        block(lambda i=i: wo_tasks(i),
              lambda i=i: _mix(final_jobs(i - 1) + (oc_jobs(i + 1) if i < 3 else []),
                                _flat([attn_quad(n, True) for n in ([30, 31] if i == 1 else [])])), 'wo')
        start([out_copy(i - 1, a) for a in range(4)])
    wait([out_copy(1, a) for a in range(4)])
    for h in range(2):
        block(nothing, lambda h=h: [final_job(3, g, n) for g in range(4 * h, 4 * h + 4) for n in range(2)], 'e3')
        start([last_copy(a, h) for a in range(4)])
    wait([out_copy(2, a) for a in range(4)])
    wait([last_copy(a, h) for h in range(2) for a in range(4)])


@jax.jit
def pallas_parallel_sum__sliding_local_dilated__glu_gated_bilinear__prompt_kernel(
    A_x: jax.Array,
    A_wqkv: jax.Array,
    A_wo: jax.Array,
    B_x: jax.Array,
    B_w_gate: jax.Array,
    B_w_up: jax.Array,
    B_w_down: jax.Array,
):
    del B_x
    x = A_x.reshape(S, D)
    hbm = pl.BlockSpec(memory_space=pl.ANY)
    dma = pltpu.SemaphoreType.DMA
    out = pl.pallas_call(
        _kernel,
        grid=(1,),
        in_specs=[pl.BlockSpec(memory_space=pltpu.SMEM)] + [hbm] * 6,
        out_specs=hbm,
        out_shape=jax.ShapeDtypeStruct((S, D), bf),
        scratch_shapes=[
            pltpu.VMEM((S, D), bf),
            pltpu.VMEM((S // 2, D), u32),
            pltpu.VMEM((NP, HB // 2, KB), u32),
            pltpu.VMEM((3, D, QW), bf),
            pltpu.VMEM((D, D), bf),
            pltpu.VMEM((D // 2, D), u32),
            pltpu.VMEM((D // 2, D), u32),
            pltpu.VMEM((8, S // 2 + PADW, 128), u32),
            pltpu.VMEM((8, S // 2 + PADW, 128), u32),
            pltpu.VMEM((8, S + PADR + 8, 128), f32),
            pltpu.VMEM((8, S + PADR + 8, 128), f32),
            pltpu.VMEM((2, D, TF), bf),
            pltpu.VMEM((2, D, TF), bf),
            pltpu.VMEM((2, TF, D), bf),
            pltpu.VMEM((2, NP, KB // 2, 2 * TB), u32),
            pltpu.VMEM((2, NP, TB // 2, KB), u32),
            pltpu.VMEM((2, NP, 2, RS + MPAD, 128), f32),
            pltpu.VMEM((2, NP, RS // 2, TB), u32),
            pltpu.VMEM((4, 16, 24, 128), f32),
            pltpu.VMEM((4, 8, 24, 128), f32),
            pltpu.VMEM((NP, 2, HB + MPAD, 128), f32),
            dma((8,)), dma((3,)), dma((1,)), dma((2,)), dma((2,)), dma((2,)), dma((16,)),
        ],
        compiler_params=pltpu.CompilerParams(
            dimension_semantics=("arbitrary",), vmem_limit_bytes=127 * 1024 * 1024,
            disable_bounds_checks=True),
        name="fused_attn_ffn",
    )(jnp.ones((1,), jnp.int32), x, A_wqkv, A_wo, B_w_gate, B_w_up, B_w_down)
    return out.reshape(1, S, D)
```

```python
import jax
import jax.numpy as jnp
from jax import lax
from jax.experimental import pallas as pl
from jax.experimental.pallas import tpu as pltpu

bf = jnp.bfloat16
f32 = jnp.float32
u32 = jnp.uint32

S, D, F = 2048, 1024, 3584
WIN = 8
NP = 49
HB = S // 4
KB = D // 4
TF = 512
TB = TF // 4
NCH = F // TF
RS = 128
NSUB = HB // RS
NT = NCH * NSUB
MPAD = 8
PADW = 8
PADR = 16
QW = 256
EPS = 1e-5
C2 = float(32 ** -0.5 * 1.4426950408889634)

A_T = [[(1, (0, 0)), (1, (1, 1))], [(1, (1, 0)), (1, (1, 1))], [(1, (0, 0))], [(1, (1, 1))],
       [(1, (0, 0)), (1, (0, 1))], [(1, (1, 0)), (-1, (0, 0))], [(1, (0, 1)), (-1, (1, 1))]]
B_T = [[(1, (0, 0)), (1, (1, 1))], [(1, (0, 0))], [(1, (0, 1)), (-1, (1, 1))], [(1, (1, 0)), (-1, (0, 0))],
       [(1, (1, 1))], [(1, (0, 0)), (1, (0, 1))], [(1, (1, 0)), (1, (1, 1))]]
C_T = {(0, 0): [(1, 0), (1, 3), (-1, 4), (1, 6)], (0, 1): [(1, 2), (1, 4)],
       (1, 0): [(1, 1), (1, 3)], (1, 1): [(1, 0), (-1, 1), (1, 2), (1, 5)]}
POS = ((0, 0), (0, 1), (1, 0), (1, 1))


def _comb(terms):
    acc = None
    for s, v in terms:
        if acc is None:
            acc = v if s > 0 else -v
        else:
            acc = acc + v if s > 0 else acc - v
    return acc


def _dot(a, b):
    return jnp.dot(a, b, preferred_element_type=f32)


def _pk(v):
    return pltpu.bitcast(v.astype(bf), u32)


def _up(w):
    return pltpu.bitcast(w, bf)


def _unpk(w):
    return pltpu.bitcast(w, bf).astype(f32)


def _as_f32(w):
    return lax.bitcast_convert_type(w, f32)


def _as_u32(v):
    return lax.bitcast_convert_type(v, u32)


def _mult(x, m):
    return x if isinstance(x, int) else pl.multiple_of(x, m)


def _opcomb(load, table, I, emit, raw):
    sub = {(r, c): _comb([(s, load(q[0] * 2 + r, q[1] * 2 + c)) for s, q in table[I]])
           for r in range(2) for c in range(2)}
    for J, t2 in enumerate(table):
        if raw is not None and len(table[I]) == 1 and len(t2) == 1:
            qo, qi = table[I][0][1], t2[0][1]
            emit(I * 7 + J, raw(qo[0] * 2 + qi[0], qo[1] * 2 + qi[1]))
        else:
            emit(I * 7 + J, _pk(_comb([(s, sub[q]) for s, q in t2])))


def _opcomb_job(load, table, emit, raw=None):
    return [(lambda I=I: _opcomb(load, table, I, emit, raw)) for I in range(7)]


def _outpos(load, pos):
    inner = [_comb([(s, load(I * 7 + J)) for s, J in C_T[pos]]) for I in range(7)]
    return {q: _comb([(s, inner[I]) for s, I in terms]) for q, terms in C_T.items()}


def _perm8(v):
    lane = lax.broadcasted_iota(jnp.int32, v[0].shape, 1)
    v = list(v)
    for cb, lb in ((2, 4), (1, 3), (0, 2)):
        sh = 1 << lb
        hi = (lane & sh) != 0
        out = [None] * 8
        for c in range(8):
            if c & (1 << cb):
                continue
            x, y = v[c], v[c | (1 << cb)]
            out[c] = jnp.where(hi, pltpu.roll(y, sh, 1), x)
            out[c | (1 << cb)] = jnp.where(hi, y, pltpu.roll(x, 128 - sh, 1))
        v = out
    return v


def _sum4(x, lane):
    x = x + jnp.where((lane & 1) != 0, pltpu.roll(x, 1, 1), pltpu.roll(x, 127, 1))
    x = x + jnp.where((lane & 2) != 0, pltpu.roll(x, 2, 1), pltpu.roll(x, 126, 1))
    return x


def _mix(a, b):
    if not b:
        return list(a)
    if not a:
        return list(b)
    out, n, m, k = [], len(a), len(b), 0
    for i, t in enumerate(a):
        out.append(t)
        tgt = (i + 1) * m // n
        while k < tgt:
            out.append(b[k])
            k += 1
    return out


def _flat(jobs, depth=1):
    return [t for j in jobs for t in j]


def _weave(mx, jobs, woff=0):
    vp = _flat(jobs)
    tot = sum(c for _, c in mx)
    n, k, acc = len(vp), 0, 0
    for t, c in mx:
        t()
        acc += c
        tgt = min(n, acc * n // tot + woff)
        while k < tgt:
            vp[k]()
            k += 1
    while k < n:
        vp[k]()
        k += 1


def _kernel(one_ref, x_hbm, wqkv_hbm, wo_hbm, wg_hbm, wu_hbm, wd_hbm, out_hbm,
            xr, xn, T, wst, wqr, wqp, wvp, R, QP, KF, VF, gst, ust, dst, B, Bd, M, H, hst, ost, acc,
            sem_x, sem_w, sem_q, sem_g, sem_u, sem_d, sem_o):

    def block(mx, jobs, name="blk", woff=0):
        with jax.named_scope(name):
            @pl.when(one_ref[0] > 0)
            def _():
                _weave(mx(), jobs(), woff)

    def x_copy(r):
        rows = pl.ds(_mult(r * 256, 256), 256)
        return pltpu.make_async_copy(x_hbm.at[rows, :], xr.at[rows, :], sem_x.at[r])

    def w_copy(j, slot):
        return pltpu.make_async_copy(wqkv_hbm.at[:, pl.ds(_mult(D + j * QW, QW), QW)], wst.at[slot], sem_w.at[slot])

    def wv_copies():
        return (pltpu.make_async_copy(wqkv_hbm.at[:, pl.ds(2 * D, TF)], gst.at[1], sem_g.at[1]),
                pltpu.make_async_copy(wqkv_hbm.at[:, pl.ds(2 * D + TF, TF)], ust.at[1], sem_u.at[1]))

    def wq_copy():
        return pltpu.make_async_copy(wqkv_hbm.at[:, pl.ds(0, D)], wqr, sem_q.at[0])

    def gu_copies(j, par):
        cols = pl.ds(_mult(j * TF, TF), TF)
        return (pltpu.make_async_copy(wg_hbm.at[:, cols], gst.at[par], sem_g.at[par]),
                pltpu.make_async_copy(wu_hbm.at[:, cols], ust.at[par], sem_u.at[par]))

    def d_copy(j, par):
        return pltpu.make_async_copy(wd_hbm.at[pl.ds(_mult(j * TF, TF), TF), :], dst.at[par], sem_d.at[par])

    def wo_copies():
        return [pltpu.make_async_copy(wo_hbm.at[:, pl.ds(q * KB + h * TB, TB)],
                                      (gst, ust)[h].at[1, :, pl.ds(q * TB, TB)], (sem_g, sem_u)[h].at[1])
                for h in range(2) for q in range(4)]

    def out_copy(i, a):
        par = i % 2
        return pltpu.make_async_copy(dst.at[par, pl.ds(a * RS, RS), :],
                                     out_hbm.at[pl.ds(_mult(a * HB + i * RS, RS), RS), :], sem_o.at[par * 4 + a])

    def last_copy(a, h):
        rows = RS // 2
        return pltpu.make_async_copy(dst.at[1, pl.ds(a * RS + h * rows, rows), :],
                                     out_hbm.at[pl.ds(a * HB + 3 * RS + h * rows, rows), :], sem_o.at[8 + h * 4 + a])

    def start(cps):
        for cp in cps:
            cp.start()

    def wait(cps):
        for cp in cps:
            cp.wait()

    def ln_job(g):
        def t():
            v = [xr[pl.ds(g * 16, 16), pl.ds(c * 128, 128)].astype(f32) for c in range(8)]
            a = v[0]
            for c in range(1, 8):
                a = a + v[c]
            mean = jnp.sum(a, axis=1, keepdims=True) * (1.0 / D)
            v = [x - mean for x in v]
            a = v[0] * v[0]
            for c in range(1, 8):
                a = a + v[c] * v[c]
            r = lax.rsqrt(jnp.sum(a, axis=1, keepdims=True) * (1.0 / D) + EPS)
            for c in range(8):
                xn[pl.ds(g * 8, 8), pl.ds(c * 128, 128)] = _pk(v[c] * r)
        return [t]

    def ln_jobs(r):
        return [ln_job(r * 16 + g) for g in range(16)]

    def t_job(wb, pos):
        w0 = _mult(wb, 16) + (pos // 2) * 8
        l0 = (pos % 2) * 128

        def raw(i, j):
            return xn[pl.ds(w0 + i * 256, 8), pl.ds(j * KB + l0, 128)]

        def emit(p, v):
            T[p, pl.ds(w0, 8), pl.ds(l0, 128)] = v
        return _opcomb_job(lambda i, j: _unpk(raw(i, j)), A_T, emit, raw)

    def b_job(par, k, g, half):
        w_ref = (gst, ust)[half]

        def src(i, q):
            return w_ref[par, pl.ds(_mult(k * 64, 64) + (i * KB + g * 16), 16), pl.ds(q * TB, TB)]

        def emit(p, v):
            B[par, p, pl.ds(_mult(k * 32, 32) + g * 8, 8), pl.ds(half * TB, TB)] = v
        return _opcomb_job(lambda i, q: src(i, q).astype(f32), B_T, emit,
                           lambda i, q: pltpu.bitcast(src(i, q), u32))

    def bd_job(par, gb, g, n):
        def src(i, q):
            return dst[par, pl.ds(_mult(gb, 16) + (i * TB + g * 16), 16), pl.ds(q * KB + n * 128, 128)]

        def emit(p, v):
            Bd[par, p, pl.ds(_mult(gb // 2, 8) + g * 8, 8), pl.ds(n * 128, 128)] = v
        return _opcomb_job(lambda i, q: src(i, q).astype(f32), B_T, emit,
                           lambda i, q: pltpu.bitcast(src(i, q), u32))

    def b_jobs(par, k):
        return [b_job(par, k, g, h) for g in range(4) for h in range(2)]

    def bd_jobs(par, k):
        return [bd_job(par, k * 32, g, n) for g in range(2) for n in range(2)]

    def kperm_job(i, a):
        def t():
            r = _perm8([R[c, pl.ds(_mult(i * 256, 256) + a * 16, 16), :] for c in range(8)])
            for c in range(8):
                KF[c, pl.ds(_mult(i * 512, 512) + (PADR + a * 32), 32), :] = _unpk(r[c])
        return [t]

    def wperm_job(which, pb, a, np_=1):
        def t():
            rows = pl.ds(_mult(pb * 32, 64) + a * 32, 32 * np_)
            if which == 'q':
                src = [wqr[rows, pl.ds(c * 128, 128)] for c in range(8)]
            else:
                src = [(gst, ust)[c // 4][1, rows, pl.ds((c % 4) * 128, 128)] for c in range(8)]
            r = _perm8([pltpu.bitcast(v, u32) for v in src])
            for c in range(8):
                (wqp if which == 'q' else wvp)[pl.ds(_mult(pb * 16, 32) + a * 16, 16 * np_), pl.ds(c * 128, 128)] = r[c]
        return [t]

    def bv_job(k, g, half):
        def raw(i, q):
            return wvp[pl.ds(_mult(k * 32, 32) + (i * (KB // 2) + g * 8), 8), pl.ds((2 * q + half) * 128, 128)]

        def emit(p, v):
            B[1, p, pl.ds(_mult(k * 32, 32) + g * 8, 8), pl.ds(half * TB, TB)] = v
        return _opcomb_job(lambda i, q: _unpk(raw(i, q)), B_T, emit, raw)

    def vcomb_job(mp, s, g):
        job = []
        for hf in range(2):
            for pos in POS:
                def t(hf=hf, pos=pos):
                    for n in range(2):
                        o = _outpos(lambda p: M[mp, p, n, pl.ds(g * 16 + hf * 8, 8), :], pos)
                        for q in o:
                            a = q[0] * 2 + pos[0]
                            ch = (q[1] * 2 + pos[1]) * 2 + n
                            VF[ch, pl.ds(_mult(s * RS, RS) + (PADR + a * HB + g * 16 + hf * 8), 8), :] = o[q]
                job.append(t)
        return job

    def vcomb_jobs(mp, s):
        return [vcomb_job(mp, s, g) for g in range(RS // 16)]

    def mzero_job(p):
        def t():
            for c in range(2):
                M[1, p, c, pl.ds(0, RS), :] = jnp.zeros((RS, 128), f32)
        return [t]

    def attn_quad(n, stack=False):
        base = _mult(((n % 8) // 2) * 256 + (n // 8) * 64 + (n % 2) * 32, 32)
        return [attn_job(base, 8 * k, k, stack) for k in range(4)]

    def attn_job(base, off, sl, stack):
        b = base + off
        rbase = _mult(base * 2, 64)
        job = []
        for h in range(2):
            st = {}
            half = lambda v, h=h: _unpk(v)[h * 8:(h + 1) * 8]

            def qk(cs, st=st, half=half, h=h):
                def t():
                    for c in cs:
                        qv = half(QP[c, pl.ds(base + off, 8), :])
                        for w in range(WIN):
                            kv = KF[c, pl.ds(rbase + (2 * off + 8 * h + PADR - 2 * w), 8), :]
                            st[w] = qv * kv if c == 0 else st[w] + qv * kv
                return t

            def sm(st=st, h=h):
                lane = lax.broadcasted_iota(jnp.int32, (8, 128), 1)
                row = lax.broadcasted_iota(jnp.int32, (8, 128), 0) + (b * 2 + h * 8)
                if stack:
                    big = jnp.concatenate([st[w] for w in range(WIN)], axis=0)
                    big = _sum4(big, lax.broadcasted_iota(jnp.int32, (8 * WIN, 128), 1))
                    ls = [big[8 * w:8 * w + 8] for w in range(WIN)]
                else:
                    ls = [_sum4(st[w], lane) for w in range(WIN)]
                ls = [ls[0]] + [jnp.where(row >= 2 * w, ls[w], -1e30) for w in range(1, WIN)]
                m = ls[0]
                for w in range(1, WIN):
                    m = jnp.maximum(m, ls[w])
                e = [jnp.exp2((l - m) * C2) for l in ls]
                den = e[0]
                for w in range(1, WIN):
                    den = den + e[w]
                inv = 1.0 / den
                st['p'] = [x * inv for x in e]

            def pv(cs, st=st, half=half, h=h):
                def t():
                    for c in cs:
                        o = None
                        for w in range(WIN):
                            a = st['p'][w] * VF[c, pl.ds(rbase + (2 * off + 8 * h + PADR - 2 * w), 8), :]
                            o = a if o is None else o + a
                        ost[sl, c, pl.ds(h * 8, 8), :] = o
                return t
            job += [qk((0, 1, 2, 3)), qk((4, 5, 6, 7)), sm, pv((0, 1, 2, 3)), pv((4, 5, 6, 7))]

        def fin():
            r = _perm8([_pk(ost[sl, c, pl.ds(0, 16), :]) for c in range(8)])
            for c in range(8):
                xn[pl.ds(_mult(b, 8), 8), pl.ds(c * 128, 128)] = r[c]
        return job + [fin]

    def comb_job(mp, g):
        sl = g % 4
        job = []
        for hf in range(2):
            for pos in POS:
                def t(hf=hf, pos=pos):
                    r = pl.ds(g * 16 + hf * 8, 8)
                    gg = _outpos(lambda p: M[mp, p, 0, r, :], pos)
                    uu = _outpos(lambda p: M[mp, p, 1, r, :], pos)
                    for q in gg:
                        hst[sl, (q[0] * 2 + pos[0]) * 4 + q[1] * 2 + pos[1], pl.ds(hf * 8, 8), :] = gg[q] * uu[q]
                job.append(t)

        def emit(p, v):
            H[mp, p, pl.ds(g * 8, 8), :] = v
        return job + _opcomb_job(lambda i, j: hst[sl, i * 4 + j, pl.ds(0, 16), :], A_T, emit)

    def comb_jobs(mp):
        return [comb_job(mp, g) for g in range(RS // 16)]

    def zero_job(p):
        def t():
            for c in range(2):
                acc[p, c, pl.ds(0, HB), :] = jnp.zeros((HB, 128), f32)
        return [t]

    def oc_job(i, g, n):
        def load(a, kb):
            return _unpk(xn[pl.ds(_mult(i * 64, 64) + (a * 256 + g * 8), 8), pl.ds(kb * KB + n * 128, 128)])

        def one(I):
            sub = {(r, c): _comb([(sg, load(q[0] * 2 + r, q[1] * 2 + c)) for sg, q in A_T[I]])
                   for r in range(2) for c in range(2)}
            for J, t2 in enumerate(A_T):
                M[i % 2, I * 7 + J, n, pl.ds(g * 16, 16), :] = _comb([(sg, sub[q]) for sg, q in t2])
        return [(lambda I=I: one(I)) for I in range(7)]

    def oc_jobs(i):
        return [oc_job(i, g, n) for g in range(RS // 16) for n in range(2)]

    def final_job(i, g, n):
        job = []
        par = i % 2
        for pos in POS:
            def t(pos=pos):
                r0 = _mult(i * RS, RS) + g * 16
                o = [_outpos(lambda p: acc[p, n, pl.ds(r0 + hf * 8, 8), :], pos) for hf in range(2)]
                for q in o[0]:
                    a = q[0] * 2 + pos[0]
                    cols = pl.ds(((q[1] * 2 + pos[1]) * 2 + n) * 128, 128)
                    res = xr[pl.ds(r0 + a * HB, 16), cols].astype(f32) + jnp.concatenate([o[0][q], o[1][q]], axis=0)
                    dst[par, pl.ds(a * RS + g * 16, 16), cols] = res.astype(bf)
            job.append(t)
        return job

    def final_jobs(i):
        return [final_job(i, g, n) for g in range(RS // 16) for n in range(2)]

    def k_tasks(slot, cbase, pieces):
        out = []
        for r in pieces:
            for ct in range(QW // 128):
                def t(r=r, ct=ct):
                    res = _dot(_up(xn[pl.ds(_mult(r * 64, 64), 64), :]), wst[slot, :, pl.ds(ct * 128, 128)])
                    for k in range(8):
                        R[cbase + ct, pl.ds(_mult(r * 64 + k * 8, 8), 8), :] = _pk(res[k * 16:(k + 1) * 16])
                out.append((t, 256))
        return out

    def q_tasks(cbase):
        out = []
        for r in range(16):
            for ct in range(QW // 128):
                def t(r=r, ct=ct):
                    res = _dot(_up(xn[pl.ds(r * 64, 64), :]),
                               _up(wqp[:, pl.ds(_mult((cbase + ct) * 128, 128), 128)]))
                    for k in range(8):
                        QP[cbase + ct, pl.ds(r * 64 + k * 8, 8), :] = _pk(res[k * 16:(k + 1) * 16])
                out.append((t, 256))
        return out

    def mm1_tasks(mp, s, par):
        out = []
        for p in range(NP):
            for c in range(2):
                def t(p=p, c=c):
                    M[mp, p, c, pl.ds(0, RS), :] = _dot(
                        _up(T[p, pl.ds(_mult(s * (RS // 2), RS // 2), RS // 2), :]),
                        _up(B[par, p, :, pl.ds(c * 128, 128)]))
                out.append((t, 64))
        return out

    def mm2_tasks(mp, s, par):
        out = []
        for p in range(NP):
            def t(p=p):
                r = _dot(_up(H[mp, p]), _up(Bd[par, p]))
                for c in range(2):
                    acc[p, c, pl.ds(_mult(s * RS, RS), RS), :] += r[:, c * 128:(c + 1) * 128]
            out.append((t, 64))
        return out

    def wo_tasks(i):
        out = []
        for p in range(NP):
            for c in range(2):
                def t(p=p, c=c):
                    lhs = jnp.concatenate([M[i % 2, p, n, pl.ds(0, RS), :] for n in range(2)], axis=1)
                    acc[p, c, pl.ds(_mult(i * RS, RS), RS), :] += lax.dot_general(
                        lhs, _up(B[1, p, :, pl.ds(c * 128, 128)]), (((1,), (0,)), ((), ())),
                        preferred_element_type=f32)
                out.append((t, 64))
        return out

    nothing = lambda: [(lambda: None, 1)]

    x_copy(0).start()
    w_copy(0, 0).start()
    for c in range(8):
        KF[c, pl.ds(0, PADR), :] = jnp.zeros((PADR, 128), f32)
        VF[c, pl.ds(0, PADR), :] = jnp.zeros((PADR, 128), f32)
    x_copy(0).wait()
    w_copy(1, 1).start()
    x_copy(1).start()
    block(nothing, lambda: ln_jobs(0), 'ln0')
    w_copy(0, 0).wait()

    def k01(pieces):
        rp = [2 * r + h for r in pieces for h in range(2)]
        return k_tasks(0, 0, rp) + k_tasks(1, 2, rp)

    block(lambda: k_tasks(0, 0, (0, 1)), lambda: [], 'p0')
    w_copy(1, 1).wait()
    x_copy(2).start()
    x_copy(1).wait()
    block(lambda: k_tasks(1, 2, (0, 1)), lambda: ln_jobs(1), 'p0')
    x_copy(3).start()
    x_copy(4).start()
    x_copy(2).wait()
    block(lambda: k01((1,)), lambda: ln_jobs(2), 'p0')
    x_copy(5).start()
    x_copy(6).start()
    x_copy(3).wait()
    x_copy(4).wait()
    block(lambda: k01((2,)), lambda: ln_jobs(3) + ln_jobs(4), 'p0')
    x_copy(7).start()
    wq_copy().start()
    x_copy(5).wait()
    x_copy(6).wait()
    block(lambda: k01((3, 4)), lambda: ln_jobs(5) + ln_jobs(6), 'p0')
    w_copy(2, 2).start()
    start(wv_copies())
    x_copy(7).wait()
    block(lambda: k01((5, 6)), lambda: ln_jobs(7), 'p0')
    wq_copy().wait()
    block(lambda: k01((7,)), lambda: [wperm_job('q', 0, a, 2) for a in range(0, 8, 2)], 'p0')

    wait(wv_copies())

    def k_body(j, c):
        w_copy(j, j % 3).wait()

        @pl.when(j == 2)
        def _():
            w_copy(3, 0).start()
            start(gu_copies(0, 0))

        @pl.when(j == 3)
        def _():
            d_copy(0, 0).start()
            d_copy(1, 1).start()
        i = j - 2

        def jobs():
            perms = _mix([wperm_job('v', i * 16, a) for a in range(16)], [wperm_job('q', 8 + 12 * i, a, 2) for a in range(0, 12, 2)])
            extra = [t_job(i * 32, a) for a in range(8)] + [mzero_job(jnp.minimum(i * 25 + a, NP - 1)) for a in range(25)]
            return _mix(perms[:-4], extra) + perms[-4:]
        block(lambda: k_tasks(j % 3, j * 2, range(16)), jobs, 'k', 0)
        return c
    lax.fori_loop(2, 4, k_body, 0)
    start(gu_copies(1, 1))

    def q_body(i, c):
        def jobs():
            extra = ([bv_job(i, g, h) for g in range(4) for h in range(2)]
                     + [t_job(64 + 48 * i, a) for a in range(12)])
            return _mix([kperm_job(i, a) for a in range(16)], extra)
        block(lambda: q_tasks(i * 2), jobs, 'q', 2)
        return c
    lax.fori_loop(0, 4, q_body, 0)

    wait(gu_copies(0, 0))
    d_copy(0, 0).wait()

    def v_slot(s, mp):
        def jobs():
            return _mix(b_jobs(0, s) + bd_jobs(0, s)[:2], [zero_job(jnp.minimum(s * 13 + a, NP - 1)) for a in range(13)]) + vcomb_jobs(1 - mp, jnp.maximum(s - 1, 0))
        block(lambda: mm1_tasks(mp, s, 1), jobs, 'v', 2)

    def v_body(it, c):
        v_slot(2 * it, 0)
        v_slot(2 * it + 1, 1)
        return c
    lax.fori_loop(0, 2, v_body, 0)

    wait(gu_copies(1, 1))
    start(gu_copies(2, 0))
    block(lambda: mm1_tasks(0, 0, 0), lambda: _mix(vcomb_jobs(1, 3), b_jobs(1, 0) + bd_jobs(0, 0)[2:] + bd_jobs(0, 1)[2:]), 'f0', 0)
    block(lambda: mm1_tasks(1, 1, 0),
          lambda: _mix(_mix(comb_jobs(0), b_jobs(1, 1) + bd_jobs(0, 2)[2:] + bd_jobs(0, 3)[2:]), attn_quad(26, True)), 'f1', 3)

    def slot(t, mp):
        j = t // 4
        s = t % 4
        par = j % 2
        if mp == 0:
            @pl.when(jnp.logical_and(s == 0, j > 0))
            def _():
                wait(gu_copies(jnp.minimum(j + 1, NCH - 1), 1 - par))

                @pl.when(j + 2 < NCH)
                def _():
                    start(gu_copies(j + 2, par))

                @pl.when(j + 2 == NCH)
                def _():
                    start(wo_copies())

            @pl.when(jnp.logical_and(s == 2, j + 1 < NCH))
            def _():
                d_copy(j + 1, 1 - par).wait()

                @pl.when(j + 2 < NCH)
                def _():
                    d_copy(j + 2, par).start()
        jd = (t + 2) // 4
        kd = (t + 2) % 4
        u = t - 2

        def jobs():
            base = _mix(comb_jobs(1 - mp), b_jobs(1 - par, s) + bd_jobs(jd % 2, kd))
            att = attn_quad(u)
            n0 = max(1, len(base) // 10)
            return base[:n0] + _mix(base[n0:-n0], att) + base[-n0:]
        block(lambda: mm1_tasks(mp, s, par) + mm2_tasks(mp, (t - 2) % 4, ((t - 2) // 4) % 2), jobs,
              'slot%d' % mp, 3)

    def steady(it, c):
        slot(2 * it + 2, 0)
        slot(2 * it + 3, 1)
        return c
    lax.fori_loop(0, (NT - 2) // 2, steady, 0)

    block(lambda: mm2_tasks(0, 2, 0), lambda: comb_jobs(1), 'e0')
    block(lambda: mm2_tasks(1, 3, 0), lambda: _mix(oc_jobs(0), attn_quad(27, True)), 'e1')
    block(lambda: wo_tasks(0),
          lambda: _mix(oc_jobs(1), _flat([attn_quad(n, True) for n in [28, 29]])), 'wo')
    for i in range(1, 3):
        block(lambda i=i: wo_tasks(i),
              lambda i=i: _mix(final_jobs(i - 1) + oc_jobs(i + 1),
                                _flat([attn_quad(n, True) for n in ([30, 31] if i == 1 else [])])), 'wo')
        start([out_copy(i - 1, a) for a in range(4)])
    wait([out_copy(0, a) for a in range(4)])
    block(lambda: wo_tasks(3)[0::2], lambda: final_jobs(2), 'wo')
    start([out_copy(2, a) for a in range(4)])
    wait([out_copy(1, a) for a in range(4)])
    block(lambda: wo_tasks(3)[1::2], lambda: [final_job(3, g, 0) for g in range(RS // 16)], 'wo')
    for h in range(2):
        block(nothing, lambda h=h: [final_job(3, g, 1) for g in range(4 * h, 4 * h + 4)], 'e3')
        start([last_copy(a, h) for a in range(4)])
    wait([out_copy(2, a) for a in range(4)])
    wait([last_copy(a, h) for h in range(2) for a in range(4)])


@jax.jit
def pallas_parallel_sum__sliding_local_dilated__glu_gated_bilinear__prompt_kernel(
    A_x: jax.Array,
    A_wqkv: jax.Array,
    A_wo: jax.Array,
    B_x: jax.Array,
    B_w_gate: jax.Array,
    B_w_up: jax.Array,
    B_w_down: jax.Array,
):
    del B_x
    x = A_x.reshape(S, D)
    hbm = pl.BlockSpec(memory_space=pl.ANY)
    dma = pltpu.SemaphoreType.DMA
    out = pl.pallas_call(
        _kernel,
        grid=(1,),
        in_specs=[pl.BlockSpec(memory_space=pltpu.SMEM)] + [hbm] * 6,
        out_specs=hbm,
        out_shape=jax.ShapeDtypeStruct((S, D), bf),
        scratch_shapes=[
            pltpu.VMEM((S, D), bf),
            pltpu.VMEM((S // 2, D), u32),
            pltpu.VMEM((NP, HB // 2, KB), u32),
            pltpu.VMEM((3, D, QW), bf),
            pltpu.VMEM((D, D), bf),
            pltpu.VMEM((D // 2, D), u32),
            pltpu.VMEM((D // 2, D), u32),
            pltpu.VMEM((8, S // 2 + PADW, 128), u32),
            pltpu.VMEM((8, S // 2 + PADW, 128), u32),
            pltpu.VMEM((8, S + PADR + 8, 128), f32),
            pltpu.VMEM((8, S + PADR + 8, 128), f32),
            pltpu.VMEM((2, D, TF), bf),
            pltpu.VMEM((2, D, TF), bf),
            pltpu.VMEM((2, TF, D), bf),
            pltpu.VMEM((2, NP, KB // 2, 2 * TB), u32),
            pltpu.VMEM((2, NP, TB // 2, KB), u32),
            pltpu.VMEM((2, NP, 2, RS + MPAD, 128), f32),
            pltpu.VMEM((2, NP, RS // 2, TB), u32),
            pltpu.VMEM((4, 16, 24, 128), f32),
            pltpu.VMEM((4, 8, 24, 128), f32),
            pltpu.VMEM((NP, 2, HB + MPAD, 128), f32),
            dma((8,)), dma((3,)), dma((1,)), dma((2,)), dma((2,)), dma((2,)), dma((16,)),
        ],
        compiler_params=pltpu.CompilerParams(
            dimension_semantics=("arbitrary",), vmem_limit_bytes=127 * 1024 * 1024,
            disable_bounds_checks=True),
        name="fused_attn_ffn",
    )(jnp.ones((1,), jnp.int32), x, A_wqkv, A_wo, B_w_gate, B_w_up, B_w_down)
    return out.reshape(1, S, D)
```
